```python
import jax
import jax.numpy as jnp

def _softmax(x, axis=-1):
    return jax.nn.softmax(x, axis=axis)

def _gelu(x):
    return jax.nn.gelu(x, approximate=True)

def _silu(x):
    return jax.nn.silu(x)

def _sigmoid(x):
    return jax.nn.sigmoid(x)

def _layernorm(x, axis=-1, eps=1e-05):
    m = jnp.mean(x, axis=axis, keepdims=True)
    v = jnp.var(x, axis=axis, keepdims=True)
    return (x - m) / jnp.sqrt(v + eps)

def _scatter_add(tgt, idx, src, axis=0):
    return tgt.at[idx].add(src)

def _segment_sum(src, seg, n):
    return jax.ops.segment_sum(src, seg, n)

class _Rng:

    def __init__(self, key):
        self._k = key

    def _next(self):
        self._k, sub = jax.random.split(self._k)
        return sub

    def normal(self, shape):
        return jax.random.normal(self._next(), shape, dtype=jnp.bfloat16)

    def randint(self, lo, hi, shape):
        return jax.random.randint(self._next(), shape, lo, hi, dtype=jnp.int32)

    def uniform(self, shape, lo=0.0, hi=1.0):
        return jax.random.uniform(self._next(), shape, jnp.bfloat16, lo, hi)

    def permutation(self, n):
        return jax.random.permutation(self._next(), n)
kernel_name = 'recurrent_scan__ssm_conv_h3__mixer_gmlp__prompt'

def setup_inputs():
    _rng = _Rng(jax.random.key(int.from_bytes(__import__("os").urandom(4), "little")))
    _w = lambda a: (lambda t: t.astype(jnp.bfloat16) if jnp.issubdtype(t.dtype, jnp.floating) else t)(jnp.asarray(a))

    def _A_setup():
        B, S, D = (1, 2048, 640)
        ks = 4
        return {'q': _w((lambda *s: _rng.normal(s) * 0.05)(B, S, D)), 'k': _w((lambda *s: _rng.normal(s) * 0.05)(B, S, D)), 'v': _w((lambda *s: _rng.normal(s) * 0.05)(B, S, D)), 'shift_k': _w((lambda *s: _rng.normal(s) * 0.05)(D, ks) * 0.5), 'ssm_k': _w((lambda *s: _rng.normal(s) * 0.05)(D, S) * (1.0 / S ** 0.5)), 'ssm_D': _w((lambda *s: _rng.normal(s) * 0.05)(D))}
    _A_in = _A_setup()

    def _B_setup():
        B, S, D, F = (1, 2048, 640, 1536)
        Fh = F // 2
        return {'x': _w((lambda *s: _rng.normal(s) * 0.05)(B, S, D)), 'w_in': _w((lambda *s: _rng.normal(s) * 0.05)(D, 2 * Fh)), 'w_sp': _w(0.01 * (lambda *s: _rng.normal(s) * 0.05)(S, S)), 'b_sp': _w(1.0 + 0.01 * (lambda *s: _rng.normal(s) * 0.05)(S)), 'w_out': _w((lambda *s: _rng.normal(s) * 0.05)(Fh, D))}
    _B_in = _B_setup()
    return {'A_q': _A_in['q'], 'A_k': _A_in['k'], 'A_v': _A_in['v'], 'A_shift_k': _A_in['shift_k'], 'A_ssm_k': _A_in['ssm_k'], 'A_ssm_D': _A_in['ssm_D'], 'B_x': _B_in['x'], 'B_w_in': _B_in['w_in'], 'B_w_sp': _B_in['w_sp'], 'B_b_sp': _B_in['b_sp'], 'B_w_out': _B_in['w_out']}

def reference(A_q, A_k, A_v, A_shift_k, A_ssm_k, A_ssm_D, B_x, B_w_in, B_w_sp, B_b_sp, B_w_out):

    def _A_ref(q, k, v, shift_k, ssm_k, ssm_D):
        B, S, D = q.shape
        ks = shift_k.shape[-1]
        k_pad = jnp.pad(k, ((0, 0), (ks - 1, 0), (0, 0)))
        k_shift = jnp.zeros_like(k)
        for t in range(ks):
            k_shift = k_shift + k_pad[:, t:t + S, :] * shift_k[:, ks - 1 - t][None, None, :]
        kv = k_shift * v
        L = 2 * S
        kv_pad = jnp.pad(kv, ((0, 0), (0, S), (0, 0)))
        kf_pad = jnp.pad(ssm_k, ((0, 0), (0, S)))
        kv_f = (lambda x, axes=(-2, -1): jnp.fft.rfft2(x.astype(jnp.float32), axes=axes))(kv_pad[:, None, :, :], axes=(1, 2))
        kf_f = (lambda x, axes=(-2, -1): jnp.fft.rfft2(x.astype(jnp.float32), axes=axes))(kf_pad[:, None, :], axes=(1, 2))
        kf_f = (lambda x, *d: x.transpose(*d))(kf_f, 1, 2, 0)
        y_f = kv_f * kf_f[None, :, :, :]
        y = (lambda x, s, axes=(-2, -1): jnp.fft.irfft2(x, s=s, axes=axes).astype(jnp.bfloat16))(y_f, (1, L), axes=(1, 2))[:, 0, :S, :]
        y = y + kv * ssm_D[None, None, :]
        return q * y

    def _B_ref(x, w_in, w_sp, b_sp, w_out):
        B, S, D = x.shape
        F = w_in.shape[-1]
        Fh = F // 2
        z = _gelu(jnp.einsum('bsd,df->bsf', x, w_in))
        z1 = z[..., :Fh].copy()
        z2 = _layernorm(z[..., Fh:], axis=-1)
        g = jnp.einsum('ts,bsf->btf', w_sp, z2) + b_sp[None, :, None]
        return jnp.einsum('bsf,fd->bsd', z1 * g, w_out)
    x = A_q
    xn = _layernorm(x, axis=-1)
    s = _A_ref(xn, A_k, A_v, A_shift_k, A_ssm_k, A_ssm_D)
    g = _silu(_B_ref(xn, B_w_in, B_w_sp, B_b_sp, B_w_out))
    return x + s * g
```

```python
import functools
import math

import jax
import jax.numpy as jnp
import numpy as np
import jax.experimental.pallas as pl
import jax.experimental.pallas.tpu as pltpu

S = 2048
D = 640
FH = 768
C = 128
NB = S // C
TM = 256
NS = S // TM
HALO = 16
EPS = 1e-5

BF = jnp.bfloat16
F32 = jnp.float32
U32 = jnp.uint32


def _dft_consts():
    m = np.arange(C)
    t = np.arange(C)
    theta = np.pi * (4 * m + 1) / (2 * C)
    ang = theta[:, None] * t[None, :]
    re = np.cos(ang)
    im = -np.sin(ang)
    f = np.stack([re.reshape(C // 8, 8, C), im.reshape(C // 8, 8, C)], axis=1).reshape(2 * C, C)
    g = f.T / C
    return f.astype(np.float32), np.ascontiguousarray(g).astype(np.float32)


def _kernel(q_hbm, k_hbm, v_hbm, sk_hbm, h_hbm, d_hbm, win_hbm, wsp_hbm, b_hbm, wout_hbm,
            f_hbm, g_hbm, o_hbm,
            q_v, k_v, v_v, sk_v, h_u, d_v, win_u, wsp_u, b_v, wout_u, f_u, g_u,
            xn_u, kv_u, z1_v, z2_u, p_v, hf_v, w_u, gg_u, o_v, b32_v,
            sem_q, sem_k, sem_v, sem_h, sem_wsp, sem_o, sem_m):
    h_v = h_u.bitcast(BF)
    win_v = win_u.bitcast(BF)
    wsp_v = wsp_u.bitcast(BF)
    wout_v = wout_u.bitcast(BF)
    f_v = f_u.bitcast(BF)
    g_v = g_u.bitcast(BF)
    xn_v = xn_u.bitcast(BF)
    kv_v = kv_u.bitcast(BF)
    z2_v = z2_u.bitcast(BF)
    w_v = w_u.bitcast(BF)
    gg_v = gg_u.bitcast(BF)

    def rows_of(i):
        if isinstance(i, int):
            return pl.ds(i * TM, TM)
        return pl.ds(pl.multiple_of(i * TM, TM), TM)

    def cp_q(i):
        return pltpu.make_async_copy(q_hbm.at[rows_of(i), :], q_v.at[rows_of(i), :], sem_q.at[i])

    def cp_k(i):
        if isinstance(i, int):
            dst = pl.ds(i * TM + HALO, TM)
        else:
            dst = pl.ds(pl.multiple_of(i * TM + HALO, HALO), TM)
        return pltpu.make_async_copy(k_hbm.at[rows_of(i), :], k_v.at[dst, :], sem_k.at[i])

    def cp_v(i):
        return pltpu.make_async_copy(v_hbm.at[rows_of(i), :], v_v.at[rows_of(i), :], sem_v.at[i])

    def cp_h(i):
        return pltpu.make_async_copy(h_hbm.at[:, rows_of(i)], h_v.at[:, rows_of(i)], sem_h.at[i])

    def cp_wsp(i):
        return pltpu.make_async_copy(wsp_hbm.at[rows_of(i), :], wsp_v.at[rows_of(i), :], sem_wsp.at[i])

    def cp_o(i):
        return pltpu.make_async_copy(o_v.at[rows_of(i), :], o_hbm.at[rows_of(i), :], sem_o.at[i])

    cp_f = pltpu.make_async_copy(f_hbm, f_v, sem_m.at[0])
    cp_sk = pltpu.make_async_copy(sk_hbm, sk_v, sem_m.at[1])
    cp_win = pltpu.make_async_copy(win_hbm, win_v, sem_m.at[2])
    cp_g = pltpu.make_async_copy(g_hbm, g_v, sem_m.at[3])
    cp_d = pltpu.make_async_copy(d_hbm, d_v, sem_m.at[4])
    cp_b = pltpu.make_async_copy(b_hbm, b_v, sem_m.at[5])
    cp_wout = pltpu.make_async_copy(wout_hbm, wout_v, sem_m.at[6])

    cp_f.start()
    cp_h(0).start()
    cp_q(0).start()
    cp_sk.start()
    cp_k(0).start()
    cp_v(0).start()
    cp_win.start()
    for i in range(1, NS):
        cp_h(i).start()
        cp_q(i).start()
        cp_k(i).start()
        cp_v(i).start()
    cp_d.start()
    cp_b.start()
    for i in range(NS):
        cp_wsp(i).start()
    cp_g.start()
    cp_wout.start()

    k_v[0:HALO, :] = jnp.zeros((HALO, D), BF)
    cp_f.wait()
    cp_sk.wait()
    cp_win.wait()

    c0 = math.sqrt(2.0 / math.pi)
    c1 = c0 * 0.044715

    def gelu2(x):
        t = jnp.tanh(x * (c0 + c1 * (x * x)))
        return x + x * t

    def phase1(i, carry):
        rows = rows_of(i)
        cp_h(i).wait()
        cp_q(i).wait()
        cp_k(i).wait()
        cp_v(i).wait()
        fm = f_v[...]

        for j in range(TM // C):
            a = i * (TM // C) + j
            cols = pl.ds(pl.multiple_of(a * C, C), C)
            hf_v[a] = jax.lax.dot_general(fm, h_v[:, cols], (((1,), (1,)), ((), ())),
                                          preferred_element_type=F32)

        x = q_v[rows, :].astype(F32)
        mu = jnp.sum(x, axis=-1, keepdims=True) * (1.0 / D)
        ex2 = jnp.sum(x * x, axis=-1, keepdims=True) * (1.0 / D)
        var = jnp.maximum(ex2 - mu * mu, 0.0)
        xn = ((x - mu) * jax.lax.rsqrt(var + EPS)).astype(BF)
        xn_v[rows, :] = xn

        kf = k_v[pl.ds(pl.multiple_of(i * TM + HALO - 8, 8), TM + 8), :].astype(F32)
        sk = sk_v[...].astype(F32)
        ks = kf[8:, :] * sk[0:1, :]
        for j in range(1, 4):
            ks = ks + pltpu.roll(kf, j, axis=0)[8:, :] * sk[j:j + 1, :]
        kv_v[rows, :] = (ks * v_v[rows, :].astype(F32)).astype(BF)

        xnl = xn_v[rows, :]
        w2 = gelu2(jnp.dot(xnl, win_v[:, FH:], preferred_element_type=F32))
        mu2 = jnp.sum(w2, axis=-1, keepdims=True) * (1.0 / FH)
        ex22 = jnp.sum(w2 * w2, axis=-1, keepdims=True) * (1.0 / FH)
        var2 = jnp.maximum(ex22 - mu2 * mu2, 0.0)
        z2_v[rows, :] = ((w2 - mu2) * (0.25 * jax.lax.rsqrt(var2 + 4.0 * EPS))).astype(BF)
        z1_v[rows, :] = gelu2(jnp.dot(xnl, win_v[:, :FH], preferred_element_type=F32))

        for j in range(TM // C):
            a = i * (TM // C) + j
            r = pl.ds(pl.multiple_of(a * C, C), C)
            p_v[a] = jnp.dot(fm, kv_v[r, :], preferred_element_type=F32)
        return carry

    jax.lax.fori_loop(0, NS, phase1, 0)

    cp_d.wait()
    cp_b.wait()
    dv = d_v[...].astype(F32)
    b32_v[...] = b_v[...].astype(F32) * 0.25
    for jt in range(2 * C // 16):
        for dt in range(D // 128):
            sl = (0, pl.ds(jt * 16, 8), pl.ds(dt * 128, 128))
            hf_v[sl] = hf_v[sl] + dv[dt:dt + 1, :]

    def conv_pos(ft, c0_, tok):
        r0 = pl.multiple_of(ft * 16, 16)
        rre = pl.ds(r0, 8)
        rim = pl.ds(r0 + 8, 8)
        cols = pl.ds(c0_, 128)
        prev = None
        for a in range(NB):
            if prev is not None:
                ar, ai = -prev[1], prev[0]
            elif tok is not None:
                ar, ai = tok
            else:
                ar = ai = None
            for dl in range(a + 1):
                hr = hf_v[dl, rre, cols]
                hi = hf_v[dl, rim, cols]
                ur = p_v[a - dl, rre, cols]
                ui = p_v[a - dl, rim, cols]
                if ar is None:
                    ar, ai = ur * hr - ui * hi, ur * hi + ui * hr
                else:
                    ar = (ar + ur * hr) - ui * hi
                    ai = (ai + ur * hi) + ui * hr
            if prev is not None:
                wr, wi = ar, ai
                prev = (wr + prev[1], wi - prev[0])
            else:
                if tok is not None:
                    ar, ai = ar - tok[0], ai - tok[1]
                wr, wi = ar, ai
                prev = (wr, wi)
            w_v[a, pl.ds(r0, 16), cols] = jnp.concatenate([wr, wi], axis=0).astype(BF)
        return prev

    def phase2a(i, carry):
        rows = rows_of(i)
        cp_wsp(i).wait()
        eye = (jax.lax.broadcasted_iota(jnp.int32, (C, C), 0)
               == jax.lax.broadcasted_iota(jnp.int32, (C, C), 1))
        bcols = []
        for j in range(TM // C):
            brow = b32_v[pl.ds(i * (TM // C) + j, 1), :]
            bcols.append(jnp.sum(jnp.where(eye, brow, 0.0), axis=-1, keepdims=True))
        bcol = jnp.concatenate(bcols, axis=0)
        g = jnp.dot(wsp_v[rows, :], z2_v[...], preferred_element_type=F32) + bcol
        gg_v[rows, :] = (z1_v[rows, :] * g).astype(BF)
        tok = None
        for ft in range(NB // NS):
            for dt in range(D // 128):
                tok = conv_pos(i * (NB // NS) + ft, dt * 128, tok)
        return carry

    jax.lax.fori_loop(0, NS, phase2a, 0)

    cp_g.wait()
    cp_wout.wait()

    def phase2b(i, carry):
        rows = rows_of(i)
        gm = g_v[...]
        ys = []
        for j in range(TM // C):
            ys.append(jnp.dot(gm, w_v[i * (TM // C) + j], preferred_element_type=F32))
        y = jnp.concatenate(ys, axis=0)
        hh = jnp.dot(gg_v[rows, :], wout_v[...], preferred_element_type=F32)
        gate = hh + hh * jnp.tanh(hh)
        s = xn_v[rows, :].astype(F32) * y
        o_v[rows, :] = (q_v[rows, :].astype(F32) + s * gate).astype(BF)
        cp_o(i).start()
        return carry

    jax.lax.fori_loop(0, NS, phase2b, 0)
    for i in range(NS):
        cp_o(i).wait()


@jax.jit
def pallas_recurrent_scan__ssm_conv_h3__mixer_gmlp__prompt_kernel(
    A_q: jax.Array,
    A_k: jax.Array,
    A_v: jax.Array,
    A_shift_k: jax.Array,
    A_ssm_k: jax.Array,
    A_ssm_D: jax.Array,
    B_x: jax.Array,
    B_w_in: jax.Array,
    B_w_sp: jax.Array,
    B_b_sp: jax.Array,
    B_w_out: jax.Array,
):
    del B_x
    fm, gm = _dft_consts()
    fm = jnp.asarray(fm, dtype=BF)
    gm = jnp.asarray(gm, dtype=BF)
    any_spec = pl.BlockSpec(memory_space=pl.ANY)
    vm = pltpu.VMEM
    out = pl.pallas_call(
        _kernel,
        out_shape=jax.ShapeDtypeStruct((S, D), BF),
        in_specs=[any_spec] * 12,
        out_specs=any_spec,
        scratch_shapes=[
            vm((S, D), BF),
            vm((S + HALO, D), BF),
            vm((S, D), BF),
            vm((4, D), BF),
            vm((D // 2, S), U32),
            vm((D // 128, 128), BF),
            vm((D // 2, 2 * FH), U32),
            vm((S // 2, S), U32),
            vm((S // 128, 128), BF),
            vm((FH // 2, D), U32),
            vm((C, C), U32),
            vm((C // 2, 2 * C), U32),
            vm((S // 2, D), U32),
            vm((S // 2, D), U32),
            vm((S, FH), F32),
            vm((S // 2, FH), U32),
            vm((NB, 2 * C, D), F32),
            vm((NB, 2 * C, D), F32),
            vm((NB, C, D), U32),
            vm((S // 2, FH), U32),
            vm((S, D), BF),
            vm((S // 128, 128), F32),
            pltpu.SemaphoreType.DMA((NS,)),
            pltpu.SemaphoreType.DMA((NS,)),
            pltpu.SemaphoreType.DMA((NS,)),
            pltpu.SemaphoreType.DMA((NS,)),
            pltpu.SemaphoreType.DMA((NS,)),
            pltpu.SemaphoreType.DMA((NS,)),
            pltpu.SemaphoreType.DMA((7,)),
        ],
        compiler_params=pltpu.CompilerParams(vmem_limit_bytes=110 * 1024 * 1024),
    )(
        A_q.reshape(S, D), A_k.reshape(S, D), A_v.reshape(S, D),
        A_shift_k.T, A_ssm_k, A_ssm_D.reshape(D // 128, 128),
        B_w_in, B_w_sp, B_b_sp.reshape(S // 128, 128), B_w_out,
        fm, gm,
    )
    return out.reshape(1, S, D)
```

```python
import math
import os

import jax
import jax.numpy as jnp
import numpy as np
import jax.experimental.pallas as pl
import jax.experimental.pallas.tpu as pltpu

S = 2048
D = 640
FH = 768
C = 128
NB = S // C
ND = D // 128
NT = FH // 128
HALO = 16
EPS = 1e-5

E = lambda k, d: int(os.environ.get(k, d))
TA = E('TA', 512)
MSA = E('MSA', 128)
GATE = E('GATE', 2)
TB = E('TB', 1024)
MSB = E('MSB', 128)
MS1 = E('MS1', 128)

BF = jnp.bfloat16
F32 = jnp.float32
U32 = jnp.uint32

QCH = [(0, 2), (2, 2), (4, 2), (6, 5), (11, 5)]
KCH = [(0, 2), (2, 4), (6, 10)]
WCH = [(6, 3), (9, 3), (0, 3), (3, 3)]
NWSP = S // TA


def _dft_consts():
    m = np.arange(C)
    t = np.arange(C)
    theta = np.pi * (4 * m + 1) / (2 * C)
    ang = theta[:, None] * t[None, :]
    re = np.cos(ang)
    im = -np.sin(ang)
    f = np.stack([re.reshape(C // 8, 8, C), im.reshape(C // 8, 8, C)], axis=1).reshape(2 * C, C)
    g = f.T / C
    fg = np.zeros((3 * C, 2 * C), np.float32)
    fg[:2 * C, :C] = f
    fg[2 * C:, :] = g
    return fg


def _kernel(q_hbm, k_hbm, v_hbm, sk_hbm, h_hbm, d_hbm, win_hbm, wsp_hbm, b_hbm, wout_hbm,
            fg_hbm, o_hbm,
            q_u, k_v, v_v, h_u, win_u, wsp_u, wout_u, fg_u,
            xn_u, z1_v, z2_u, p_v, hf_v, w_u, gg_u, o_v, b32_v, b_v, sk_v, d_v,
            sem_q, sem_k, sem_v, sem_h, sem_w, sem_wsp, sem_o, sem_m):
    q_v = q_u.bitcast(BF)
    h_v = h_u.bitcast(BF)
    win_v = win_u.bitcast(BF)
    wsp_v = wsp_u.bitcast(BF)
    wout_v = wout_u.bitcast(BF)
    fg_v = fg_u.bitcast(BF)
    xn_v = xn_u.bitcast(BF)
    z2_v = z2_u.bitcast(BF)
    w_v = w_u.bitcast(BF)
    gg_v = gg_u.bitcast(BF)

    def ds(start, size, mult):
        if isinstance(start, int):
            return pl.ds(start, size)
        return pl.ds(pl.multiple_of(start, mult), size)

    def blocks(ch):
        return pl.ds(ch[0] * C, ch[1] * C)

    def cp_q(c):
        r = blocks(QCH[c])
        return pltpu.make_async_copy(q_hbm.at[r, :], q_v.at[r, :], sem_q.at[c])

    def cp_k(c):
        b0, n = KCH[c]
        return pltpu.make_async_copy(k_hbm.at[blocks(KCH[c]), :], k_v.at[pl.ds(b0 * C + HALO, n * C), :],
                                     sem_k.at[c])

    def cp_v(c):
        r = blocks(KCH[c])
        return pltpu.make_async_copy(v_hbm.at[r, :], v_v.at[r, :], sem_v.at[c])

    def cp_h(c):
        r = blocks(KCH[c])
        return pltpu.make_async_copy(h_hbm.at[:, r], h_v.at[:, r], sem_h.at[c])

    def cp_w(c):
        r = blocks(WCH[c])
        return pltpu.make_async_copy(win_hbm.at[:, r], win_v.at[:, r], sem_w.at[c])

    def cp_wsp(i):
        r = ds(i * TA, TA, TA)
        return pltpu.make_async_copy(wsp_hbm.at[r, :], wsp_v.at[r, :], sem_wsp.at[i])

    def cp_o(a):
        r = ds(a * C, C, C)
        return pltpu.make_async_copy(o_v.at[r, :], o_hbm.at[r, :], sem_o.at[a])

    cp_f = pltpu.make_async_copy(fg_hbm, fg_v, sem_m.at[0])
    cp_sk = pltpu.make_async_copy(sk_hbm, sk_v.at[:, 0:D], sem_m.at[1])
    cp_d = pltpu.make_async_copy(d_hbm, d_v, sem_m.at[2])
    cp_b = pltpu.make_async_copy(b_hbm, b_v, sem_m.at[3])
    cp_wout = pltpu.make_async_copy(wout_hbm, wout_v, sem_m.at[4])

    def hkv(c):
        return [cp_h(c), cp_k(c), cp_v(c)]

    groups = [
        [cp_q(0)], [cp_w(0)], [cp_w(1)], [cp_w(2)], [cp_q(1), cp_w(3)],
        [cp_f, cp_sk, cp_d, cp_b, cp_q(2)] + hkv(0),
        [cp_q(3)] + hkv(1),
        [cp_q(4)] + hkv(2),
    ]
    for grp in groups:
        for cp in grp:
            cp.start()

    def wait(g):
        for cp in groups[g]:
            cp.wait()

    for i in range(NWSP):
        cp_wsp(i).start()
    cp_wout.start()

    k_v[0:HALO, :] = jnp.zeros((HALO, D), BF)

    c0 = math.sqrt(2.0 / math.pi)
    c1 = c0 * 0.044715

    def gelu2(x):
        t = jnp.tanh(x * (c0 + c1 * (x * x)))
        return x + x * t

    def brows(a):
        return pl.ds(a * C, C)

    def h_dft(a, dt):
        cols = slice(dt * 128, (dt + 1) * 128)
        res = jax.lax.dot_general(fg_v[0:2 * C, 0:C], h_v[cols, brows(a)], (((1,), (1,)), ((), ())),
                                  preferred_element_type=F32)
        hf_v[:, a, :, cols] = res.reshape(NB, 16, 128)

    def ln_q(a, after=None):
        r = brows(a)
        x = q_v[r, :]
        if after is not None:
            au = pltpu.bitcast(after, U32)
            tok = au[:, 0:128]
            for n in range(1, NT if GATE else 1):
                tok = tok | au[:, n * 128:(n + 1) * 128]
            zero = tok & jnp.tile(pltpu.bitcast(k_v[0:HALO, 0:128], U32), (C // 16, 1))
            x = pltpu.bitcast(pltpu.bitcast(x, U32) | jnp.tile(zero, (1, ND)), BF)
        x = x.astype(F32)
        mu = jnp.sum(x, axis=-1, keepdims=True) * (1.0 / D)
        ex2 = jnp.sum(x * x, axis=-1, keepdims=True) * (1.0 / D)
        var = jnp.maximum(ex2 - mu * mu, 0.0)
        xn_v[r, :] = ((x - mu) * jax.lax.rsqrt(var + EPS)).astype(BF)

    def u_dft(a, dt):
        cols = slice(dt * 128, (dt + 1) * 128)
        kf = k_v[pl.ds(a * C + HALO - 8, C + 8), cols].astype(F32)
        sk = sk_v[:, cols].astype(F32)
        ks = kf[8:, :] * sk[0:1, :]
        for t in range(1, 4):
            ks = ks + pltpu.roll(kf, t, axis=0)[8:, :] * sk[t:t + 1, :]
        kv = (ks * v_v[brows(a), cols].astype(F32)).astype(BF)
        res = jnp.dot(fg_v[0:2 * C, 0:C], kv, preferred_element_type=F32)
        p_v[:, a, :, cols] = res.reshape(NB, 16, 128)

    def proj(a, n):
        return gelu2(jnp.dot(xn_v[brows(a), :], win_v[:, n * 128:(n + 1) * 128],
                             preferred_element_type=F32))

    def z2_tile(a, n):
        t = proj(a, NT + n)
        z1_v[pl.ds(S + (a % 2) * C, C), n * 128:(n + 1) * 128] = t
        return t

    def z1_tile(a, n):
        z1_v[brows(a), n * 128:(n + 1) * 128] = proj(a, n)

    def ln_z2(a):
        w2 = z1_v[pl.ds(S + (a % 2) * C, C), :]
        mu2 = jnp.sum(w2, axis=-1, keepdims=True) * (1.0 / FH)
        ex22 = jnp.sum(w2 * w2, axis=-1, keepdims=True) * (1.0 / FH)
        var2 = jnp.maximum(ex22 - mu2 * mu2, 0.0)
        rs2 = 0.25 * jax.lax.rsqrt(var2 + 4.0 * EPS)
        z2n = ((w2 - mu2) * rs2).astype(BF)
        z2_v[brows(a), :] = z2n
        return z2n

    with jax.named_scope('phase1'):
        wait(0)
        ln_q(0)
        ln_q(1)
        for c in range(2):
            wait(1 + c)
            for n in range(3 * c, 3 * c + 3):
                z2_tile(0, n)
                z2_tile(1, n)
        wait(3)
        ln_z2(0)
        ln_z2(1)
        for n in range(3):
            z1_tile(0, n)
            z1_tile(1, n)

        def region(blks, dfts, pre=()):
            hs = [(a, dt) for a in dfts for dt in range(ND)]
            us = list(hs)
            nb = len(blks)
            for f in pre:
                f()
            for bi, a in enumerate(blks):
                last = bi == nb - 1
                nh = len(hs) // (nb - bi)
                nu = len(us) // (nb - bi)
                slots = 2 * NT - (1 if last else 0)
                cnt = [nu * (j + 1) // slots - nu * j // slots for j in range(slots)] + [0]
                for n in range(NT):
                    z2_tile(a, n)
                    for _ in range(cnt[n]):
                        u_dft(*us.pop(0))
                nh_mid = nh if not last else max(nh - 4, 0)
                for _ in range(nh_mid):
                    h_dft(*hs.pop(0))
                z2n = ln_z2(a)
                if a + 1 < NB:
                    ln_q(a + 1, z2n)
                for n in range(NT):
                    z1_tile(a, n)
                    for _ in range(cnt[NT + n]):
                        u_dft(*us.pop(0))
                for _ in range(nh - nh_mid):
                    h_dft(*hs.pop(0))
            assert not hs and not us

        wait(4)
        pre = [lambda: ln_q(2)]
        for n in range(3, 6):
            pre += [lambda n=n: z1_tile(0, n), lambda n=n: z1_tile(1, n)]
        region([2], [], pre)
        wait(5)
        region([3, 4], [0, 1])
        wait(6)
        region([5, 6, 7, 8, 9], [2, 3, 4, 5])
        wait(7)
        region(list(range(10, 16)), list(range(6, 16)))

        dv = d_v[0:ND, :].astype(F32)
        b32_v[0:NB, :] = b_v[0:NB, :].astype(F32) * 0.25
        for dt in range(ND):
            cols = slice(dt * 128, (dt + 1) * 128)
            hf_v[:, 0, 0:8, cols] = hf_v[:, 0, 0:8, cols] + dv[dt:dt + 1, :][None]

    def conv_pos(ft, dt):
        cols = slice(dt * 128, (dt + 1) * 128)
        prev = None
        for a in range(NB):
            if prev is not None:
                ar, ai = -prev[1], prev[0]
            else:
                ar = ai = None
            for dl in range(a + 1):
                hr = hf_v[ft, dl, 0:8, cols]
                hi = hf_v[ft, dl, 8:16, cols]
                ur = p_v[ft, a - dl, 0:8, cols]
                ui = p_v[ft, a - dl, 8:16, cols]
                if ar is None:
                    ar, ai = ur * hr - ui * hi, ur * hi + ui * hr
                else:
                    ar = (ar + ur * hr) - ui * hi
                    ai = (ai + ur * hi) + ui * hr
            prev = (ar, ai) if prev is None else (ar + prev[1], ai - prev[0])
            w_v[ds(a * 2 * C + ft * 16, 16, 16), cols] = jnp.concatenate([ar, ai], axis=0).astype(BF)

    def phase2a(i, carry):
        cp_wsp(i).wait()
        eye = (jax.lax.broadcasted_iota(jnp.int32, (C, C), 0)
               == jax.lax.broadcasted_iota(jnp.int32, (C, C), 1))
        for m in range(TA // MSA):
            rows = ds(i * TA + m * MSA, MSA, MSA)
            bcols = []
            for j in range(MSA // C):
                brow = b32_v[pl.ds(i * (TA // C) + m * (MSA // C) + j, 1), :]
                bcols.append(jnp.sum(jnp.where(eye, brow, 0.0), axis=-1, keepdims=True))
            bcol = jnp.concatenate(bcols, axis=0)
            for n in range(NT):
                cols = slice(n * 128, (n + 1) * 128)
                g = jnp.dot(wsp_v[rows, :], z2_v[:, cols], preferred_element_type=F32) + bcol
                gg_v[rows, cols] = (z1_v[rows, cols] * g).astype(BF)
        nft = NB * TA // S
        for ft in range(nft):
            for dt in range(ND):
                conv_pos(i * nft + ft, dt)
        return carry

    with jax.named_scope('phase2a'):
        jax.lax.fori_loop(0, S // TA, phase2a, 0)

    cp_wout.wait()

    def phase2b(i, carry):
        for m in range(TB // MSB):
            rows = ds(i * TB + m * MSB, MSB, MSB)
            for dt in range(ND):
                cols = slice(dt * 128, (dt + 1) * 128)
                ys = []
                for j in range(MSB // C):
                    a = i * (TB // C) + m * (MSB // C) + j
                    ys.append(jnp.dot(fg_v[2 * C:3 * C, :], w_v[ds(a * 2 * C, 2 * C, 2 * C), cols],
                                      preferred_element_type=F32))
                y = jnp.concatenate(ys, axis=0)
                hh = jnp.dot(gg_v[rows, :], wout_v[:, cols], preferred_element_type=F32)
                gate = hh + hh * jnp.tanh(hh)
                s = xn_v[rows, cols].astype(F32) * y
                o_v[rows, cols] = (q_v[rows, cols].astype(F32) + s * gate).astype(BF)
            for j in range(MSB // C):
                cp_o(i * (TB // C) + m * (MSB // C) + j).start()
        return carry

    with jax.named_scope('phase2b'):
        jax.lax.fori_loop(0, S // TB, phase2b, 0)
    for a in range(NB):
        cp_o(a).wait()


@jax.jit
def pallas_recurrent_scan__ssm_conv_h3__mixer_gmlp__prompt_kernel(
    A_q, A_k, A_v, A_shift_k, A_ssm_k, A_ssm_D, B_x, B_w_in, B_w_sp, B_b_sp, B_w_out,
):
    del B_x
    fg = jnp.asarray(_dft_consts(), dtype=BF)
    any_spec = pl.BlockSpec(memory_space=pl.ANY)
    vm = pltpu.VMEM
    dma = pltpu.SemaphoreType.DMA
    out = pl.pallas_call(
        _kernel,
        out_shape=jax.ShapeDtypeStruct((S, D), BF),
        in_specs=[any_spec] * 11,
        out_specs=any_spec,
        scratch_shapes=[
            vm((S // 2, D), U32),
            vm((S + 64, D), BF),
            vm((S, D), BF),
            vm((D // 2, S), U32),
            vm((D // 2, 2 * FH), U32),
            vm((S // 2, S), U32),
            vm((FH // 2, D), U32),
            vm((3 * C // 2, 2 * C), U32),
            vm((S // 2, D), U32),
            vm((S + 2 * C, FH), F32),
            vm((S // 2, FH), U32),
            vm((NB, NB, 16, D), F32),
            vm((NB, NB, 16, D), F32),
            vm((NB * C, 1024), U32),
            vm((S // 2, FH), U32),
            vm((S, D), BF),
            vm((S // 128, 128), F32),
            vm((S // 128, 128), BF),
            vm((4, 18 * 128), BF),
            vm((D // 128, 128), BF),
            dma((len(QCH),)), dma((len(KCH),)), dma((len(KCH),)), dma((len(KCH),)),
            dma((len(WCH),)), dma((NWSP,)), dma((NB,)), dma((5,)),
        ],
        compiler_params=pltpu.CompilerParams(vmem_limit_bytes=110 * 1024 * 1024),
    )(
        A_q.reshape(S, D), A_k.reshape(S, D), A_v.reshape(S, D),
        A_shift_k.T, A_ssm_k, A_ssm_D.reshape(D // 128, 128),
        B_w_in, B_w_sp, B_b_sp.reshape(S // 128, 128), B_w_out,
        fg,
    )
    return out.reshape(1, S, D)
```

```python
import math
import os

import jax
import jax.numpy as jnp
import numpy as np
import jax.experimental.pallas as pl
import jax.experimental.pallas.tpu as pltpu

S = 2048
D = 640
FH = 768
C = 128
NB = S // C
ND = D // 128
NT = FH // 128
HALO = 16
EPS = 1e-5

E = lambda k, d: int(os.environ.get(k, d))
TA = E('TA', 512)
MSA = E('MSA', 128)
GATE = E('GATE', 0)
CH = E('CH', 0)
FINE = E('FINE', 2)
NOCHK = E('NOCHK', 3)
TB = E('TB', 1024)
MSB = E('MSB', 128)
MS1 = E('MS1', 128)

BF = jnp.bfloat16
F32 = jnp.float32
U32 = jnp.uint32

QCH = [(0, 2), (2, 2), (4, 2), (6, 5), (11, 5)]
KCH = [(0, 2), (2, 4), (6, 10)]
WCH = [(6, 2), (8, 4), (0, 4), (4, 2)]
NWSP = S // TA


def _dft_consts():
    m = np.arange(C)
    t = np.arange(C)
    theta = np.pi * (4 * m + 1) / (2 * C)

    def fwd(tt):
        ang = theta[:, None] * tt[None, :]
        re = np.cos(ang).reshape(C // 8, 8, C)
        im = -np.sin(ang).reshape(C // 8, 8, C)
        return np.stack([re, im], axis=1).reshape(2 * C, C)

    fg = np.zeros((2 * C + C // 2, 2 * C), np.float32)
    fg[:2 * C, :C] = fwd(t - (C - 1) / 2)
    fg[:2 * C, C:] = fwd(t)
    ang = (np.arange(C // 2) + 0.5)[:, None] * theta[None, :]
    fg[2 * C:, :C] = np.cos(ang) / C
    fg[2 * C:, C:] = -np.sin(ang) / C
    return fg


def _kernel(q_hbm, k_hbm, v_hbm, sk_hbm, h_hbm, d_hbm, win_hbm, wsp_hbm, b_hbm, wout_hbm,
            fg_hbm, o_hbm,
            q_u, k_v, v_v, h_u, win_u, wsp_u, wout_u, fg_u,
            xn_u, z1_v, z2_u, p_v, hf_v, w_u, gg_u, o_v, b32_v, b_v, sk_v, d_v,
            sem_q, sem_k, sem_v, sem_h, sem_w, sem_wsp, sem_o, sem_m):
    q_v = q_u.bitcast(BF)
    h_v = h_u.bitcast(BF)
    win_v = win_u.bitcast(BF)
    wsp_v = wsp_u.bitcast(BF)
    wout_v = wout_u.bitcast(BF)
    fg_v = fg_u.bitcast(BF)
    xn_v = xn_u.bitcast(BF)
    z2_v = z2_u.bitcast(BF)
    w_v = w_u.bitcast(BF)
    gg_v = gg_u.bitcast(BF)

    def ds(start, size, mult):
        if isinstance(start, int):
            return pl.ds(start, size)
        return pl.ds(pl.multiple_of(start, mult), size)

    def blocks(ch):
        return pl.ds(ch[0] * C, ch[1] * C)

    def cp_q(c):
        r = blocks(QCH[c])
        return pltpu.make_async_copy(q_hbm.at[r, :], q_v.at[r, :], sem_q.at[c])

    def cp_k(c):
        b0, n = KCH[c]
        return pltpu.make_async_copy(k_hbm.at[blocks(KCH[c]), :], k_v.at[pl.ds(b0 * C + HALO, n * C), :],
                                     sem_k.at[c])

    def cp_v(c):
        r = blocks(KCH[c])
        return pltpu.make_async_copy(v_hbm.at[r, :], v_v.at[r, :], sem_v.at[c])

    def cp_h(c):
        r = blocks(KCH[c])
        return pltpu.make_async_copy(h_hbm.at[:, r], h_v.at[:, r], sem_h.at[c])

    def cp_w(c):
        r = blocks(WCH[c])
        return pltpu.make_async_copy(win_hbm.at[:, r], win_v.at[:, r], sem_w.at[c])

    def cp_wsp(i):
        r = ds(i * TA, TA, TA)
        return pltpu.make_async_copy(wsp_hbm.at[r, :], wsp_v.at[r, :], sem_wsp.at[i])

    def cp_o(a, cols=slice(None)):
        r = ds(a * C, C, C)
        return pltpu.make_async_copy(o_v.at[r, cols], o_hbm.at[r, cols], sem_o.at[0])

    cp_f = pltpu.make_async_copy(fg_hbm, fg_v, sem_m.at[0])
    cp_sk = pltpu.make_async_copy(sk_hbm, sk_v.at[:, 0:D], sem_m.at[1])
    cp_d = pltpu.make_async_copy(d_hbm, d_v, sem_m.at[2])
    cp_b = pltpu.make_async_copy(b_hbm, b_v, sem_m.at[3])
    cp_wout = pltpu.make_async_copy(wout_hbm, wout_v, sem_m.at[4])

    def hkv(c):
        return [cp_h(c), cp_k(c), cp_v(c)]

    groups = [
        [cp_q(0)], [cp_w(0)], [cp_w(1)], [cp_w(2)], [cp_q(1), cp_w(3)],
        [cp_f, cp_sk, cp_d, cp_b, cp_q(2)] + hkv(0),
        [cp_q(3)] + hkv(1),
        [cp_q(4)] + hkv(2),
    ]
    for grp in groups:
        for cp in grp:
            cp.start()

    def wait(g):
        with jax.named_scope(f'w{g}'):
            for cp in groups[g]:
                cp.wait()

    for i in range(NWSP):
        cp_wsp(i).start()
    cp_wout.start()

    k_v[0:HALO, :] = jnp.zeros((HALO, D), BF)

    c0 = math.sqrt(2.0 / math.pi)
    c1 = c0 * 0.044715

    def gelu2(x):
        t = jnp.tanh(x * (c0 + c1 * (x * x)))
        return x + x * t

    def brows(a):
        return pl.ds(a * C, C)

    def h_dft(a, dt):
        cols = slice(dt * 128, (dt + 1) * 128)
        res = jax.lax.dot_general(fg_v[0:2 * C, C:2 * C], h_v[cols, brows(a)], (((1,), (1,)), ((), ())),
                                  preferred_element_type=F32)
        hf_v[:, a, :, cols] = res.reshape(NB, 16, 128)

    def fence(tok):
        t = tok[0:8, :]
        for g in range(1, tok.shape[0] // 8):
            t = t | tok[g * 8:(g + 1) * 8, :]
        return t & pltpu.bitcast(k_v[0:HALO, 0:128], U32)

    def z2_done(a):
        return fence(pltpu.bitcast(z2_v[brows(a), 0:128], U32))

    def ln_q(a, after=None):
        r = brows(a)
        x = q_v[r, :]
        if after is not None:
            tok = pltpu.bitcast(z2_v[brows(after[0]), 0:128], U32)
            for b in after[1:]:
                tok = tok | pltpu.bitcast(z2_v[brows(b), 0:128], U32)
            zero = tok & jnp.tile(pltpu.bitcast(k_v[0:HALO, 0:128], U32), (C // 16, 1))
            x = pltpu.bitcast(pltpu.bitcast(x, U32) | jnp.tile(zero, (1, ND)), BF)
        x = x.astype(F32)
        mu = jnp.sum(x, axis=-1, keepdims=True) * (1.0 / D)
        ex2 = jnp.sum(x * x, axis=-1, keepdims=True) * (1.0 / D)
        var = jnp.maximum(ex2 - mu * mu, 0.0)
        xn_v[r, :] = ((x - mu) * jax.lax.rsqrt(var + EPS)).astype(BF)

    def u_dft(a, dt):
        cols = slice(dt * 128, (dt + 1) * 128)
        kf = k_v[pl.ds(a * C + HALO - 8, C + 8), cols].astype(F32)
        sk = sk_v[:, cols].astype(F32)
        ks = kf[8:, :] * sk[0:1, :]
        for t in range(1, 4):
            ks = ks + pltpu.roll(kf, t, axis=0)[8:, :] * sk[t:t + 1, :]
        kv = (ks * v_v[brows(a), cols].astype(F32)).astype(BF)
        res = jnp.dot(fg_v[0:2 * C, 0:C], kv, preferred_element_type=F32)
        p_v[:, a, :, cols] = res.reshape(NB, 16, 128)

    def proj(a, n, gate=None):
        lhs = xn_v[brows(a), :]
        if gate is not None:
            top = pltpu.bitcast(pltpu.bitcast(lhs[0:16, :], U32) | jnp.tile(gate, (1, ND)), BF)
            lhs = jnp.concatenate([top, lhs[16:, :]], axis=0)
        return gelu2(jnp.dot(lhs, win_v[:, n * 128:(n + 1) * 128], preferred_element_type=F32))

    def z2_tile(a, n):
        t = proj(a, NT + n)
        z1_v[pl.ds(S + (a % 2) * C, C), n * 128:(n + 1) * 128] = t
        return t

    def z1_tile(a, n, gate=None):
        t = proj(a, n, gate)
        z1_v[brows(a), n * 128:(n + 1) * 128] = t
        return t

    def ln_z2(a, gate=None):
        w2 = z1_v[pl.ds(S + (a % 2) * C, C), :]
        if gate is not None:
            left = pltpu.bitcast(pltpu.bitcast(w2[:, 0:128], U32) | jnp.tile(gate, (C // 8, 1)), F32)
            w2 = jnp.concatenate([left, w2[:, 128:]], axis=1)
        mu2 = jnp.sum(w2, axis=-1, keepdims=True) * (1.0 / FH)
        ex22 = jnp.sum(w2 * w2, axis=-1, keepdims=True) * (1.0 / FH)
        var2 = jnp.maximum(ex22 - mu2 * mu2, 0.0)
        rs2 = 0.25 * jax.lax.rsqrt(var2 + 4.0 * EPS)
        z2_v[brows(a), :] = ((w2 - mu2) * rs2).astype(BF)

    with jax.named_scope('phase1'):
        wait(0)
        ln_q(0)
        ln_q(1)
        for c in range(2):
            wait(1 + c)
            for n in range(WCH[c][0], WCH[c][0] + WCH[c][1]):
                for a in range(2):
                    z2_tile(a, n - NT)
        wait(3)
        ln_z2(0)
        z1_tile(0, 0)
        t = z1_tile(1, 0)
        z1_tile(0, 1, z2_done(0))
        ln_z2(1, fence(pltpu.bitcast(t[0:8, :], U32)) if CH else None)
        z1_tile(1, 1)
        z1_tile(0, 2)
        z1_tile(1, 2)
        z1_tile(0, 3, z2_done(1))
        z1_tile(1, 3)

        def region(blks, dfts, pre=()):
            hs = [(a, dt) for a in dfts for dt in range(ND)]
            us = list(hs)
            nb = len(blks)
            for f in pre:
                f()
            for bi, a in enumerate(blks):
                last = bi == nb - 1
                nh = len(hs) // (nb - bi)
                nu = len(us) // (nb - bi)
                slots = 2 * NT - (1 if last else 0)
                cnt = [nu * (j + 1) // slots - nu * j // slots for j in range(slots)] + [0]
                for n in range(NT):
                    z2_tile(a, n)
                    for _ in range(cnt[n]):
                        u_dft(*us.pop(0))
                nh_mid = nh if not last else max(nh - 4, 0)
                for _ in range(nh_mid):
                    h_dft(*hs.pop(0))
                ln_z2(a)
                if a + 1 < NB:
                    ln_q(a + 1, [a])
                for n in range(NT):
                    z1_tile(a, n)
                    for _ in range(cnt[NT + n]):
                        u_dft(*us.pop(0))
                for _ in range(nh - nh_mid):
                    h_dft(*hs.pop(0))
            assert not hs and not us

        wait(4)
        pre = [lambda: ln_q(2)]
        for n in range(WCH[3][0], WCH[3][0] + WCH[3][1]):
            pre += [lambda n=n: z1_tile(0, n), lambda n=n: z1_tile(1, n)]
        region([2], [], pre)
        wait(5)
        region([3, 4], [0, 1])
        wait(6)
        region([5, 6, 7, 8, 9], [2, 3, 4, 5])
        wait(7)
        region(list(range(10, 16)), list(range(6, 16)))

        dv = d_v[0:ND, :].astype(F32)
        b32_v[0:NB, :] = b_v[0:NB, :].astype(F32) * 0.25
        for dt in range(ND):
            cols = slice(dt * 128, (dt + 1) * 128)
            hf_v[:, 0, 0:8, cols] = hf_v[:, 0, 0:8, cols] + dv[dt:dt + 1, :][None]

    def conv_pos(ft, ft2, par, dt):
        cols = slice(dt * 128, (dt + 1) * 128)
        prev = None
        for a in range(NB):
            if prev is not None:
                ar, ai = -prev[1], prev[0]
            else:
                ar = ai = None
            for dl in range(a + 1):
                hr = hf_v[ft, dl, 0:8, cols]
                hi = hf_v[ft, dl, 8:16, cols]
                ur = p_v[ft, a - dl, 0:8, cols]
                ui = p_v[ft, a - dl, 8:16, cols]
                if ar is None:
                    ar, ai = ur * hr - ui * hi, ur * hi + ui * hr
                else:
                    ar = (ar + ur * hr) - ui * hi
                    ai = (ai + ur * hi) + ui * hr
            prev = (ar, ai) if prev is None else (ar + prev[1], ai - prev[0])
            w_v[a * 16 + ft2, par * 8:(par + 1) * 8, cols] = ar.astype(BF)
            w_v[a * 16 + 8 + ft2, par * 8:(par + 1) * 8, cols] = ai.astype(BF)

    def phase2a(i, carry):
        cp_wsp(i).wait()
        eye = (jax.lax.broadcasted_iota(jnp.int32, (C, C), 0)
               == jax.lax.broadcasted_iota(jnp.int32, (C, C), 1))
        for m in range(TA // MSA):
            rows = ds(i * TA + m * MSA, MSA, MSA)
            bcols = []
            for j in range(MSA // C):
                brow = b32_v[pl.ds(i * (TA // C) + m * (MSA // C) + j, 1), :]
                bcols.append(jnp.sum(jnp.where(eye, brow, 0.0), axis=-1, keepdims=True))
            bcol = jnp.concatenate(bcols, axis=0)
            for n in range(NT):
                cols = slice(n * 128, (n + 1) * 128)
                g = jnp.dot(wsp_v[rows, :], z2_v[:, cols], preferred_element_type=F32) + bcol
                gg_v[rows, cols] = (z1_v[rows, cols] * g).astype(BF)
        nft = NB * TA // S
        for ft in range(nft):
            for dt in range(ND):
                conv_pos(i * nft + ft, i * (nft // 2) + ft // 2, ft % 2, dt)
        return carry

    with jax.named_scope('phase2a'):
        jax.lax.fori_loop(0, S // TA, phase2a, 0)

    cp_wout.wait()

    def phase2b(i, carry):
        rev = 7 - jax.lax.broadcasted_iota(jnp.int32, (8, 128), 0)
        for m in range(TB // MSB):
            rows = ds(i * TB + m * MSB, MSB, MSB)
            for dt in range(ND):
                cols = slice(dt * 128, (dt + 1) * 128)
                ys = []
                for j in range(MSB // C):
                    a = i * (TB // C) + m * (MSB // C) + j
                    ev = jnp.dot(fg_v[2 * C:2 * C + C // 2, 0:C], w_v[ds(a * 16, 8, 8), :, cols].reshape(C, 128),
                                 preferred_element_type=F32)
                    od = jnp.dot(fg_v[2 * C:2 * C + C // 2, C:2 * C], w_v[ds(a * 16 + 8, 8, 8), :, cols].reshape(C, 128),
                                 preferred_element_type=F32)
                    lo = ev - od
                    for g in range(C // 16 - 1, -1, -1):
                        ys.append(jnp.take_along_axis(lo[g * 8:(g + 1) * 8, :], rev, axis=0))
                    ys.append(ev + od)
                y = jnp.concatenate(ys, axis=0)
                hh = jnp.dot(gg_v[rows, :], wout_v[:, cols], preferred_element_type=F32)
                gate = hh + hh * jnp.tanh(hh)
                s = xn_v[rows, cols].astype(F32) * y
                o_v[rows, cols] = (q_v[rows, cols].astype(F32) + s * gate).astype(BF)
                if FINE == 1 and m == TB // MSB - 1 and dt >= ND - 2:
                    cp_o(i * (TB // C) + m, slice(0, (ND - 1) * 128) if dt == ND - 2 else cols).start()
                if FINE == 2 and m == TB // MSB - 1:
                    cp_o(i * (TB // C) + m, cols).start()
            if not (FINE and m == TB // MSB - 1):
                cp_o(i * (TB // C) + m).start()
        return carry

    with jax.named_scope('phase2b'):
        jax.lax.fori_loop(0, S // TB, phase2b, 0)
    pltpu.make_async_copy(o_v, o_hbm, sem_o.at[0]).wait()


@jax.jit
def pallas_recurrent_scan__ssm_conv_h3__mixer_gmlp__prompt_kernel(
    A_q, A_k, A_v, A_shift_k, A_ssm_k, A_ssm_D, B_x, B_w_in, B_w_sp, B_b_sp, B_w_out,
):
    del B_x
    fg = jnp.asarray(_dft_consts(), dtype=BF)
    any_spec = pl.BlockSpec(memory_space=pl.ANY)
    vm = pltpu.VMEM
    dma = pltpu.SemaphoreType.DMA
    out = pl.pallas_call(
        _kernel,
        out_shape=jax.ShapeDtypeStruct((S, D), BF),
        in_specs=[any_spec] * 11,
        out_specs=any_spec,
        scratch_shapes=[
            vm((S // 2, D), U32),
            vm((S + 64, D), BF),
            vm((S, D), BF),
            vm((D // 2, S), U32),
            vm((D // 2, 2 * FH), U32),
            vm((S // 2, S), U32),
            vm((FH // 2, D), U32),
            vm(((2 * C + C // 2) // 2, 2 * C), U32),
            vm((S // 2, D), U32),
            vm((S + 2 * C, FH), F32),
            vm((S // 2, FH), U32),
            vm((NB, NB, 16, D), F32),
            vm((NB, NB, 16, D), F32),
            vm((NB * 16, 8, 1024), U32),
            vm((S // 2, FH), U32),
            vm((S, D), BF),
            vm((S // 128, 128), F32),
            vm((S // 128, 128), BF),
            vm((4, 18 * 128), BF),
            vm((D // 128, 128), BF),
            dma((len(QCH),)), dma((len(KCH),)), dma((len(KCH),)), dma((len(KCH),)),
            dma((len(WCH),)), dma((NWSP,)), dma((1,)), dma((5,)),
        ],
        compiler_params=pltpu.CompilerParams(vmem_limit_bytes=110 * 1024 * 1024,
                                             disable_semaphore_checks=bool(NOCHK & 1), disable_bounds_checks=bool(NOCHK & 2)),
    )(
        A_q.reshape(S, D), A_k.reshape(S, D), A_v.reshape(S, D),
        A_shift_k.T, A_ssm_k, A_ssm_D.reshape(D // 128, 128),
        B_w_in, B_w_sp, B_b_sp.reshape(S // 128, 128), B_w_out,
        fg,
    )
    return out.reshape(1, S, D)
```

```python
import math

import jax
import jax.numpy as jnp
import numpy as np
import jax.experimental.pallas as pl
import jax.experimental.pallas.tpu as pltpu

S = 2048
D = 640
FH = 768
C = 128
NB = S // C
ND = D // 128
NT = FH // 128
HALO = 16
EPS = 1e-5
TA = 512
TB = 1024
NLQ = 4

BF = jnp.bfloat16
F32 = jnp.float32
U32 = jnp.uint32

QCH = [(0, 2), (2, 2), (4, 2), (6, 5), (11, 5)]
HCH = [(0, 2), (2, 5), (7, 9)]
KCH = [(0, 2), (2, 3), (5, 11)]
WCH = [(6, 2), (8, 2), (10, 2), (0, 4), (4, 2)]


def _dft_consts():
    theta = np.pi * (4 * np.arange(C) + 1) / (2 * C)

    def fwd(t):
        ang = theta[:, None] * t[None, :]
        re = np.cos(ang).reshape(C // 8, 8, C)
        im = -np.sin(ang).reshape(C // 8, 8, C)
        return np.stack([re, im], axis=1).reshape(2 * C, C)

    fg = np.zeros((2 * C + C // 2, 2 * C), np.float64)
    fg[:2 * C, :C] = fwd(np.arange(C) - (C - 1) / 2)
    fg[:2 * C, C:] = fwd(np.arange(C))
    ang = (np.arange(C // 2) + 0.5)[:, None] * theta[None, :]
    fg[2 * C:, :C] = np.cos(ang) / C
    fg[2 * C:, C:] = -np.sin(ang) / C
    return fg.astype(np.float32).astype(BF)


def _kernel(q_hbm, k_hbm, v_hbm, sk_hbm, h_hbm, d_hbm, win_hbm, wsp_hbm, b_hbm, wout_hbm,
            fg_hbm, o_hbm,
            q_u, k_v, v_v, h_u, win_u, wsp_u, wout_u, fg_u,
            xn_u, z1_v, z2_u, p_v, hf_v, w_u, gg_u, o_v, b32_v, b_v, sk_v, d_v,
            sem_q, sem_k, sem_v, sem_h, sem_w, sem_wsp, sem_o, sem_m):
    q_v = q_u.bitcast(BF)
    h_v = h_u.bitcast(BF)
    win_v = win_u.bitcast(BF)
    wsp_v = wsp_u.bitcast(BF)
    wout_v = wout_u.bitcast(BF)
    fg_v = fg_u.bitcast(BF)
    xn_v = xn_u.bitcast(BF)
    z2_v = z2_u.bitcast(BF)
    w_v = w_u.bitcast(BF)
    gg_v = gg_u.bitcast(BF)

    def ds(start, size):
        if isinstance(start, int):
            return pl.ds(start, size)
        return pl.ds(pl.multiple_of(start, size), size)

    def lanes(n):
        return slice(n * 128, (n + 1) * 128)

    def blocks(ch):
        return pl.ds(ch[0] * C, ch[1] * C)

    def brows(a):
        return ds(a * C, C)

    def cp_q(c):
        r = blocks(QCH[c])
        return pltpu.make_async_copy(q_hbm.at[r, :], q_v.at[r, :], sem_q.at[c])

    def cp_k(c):
        b0, n = KCH[c]
        return pltpu.make_async_copy(k_hbm.at[blocks(KCH[c]), :],
                                     k_v.at[pl.ds(b0 * C + HALO, n * C), :], sem_k.at[c])

    def cp_v(c):
        r = blocks(KCH[c])
        return pltpu.make_async_copy(v_hbm.at[r, :], v_v.at[r, :], sem_v.at[c])

    def cp_h(c):
        r = blocks(HCH[c])
        return pltpu.make_async_copy(h_hbm.at[:, r], h_v.at[:, r], sem_h.at[c])

    def cp_w(c):
        r = blocks(WCH[c])
        return pltpu.make_async_copy(win_hbm.at[:, r], win_v.at[:, r], sem_w.at[c])

    def cp_wsp(i):
        r = ds(i * TA, TA)
        return pltpu.make_async_copy(wsp_hbm.at[r, :], wsp_v.at[r, :], sem_wsp.at[i])

    def cp_o(a, cols=slice(None)):
        r = brows(a)
        return pltpu.make_async_copy(o_v.at[r, cols], o_hbm.at[r, cols], sem_o.at[0])

    cp_f = pltpu.make_async_copy(fg_hbm, fg_v, sem_m.at[0])
    cp_sk = pltpu.make_async_copy(sk_hbm, sk_v.at[:, 0:D], sem_m.at[1])
    cp_d = pltpu.make_async_copy(d_hbm, d_v, sem_m.at[2])
    cp_b = pltpu.make_async_copy(b_hbm, b_v, sem_m.at[3])
    cp_wout = pltpu.make_async_copy(wout_hbm, wout_v, sem_m.at[4])

    groups = [
        [cp_q(0)], [cp_w(0)], [cp_w(1)], [cp_w(2)], [cp_w(3)], [cp_q(1), cp_w(4)],
        [cp_f, cp_sk, cp_d, cp_b, cp_q(2), cp_h(0), cp_k(0), cp_v(0)],
        [cp_q(3), cp_h(1), cp_k(1), cp_v(1)],
        [cp_q(4), cp_h(2), cp_k(2), cp_v(2)],
    ]
    for grp in groups:
        for cp in grp:
            cp.start()
    for i in range(S // TA):
        cp_wsp(i).start()
    cp_wout.start()

    def wait(g):
        for cp in groups[g]:
            cp.wait()

    k_v[0:HALO, :] = jnp.zeros((HALO, D), BF)

    c0 = math.sqrt(2.0 / math.pi)
    c1 = c0 * 0.044715

    def gelu2(x):
        return x + x * jnp.tanh(x * (c0 + c1 * (x * x)))

    def fence(tok):
        t = tok[0:8, :]
        for g in range(1, tok.shape[0] // 8):
            t = t | tok[g * 8:(g + 1) * 8, :]
        return t & pltpu.bitcast(k_v[0:HALO, 0:128], U32)

    def z2_words(a):
        return pltpu.bitcast(z2_v[brows(a), 0:128], U32)

    def ln_q(a, gate=None, part=0, nparts=1):
        n = C // nparts
        r = pl.ds(a * C + part * n, n)
        x = q_v[r, :]
        if gate is not None:
            x = pltpu.bitcast(pltpu.bitcast(x, U32) | jnp.tile(gate, (n // 16, ND)), BF)
        x = x.astype(F32)
        mu = jnp.sum(x, axis=-1, keepdims=True) * (1.0 / D)
        ex2 = jnp.sum(x * x, axis=-1, keepdims=True) * (1.0 / D)
        var = jnp.maximum(ex2 - mu * mu, 0.0)
        xn_v[r, :] = ((x - mu) * jax.lax.rsqrt(var + EPS)).astype(BF)

    def h_dft(a, dt):
        res = jax.lax.dot_general(fg_v[0:2 * C, C:2 * C], h_v[lanes(dt), brows(a)],
                                  (((1,), (1,)), ((), ())), preferred_element_type=F32)
        hf_v[:, a, :, lanes(dt)] = res.reshape(NB, 16, 128)

    def u_dft(a, dt):
        cols = lanes(dt)
        kf = k_v[pl.ds(a * C + HALO - 8, C + 8), cols].astype(F32)
        sk = sk_v[:, cols].astype(F32)
        ks = kf[8:, :] * sk[0:1, :]
        for t in range(1, 4):
            ks = ks + pltpu.roll(kf, t, axis=0)[8:, :] * sk[t:t + 1, :]
        kv = (ks * v_v[brows(a), cols].astype(F32)).astype(BF)
        res = jnp.dot(fg_v[0:2 * C, 0:C], kv, preferred_element_type=F32)
        p_v[:, a, :, cols] = res.reshape(NB, 16, 128)

    def proj(a, n, gate=None):
        lhs = xn_v[brows(a), :]
        if gate is not None:
            top = pltpu.bitcast(pltpu.bitcast(lhs[0:16, :], U32) | jnp.tile(gate, (1, ND)), BF)
            lhs = jnp.concatenate([top, lhs[16:, :]], axis=0)
        return gelu2(jnp.dot(lhs, win_v[:, lanes(n)], preferred_element_type=F32))

    def w2_rows(a):
        return pl.ds(S + (a % 2) * C, C)

    def z2_tile(a, n):
        z1_v[w2_rows(a), lanes(n)] = proj(a, NT + n)

    def z1_tile(a, n, gate=None):
        t = proj(a, n, gate)
        z1_v[brows(a), lanes(n)] = t
        return t

    def ln_z2(a):
        w2 = z1_v[w2_rows(a), :]
        mu = jnp.sum(w2, axis=-1, keepdims=True) * (1.0 / FH)
        ex2 = jnp.sum(w2 * w2, axis=-1, keepdims=True) * (1.0 / FH)
        var = jnp.maximum(ex2 - mu * mu, 0.0)
        rs = 0.25 * jax.lax.rsqrt(var + 4.0 * EPS)
        z2_v[brows(a), :] = ((w2 - mu) * rs).astype(BF)

    def region(blks, hch=(0, 0), kch=(0, 0)):
        hs = [(a, dt) for a in range(hch[0], hch[0] + hch[1]) for dt in range(ND)]
        us = [(a, dt) for a in range(kch[0], kch[0] + kch[1]) for dt in range(ND)]
        for bi, a in enumerate(blks):
            last = bi == len(blks) - 1
            nh = len(hs) // (len(blks) - bi)
            nu = len(us) // (len(blks) - bi)
            slots = 2 * NT - (1 if last else 0)
            cnt = [nu * (j + 1) // slots - nu * j // slots for j in range(slots)] + [0]
            for n in range(NT):
                z2_tile(a, n)
                for _ in range(cnt[n]):
                    u_dft(*us.pop(0))
            nh_mid = max(nh - 4, 0) if last else nh
            for _ in range(nh_mid):
                h_dft(*hs.pop(0))
            ln_z2(a)
            for n in range(NT):
                t = z1_tile(a, n)
                if a + 1 < NB and n < NLQ:
                    tok = pltpu.bitcast(t[0:8, :], U32)
                    if n == 0:
                        tok = jnp.concatenate([tok, z2_words(a)], axis=0)
                    ln_q(a + 1, fence(tok), n, NLQ)
                for _ in range(cnt[NT + n]):
                    u_dft(*us.pop(0))
            for _ in range(nh - nh_mid):
                h_dft(*hs.pop(0))
        assert not hs and not us

    wait(0)
    ln_q(0)
    ln_q(1)
    for c in range(3):
        wait(1 + c)
        for n in range(WCH[c][0], WCH[c][0] + WCH[c][1]):
            z2_tile(0, n - NT)
            z2_tile(1, n - NT)
    wait(4)
    ln_z2(0)
    ln_z2(1)
    z1_tile(0, 0)
    z1_tile(1, 0)
    z1_tile(0, 1, fence(z2_words(0)))
    z1_tile(1, 1)
    z1_tile(0, 2)
    z1_tile(1, 2)
    z1_tile(0, 3, fence(z2_words(1)))
    z1_tile(1, 3)
    wait(5)
    ln_q(2)
    for n in range(WCH[4][0], WCH[4][0] + WCH[4][1]):
        z1_tile(0, n)
        z1_tile(1, n)
    region([2])
    wait(6)
    region([3, 4], HCH[0], KCH[0])
    wait(7)
    region(list(range(5, QCH[4][0] - 1)), HCH[1], KCH[1])
    wait(8)
    region(list(range(QCH[4][0] - 1, NB)), HCH[2], KCH[2])

    dv = d_v[...].astype(F32)
    for dt in range(ND):
        hf_v[:, 0, 0:8, lanes(dt)] = hf_v[:, 0, 0:8, lanes(dt)] + dv[dt:dt + 1, :][None]
    b32_v[...] = b_v[...].astype(F32) * 0.25

    def conv_pos(ft, ft2, par, dt):
        cols = lanes(dt)
        prev = None
        for a in range(NB):
            ar, ai = (None, None) if prev is None else (-prev[1], prev[0])
            for dl in range(a + 1):
                hr = hf_v[ft, dl, 0:8, cols]
                hi = hf_v[ft, dl, 8:16, cols]
                ur = p_v[ft, a - dl, 0:8, cols]
                ui = p_v[ft, a - dl, 8:16, cols]
                if ar is None:
                    ar, ai = ur * hr - ui * hi, ur * hi + ui * hr
                else:
                    ar = (ar + ur * hr) - ui * hi
                    ai = (ai + ur * hi) + ui * hr
            prev = (ar, ai) if prev is None else (ar + prev[1], ai - prev[0])
            w_v[a * 16 + ft2, par * 8:(par + 1) * 8, cols] = ar.astype(BF)
            w_v[a * 16 + 8 + ft2, par * 8:(par + 1) * 8, cols] = ai.astype(BF)

    def phase2a(i, carry):
        cp_wsp(i).wait()
        eye = (jax.lax.broadcasted_iota(jnp.int32, (C, C), 0)
               == jax.lax.broadcasted_iota(jnp.int32, (C, C), 1))
        for m in range(TA // C):
            a = i * (TA // C) + m
            rows = brows(a)
            bcol = jnp.sum(jnp.where(eye, b32_v[pl.ds(a, 1), :], 0.0), axis=-1, keepdims=True)
            for n in range(NT):
                g = jnp.dot(wsp_v[rows, :], z2_v[:, lanes(n)], preferred_element_type=F32) + bcol
                gg_v[rows, lanes(n)] = (z1_v[rows, lanes(n)] * g).astype(BF)
        nft = NB * TA // S
        for ft in range(nft):
            for dt in range(ND):
                conv_pos(i * nft + ft, i * (nft // 2) + ft // 2, ft % 2, dt)
        return carry

    jax.lax.fori_loop(0, S // TA, phase2a, 0)

    cp_wout.wait()

    def phase2b(i, carry):
        rev = 7 - jax.lax.broadcasted_iota(jnp.int32, (8, 128), 0)
        for m in range(TB // C):
            a = i * (TB // C) + m
            rows = brows(a)
            last = m == TB // C - 1
            for dt in range(ND):
                cols = lanes(dt)
                ev = jnp.dot(fg_v[2 * C:2 * C + C // 2, 0:C],
                             w_v[ds(a * 16, 8), :, cols].reshape(C, 128), preferred_element_type=F32)
                od = jnp.dot(fg_v[2 * C:2 * C + C // 2, C:2 * C],
                             w_v[ds(a * 16 + 8, 8), :, cols].reshape(C, 128), preferred_element_type=F32)
                lo = ev - od
                ys = [jnp.take_along_axis(lo[g * 8:(g + 1) * 8, :], rev, axis=0)
                      for g in range(C // 16 - 1, -1, -1)]
                y = jnp.concatenate(ys + [ev + od], axis=0)
                hh = jnp.dot(gg_v[rows, :], wout_v[:, cols], preferred_element_type=F32)
                gate = hh + hh * jnp.tanh(hh)
                s = xn_v[rows, cols].astype(F32) * y
                o_v[rows, cols] = (q_v[rows, cols].astype(F32) + s * gate).astype(BF)
                if last:
                    cp_o(a, cols).start()
            if not last:
                cp_o(a).start()
        return carry

    jax.lax.fori_loop(0, S // TB, phase2b, 0)
    pltpu.make_async_copy(o_v, o_hbm, sem_o.at[0]).wait()


@jax.jit
def pallas_recurrent_scan__ssm_conv_h3__mixer_gmlp__prompt_kernel(
    A_q: jax.Array,
    A_k: jax.Array,
    A_v: jax.Array,
    A_shift_k: jax.Array,
    A_ssm_k: jax.Array,
    A_ssm_D: jax.Array,
    B_x: jax.Array,
    B_w_in: jax.Array,
    B_w_sp: jax.Array,
    B_b_sp: jax.Array,
    B_w_out: jax.Array,
):
    del B_x
    any_spec = pl.BlockSpec(memory_space=pl.ANY)
    vm = pltpu.VMEM
    dma = pltpu.SemaphoreType.DMA
    out = pl.pallas_call(
        _kernel,
        out_shape=jax.ShapeDtypeStruct((S, D), BF),
        in_specs=[any_spec] * 11,
        out_specs=any_spec,
        scratch_shapes=[
            vm((S // 2, D), U32),
            vm((S + 64, D), BF),
            vm((S, D), BF),
            vm((D // 2, S), U32),
            vm((D // 2, 2 * FH), U32),
            vm((S // 2, S), U32),
            vm((FH // 2, D), U32),
            vm(((2 * C + C // 2) // 2, 2 * C), U32),
            vm((S // 2, D), U32),
            vm((S + 2 * C, FH), F32),
            vm((S // 2, FH), U32),
            vm((NB, NB, 16, D), F32),
            vm((NB, NB, 16, D), F32),
            vm((NB * 16, 8, 1024), U32),
            vm((S // 2, FH), U32),
            vm((S, D), BF),
            vm((NB, 128), F32),
            vm((NB, 128), BF),
            vm((4, 18 * 128), BF),
            vm((ND, 128), BF),
            dma((len(QCH),)), dma((len(KCH),)), dma((len(KCH),)), dma((len(HCH),)),
            dma((len(WCH),)), dma((S // TA,)), dma((1,)), dma((5,)),
        ],
        compiler_params=pltpu.CompilerParams(
            vmem_limit_bytes=110 * 1024 * 1024,
            disable_bounds_checks=True,
            disable_semaphore_checks=True,
        ),
    )(
        A_q.reshape(S, D), A_k.reshape(S, D), A_v.reshape(S, D),
        A_shift_k.T, A_ssm_k, A_ssm_D.reshape(ND, 128),
        B_w_in, B_w_sp, B_b_sp.reshape(NB, 128), B_w_out,
        _dft_consts(),
    )
    return out.reshape(1, S, D)
```

```python
import math

import jax
import jax.numpy as jnp
import numpy as np
import jax.experimental.pallas as pl
import jax.experimental.pallas.tpu as pltpu

S = 2048
D = 640
FH = 768
C = 128
NB = S // C
ND = D // 128
NT = FH // 128
HALO = 16
EPS = 1e-5
TA = 512
TB = 1024
NLQ = 4

BF = jnp.bfloat16
F32 = jnp.float32
U32 = jnp.uint32

QCH = [(0, 2), (2, 2), (4, 2), (6, 5), (11, 5)]
HCH = [(0, 2), (2, 5), (7, 9)]
KCH = [(0, 2), (2, 3), (5, 11)]
WCH = [(6, 2), (8, 2), (10, 2), (0, 4), (4, 2)]
U_SLOTS = [1, 3, 0, 2, 4, 11, 12, 5, 6, 6, 10, 9]
U_SLOTS_EARLY = [1, 3, 8, 10, 0, 2, 7, 9, 11, 4, 12, 5]


def _dft_consts():
    theta = np.pi * (4 * np.arange(C) + 1) / (2 * C)

    def fwd(t):
        ang = theta[:, None] * t[None, :]
        re = np.cos(ang).reshape(C // 8, 8, C)
        im = -np.sin(ang).reshape(C // 8, 8, C)
        return np.stack([re, im], axis=1).reshape(2 * C, C)

    fg = np.zeros((2 * C + C // 2, 2 * C), np.float64)
    fg[:2 * C, :C] = fwd(np.arange(C) - (C - 1) / 2)
    fg[:2 * C, C:] = fwd(np.arange(C))
    ang = (np.arange(C // 2) + 0.5)[:, None] * theta[None, :]
    fg[2 * C:, :C] = np.cos(ang) / C
    fg[2 * C:, C:] = -np.sin(ang) / C
    return fg.astype(np.float32).astype(BF)


def _kernel(q_hbm, k_hbm, v_hbm, sk_hbm, h_hbm, d_hbm, win_hbm, wsp_hbm, b_hbm, wout_hbm,
            fg_hbm, o_hbm,
            q_u, k_v, v_v, h_u, win_u, wsp_u, wout_u, fg_u,
            xn_u, z1_v, z2_u, p_v, hf_v, w_u, gg_u, o_v, b32_v, b_v, sk_v, d_v,
            sem_q, sem_k, sem_v, sem_h, sem_w, sem_wsp, sem_o, sem_m):
    q_v = q_u.bitcast(BF)
    h_v = h_u.bitcast(BF)
    win_v = win_u.bitcast(BF)
    wsp_v = wsp_u.bitcast(BF)
    wout_v = wout_u.bitcast(BF)
    fg_v = fg_u.bitcast(BF)
    xn_v = xn_u.bitcast(BF)
    z2_v = z2_u.bitcast(BF)
    w_v = w_u.bitcast(BF)
    gg_v = gg_u.bitcast(BF)

    def ds(start, size):
        if isinstance(start, int):
            return pl.ds(start, size)
        return pl.ds(pl.multiple_of(start, size), size)

    def lanes(n):
        return slice(n * 128, (n + 1) * 128)

    def blocks(ch):
        return pl.ds(ch[0] * C, ch[1] * C)

    def brows(a):
        return ds(a * C, C)

    def cp_q(c):
        r = blocks(QCH[c])
        return pltpu.make_async_copy(q_hbm.at[r, :], q_v.at[r, :], sem_q.at[c])

    def cp_k(c):
        b0, n = KCH[c]
        return pltpu.make_async_copy(k_hbm.at[blocks(KCH[c]), :],
                                     k_v.at[pl.ds(b0 * C + HALO, n * C), :], sem_k.at[c])

    def cp_v(c):
        r = blocks(KCH[c])
        return pltpu.make_async_copy(v_hbm.at[r, :], v_v.at[r, :], sem_v.at[c])

    def cp_h(c):
        r = blocks(HCH[c])
        return pltpu.make_async_copy(h_hbm.at[:, r], h_v.at[:, r], sem_h.at[c])

    def cp_w(c):
        r = blocks(WCH[c])
        return pltpu.make_async_copy(win_hbm.at[:, r], win_v.at[:, r], sem_w.at[c])

    def cp_wsp(i):
        r = ds(i * TA, TA)
        return pltpu.make_async_copy(wsp_hbm.at[r, :], wsp_v.at[r, :], sem_wsp.at[i])

    def cp_o(a, cols=slice(None)):
        r = brows(a)
        return pltpu.make_async_copy(o_v.at[r, cols], o_hbm.at[r, cols], sem_o.at[0])

    cp_f = pltpu.make_async_copy(fg_hbm, fg_v, sem_m.at[0])
    cp_sk = pltpu.make_async_copy(sk_hbm, sk_v.at[:, 0:D], sem_m.at[1])
    cp_d = pltpu.make_async_copy(d_hbm, d_v, sem_m.at[2])
    cp_b = pltpu.make_async_copy(b_hbm, b_v, sem_m.at[3])
    cp_wout = pltpu.make_async_copy(wout_hbm, wout_v, sem_m.at[4])

    groups = [
        [cp_q(0)], [cp_w(0)], [cp_w(1)], [cp_w(2)], [cp_w(3)], [cp_q(1), cp_w(4)],
        [cp_f, cp_sk, cp_d, cp_b, cp_q(2), cp_h(0), cp_k(0), cp_v(0)],
        [cp_q(3), cp_h(1), cp_k(1), cp_v(1)],
        [cp_q(4), cp_h(2), cp_k(2), cp_v(2)],
    ]
    for grp in groups:
        for cp in grp:
            cp.start()
    for i in range(S // TA):
        cp_wsp(i).start()
    cp_wout.start()

    def wait(g):
        for cp in groups[g]:
            cp.wait()

    k_v[0:HALO, :] = jnp.zeros((HALO, D), BF)

    c0 = math.sqrt(2.0 / math.pi)
    c1 = c0 * 0.044715

    def gelu2(x):
        return x + x * jnp.tanh(x * (c0 + c1 * (x * x)))

    def fence(tok):
        t = tok[0:8, :]
        for g in range(1, tok.shape[0] // 8):
            t = t | tok[g * 8:(g + 1) * 8, :]
        return t & pltpu.bitcast(k_v[0:HALO, 0:128], U32)

    def z2_words(a):
        return pltpu.bitcast(z2_v[brows(a), 0:128], U32)

    def ln_q(a, gate=None, part=0, nparts=1):
        n = C // nparts
        r = pl.ds(a * C + part * n, n)
        x = q_v[r, :]
        if gate is not None:
            x = pltpu.bitcast(pltpu.bitcast(x, U32) | jnp.tile(gate, (n // 16, ND)), BF)
        x = x.astype(F32)
        mu = jnp.sum(x, axis=-1, keepdims=True) * (1.0 / D)
        ex2 = jnp.sum(x * x, axis=-1, keepdims=True) * (1.0 / D)
        var = jnp.maximum(ex2 - mu * mu, 0.0)
        xn_v[r, :] = ((x - mu) * jax.lax.rsqrt(var + EPS)).astype(BF)

    def h_dft(a, dt):
        res = jax.lax.dot_general(fg_v[0:2 * C, C:2 * C], h_v[lanes(dt), brows(a)],
                                  (((1,), (1,)), ((), ())), preferred_element_type=F32)
        hf_v[:, a, :, lanes(dt)] = res.reshape(NB, 16, 128)
        return res

    def u_dft(a, dt):
        cols = lanes(dt)
        kf = k_v[pl.ds(a * C + HALO - 8, C + 8), cols].astype(F32)
        sk = sk_v[:, cols].astype(F32)
        ks = kf[8:, :] * sk[0:1, :]
        for t in range(1, 4):
            ks = ks + pltpu.roll(kf, t, axis=0)[8:, :] * sk[t:t + 1, :]
        kv = (ks * v_v[brows(a), cols].astype(F32)).astype(BF)
        res = jnp.dot(fg_v[0:2 * C, 0:C], kv, preferred_element_type=F32)
        p_v[:, a, :, cols] = res.reshape(NB, 16, 128)

    def proj(a, n, gate=None):
        lhs = xn_v[brows(a), :]
        if gate is not None:
            top = pltpu.bitcast(pltpu.bitcast(lhs[0:16, :], U32) | jnp.tile(gate, (1, ND)), BF)
            lhs = jnp.concatenate([top, lhs[16:, :]], axis=0)
        return gelu2(jnp.dot(lhs, win_v[:, lanes(n)], preferred_element_type=F32))

    def w2_rows(a):
        return pl.ds(S + (a % 2) * C, C)

    def z2_tile(a, n):
        z1_v[w2_rows(a), lanes(n)] = proj(a, NT + n)

    def z1_tile(a, n, gate=None):
        t = proj(a, n, gate)
        z1_v[brows(a), lanes(n)] = t
        return t

    def ln_z2(a):
        w2 = z1_v[w2_rows(a), :]
        mu = jnp.sum(w2, axis=-1, keepdims=True) * (1.0 / FH)
        ex2 = jnp.sum(w2 * w2, axis=-1, keepdims=True) * (1.0 / FH)
        var = jnp.maximum(ex2 - mu * mu, 0.0)
        rs = 0.25 * jax.lax.rsqrt(var + 4.0 * EPS)
        z2_v[brows(a), :] = ((w2 - mu) * rs).astype(BF)

    def region(blks, hch=(0, 0), kch=(0, 0)):
        hs = [(a, dt) for a in range(hch[0], hch[0] + hch[1]) for dt in range(ND)]
        us = [(a, dt) for a in range(kch[0], kch[0] + kch[1]) for dt in range(ND)]

        def next_ln_q(a, n, t):
            tok = pltpu.bitcast(t, U32)
            if n == 0:
                tok = jnp.concatenate([tok, z2_words(a)], axis=0)
            ln_q(a + 1, fence(tok), n, NLQ)

        for bi, a in enumerate(blks):
            last = bi == len(blks) - 1
            nh = len(hs) // (len(blks) - bi)
            nu = len(us) // (len(blks) - bi)
            nh_mid = max(nh - 4, 0) if last else nh
            early_ln = nh_mid >= 6 and a + 1 < NB
            slots = [x for x in (U_SLOTS_EARLY if early_ln else U_SLOTS) if not (last and x == 2 * NT)]
            cnt = [0] * (2 * NT + 1)
            for j in range(nu):
                cnt[slots[j % len(slots)]] += 1
            for n in range(NT):
                z2_tile(a, n)
                for _ in range(cnt[n]):
                    u_dft(*us.pop(0))
            hres = [h_dft(*hs.pop(0)) for _ in range(nh_mid)]
            for _ in range(cnt[NT]):
                u_dft(*us.pop(0))
            ln_z2(a)
            if early_ln:
                for n in range(NLQ):
                    next_ln_q(a, n, hres[4][n * 64:n * 64 + 8, :])
            for n in range(NT):
                t = z1_tile(a, n)
                if a + 1 < NB and n < NLQ and not early_ln:
                    next_ln_q(a, n, t[0:8, :])
                for _ in range(cnt[NT + 1 + n]):
                    u_dft(*us.pop(0))
            for _ in range(nh - nh_mid):
                h_dft(*hs.pop(0))
        assert not hs and not us

    wait(0)
    ln_q(0)
    ln_q(1)
    for c in range(3):
        wait(1 + c)
        for n in range(WCH[c][0], WCH[c][0] + WCH[c][1]):
            z2_tile(0, n - NT)
            z2_tile(1, n - NT)
    wait(4)
    ln_z2(0)
    ln_z2(1)
    z1_tile(0, 0)
    z1_tile(1, 0)
    z1_tile(0, 1, fence(z2_words(0)))
    z1_tile(1, 1)
    z1_tile(0, 2)
    z1_tile(1, 2)
    z1_tile(0, 3, fence(z2_words(1)))
    z1_tile(1, 3)
    wait(5)
    ln_q(2)
    for n in range(WCH[4][0], WCH[4][0] + WCH[4][1]):
        z1_tile(0, n)
        z1_tile(1, n)
    region([2])
    wait(6)
    region([3, 4], HCH[0], KCH[0])
    wait(7)
    region(list(range(5, QCH[4][0] - 1)), HCH[1], KCH[1])
    wait(8)
    region(list(range(QCH[4][0] - 1, NB)), HCH[2], KCH[2])

    dv = d_v[...].astype(F32)
    for dt in range(ND):
        hf_v[:, 0, 0:8, lanes(dt)] = hf_v[:, 0, 0:8, lanes(dt)] + dv[dt:dt + 1, :][None]
    b32_v[...] = b_v[...].astype(F32) * 0.25

    def conv_pos(ft, ft2, par, dt, after):
        cols = lanes(dt)
        prev = None
        for a in range(NB):
            ar, ai = (None, None) if prev is None else (-prev[1], prev[0])
            for dl in range(a + 1):
                hr = hf_v[ft, dl, 0:8, cols]
                hi = hf_v[ft, dl, 8:16, cols]
                ur = p_v[ft, a - dl, 0:8, cols]
                ui = p_v[ft, a - dl, 8:16, cols]
                if ar is None:
                    ar, ai = ur * hr - ui * hi, ur * hi + ui * hr
                    if after is not None:
                        z = fence(pltpu.bitcast(after, U32))
                        ar = pltpu.bitcast(pltpu.bitcast(ar, U32) | z, F32)
                        ai = pltpu.bitcast(pltpu.bitcast(ai, U32) | z, F32)
                else:
                    ar = (ar + ur * hr) - ui * hi
                    ai = (ai + ur * hi) + ui * hr
            prev = (ar, ai) if prev is None else (ar + prev[1], ai - prev[0])
            w_v[a * 16 + ft2, par * 8:(par + 1) * 8, cols] = ar.astype(BF)
            w_v[a * 16 + 8 + ft2, par * 8:(par + 1) * 8, cols] = ai.astype(BF)
        return prev[0]

    def phase2a(i, carry):
        cp_wsp(i).wait()
        eye = (jax.lax.broadcasted_iota(jnp.int32, (C, C), 0)
               == jax.lax.broadcasted_iota(jnp.int32, (C, C), 1))
        for m in range(TA // C):
            a = i * (TA // C) + m
            rows = brows(a)
            bcol = jnp.sum(jnp.where(eye, b32_v[pl.ds(a, 1), :], 0.0), axis=-1, keepdims=True)
            for n in range(NT):
                g = jnp.dot(wsp_v[rows, :], z2_v[:, lanes(n)], preferred_element_type=F32) + bcol
                gg_v[rows, lanes(n)] = (z1_v[rows, lanes(n)] * g).astype(BF)
        nft = NB * TA // S
        last = None
        for ft in range(nft):
            for dt in range(ND):
                last = conv_pos(i * nft + ft, i * (nft // 2) + ft // 2, ft % 2, dt, last)
        return carry

    jax.lax.fori_loop(0, S // TA, phase2a, 0)

    cp_wout.wait()

    def phase2b(i, carry):
        rev = 7 - jax.lax.broadcasted_iota(jnp.int32, (8, 128), 0)
        for m in range(TB // C):
            a = i * (TB // C) + m
            rows = brows(a)
            last = m == TB // C - 1
            for dt in range(ND):
                cols = lanes(dt)
                ev = jnp.dot(fg_v[2 * C:2 * C + C // 2, 0:C],
                             w_v[ds(a * 16, 8), :, cols].reshape(C, 128), preferred_element_type=F32)
                od = jnp.dot(fg_v[2 * C:2 * C + C // 2, C:2 * C],
                             w_v[ds(a * 16 + 8, 8), :, cols].reshape(C, 128), preferred_element_type=F32)
                lo = ev - od
                ys = [jnp.take_along_axis(lo[g * 8:(g + 1) * 8, :], rev, axis=0)
                      for g in range(C // 16 - 1, -1, -1)]
                y = jnp.concatenate(ys + [ev + od], axis=0)
                hh = jnp.dot(gg_v[rows, :], wout_v[:, cols], preferred_element_type=F32)
                gate = hh + hh * jnp.tanh(hh)
                s = xn_v[rows, cols].astype(F32) * y
                o_v[rows, cols] = (q_v[rows, cols].astype(F32) + s * gate).astype(BF)
                if last:
                    cp_o(a, cols).start()
            if not last:
                cp_o(a).start()
        return carry

    jax.lax.fori_loop(0, S // TB, phase2b, 0)
    pltpu.make_async_copy(o_v, o_hbm, sem_o.at[0]).wait()


@jax.jit
def pallas_recurrent_scan__ssm_conv_h3__mixer_gmlp__prompt_kernel(
    A_q: jax.Array,
    A_k: jax.Array,
    A_v: jax.Array,
    A_shift_k: jax.Array,
    A_ssm_k: jax.Array,
    A_ssm_D: jax.Array,
    B_x: jax.Array,
    B_w_in: jax.Array,
    B_w_sp: jax.Array,
    B_b_sp: jax.Array,
    B_w_out: jax.Array,
):
    del B_x
    any_spec = pl.BlockSpec(memory_space=pl.ANY)
    vm = pltpu.VMEM
    dma = pltpu.SemaphoreType.DMA
    out = pl.pallas_call(
        _kernel,
        out_shape=jax.ShapeDtypeStruct((S, D), BF),
        in_specs=[any_spec] * 11,
        out_specs=any_spec,
        scratch_shapes=[
            vm((S // 2, D), U32),
            vm((S + 64, D), BF),
            vm((S, D), BF),
            vm((D // 2, S), U32),
            vm((D // 2, 2 * FH), U32),
            vm((S // 2, S), U32),
            vm((FH // 2, D), U32),
            vm(((2 * C + C // 2) // 2, 2 * C), U32),
            vm((S // 2, D), U32),
            vm((S + 2 * C, FH), F32),
            vm((S // 2, FH), U32),
            vm((NB, NB, 16, D), F32),
            vm((NB, NB, 16, D), F32),
            vm((NB * 16, 8, 1024), U32),
            vm((S // 2, FH), U32),
            vm((S, D), BF),
            vm((NB, 128), F32),
            vm((NB, 128), BF),
            vm((4, 18 * 128), BF),
            vm((ND, 128), BF),
            dma((len(QCH),)), dma((len(KCH),)), dma((len(KCH),)), dma((len(HCH),)),
            dma((len(WCH),)), dma((S // TA,)), dma((1,)), dma((5,)),
        ],
        compiler_params=pltpu.CompilerParams(
            vmem_limit_bytes=110 * 1024 * 1024,
            disable_bounds_checks=True,
            disable_semaphore_checks=True,
        ),
    )(
        A_q.reshape(S, D), A_k.reshape(S, D), A_v.reshape(S, D),
        A_shift_k.T, A_ssm_k, A_ssm_D.reshape(ND, 128),
        B_w_in, B_w_sp, B_b_sp.reshape(NB, 128), B_w_out,
        _dft_consts(),
    )
    return out.reshape(1, S, D)
```

```python
import math

import jax
import jax.numpy as jnp
import numpy as np
import jax.experimental.pallas as pl
import jax.experimental.pallas.tpu as pltpu

S = 2048
D = 640
FH = 768
C = 128
NB = S // C
ND = D // 128
NT = FH // 128
HALO = 16
EPS = 1e-5
TA = 512
TB = 1024
NLQ = 4

BF = jnp.bfloat16
F32 = jnp.float32
U32 = jnp.uint32

QCH = [(0, 2), (2, 2), (4, 2), (6, 5), (11, 5)]
HCH = [(0, 2), (2, 5), (7, 9)]
KCH = [(0, 2), (2, 3), (5, 11)]
WCH = [(6, 2), (8, 2), (10, 2), (0, 4), (4, 2)]
U_SLOTS = [1, 3, 0, 2, 4, 11, 12, 5, 6, 6, 10, 9]
U_SLOTS_EARLY = [1, 3, 7, 9, 0, 2, 11, 12, 4, 5, 8, 10]


def _dft_consts():
    theta = np.pi * (4 * np.arange(C) + 1) / (2 * C)

    def fwd(t):
        ang = theta[:, None] * t[None, :]
        re = np.cos(ang).reshape(C // 8, 8, C)
        im = -np.sin(ang).reshape(C // 8, 8, C)
        return np.stack([re, im], axis=1).reshape(2 * C, C)

    fg = np.zeros((2 * C + C // 2, 2 * C), np.float64)
    fg[:2 * C, :C] = fwd(np.arange(C) - (C - 1) / 2)
    fg[:2 * C, C:] = fwd(np.arange(C))
    ang = (np.arange(C // 2) + 0.5)[:, None] * theta[None, :]
    fg[2 * C:, :C] = np.cos(ang) / C
    fg[2 * C:, C:] = -np.sin(ang) / C
    return fg.astype(np.float32).astype(BF)


def _kernel(q_hbm, k_hbm, v_hbm, sk_hbm, h_hbm, d_hbm, win_hbm, wsp_hbm, b_hbm, wout_hbm,
            fg_hbm, o_hbm,
            q_u, k_v, v_v, h_u, win_u, wsp_u, wout_u, fg_u,
            xn_u, z1_v, z2_u, p_v, hf_v, w_u, gg_u, o_v, b32_v, b_v, sk_v, d_v,
            sem_q, sem_k, sem_v, sem_h, sem_w, sem_wsp, sem_o, sem_m):
    q_v = q_u.bitcast(BF)
    h_v = h_u.bitcast(BF)
    win_v = win_u.bitcast(BF)
    wsp_v = wsp_u.bitcast(BF)
    wout_v = wout_u.bitcast(BF)
    fg_v = fg_u.bitcast(BF)
    xn_v = xn_u.bitcast(BF)
    z2_v = z2_u.bitcast(BF)
    w_v = w_u.bitcast(BF)
    gg_v = gg_u.bitcast(BF)

    def ds(start, size):
        if isinstance(start, int):
            return pl.ds(start, size)
        return pl.ds(pl.multiple_of(start, size), size)

    def lanes(n):
        return slice(n * 128, (n + 1) * 128)

    def blocks(ch):
        return pl.ds(ch[0] * C, ch[1] * C)

    def brows(a):
        return ds(a * C, C)

    def cp_q(c):
        r = blocks(QCH[c])
        return pltpu.make_async_copy(q_hbm.at[r, :], q_v.at[r, :], sem_q.at[c])

    def cp_k(c):
        b0, n = KCH[c]
        return pltpu.make_async_copy(k_hbm.at[blocks(KCH[c]), :],
                                     k_v.at[pl.ds(b0 * C + HALO, n * C), :], sem_k.at[c])

    def cp_v(c):
        r = blocks(KCH[c])
        return pltpu.make_async_copy(v_hbm.at[r, :], v_v.at[r, :], sem_v.at[c])

    def cp_h(c):
        r = blocks(HCH[c])
        return pltpu.make_async_copy(h_hbm.at[:, r], h_v.at[:, r], sem_h.at[c])

    def cp_w(c):
        r = blocks(WCH[c])
        return pltpu.make_async_copy(win_hbm.at[:, r], win_v.at[:, r], sem_w.at[c])

    def cp_wsp(i):
        r = ds(i * TA, TA)
        return pltpu.make_async_copy(wsp_hbm.at[r, :], wsp_v.at[r, :], sem_wsp.at[i])

    def cp_o(a, cols=slice(None)):
        r = brows(a)
        return pltpu.make_async_copy(o_v.at[r, cols], o_hbm.at[r, cols], sem_o.at[0])

    cp_f = pltpu.make_async_copy(fg_hbm, fg_v, sem_m.at[0])
    cp_sk = pltpu.make_async_copy(sk_hbm, sk_v.at[:, 0:D], sem_m.at[1])
    cp_d = pltpu.make_async_copy(d_hbm, d_v, sem_m.at[2])
    cp_b = pltpu.make_async_copy(b_hbm, b_v, sem_m.at[3])
    cp_wout = pltpu.make_async_copy(wout_hbm, wout_v, sem_m.at[4])

    groups = [
        [cp_q(0)], [cp_w(0)], [cp_w(1)], [cp_w(2)], [cp_w(3)], [cp_q(1), cp_w(4)],
        [cp_f, cp_sk, cp_d, cp_b, cp_q(2), cp_h(0), cp_k(0), cp_v(0)],
        [cp_q(3), cp_h(1), cp_k(1), cp_v(1)],
        [cp_q(4), cp_h(2), cp_k(2), cp_v(2)],
    ]
    for grp in groups:
        for cp in grp:
            cp.start()
    for i in range(S // TA):
        cp_wsp(i).start()
    cp_wout.start()

    def wait(g):
        for cp in groups[g]:
            cp.wait()

    k_v[0:HALO, :] = jnp.zeros((HALO, D), BF)

    c0 = math.sqrt(2.0 / math.pi)
    c1 = c0 * 0.044715

    def gelu2(x):
        return x + x * jnp.tanh(x * (c0 + c1 * (x * x)))

    def fence(tok):
        t = tok[0:8, :]
        for g in range(1, tok.shape[0] // 8):
            t = t | tok[g * 8:(g + 1) * 8, :]
        return t & pltpu.bitcast(k_v[0:HALO, 0:128], U32)

    def z2_words(a):
        return pltpu.bitcast(z2_v[brows(a), 0:128], U32)

    def ln_q(a, gate=None, part=0, nparts=1):
        n = C // nparts
        r = pl.ds(a * C + part * n, n)
        x = q_v[r, :]
        if gate is not None:
            x = pltpu.bitcast(pltpu.bitcast(x, U32) | jnp.tile(gate, (n // 16, ND)), BF)
        x = x.astype(F32)
        mu = jnp.sum(x, axis=-1, keepdims=True) * (1.0 / D)
        ex2 = jnp.sum(x * x, axis=-1, keepdims=True) * (1.0 / D)
        var = jnp.maximum(ex2 - mu * mu, 0.0)
        xn_v[r, :] = ((x - mu) * jax.lax.rsqrt(var + EPS)).astype(BF)

    def h_dft(a, dt):
        res = jax.lax.dot_general(fg_v[0:2 * C, C:2 * C], h_v[lanes(dt), brows(a)],
                                  (((1,), (1,)), ((), ())), preferred_element_type=F32)
        hf_v[:, a, :, lanes(dt)] = res.reshape(NB, 16, 128)
        return res

    def u_dft(a, dt):
        cols = lanes(dt)
        kf = k_v[pl.ds(a * C + HALO - 8, C + 8), cols].astype(F32)
        sk = sk_v[:, cols].astype(F32)
        ks = kf[8:, :] * sk[0:1, :]
        for t in range(1, 4):
            ks = ks + pltpu.roll(kf, t, axis=0)[8:, :] * sk[t:t + 1, :]
        kv = (ks * v_v[brows(a), cols].astype(F32)).astype(BF)
        res = jnp.dot(fg_v[0:2 * C, 0:C], kv, preferred_element_type=F32)
        p_v[:, a, :, cols] = res.reshape(NB, 16, 128)

    def proj(a, n, gate=None):
        lhs = xn_v[brows(a), :]
        if gate is not None:
            top = pltpu.bitcast(pltpu.bitcast(lhs[0:16, :], U32) | jnp.tile(gate, (1, ND)), BF)
            lhs = jnp.concatenate([top, lhs[16:, :]], axis=0)
        return gelu2(jnp.dot(lhs, win_v[:, lanes(n)], preferred_element_type=F32))

    def w2_rows(a):
        return pl.ds(S + (a % 2) * C, C)

    def z2_tile(a, n):
        z1_v[w2_rows(a), lanes(n)] = proj(a, NT + n)

    def z1_tile(a, n, gate=None):
        t = proj(a, n, gate)
        z1_v[brows(a), lanes(n)] = t
        return t

    def ln_z2(a):
        w2 = z1_v[w2_rows(a), :]
        mu = jnp.sum(w2, axis=-1, keepdims=True) * (1.0 / FH)
        ex2 = jnp.sum(w2 * w2, axis=-1, keepdims=True) * (1.0 / FH)
        var = jnp.maximum(ex2 - mu * mu, 0.0)
        rs = 0.25 * jax.lax.rsqrt(var + 4.0 * EPS)
        z2_v[brows(a), :] = ((w2 - mu) * rs).astype(BF)

    def region(blks, hch=(0, 0), kch=(0, 0)):
        hs = [(a, dt) for a in range(hch[0], hch[0] + hch[1]) for dt in range(ND)]
        us = [(a, dt) for a in range(kch[0], kch[0] + kch[1]) for dt in range(ND)]

        def next_ln_q(a, n, t):
            tok = pltpu.bitcast(t, U32)
            if n == 0:
                tok = jnp.concatenate([tok, z2_words(a)], axis=0)
            ln_q(a + 1, fence(tok), n, NLQ)

        for bi, a in enumerate(blks):
            last = bi == len(blks) - 1
            nh = len(hs) // (len(blks) - bi)
            nu = len(us) // (len(blks) - bi)
            nh_mid = max(nh - 4, 0) if last else nh
            early_ln = nh_mid >= 6 and a + 1 < NB
            slots = [x for x in (U_SLOTS_EARLY if early_ln else U_SLOTS) if not (last and x == 2 * NT)]
            cnt = [0] * (2 * NT + 1)
            for j in range(nu):
                cnt[slots[j % len(slots)]] += 1
            for n in range(NT):
                z2_tile(a, n)
                for _ in range(cnt[n]):
                    u_dft(*us.pop(0))
            hres = [h_dft(*hs.pop(0)) for _ in range(nh_mid)]
            for _ in range(cnt[NT]):
                u_dft(*us.pop(0))
            ln_z2(a)
            if early_ln:
                next_ln_q(a, 0, hres[4][64:72, :])
                next_ln_q(a, 1, hres[4][248:256, :])
            for n in range(NT):
                t = z1_tile(a, n)
                if early_ln and n in (1, 3):
                    next_ln_q(a, 2 + n // 2, t[0:8, :])
                if a + 1 < NB and n < NLQ and not early_ln:
                    next_ln_q(a, n, t[0:8, :])
                for _ in range(cnt[NT + 1 + n]):
                    u_dft(*us.pop(0))
            for _ in range(nh - nh_mid):
                h_dft(*hs.pop(0))
        assert not hs and not us

    wait(0)
    ln_q(0)
    ln_q(1)
    for c in range(3):
        wait(1 + c)
        for n in range(WCH[c][0], WCH[c][0] + WCH[c][1]):
            z2_tile(0, n - NT)
            z2_tile(1, n - NT)
    wait(4)
    ln_z2(0)
    ln_z2(1)
    z1_tile(0, 0)
    z1_tile(1, 0)
    z1_tile(0, 1, fence(z2_words(0)))
    z1_tile(1, 1)
    z1_tile(0, 2)
    z1_tile(1, 2)
    z1_tile(0, 3, fence(z2_words(1)))
    z1_tile(1, 3)
    wait(5)
    ln_q(2)
    for n in range(WCH[4][0], WCH[4][0] + WCH[4][1]):
        z1_tile(0, n)
        z1_tile(1, n)
    region([2])
    wait(6)
    region([3, 4], HCH[0], KCH[0])
    wait(7)
    region(list(range(5, QCH[4][0] - 1)), HCH[1], KCH[1])
    wait(8)
    region(list(range(QCH[4][0] - 1, NB)), HCH[2], KCH[2])

    dv = d_v[...].astype(F32)
    for dt in range(ND):
        hf_v[:, 0, 0:8, lanes(dt)] = hf_v[:, 0, 0:8, lanes(dt)] + dv[dt:dt + 1, :][None]
    b32_v[...] = b_v[...].astype(F32) * 0.25

    def conv_pos(ft, ft2, par, dt, after):
        cols = lanes(dt)
        prev = None
        for a in range(NB):
            ar, ai = (None, None) if prev is None else (-prev[1], prev[0])
            for dl in range(a + 1):
                hr = hf_v[ft, dl, 0:8, cols]
                hi = hf_v[ft, dl, 8:16, cols]
                ur = p_v[ft, a - dl, 0:8, cols]
                ui = p_v[ft, a - dl, 8:16, cols]
                if ar is None:
                    ar, ai = ur * hr - ui * hi, ur * hi + ui * hr
                    if after is not None:
                        z = fence(pltpu.bitcast(after, U32))
                        ar = pltpu.bitcast(pltpu.bitcast(ar, U32) | z, F32)
                        ai = pltpu.bitcast(pltpu.bitcast(ai, U32) | z, F32)
                else:
                    ar = (ar + ur * hr) - ui * hi
                    ai = (ai + ur * hi) + ui * hr
            prev = (ar, ai) if prev is None else (ar + prev[1], ai - prev[0])
            w_v[a * 16 + ft2, par * 8:(par + 1) * 8, cols] = ar.astype(BF)
            w_v[a * 16 + 8 + ft2, par * 8:(par + 1) * 8, cols] = ai.astype(BF)
        return prev[0]

    def phase2a(i, carry):
        cp_wsp(i).wait()
        eye = (jax.lax.broadcasted_iota(jnp.int32, (C, C), 0)
               == jax.lax.broadcasted_iota(jnp.int32, (C, C), 1))
        for m in range(TA // C):
            a = i * (TA // C) + m
            rows = brows(a)
            bcol = jnp.sum(jnp.where(eye, b32_v[pl.ds(a, 1), :], 0.0), axis=-1, keepdims=True)
            for n in range(NT):
                g = jnp.dot(wsp_v[rows, :], z2_v[:, lanes(n)], preferred_element_type=F32) + bcol
                gg_v[rows, lanes(n)] = (z1_v[rows, lanes(n)] * g).astype(BF)
        nft = NB * TA // S
        last = None
        for ft in range(nft):
            for dt in range(ND):
                last = conv_pos(i * nft + ft, i * (nft // 2) + ft // 2, ft % 2, dt, last)
        return carry

    jax.lax.fori_loop(0, S // TA, phase2a, 0)

    cp_wout.wait()

    def phase2b(i, carry):
        rev = 7 - jax.lax.broadcasted_iota(jnp.int32, (8, 128), 0)
        for m in range(TB // C):
            a = i * (TB // C) + m
            rows = brows(a)
            last = m == TB // C - 1
            for dt in range(ND):
                cols = lanes(dt)
                ev = jnp.dot(fg_v[2 * C:2 * C + C // 2, 0:C],
                             w_v[ds(a * 16, 8), :, cols].reshape(C, 128), preferred_element_type=F32)
                od = jnp.dot(fg_v[2 * C:2 * C + C // 2, C:2 * C],
                             w_v[ds(a * 16 + 8, 8), :, cols].reshape(C, 128), preferred_element_type=F32)
                lo = ev - od
                ys = [jnp.take_along_axis(lo[g * 8:(g + 1) * 8, :], rev, axis=0)
                      for g in range(C // 16 - 1, -1, -1)]
                y = jnp.concatenate(ys + [ev + od], axis=0)
                hh = jnp.dot(gg_v[rows, :], wout_v[:, cols], preferred_element_type=F32)
                gate = hh + hh * jnp.tanh(hh)
                s = xn_v[rows, cols].astype(F32) * y
                o_v[rows, cols] = (q_v[rows, cols].astype(F32) + s * gate).astype(BF)
                if last:
                    cp_o(a, cols).start()
            if not last:
                cp_o(a).start()
        return carry

    jax.lax.fori_loop(0, S // TB, phase2b, 0)
    pltpu.make_async_copy(o_v, o_hbm, sem_o.at[0]).wait()


@jax.jit
def pallas_recurrent_scan__ssm_conv_h3__mixer_gmlp__prompt_kernel(
    A_q: jax.Array,
    A_k: jax.Array,
    A_v: jax.Array,
    A_shift_k: jax.Array,
    A_ssm_k: jax.Array,
    A_ssm_D: jax.Array,
    B_x: jax.Array,
    B_w_in: jax.Array,
    B_w_sp: jax.Array,
    B_b_sp: jax.Array,
    B_w_out: jax.Array,
):
    del B_x
    any_spec = pl.BlockSpec(memory_space=pl.ANY)
    vm = pltpu.VMEM
    dma = pltpu.SemaphoreType.DMA
    out = pl.pallas_call(
        _kernel,
        out_shape=jax.ShapeDtypeStruct((S, D), BF),
        in_specs=[any_spec] * 11,
        out_specs=any_spec,
        scratch_shapes=[
            vm((S // 2, D), U32),
            vm((S + 64, D), BF),
            vm((S, D), BF),
            vm((D // 2, S), U32),
            vm((D // 2, 2 * FH), U32),
            vm((S // 2, S), U32),
            vm((FH // 2, D), U32),
            vm(((2 * C + C // 2) // 2, 2 * C), U32),
            vm((S // 2, D), U32),
            vm((S + 2 * C, FH), F32),
            vm((S // 2, FH), U32),
            vm((NB, NB, 16, D), F32),
            vm((NB, NB, 16, D), F32),
            vm((NB * 16, 8, 1024), U32),
            vm((S // 2, FH), U32),
            vm((S, D), BF),
            vm((NB, 128), F32),
            vm((NB, 128), BF),
            vm((4, 18 * 128), BF),
            vm((ND, 128), BF),
            dma((len(QCH),)), dma((len(KCH),)), dma((len(KCH),)), dma((len(HCH),)),
            dma((len(WCH),)), dma((S // TA,)), dma((1,)), dma((5,)),
        ],
        compiler_params=pltpu.CompilerParams(
            vmem_limit_bytes=110 * 1024 * 1024,
            disable_bounds_checks=True,
            disable_semaphore_checks=True,
        ),
    )(
        A_q.reshape(S, D), A_k.reshape(S, D), A_v.reshape(S, D),
        A_shift_k.T, A_ssm_k, A_ssm_D.reshape(ND, 128),
        B_w_in, B_w_sp, B_b_sp.reshape(NB, 128), B_w_out,
        _dft_consts(),
    )
    return out.reshape(1, S, D)
```

```python
import math

import jax
import jax.numpy as jnp
import numpy as np
import jax.experimental.pallas as pl
import jax.experimental.pallas.tpu as pltpu

S = 2048
D = 640
FH = 768
C = 128
NB = S // C
ND = D // 128
NT = FH // 128
HALO = 16
EPS = 1e-5
TA = 512
NOP = 3
NLQ = 4

BF = jnp.bfloat16
F32 = jnp.float32
U32 = jnp.uint32

QCH = [(0, 2), (2, 2), (4, 2), (6, 5), (11, 5)]
HCH = [(0, 2), (2, 5), (7, 9)]
KCH = [(0, 2), (2, 3), (5, 11)]
WCH = [(6, 2), (8, 2), (10, 2), (0, 4), (4, 2)]
U_SLOTS = [1, 3, 0, 2, 4, 11, 12, 5, 6, 6, 10, 9]
U_SLOTS_EARLY = [1, 3, 7, 9, 0, 2, 11, 12, 4, 5, 8, 10]


def _dft_consts():
    theta = np.pi * (4 * np.arange(C) + 1) / (2 * C)

    def fwd(t):
        ang = theta[:, None] * t[None, :]
        re = np.cos(ang).reshape(C // 8, 8, C)
        im = -np.sin(ang).reshape(C // 8, 8, C)
        return np.stack([re, im], axis=1).reshape(2 * C, C)

    fg = np.zeros((2 * C + C // 2, 2 * C), np.float64)
    fg[:2 * C, :C] = fwd(np.arange(C) - (C - 1) / 2)
    fg[:2 * C, C:] = fwd(np.arange(C))
    ang = (np.arange(C // 2) + 0.5)[:, None] * theta[None, :]
    fg[2 * C:, :C] = np.cos(ang) / C
    fg[2 * C:, C:] = -np.sin(ang) / C
    return fg.astype(np.float32).astype(BF)


def _kernel(q_hbm, k_hbm, v_hbm, sk_hbm, h_hbm, d_hbm, win_hbm, wsp_hbm, b_hbm, wout_hbm,
            fg_hbm, o_hbm,
            q_u, k_v, v_v, h_u, win_u, wsp_u, wout_u, fg_u,
            xn_u, z1_v, z2_u, p_v, hf_v, w_u, gg_u, xg_v, o_v, b32_v, b_v, sk_v, d_v,
            sem_q, sem_k, sem_v, sem_h, sem_w, sem_wsp, sem_o, sem_m):
    q_v = q_u.bitcast(BF)
    h_v = h_u.bitcast(BF)
    win_v = win_u.bitcast(BF)
    wsp_v = wsp_u.bitcast(BF)
    wout_v = wout_u.bitcast(BF)
    fg_v = fg_u.bitcast(BF)
    xn_v = xn_u.bitcast(BF)
    z2_v = z2_u.bitcast(BF)
    w_v = w_u.bitcast(BF)
    gg_v = gg_u.bitcast(BF)

    def ds(start, size):
        if isinstance(start, int):
            return pl.ds(start, size)
        return pl.ds(pl.multiple_of(start, size), size)

    def lanes(n):
        return slice(n * 128, (n + 1) * 128)

    def blocks(ch):
        return pl.ds(ch[0] * C, ch[1] * C)

    def brows(a):
        return ds(a * C, C)

    def cp_q(c):
        r = blocks(QCH[c])
        return pltpu.make_async_copy(q_hbm.at[r, :], q_v.at[r, :], sem_q.at[c])

    def cp_k(c):
        b0, n = KCH[c]
        return pltpu.make_async_copy(k_hbm.at[blocks(KCH[c]), :],
                                     k_v.at[pl.ds(b0 * C + HALO, n * C), :], sem_k.at[c])

    def cp_v(c):
        r = blocks(KCH[c])
        return pltpu.make_async_copy(v_hbm.at[r, :], v_v.at[r, :], sem_v.at[c])

    def cp_h(c):
        r = blocks(HCH[c])
        return pltpu.make_async_copy(h_hbm.at[:, r], h_v.at[:, r], sem_h.at[c])

    def cp_w(c):
        r = blocks(WCH[c])
        return pltpu.make_async_copy(win_hbm.at[:, r], win_v.at[:, r], sem_w.at[c])

    def cp_wsp(i):
        r = ds(i * TA, TA)
        return pltpu.make_async_copy(wsp_hbm.at[r, :], wsp_v.at[r, :], sem_wsp.at[i])

    def cp_o(a, cols=slice(None)):
        r = brows(a)
        return pltpu.make_async_copy(o_v.at[r, cols], o_hbm.at[r, cols], sem_o.at[0])

    cp_f = pltpu.make_async_copy(fg_hbm, fg_v, sem_m.at[0])
    cp_sk = pltpu.make_async_copy(sk_hbm, sk_v.at[:, 0:D], sem_m.at[1])
    cp_d = pltpu.make_async_copy(d_hbm, d_v, sem_m.at[2])
    cp_b = pltpu.make_async_copy(b_hbm, b_v, sem_m.at[3])
    cp_wout = pltpu.make_async_copy(wout_hbm, wout_v.at[0:FH, 0:D], sem_m.at[4])

    groups = [
        [cp_q(0)], [cp_w(0)], [cp_w(1)], [cp_w(2)], [cp_w(3)], [cp_q(1), cp_w(4)],
        [cp_f, cp_sk, cp_d, cp_b, cp_q(2), cp_h(0), cp_k(0), cp_v(0)],
        [cp_q(3), cp_h(1), cp_k(1), cp_v(1)],
        [cp_q(4), cp_h(2), cp_k(2), cp_v(2)],
    ]
    for grp in groups:
        for cp in grp:
            cp.start()
    cp_wout.start()
    for i in range(S // TA):
        cp_wsp(i).start()

    def wait(g):
        for cp in groups[g]:
            cp.wait()

    k_v[0:HALO, :] = jnp.zeros((HALO, D), BF)

    c0 = math.sqrt(2.0 / math.pi)
    c1 = c0 * 0.044715

    def gelu2(x):
        return x + x * jnp.tanh(x * (c0 + c1 * (x * x)))

    def fence(tok):
        t = tok[0:8, :]
        for g in range(1, tok.shape[0] // 8):
            t = t | tok[g * 8:(g + 1) * 8, :]
        return t & pltpu.bitcast(k_v[0:HALO, 0:128], U32)

    def z2_words(a):
        return pltpu.bitcast(z2_v[brows(a), 0:128], U32)

    def ln_q(a, gate=None, part=0, nparts=1):
        n = C // nparts
        r = pl.ds(a * C + part * n, n)
        x = q_v[r, :]
        if gate is not None:
            x = pltpu.bitcast(pltpu.bitcast(x, U32) | jnp.tile(gate, (n // 16, ND)), BF)
        x = x.astype(F32)
        mu = jnp.sum(x, axis=-1, keepdims=True) * (1.0 / D)
        ex2 = jnp.sum(x * x, axis=-1, keepdims=True) * (1.0 / D)
        var = jnp.maximum(ex2 - mu * mu, 0.0)
        mu = mu.astype(BF).astype(F32)
        xn_v[r, :] = ((x - mu) * jax.lax.rsqrt(var + EPS)).astype(BF)

    def h_dft(a, dt):
        res = jax.lax.dot_general(fg_v[0:2 * C, C:2 * C], h_v[lanes(dt), brows(a)],
                                  (((1,), (1,)), ((), ())), preferred_element_type=F32)
        hf_v[:, a, :, lanes(dt)] = res.reshape(NB, 16, 128)
        return res

    def u_dft(a, dt):
        cols = lanes(dt)
        kf = k_v[pl.ds(a * C + HALO - 8, C + 8), cols].astype(F32)
        sk = sk_v[:, cols].astype(F32)
        ks = kf[8:, :] * sk[0:1, :]
        for t in range(1, 4):
            ks = ks + pltpu.roll(kf, t, axis=0)[8:, :] * sk[t:t + 1, :]
        kv = (ks * v_v[brows(a), cols].astype(F32)).astype(BF)
        res = jnp.dot(fg_v[0:2 * C, 0:C], kv, preferred_element_type=F32)
        p_v[:, a, :, cols] = res.reshape(NB, 16, 128)

    def proj(a, n, gate=None):
        lhs = xn_v[brows(a), :]
        if gate is not None:
            top = pltpu.bitcast(pltpu.bitcast(lhs[0:16, :], U32) | jnp.tile(gate, (1, ND)), BF)
            lhs = jnp.concatenate([top, lhs[16:, :]], axis=0)
        return gelu2(jnp.dot(lhs, win_v[:, lanes(n)], preferred_element_type=F32))

    def w2_rows(a):
        return pl.ds(S + (a % 2) * C, C)

    def z2_tile(a, n):
        z1_v[w2_rows(a), lanes(n)] = proj(a, NT + n)

    def z1_tile(a, n, gate=None):
        t = proj(a, n, gate)
        z1_v[brows(a), lanes(n)] = t
        return t

    def ln_z2(a):
        w2 = z1_v[w2_rows(a), :]
        mu = jnp.sum(w2, axis=-1, keepdims=True) * (1.0 / FH)
        ex2 = jnp.sum(w2 * w2, axis=-1, keepdims=True) * (1.0 / FH)
        var = jnp.maximum(ex2 - mu * mu, 0.0)
        rs = 0.25 * jax.lax.rsqrt(var + 4.0 * EPS)
        z2_v[brows(a), :] = ((w2 - mu) * rs).astype(BF)

    def region(blks, hch=(0, 0), kch=(0, 0)):
        hs = [(a, dt) for a in range(hch[0], hch[0] + hch[1]) for dt in range(ND)]
        us = [(a, dt) for a in range(kch[0], kch[0] + kch[1]) for dt in range(ND)]

        def next_ln_q(a, n, t):
            tok = pltpu.bitcast(t, U32)
            if n == 0:
                tok = jnp.concatenate([tok, z2_words(a)], axis=0)
            ln_q(a + 1, fence(tok), n, NLQ)

        for bi, a in enumerate(blks):
            last = bi == len(blks) - 1
            nh = len(hs) // (len(blks) - bi)
            nu = len(us) // (len(blks) - bi)
            nh_mid = max(nh - 4, 0) if last else nh
            early_ln = nh_mid >= 6 and a + 1 < NB
            slots = [x for x in (U_SLOTS_EARLY if early_ln else U_SLOTS) if not (last and x == 2 * NT)]
            cnt = [0] * (2 * NT + 1)
            for j in range(nu):
                cnt[slots[j % len(slots)]] += 1
            for n in range(NT):
                z2_tile(a, n)
                for _ in range(cnt[n]):
                    u_dft(*us.pop(0))
            hres = [h_dft(*hs.pop(0)) for _ in range(nh_mid)]
            for _ in range(cnt[NT]):
                u_dft(*us.pop(0))
            ln_z2(a)
            if early_ln:
                next_ln_q(a, 0, hres[4][64:72, :])
                next_ln_q(a, 1, hres[4][248:256, :])
            for n in range(NT):
                t = z1_tile(a, n)
                if early_ln and n in (1, 3):
                    next_ln_q(a, 2 + n // 2, t[0:8, :])
                if a + 1 < NB and n < NLQ and not early_ln:
                    next_ln_q(a, n, t[0:8, :])
                for _ in range(cnt[NT + 1 + n]):
                    u_dft(*us.pop(0))
            for _ in range(nh - nh_mid):
                h_dft(*hs.pop(0))
        assert not hs and not us

    wait(0)
    ln_q(0)
    ln_q(1)
    for c in range(3):
        wait(1 + c)
        for n in range(WCH[c][0], WCH[c][0] + WCH[c][1]):
            z2_tile(0, n - NT)
            z2_tile(1, n - NT)
    wait(4)
    ln_z2(0)
    ln_z2(1)
    z1_tile(0, 0)
    z1_tile(1, 0)
    z1_tile(0, 1, fence(z2_words(0)))
    z1_tile(1, 1)
    z1_tile(0, 2)
    z1_tile(1, 2)
    z1_tile(0, 3, fence(z2_words(1)))
    z1_tile(1, 3)
    wait(5)
    ln_q(2)
    for n in range(WCH[4][0], WCH[4][0] + WCH[4][1]):
        z1_tile(0, n)
        z1_tile(1, n)
    region([2])
    wait(6)
    region([3, 4], HCH[0], KCH[0])
    wait(7)
    region(list(range(5, QCH[4][0] - 1)), HCH[1], KCH[1])
    wait(8)
    region(list(range(QCH[4][0] - 1, NB)), HCH[2], KCH[2])

    dv = d_v[...].astype(F32)
    for dt in range(ND):
        hf_v[:, 0, 0:8, lanes(dt)] = hf_v[:, 0, 0:8, lanes(dt)] + dv[dt:dt + 1, :][None]
    b32_v[...] = b_v[...].astype(F32) * 0.25

    def conv_pos(ft, ft2, par, dt, after):
        cols = lanes(dt)
        prev = None
        for a in range(NB):
            ar, ai = (None, None) if prev is None else (-prev[1], prev[0])
            for dl in range(a + 1):
                hr = hf_v[ft, dl, 0:8, cols]
                hi = hf_v[ft, dl, 8:16, cols]
                ur = p_v[ft, a - dl, 0:8, cols]
                ui = p_v[ft, a - dl, 8:16, cols]
                if ar is None:
                    ar, ai = ur * hr - ui * hi, ur * hi + ui * hr
                    if after is not None:
                        z = fence(pltpu.bitcast(after, U32))
                        ar = pltpu.bitcast(pltpu.bitcast(ar, U32) | z, F32)
                        ai = pltpu.bitcast(pltpu.bitcast(ai, U32) | z, F32)
                else:
                    ar = (ar + ur * hr) - ui * hi
                    ai = (ai + ur * hi) + ui * hr
            prev = (ar, ai) if prev is None else (ar + prev[1], ai - prev[0])
            w_v[a * 16 + ft2, par * 8:(par + 1) * 8, cols] = ar.astype(BF)
            w_v[a * 16 + 8 + ft2, par * 8:(par + 1) * 8, cols] = ai.astype(BF)
        return prev[0]

    gl_v = wout_v
    GL0 = FH

    def xn_gate(a, dt, g_ref, g_rows):
        rows = brows(a)
        hh = jnp.dot(g_ref[g_rows, :], wout_v[0:FH, lanes(dt)], preferred_element_type=F32)
        return xn_v[rows, lanes(dt)].astype(F32) * (hh + hh * jnp.tanh(hh))

    def phase2a(i, carry):
        cp_wsp(i).wait()
        eye = (jax.lax.broadcasted_iota(jnp.int32, (C, C), 0)
               == jax.lax.broadcasted_iota(jnp.int32, (C, C), 1))
        bcols = {}

        def g_tile(m, n):
            a = i * (TA // C) + m
            rows = brows(a)
            if m not in bcols:
                bcols[m] = jnp.sum(jnp.where(eye, b32_v[pl.ds(a, 1), :], 0.0), axis=-1, keepdims=True)
            g = jnp.dot(wsp_v[rows, :], z2_v[:, lanes(n)], preferred_element_type=F32) + bcols[m]
            g = (z1_v[rows, lanes(n)] * g).astype(BF)
            if m < NOP:
                gl_v[GL0 + m * C:GL0 + (m + 1) * C, lanes(n)] = g
            else:
                gg_v[ds(i * C, C), lanes(n)] = g

        tiles = [(m, n) for m in range(TA // C) for n in range(NT)]
        for m, n in tiles[:-1]:
            g_tile(m, n)
        for m in range(NOP):
            a = i * (TA // C) + m
            for dt in range(ND):
                xg_v[brows(a), lanes(dt)] = xn_gate(a, dt, gl_v, pl.ds(GL0 + m * C, C))
        g_tile(*tiles[-1])
        nft = NB * TA // S
        last = None
        for ft in range(nft):
            for dt in range(ND):
                last = conv_pos(i * nft + ft, i * (nft // 2) + ft // 2, ft % 2, dt, last)
        return carry

    cp_wout.wait()
    jax.lax.fori_loop(0, S // TA, phase2a, 0)

    rev = 7 - jax.lax.broadcasted_iota(jnp.int32, (8, 128), 0)
    for a in range(NB):
        rows = brows(a)
        for dt in range(ND):
            cols = lanes(dt)
            ev = jnp.dot(fg_v[2 * C:2 * C + C // 2, 0:C],
                         w_v[ds(a * 16, 8), :, cols].reshape(C, 128), preferred_element_type=F32)
            od = jnp.dot(fg_v[2 * C:2 * C + C // 2, C:2 * C],
                         w_v[ds(a * 16 + 8, 8), :, cols].reshape(C, 128), preferred_element_type=F32)
            lo = ev - od
            ys = [jnp.take_along_axis(lo[g * 8:(g + 1) * 8, :], rev, axis=0)
                  for g in range(C // 16 - 1, -1, -1)]
            y = jnp.concatenate(ys + [ev + od], axis=0)
            xg = xg_v[rows, cols] if a % (TA // C) < NOP else xn_gate(a, dt, gg_v, brows(a // (TA // C)))
            o_v[rows, cols] = (q_v[rows, cols].astype(F32) + xg * y).astype(BF)
            if a == NB - 1:
                cp_o(a, cols).start()
        if a < NB - 1:
            cp_o(a).start()
    pltpu.make_async_copy(o_v, o_hbm, sem_o.at[0]).wait()


@jax.jit
def pallas_recurrent_scan__ssm_conv_h3__mixer_gmlp__prompt_kernel(
    A_q: jax.Array,
    A_k: jax.Array,
    A_v: jax.Array,
    A_shift_k: jax.Array,
    A_ssm_k: jax.Array,
    A_ssm_D: jax.Array,
    B_x: jax.Array,
    B_w_in: jax.Array,
    B_w_sp: jax.Array,
    B_b_sp: jax.Array,
    B_w_out: jax.Array,
):
    del B_x
    any_spec = pl.BlockSpec(memory_space=pl.ANY)
    vm = pltpu.VMEM
    dma = pltpu.SemaphoreType.DMA
    out = pl.pallas_call(
        _kernel,
        out_shape=jax.ShapeDtypeStruct((S, D), BF),
        in_specs=[any_spec] * 11,
        out_specs=any_spec,
        scratch_shapes=[
            vm((S // 2, D), U32),
            vm((S + 64, D), BF),
            vm((S, D), BF),
            vm((D // 2, S), U32),
            vm((D // 2, 2 * FH), U32),
            vm((S // 2, S), U32),
            vm(((FH + 512) // 2, FH), U32),
            vm(((2 * C + C // 2) // 2, 2 * C), U32),
            vm((S // 2, D), U32),
            vm((S + 2 * C, FH), F32),
            vm((S // 2, FH), U32),
            vm((NB, NB, 16, D), F32),
            vm((NB, NB, 16, D), F32),
            vm((NB * 16, 8, 1024), U32),
            vm((S // TA * C // 2, FH), U32),
            vm((S, D), F32),
            vm((S, D), BF),
            vm((NB, 128), F32),
            vm((NB, 128), BF),
            vm((4, 18 * 128), BF),
            vm((ND, 128), BF),
            dma((len(QCH),)), dma((len(KCH),)), dma((len(KCH),)), dma((len(HCH),)),
            dma((len(WCH),)), dma((S // TA,)), dma((1,)), dma((5,)),
        ],
        compiler_params=pltpu.CompilerParams(
            vmem_limit_bytes=110 * 1024 * 1024,
            disable_bounds_checks=True,
            disable_semaphore_checks=True,
        ),
    )(
        A_q.reshape(S, D), A_k.reshape(S, D), A_v.reshape(S, D),
        A_shift_k.T, A_ssm_k, A_ssm_D.reshape(ND, 128),
        B_w_in, B_w_sp, B_b_sp.reshape(NB, 128), B_w_out,
        _dft_consts(),
    )
    return out.reshape(1, S, D)
```

```python
import math

import jax
import jax.numpy as jnp
import numpy as np
import jax.experimental.pallas as pl
import jax.experimental.pallas.tpu as pltpu

S = 2048
D = 640
FH = 768
C = 128
NB = S // C
ND = D // 128
NT = FH // 128
HALO = 16
EPS = 1e-5
TA = 512
NOP = 3
NLQ = 4

BF = jnp.bfloat16
F32 = jnp.float32
U32 = jnp.uint32

QCH = [(0, 2), (2, 2), (4, 2), (6, 5), (11, 5)]
HCH = [(0, 2), (2, 5), (7, 9)]
KCH = [(0, 2), (2, 3), (5, 11)]
WCH = [(6, 2), (8, 2), (10, 2), (0, 4), (4, 2)]
U_SLOTS = [1, 3, 0, 2, 4, 11, 12, 5, 6, 6, 10, 9]
U_SLOTS_EARLY = [1, 3, 7, 9, 0, 2, 11, 12, 4, 5, 8, 10]


def _dft_consts():
    theta = np.pi * (4 * np.arange(C) + 1) / (2 * C)

    def fwd(t):
        ang = theta[:, None] * t[None, :]
        re = np.cos(ang).reshape(C // 8, 8, C)
        im = -np.sin(ang).reshape(C // 8, 8, C)
        return np.stack([re, im], axis=1).reshape(2 * C, C)

    fg = np.zeros((2 * C + C // 2, 2 * C), np.float64)
    fg[:2 * C, :C] = fwd(np.arange(C) - (C - 1) / 2)
    fg[:2 * C, C:] = fwd(np.arange(C))
    ang = (np.arange(C // 2) + 0.5)[:, None] * theta[None, :]
    fg[2 * C:, :C] = np.cos(ang) / C
    fg[2 * C:, C:] = -np.sin(ang) / C
    return fg.astype(np.float32).astype(BF)


def _kernel(q_hbm, k_hbm, v_hbm, sk_hbm, h_hbm, d_hbm, win_hbm, wsp_hbm, b_hbm, wout_hbm,
            fg_hbm, o_hbm,
            q_u, k_v, v_v, h_u, win_u, wsp_u, wout_u, fg_u,
            xn_u, z1_v, z2_u, p_v, hf_v, w_u, gg_u, xg_v, o_v, b32_v, b_v, sk_v, d_v,
            sem_q, sem_k, sem_v, sem_h, sem_w, sem_wsp, sem_o, sem_m):
    q_v = q_u.bitcast(BF)
    h_v = h_u.bitcast(BF)
    win_v = win_u.bitcast(BF)
    wsp_v = wsp_u.bitcast(BF)
    wout_v = wout_u.bitcast(BF)
    fg_v = fg_u.bitcast(BF)
    xn_v = xn_u.bitcast(BF)
    z2_v = z2_u.bitcast(BF)
    w_v = w_u.bitcast(BF)
    gg_v = gg_u.bitcast(BF)

    def ds(start, size):
        if isinstance(start, int):
            return pl.ds(start, size)
        return pl.ds(pl.multiple_of(start, size), size)

    def lanes(n):
        return slice(n * 128, (n + 1) * 128)

    def blocks(ch):
        return pl.ds(ch[0] * C, ch[1] * C)

    def brows(a):
        return ds(a * C, C)

    def cp_q(c):
        r = blocks(QCH[c])
        return pltpu.make_async_copy(q_hbm.at[r, :], q_v.at[r, :], sem_q.at[c])

    def cp_k(c):
        b0, n = KCH[c]
        return pltpu.make_async_copy(k_hbm.at[blocks(KCH[c]), :],
                                     k_v.at[pl.ds(b0 * C + HALO, n * C), :], sem_k.at[c])

    def cp_v(c):
        r = blocks(KCH[c])
        return pltpu.make_async_copy(v_hbm.at[r, :], v_v.at[r, :], sem_v.at[c])

    def cp_h(c):
        r = blocks(HCH[c])
        return pltpu.make_async_copy(h_hbm.at[:, r], h_v.at[:, r], sem_h.at[c])

    def cp_w(c):
        r = blocks(WCH[c])
        return pltpu.make_async_copy(win_hbm.at[:, r], win_v.at[:, r], sem_w.at[c])

    def cp_wsp(i):
        r = ds(i * TA, TA)
        return pltpu.make_async_copy(wsp_hbm.at[r, :], wsp_v.at[r, :], sem_wsp.at[i])

    def cp_o(a, cols=slice(None)):
        r = brows(a)
        return pltpu.make_async_copy(o_v.at[r, cols], o_hbm.at[r, cols], sem_o.at[0])

    cp_f = pltpu.make_async_copy(fg_hbm, fg_v, sem_m.at[0])
    cp_sk = pltpu.make_async_copy(sk_hbm, sk_v.at[:, 0:D], sem_m.at[1])
    cp_d = pltpu.make_async_copy(d_hbm, d_v, sem_m.at[2])
    cp_b = pltpu.make_async_copy(b_hbm, b_v, sem_m.at[3])
    cp_wout = pltpu.make_async_copy(wout_hbm, wout_v.at[0:FH, 0:D], sem_m.at[4])

    groups = [
        [cp_q(0)], [cp_w(0)], [cp_w(1)], [cp_w(2)], [cp_w(3)], [cp_q(1), cp_w(4)],
        [cp_f, cp_sk, cp_d, cp_b, cp_q(2), cp_h(0), cp_k(0), cp_v(0)],
        [cp_q(3), cp_h(1), cp_k(1), cp_v(1)],
        [cp_q(4), cp_h(2), cp_k(2), cp_v(2)],
    ]
    def wait(g):
        for cp in groups[g]:
            cp.wait()

    c0 = math.sqrt(2.0 / math.pi)
    c1 = c0 * 0.044715

    def gelu2(x):
        return x + x * jnp.tanh(x * (c0 + c1 * (x * x)))

    def fence(tok):
        t = tok[0:8, :]
        for g in range(1, tok.shape[0] // 8):
            t = t | tok[g * 8:(g + 1) * 8, :]
        return t & pltpu.bitcast(k_v[0:HALO, 0:128], U32)

    def z2_words(a):
        return pltpu.bitcast(z2_v[brows(a), 0:128], U32)

    def ln_q(a, gate=None, part=0, nparts=1):
        n = C // nparts
        r = pl.ds(a * C + part * n, n)
        x = q_v[r, :]
        if gate is not None:
            x = pltpu.bitcast(pltpu.bitcast(x, U32) | jnp.tile(gate, (n // 16, ND)), BF)
        x = x.astype(F32)
        mu = jnp.sum(x, axis=-1, keepdims=True) * (1.0 / D)
        ex2 = jnp.sum(x * x, axis=-1, keepdims=True) * (1.0 / D)
        var = jnp.maximum(ex2 - mu * mu, 0.0)
        mu = mu.astype(BF).astype(F32)
        xn_v[r, :] = ((x - mu) * jax.lax.rsqrt(var + EPS)).astype(BF)

    def h_dft(a, dt):
        res = jax.lax.dot_general(fg_v[0:2 * C, C:2 * C], h_v[lanes(dt), brows(a)],
                                  (((1,), (1,)), ((), ())), preferred_element_type=F32)
        hf_v[:, a, :, lanes(dt)] = res.reshape(NB, 16, 128)
        return res

    def u_dft(a, dt):
        cols = lanes(dt)
        kf = k_v[pl.ds(a * C + HALO - 8, C + 8), cols].astype(F32)
        sk = sk_v[:, cols].astype(F32)
        ks = kf[8:, :] * sk[0:1, :]
        for t in range(1, 4):
            ks = ks + pltpu.roll(kf, t, axis=0)[8:, :] * sk[t:t + 1, :]
        kv = (ks * v_v[brows(a), cols].astype(F32)).astype(BF)
        res = jnp.dot(fg_v[0:2 * C, 0:C], kv, preferred_element_type=F32)
        p_v[:, a, :, cols] = res.reshape(NB, 16, 128)

    def proj(a, n, gate=None):
        lhs = xn_v[brows(a), :]
        if gate is not None:
            top = pltpu.bitcast(pltpu.bitcast(lhs[0:16, :], U32) | jnp.tile(gate, (1, ND)), BF)
            lhs = jnp.concatenate([top, lhs[16:, :]], axis=0)
        return gelu2(jnp.dot(lhs, win_v[:, lanes(n)], preferred_element_type=F32))

    def w2_rows(a):
        return pl.ds(S + (a % 2) * C, C)

    def z2_tile(a, n):
        z1_v[w2_rows(a), lanes(n)] = proj(a, NT + n)

    def z1_tile(a, n, gate=None):
        t = proj(a, n, gate)
        z1_v[brows(a), lanes(n)] = t
        return t

    def ln_z2(a):
        w2 = z1_v[w2_rows(a), :]
        mu = jnp.sum(w2, axis=-1, keepdims=True) * (1.0 / FH)
        ex2 = jnp.sum(w2 * w2, axis=-1, keepdims=True) * (1.0 / FH)
        var = jnp.maximum(ex2 - mu * mu, 0.0)
        rs = 0.25 * jax.lax.rsqrt(var + 4.0 * EPS)
        z2_v[brows(a), :] = ((w2 - mu) * rs).astype(BF)

    def region(blks, hch=(0, 0), kch=(0, 0)):
        hs = [(a, dt) for a in range(hch[0], hch[0] + hch[1]) for dt in range(ND)]
        us = [(a, dt) for a in range(kch[0], kch[0] + kch[1]) for dt in range(ND)]

        def next_ln_q(a, n, t):
            tok = pltpu.bitcast(t, U32)
            if n == 0:
                tok = jnp.concatenate([tok, z2_words(a)], axis=0)
            ln_q(a + 1, fence(tok), n, NLQ)

        for bi, a in enumerate(blks):
            last = bi == len(blks) - 1
            nh = len(hs) // (len(blks) - bi)
            nu = len(us) // (len(blks) - bi)
            nh_mid = max(nh - 4, 0) if last else nh
            early_ln = nh_mid >= 6 and a + 1 < NB
            slots = [x for x in (U_SLOTS_EARLY if early_ln else U_SLOTS) if not (last and x == 2 * NT)]
            cnt = [0] * (2 * NT + 1)
            for j in range(nu):
                cnt[slots[j % len(slots)]] += 1
            for n in range(NT):
                z2_tile(a, n)
                for _ in range(cnt[n]):
                    u_dft(*us.pop(0))
            hres = [h_dft(*hs.pop(0)) for _ in range(nh_mid)]
            for _ in range(cnt[NT]):
                u_dft(*us.pop(0))
            ln_z2(a)
            if early_ln:
                next_ln_q(a, 0, hres[4][64:72, :])
                next_ln_q(a, 1, hres[4][248:256, :])
            for n in range(NT):
                t = z1_tile(a, n)
                if early_ln and n in (1, 3):
                    next_ln_q(a, 2 + n // 2, t[0:8, :])
                if a + 1 < NB and n < NLQ and not early_ln:
                    next_ln_q(a, n, t[0:8, :])
                for _ in range(cnt[NT + 1 + n]):
                    u_dft(*us.pop(0))
            for _ in range(nh - nh_mid):
                h_dft(*hs.pop(0))
        assert not hs and not us

    def conv_pos(ft, ft2, par, dt, after):
        cols = lanes(dt)
        prev = None
        for a in range(NB):
            ar, ai = (None, None) if prev is None else (-prev[1], prev[0])
            for dl in range(a + 1):
                hr = hf_v[ft, dl, 0:8, cols]
                hi = hf_v[ft, dl, 8:16, cols]
                ur = p_v[ft, a - dl, 0:8, cols]
                ui = p_v[ft, a - dl, 8:16, cols]
                if ar is None:
                    ar, ai = ur * hr - ui * hi, ur * hi + ui * hr
                    if after is not None:
                        z = fence(pltpu.bitcast(after, U32))
                        ar = pltpu.bitcast(pltpu.bitcast(ar, U32) | z, F32)
                        ai = pltpu.bitcast(pltpu.bitcast(ai, U32) | z, F32)
                else:
                    ar = (ar + ur * hr) - ui * hi
                    ai = (ai + ur * hi) + ui * hr
            prev = (ar, ai) if prev is None else (ar + prev[1], ai - prev[0])
            w_v[a * 16 + ft2, par * 8:(par + 1) * 8, cols] = ar.astype(BF)
            w_v[a * 16 + 8 + ft2, par * 8:(par + 1) * 8, cols] = ai.astype(BF)
        return prev[0]

    gl_v = wout_v
    GL0 = FH

    def xn_gate(a, dt, g_ref, g_rows):
        rows = brows(a)
        hh = jnp.dot(g_ref[g_rows, :], wout_v[0:FH, lanes(dt)], preferred_element_type=F32)
        return xn_v[rows, lanes(dt)].astype(F32) * (hh + hh * jnp.tanh(hh))

    def phase2a(i, carry):
        cp_wsp(i).wait()
        eye = (jax.lax.broadcasted_iota(jnp.int32, (C, C), 0)
               == jax.lax.broadcasted_iota(jnp.int32, (C, C), 1))
        bcols = {}

        def g_tile(m, n):
            a = i * (TA // C) + m
            rows = brows(a)
            if m not in bcols:
                bcols[m] = jnp.sum(jnp.where(eye, b32_v[pl.ds(a, 1), :], 0.0), axis=-1, keepdims=True)
            g = jnp.dot(wsp_v[rows, :], z2_v[:, lanes(n)], preferred_element_type=F32) + bcols[m]
            g = (z1_v[rows, lanes(n)] * g).astype(BF)
            if m < NOP:
                gl_v[GL0 + m * C:GL0 + (m + 1) * C, lanes(n)] = g
            else:
                gg_v[ds(i * C, C), lanes(n)] = g

        tiles = [(m, n) for m in range(TA // C) for n in range(NT)]
        for m, n in tiles[:-1]:
            g_tile(m, n)
        for m in range(NOP):
            a = i * (TA // C) + m
            for dt in range(ND):
                xg_v[brows(a), lanes(dt)] = xn_gate(a, dt, gl_v, pl.ds(GL0 + m * C, C))
        g_tile(*tiles[-1])
        nft = NB * TA // S
        last = None
        for ft in range(nft):
            for dt in range(ND):
                last = conv_pos(i * nft + ft, i * (nft // 2) + ft // 2, ft % 2, dt, last)
        return carry

    step = pl.program_id(0)

    @pl.when(step == 0)
    def _():
        for grp in groups:
            for cp in grp:
                cp.start()
        cp_wout.start()
        for i in range(S // TA):
            cp_wsp(i).start()
        k_v[0:HALO, :] = jnp.zeros((HALO, D), BF)

    @pl.when(step == 1)
    def _():
        cp_wout.wait()
        jax.lax.fori_loop(0, S // TA, phase2a, 0)

        rev = 7 - jax.lax.broadcasted_iota(jnp.int32, (8, 128), 0)
        for a in range(NB):
            rows = brows(a)
            for dt in range(ND):
                cols = lanes(dt)
                ev = jnp.dot(fg_v[2 * C:2 * C + C // 2, 0:C],
                             w_v[ds(a * 16, 8), :, cols].reshape(C, 128), preferred_element_type=F32)
                od = jnp.dot(fg_v[2 * C:2 * C + C // 2, C:2 * C],
                             w_v[ds(a * 16 + 8, 8), :, cols].reshape(C, 128), preferred_element_type=F32)
                lo = ev - od
                ys = [jnp.take_along_axis(lo[g * 8:(g + 1) * 8, :], rev, axis=0)
                      for g in range(C // 16 - 1, -1, -1)]
                y = jnp.concatenate(ys + [ev + od], axis=0)
                xg = xg_v[rows, cols] if a % (TA // C) < NOP else xn_gate(a, dt, gg_v, brows(a // (TA // C)))
                o_v[rows, cols] = (q_v[rows, cols].astype(F32) + xg * y).astype(BF)
                if a == NB - 1:
                    cp_o(a, cols).start()
            if a < NB - 1:
                cp_o(a).start()
        pltpu.make_async_copy(o_v, o_hbm, sem_o.at[0]).wait()

    @pl.when(step == 0)
    def _():
        wait(0)
        ln_q(0)
        ln_q(1)
        for c in range(3):
            wait(1 + c)
            for n in range(WCH[c][0], WCH[c][0] + WCH[c][1]):
                z2_tile(0, n - NT)
                z2_tile(1, n - NT)
        wait(4)
        ln_z2(0)
        ln_z2(1)
        z1_tile(0, 0)
        z1_tile(1, 0)
        z1_tile(0, 1, fence(z2_words(0)))
        z1_tile(1, 1)
        z1_tile(0, 2)
        z1_tile(1, 2)
        z1_tile(0, 3, fence(z2_words(1)))
        z1_tile(1, 3)
        wait(5)
        ln_q(2)
        for n in range(WCH[4][0], WCH[4][0] + WCH[4][1]):
            z1_tile(0, n)
            z1_tile(1, n)
        region([2])
        wait(6)
        region([3, 4], HCH[0], KCH[0])
        wait(7)
        region(list(range(5, QCH[4][0] - 1)), HCH[1], KCH[1])
        wait(8)
        region(list(range(QCH[4][0] - 1, NB)), HCH[2], KCH[2])

        dv = d_v[...].astype(F32)
        for dt in range(ND):
            hf_v[:, 0, 0:8, lanes(dt)] = hf_v[:, 0, 0:8, lanes(dt)] + dv[dt:dt + 1, :][None]
        b32_v[...] = b_v[...].astype(F32) * 0.25


@jax.jit
def pallas_recurrent_scan__ssm_conv_h3__mixer_gmlp__prompt_kernel(
    A_q: jax.Array,
    A_k: jax.Array,
    A_v: jax.Array,
    A_shift_k: jax.Array,
    A_ssm_k: jax.Array,
    A_ssm_D: jax.Array,
    B_x: jax.Array,
    B_w_in: jax.Array,
    B_w_sp: jax.Array,
    B_b_sp: jax.Array,
    B_w_out: jax.Array,
):
    del B_x
    any_spec = pl.BlockSpec(memory_space=pl.ANY)
    vm = pltpu.VMEM
    dma = pltpu.SemaphoreType.DMA
    out = pl.pallas_call(
        _kernel,
        out_shape=jax.ShapeDtypeStruct((S, D), BF),
        grid=(2,),
        in_specs=[any_spec] * 11,
        out_specs=any_spec,
        scratch_shapes=[
            vm((S // 2, D), U32),
            vm((S + 64, D), BF),
            vm((S, D), BF),
            vm((D // 2, S), U32),
            vm((D // 2, 2 * FH), U32),
            vm((S // 2, S), U32),
            vm(((FH + 512) // 2, FH), U32),
            vm(((2 * C + C // 2) // 2, 2 * C), U32),
            vm((S // 2, D), U32),
            vm((S + 2 * C, FH), F32),
            vm((S // 2, FH), U32),
            vm((NB, NB, 16, D), F32),
            vm((NB, NB, 16, D), F32),
            vm((NB * 16, 8, 1024), U32),
            vm((S // TA * C // 2, FH), U32),
            vm((S, D), F32),
            vm((S, D), BF),
            vm((NB, 128), F32),
            vm((NB, 128), BF),
            vm((4, 18 * 128), BF),
            vm((ND, 128), BF),
            dma((len(QCH),)), dma((len(KCH),)), dma((len(KCH),)), dma((len(HCH),)),
            dma((len(WCH),)), dma((S // TA,)), dma((1,)), dma((5,)),
        ],
        compiler_params=pltpu.CompilerParams(
            dimension_semantics=("arbitrary",),
            vmem_limit_bytes=110 * 1024 * 1024,
            disable_bounds_checks=True,
            disable_semaphore_checks=True,
        ),
    )(
        A_q.reshape(S, D), A_k.reshape(S, D), A_v.reshape(S, D),
        A_shift_k.T, A_ssm_k, A_ssm_D.reshape(ND, 128),
        B_w_in, B_w_sp, B_b_sp.reshape(NB, 128), B_w_out,
        _dft_consts(),
    )
    return out.reshape(1, S, D)
```

```python
import math

import jax
import jax.numpy as jnp
import numpy as np
import jax.experimental.pallas as pl
import jax.experimental.pallas.tpu as pltpu

S = 2048
D = 640
FH = 768
C = 128
NB = S // C
ND = D // 128
NT = FH // 128
HALO = 16
EPS = 1e-5
TA = 512
NOP = 3
NLQ = 4

BF = jnp.bfloat16
F32 = jnp.float32
U32 = jnp.uint32

QCH = [(0, 2), (2, 2), (4, 2), (6, 5), (11, 5)]
HCH = [(0, 2), (2, 5), (7, 9)]
KCH = [(0, 2), (2, 3), (5, 11)]
WCH = [(6, 2), (8, 2), (10, 2), (0, 4), (4, 2)]
U_SLOTS = [1, 3, 0, 2, 4, 11, 12, 5, 6, 6, 10, 9]
U_SLOTS_EARLY = [1, 3, 7, 9, 0, 2, 11, 12, 4, 5, 8, 10]
U_SLOTS_FINAL = [1, 3, 8, 10, 0, 2, 9, 11, 4, 7, 5]
LNQ_MANY_H = [('h', 4, 128), ('h', 5, 248), ('z', 1, 0), ('z', 3, 0)]
LNQ_SOME_H = [('h', 4, 128), ('z', 0, 64), ('z', 1, 120), ('z', 3, 0)]
LNQ_NO_H = [('z', 0, 120), ('z', 1, 120), ('z', 2, 120), ('z', 3, 120)]


def _dft_consts():
    theta = np.pi * (4 * np.arange(C) + 1) / (2 * C)

    def fwd(t):
        ang = theta[:, None] * t[None, :]
        re = np.cos(ang).reshape(C // 8, 8, C)
        im = -np.sin(ang).reshape(C // 8, 8, C)
        return np.stack([re, im], axis=1).reshape(2 * C, C)

    fg = np.zeros((2 * C + C // 2, 2 * C), np.float64)
    fg[:2 * C, :C] = fwd(np.arange(C) - (C - 1) / 2)
    fg[:2 * C, C:] = fwd(np.arange(C))
    ang = (np.arange(C // 2) + 0.5)[:, None] * theta[None, :]
    fg[2 * C:, :C] = np.cos(ang) / C
    fg[2 * C:, C:] = -np.sin(ang) / C
    return fg.astype(np.float32).astype(BF)


def _kernel(q_hbm, k_hbm, v_hbm, sk_hbm, h_hbm, d_hbm, win_hbm, wsp_hbm, b_hbm, wout_hbm,
            fg_hbm, o_hbm,
            q_u, k_v, v_v, h_u, win_u, wsp_u, wout_u, fg_u,
            xn_u, z1_v, z2_u, p_v, hf_v, w_u, gg_u, xg_v, o_v, b32_v, b_v, sk_v, d_v,
            sem_q, sem_k, sem_v, sem_h, sem_w, sem_wsp, sem_o, sem_m):
    q_v = q_u.bitcast(BF)
    h_v = h_u.bitcast(BF)
    win_v = win_u.bitcast(BF)
    wsp_v = wsp_u.bitcast(BF)
    wout_v = wout_u.bitcast(BF)
    fg_v = fg_u.bitcast(BF)
    xn_v = xn_u.bitcast(BF)
    z2_v = z2_u.bitcast(BF)
    w_v = w_u.bitcast(BF)
    gg_v = gg_u.bitcast(BF)

    def ds(start, size):
        if isinstance(start, int):
            return pl.ds(start, size)
        return pl.ds(pl.multiple_of(start, size), size)

    def lanes(n):
        return slice(n * 128, (n + 1) * 128)

    def blocks(ch):
        return pl.ds(ch[0] * C, ch[1] * C)

    def brows(a):
        return ds(a * C, C)

    def cp_q(c):
        r = blocks(QCH[c])
        return pltpu.make_async_copy(q_hbm.at[r, :], q_v.at[r, :], sem_q.at[c])

    def cp_k(c):
        b0, n = KCH[c]
        return pltpu.make_async_copy(k_hbm.at[blocks(KCH[c]), :],
                                     k_v.at[pl.ds(b0 * C + HALO, n * C), :], sem_k.at[c])

    def cp_v(c):
        r = blocks(KCH[c])
        return pltpu.make_async_copy(v_hbm.at[r, :], v_v.at[r, :], sem_v.at[c])

    def cp_h(c):
        r = blocks(HCH[c])
        return pltpu.make_async_copy(h_hbm.at[:, r], h_v.at[:, r], sem_h.at[c])

    def cp_w(c):
        r = blocks(WCH[c])
        return pltpu.make_async_copy(win_hbm.at[:, r], win_v.at[:, r], sem_w.at[c])

    def cp_wsp(i):
        r = ds(i * TA, TA)
        return pltpu.make_async_copy(wsp_hbm.at[r, :], wsp_v.at[r, :], sem_wsp.at[i])

    def cp_o(a, cols=slice(None)):
        r = brows(a)
        return pltpu.make_async_copy(o_v.at[r, cols], o_hbm.at[r, cols], sem_o.at[0])

    cp_f = pltpu.make_async_copy(fg_hbm, fg_v, sem_m.at[0])
    cp_sk = pltpu.make_async_copy(sk_hbm, sk_v.at[:, 0:D], sem_m.at[1])
    cp_d = pltpu.make_async_copy(d_hbm, d_v, sem_m.at[2])
    cp_b = pltpu.make_async_copy(b_hbm, b_v, sem_m.at[3])
    cp_wout = pltpu.make_async_copy(wout_hbm, wout_v.at[0:FH, 0:D], sem_m.at[4])

    groups = [
        [cp_q(0)], [cp_w(0)], [cp_w(1)], [cp_w(2)], [cp_w(3)], [cp_q(1), cp_w(4)],
        [cp_f, cp_sk, cp_d, cp_b, cp_q(2), cp_h(0), cp_k(0), cp_v(0)],
        [cp_q(3), cp_h(1), cp_k(1), cp_v(1)],
        [cp_q(4), cp_h(2), cp_k(2), cp_v(2)],
    ]
    def wait(g):
        for cp in groups[g]:
            cp.wait()

    c0 = math.sqrt(2.0 / math.pi)
    c1 = c0 * 0.044715

    def gelu2(x):
        return x + x * jnp.tanh(x * (c0 + c1 * (x * x)))

    def fence(tok):
        t = tok[0:8, :]
        for g in range(1, tok.shape[0] // 8):
            t = t | tok[g * 8:(g + 1) * 8, :]
        return t & pltpu.bitcast(k_v[0:HALO, 0:128], U32)

    def z2_words(a):
        return pltpu.bitcast(z2_v[brows(a), 0:128], U32)

    def ln_q(a, gate=None, part=0, nparts=1):
        n = C // nparts
        r = pl.ds(a * C + part * n, n)
        x = q_v[r, :]
        if gate is not None:
            x = pltpu.bitcast(pltpu.bitcast(x, U32) | jnp.tile(gate, (n // 16, ND)), BF)
        x = x.astype(F32)
        mu = jnp.sum(x, axis=-1, keepdims=True) * (1.0 / D)
        ex2 = jnp.sum(x * x, axis=-1, keepdims=True) * (1.0 / D)
        var = jnp.maximum(ex2 - mu * mu, 0.0)
        mu = mu.astype(BF).astype(F32)
        xn_v[r, :] = ((x - mu) * jax.lax.rsqrt(var + EPS)).astype(BF)

    def h_dft(a, dt):
        res = jax.lax.dot_general(fg_v[0:2 * C, C:2 * C], h_v[lanes(dt), brows(a)],
                                  (((1,), (1,)), ((), ())), preferred_element_type=F32)
        spec = res.reshape(NB, 16, 128)
        if a == 0:
            dv = d_v[...].astype(F32)[dt:dt + 1, :]
            spec = jnp.concatenate([spec[:, 0:8, :] + dv[None], spec[:, 8:16, :]], axis=1)
        hf_v[:, a, :, lanes(dt)] = spec
        return res

    def u_dft(a, dt):
        cols = lanes(dt)
        kf = k_v[pl.ds(a * C + HALO - 8, C + 8), cols].astype(F32)
        sk = sk_v[:, cols].astype(F32)
        ks = kf[8:, :] * sk[0:1, :]
        for t in range(1, 4):
            ks = ks + pltpu.roll(kf, t, axis=0)[8:, :] * sk[t:t + 1, :]
        kv = (ks * v_v[brows(a), cols].astype(F32)).astype(BF)
        res = jnp.dot(fg_v[0:2 * C, 0:C], kv, preferred_element_type=F32)
        p_v[:, a, :, cols] = res.reshape(NB, 16, 128)

    def proj(a, n, gate=None):
        lhs = xn_v[brows(a), :]
        if gate is not None:
            top = pltpu.bitcast(pltpu.bitcast(lhs[0:16, :], U32) | jnp.tile(gate, (1, ND)), BF)
            lhs = jnp.concatenate([top, lhs[16:, :]], axis=0)
        return gelu2(jnp.dot(lhs, win_v[:, lanes(n)], preferred_element_type=F32))

    def w2_rows(a):
        return pl.ds(S + (a % 2) * C, C)

    def z2_tile(a, n):
        z1_v[w2_rows(a), lanes(n)] = proj(a, NT + n)

    def z1_tile(a, n, gate=None):
        t = proj(a, n, gate)
        z1_v[brows(a), lanes(n)] = t
        return t

    def ln_z2(a):
        w2 = z1_v[w2_rows(a), :]
        mu = jnp.sum(w2, axis=-1, keepdims=True) * (1.0 / FH)
        ex2 = jnp.sum(w2 * w2, axis=-1, keepdims=True) * (1.0 / FH)
        var = jnp.maximum(ex2 - mu * mu, 0.0)
        rs = 0.25 * jax.lax.rsqrt(var + 4.0 * EPS)
        z2_v[brows(a), :] = ((w2 - mu) * rs).astype(BF)

    def region(blks, hch=(0, 0), kch=(0, 0)):
        hs = [(a, dt) for a in range(hch[0], hch[0] + hch[1]) for dt in range(ND)]
        us = [(a, dt) for a in range(kch[0], kch[0] + kch[1]) for dt in range(ND)]

        def next_ln_q(a, n, t):
            tok = pltpu.bitcast(t, U32)
            if n == 0:
                tok = jnp.concatenate([tok, z2_words(a)], axis=0)
            ln_q(a + 1, fence(tok), n, NLQ)

        for bi, a in enumerate(blks):
            last = bi == len(blks) - 1
            nh = len(hs) // (len(blks) - bi)
            nu = len(us) // (len(blks) - bi)
            nh_mid = max(nh - 4, 0) if last else nh
            if a == NB - 1:
                slots, marks = U_SLOTS_FINAL, []
            elif nh_mid >= 6:
                slots, marks = U_SLOTS_EARLY, LNQ_MANY_H
            else:
                slots, marks = U_SLOTS, LNQ_SOME_H if nh_mid >= 5 else LNQ_NO_H
            slots = [x for x in slots if not (last and x == 2 * NT)]
            cnt = [0] * (2 * NT + 1)
            for j in range(nu):
                cnt[slots[j % len(slots)]] += 1
            for n in range(NT):
                z2_tile(a, n)
                for _ in range(cnt[n]):
                    u_dft(*us.pop(0))
            hres = [h_dft(*hs.pop(0)) for _ in range(nh_mid)]
            for _ in range(cnt[NT]):
                u_dft(*us.pop(0))
            ln_z2(a)
            for part, (kind, tile, row) in enumerate(marks):
                if kind == 'h':
                    next_ln_q(a, part, hres[tile][row:row + 8, :])
            for n in range(NT):
                t = z1_tile(a, n)
                for part, (kind, tile, row) in enumerate(marks):
                    if kind == 'z' and tile == n:
                        next_ln_q(a, part, t[row:row + 8, :])
                for _ in range(cnt[NT + 1 + n]):
                    u_dft(*us.pop(0))
            for _ in range(nh - nh_mid):
                h_dft(*hs.pop(0))
        assert not hs and not us

    def conv_pos(ft, ft2, par, dt, after):
        cols = lanes(dt)
        prev = None
        for a in range(NB):
            ar, ai = (None, None) if prev is None else (-prev[1], prev[0])
            for dl in range(a + 1):
                hr = hf_v[ft, dl, 0:8, cols]
                hi = hf_v[ft, dl, 8:16, cols]
                ur = p_v[ft, a - dl, 0:8, cols]
                ui = p_v[ft, a - dl, 8:16, cols]
                if ar is None:
                    ar, ai = ur * hr - ui * hi, ur * hi + ui * hr
                    if after is not None:
                        z = fence(pltpu.bitcast(after, U32))
                        ar = pltpu.bitcast(pltpu.bitcast(ar, U32) | z, F32)
                        ai = pltpu.bitcast(pltpu.bitcast(ai, U32) | z, F32)
                else:
                    ar = (ar + ur * hr) - ui * hi
                    ai = (ai + ur * hi) + ui * hr
            prev = (ar, ai) if prev is None else (ar + prev[1], ai - prev[0])
            w_v[a * 16 + ft2, par * 8:(par + 1) * 8, cols] = ar.astype(BF)
            w_v[a * 16 + 8 + ft2, par * 8:(par + 1) * 8, cols] = ai.astype(BF)
        return prev[0]

    gl_v = wout_v
    GL0 = FH

    def xn_gate(a, dt, g_ref, g_rows):
        rows = brows(a)
        hh = jnp.dot(g_ref[g_rows, :], wout_v[0:FH, lanes(dt)], preferred_element_type=F32)
        return xn_v[rows, lanes(dt)].astype(F32) * (hh + hh * jnp.tanh(hh))

    def phase2a(i, carry):
        cp_wsp(i).wait()
        eye = (jax.lax.broadcasted_iota(jnp.int32, (C, C), 0)
               == jax.lax.broadcasted_iota(jnp.int32, (C, C), 1))
        bcols = {}

        def g_tile(m, n):
            a = i * (TA // C) + m
            rows = brows(a)
            if m not in bcols:
                bcols[m] = jnp.sum(jnp.where(eye, b32_v[pl.ds(a, 1), :], 0.0), axis=-1, keepdims=True)
            g = jnp.dot(wsp_v[rows, :], z2_v[:, lanes(n)], preferred_element_type=F32) + bcols[m]
            g = (z1_v[rows, lanes(n)] * g).astype(BF)
            if m < NOP:
                gl_v[GL0 + m * C:GL0 + (m + 1) * C, lanes(n)] = g
            else:
                gg_v[ds(i * C, C), lanes(n)] = g

        tiles = [(m, n) for m in range(TA // C) for n in range(NT)]
        for m, n in tiles[:-1]:
            g_tile(m, n)
        for m in range(NOP):
            a = i * (TA // C) + m
            for dt in range(ND):
                xg_v[brows(a), lanes(dt)] = xn_gate(a, dt, gl_v, pl.ds(GL0 + m * C, C))
        g_tile(*tiles[-1])
        nft = NB * TA // S
        last = None
        for ft in range(nft):
            for dt in range(ND):
                last = conv_pos(i * nft + ft, i * (nft // 2) + ft // 2, ft % 2, dt, last)
        return carry

    step = pl.program_id(0)

    @pl.when(step == 0)
    def _():
        for grp in groups:
            for cp in grp:
                cp.start()
        cp_wout.start()
        for i in range(S // TA):
            cp_wsp(i).start()
        k_v[0:HALO, :] = jnp.zeros((HALO, D), BF)

    @pl.when(step == 1)
    def _():
        cp_wout.wait()
        jax.lax.fori_loop(0, S // TA, phase2a, 0)

        rev = 7 - jax.lax.broadcasted_iota(jnp.int32, (8, 128), 0)
        for a in range(NB):
            rows = brows(a)
            for dt in range(ND):
                cols = lanes(dt)
                ev = jnp.dot(fg_v[2 * C:2 * C + C // 2, 0:C],
                             w_v[ds(a * 16, 8), :, cols].reshape(C, 128), preferred_element_type=F32)
                od = jnp.dot(fg_v[2 * C:2 * C + C // 2, C:2 * C],
                             w_v[ds(a * 16 + 8, 8), :, cols].reshape(C, 128), preferred_element_type=F32)
                lo = ev - od
                ys = [jnp.take_along_axis(lo[g * 8:(g + 1) * 8, :], rev, axis=0)
                      for g in range(C // 16 - 1, -1, -1)]
                y = jnp.concatenate(ys + [ev + od], axis=0)
                xg = xg_v[rows, cols] if a % (TA // C) < NOP else xn_gate(a, dt, gg_v, brows(a // (TA // C)))
                o_v[rows, cols] = (q_v[rows, cols].astype(F32) + xg * y).astype(BF)
                if a == NB - 1:
                    cp_o(a, cols).start()
            if a < NB - 1:
                cp_o(a).start()
        pltpu.make_async_copy(o_v, o_hbm, sem_o.at[0]).wait()

    @pl.when(step == 0)
    def _():
        wait(0)
        ln_q(0)
        ln_q(1)
        for c in range(3):
            wait(1 + c)
            for n in range(WCH[c][0], WCH[c][0] + WCH[c][1]):
                z2_tile(0, n - NT)
                z2_tile(1, n - NT)
        wait(4)
        ln_z2(0)
        ln_z2(1)
        for n in range(WCH[3][0], WCH[3][0] + WCH[3][1]):
            z1_tile(0, n, fence(z2_words(0)) if n == 2 else None)
            z1_tile(1, n, fence(z2_words(1)) if n == 3 else None)
        wait(5)
        ln_q(2)
        for n in range(WCH[4][0], WCH[4][0] + WCH[4][1]):
            z1_tile(0, n)
            z1_tile(1, n)
        region([2])
        wait(6)
        b32_v[...] = b_v[...].astype(F32) * 0.25
        region([3, 4], HCH[0], KCH[0])
        wait(7)
        region(list(range(5, QCH[4][0] - 1)), HCH[1], KCH[1])
        wait(8)
        region(list(range(QCH[4][0] - 1, NB)), HCH[2], KCH[2])


@jax.jit
def pallas_recurrent_scan__ssm_conv_h3__mixer_gmlp__prompt_kernel(
    A_q: jax.Array,
    A_k: jax.Array,
    A_v: jax.Array,
    A_shift_k: jax.Array,
    A_ssm_k: jax.Array,
    A_ssm_D: jax.Array,
    B_x: jax.Array,
    B_w_in: jax.Array,
    B_w_sp: jax.Array,
    B_b_sp: jax.Array,
    B_w_out: jax.Array,
):
    del B_x
    any_spec = pl.BlockSpec(memory_space=pl.ANY)
    vm = pltpu.VMEM
    dma = pltpu.SemaphoreType.DMA
    out = pl.pallas_call(
        _kernel,
        out_shape=jax.ShapeDtypeStruct((S, D), BF),
        grid=(2,),
        in_specs=[any_spec] * 11,
        out_specs=any_spec,
        scratch_shapes=[
            vm((S // 2, D), U32),
            vm((S + 64, D), BF),
            vm((S, D), BF),
            vm((D // 2, S), U32),
            vm((D // 2, 2 * FH), U32),
            vm((S // 2, S), U32),
            vm(((FH + 512) // 2, FH), U32),
            vm(((2 * C + C // 2) // 2, 2 * C), U32),
            vm((S // 2, D), U32),
            vm((S + 2 * C, FH), F32),
            vm((S // 2, FH), U32),
            vm((NB, NB, 16, D), F32),
            vm((NB, NB, 16, D), F32),
            vm((NB * 16, 8, 1024), U32),
            vm((S // TA * C // 2, FH), U32),
            vm((S, D), F32),
            vm((S, D), BF),
            vm((NB, 128), F32),
            vm((NB, 128), BF),
            vm((4, 18 * 128), BF),
            vm((ND, 128), BF),
            dma((len(QCH),)), dma((len(KCH),)), dma((len(KCH),)), dma((len(HCH),)),
            dma((len(WCH),)), dma((S // TA,)), dma((1,)), dma((5,)),
        ],
        compiler_params=pltpu.CompilerParams(
            dimension_semantics=("arbitrary",),
            vmem_limit_bytes=110 * 1024 * 1024,
            disable_bounds_checks=True,
            disable_semaphore_checks=True,
        ),
    )(
        A_q.reshape(S, D), A_k.reshape(S, D), A_v.reshape(S, D),
        A_shift_k.T, A_ssm_k, A_ssm_D.reshape(ND, 128),
        B_w_in, B_w_sp, B_b_sp.reshape(NB, 128), B_w_out,
        _dft_consts(),
    )
    return out.reshape(1, S, D)
```

```python
import math

import jax
import jax.numpy as jnp
import numpy as np
import jax.experimental.pallas as pl
import jax.experimental.pallas.tpu as pltpu

S = 2048
D = 640
FH = 768
C = 128
NB = S // C
ND = D // 128
NT = FH // 128
HALO = 16
EPS = 1e-5
TA = 512
NOP = 3
NLQ = 4

BF = jnp.bfloat16
F32 = jnp.float32
U32 = jnp.uint32

QCH = [(0, 2), (2, 1), (3, 1), (4, 2), (6, 6), (12, 4)]
HCH = [(0, 5), (5, 11)]
KCH = [(0, 3), (3, 13)]
WCH = [(6, 2), (8, 2), (10, 2), (0, 1), (1, 5)]
U_SLOTS = [1, 3, 0, 2, 4, 11, 12, 5, 6, 6, 10, 9]
U_SLOTS_EARLY = [1, 3, 7, 9, 0, 2, 11, 12, 4, 5, 8, 10, 6, 6]
U_SLOTS_FINAL = [1, 3, 8, 10, 0, 2, 9, 11, 4, 7, 5]
LNQ_MANY_H = [('h', 4, 128), ('h', 5, 248), ('z', 1, 0), ('z', 3, 0)]
LNQ_SOME_H = [('h', 3, 248), ('z', 0, 64), ('z', 1, 120), ('z', 3, 0)]
LNQ_NO_H = [('z', 0, 64), ('z', 1, 64), ('z', 2, 64), ('z', 3, 0)]


def _dft_consts():
    theta = np.pi * (4 * np.arange(C) + 1) / (2 * C)

    def fwd(t):
        ang = theta[:, None] * t[None, :]
        re = np.cos(ang).reshape(C // 8, 8, C)
        im = -np.sin(ang).reshape(C // 8, 8, C)
        return np.stack([re, im], axis=1).reshape(2 * C, C)

    fg = np.zeros((2 * C + C // 2, 2 * C), np.float64)
    fg[:2 * C, :C] = fwd(np.arange(C) - (C - 1) / 2)
    fg[:2 * C, C:] = fwd(np.arange(C))
    ang = (np.arange(C // 2) + 0.5)[:, None] * theta[None, :]
    fg[2 * C:, :C] = np.cos(ang) / C
    fg[2 * C:, C:] = -np.sin(ang) / C
    return fg.astype(np.float32).astype(BF)


def _kernel(q_hbm, k_hbm, v_hbm, sk_hbm, h_hbm, d_hbm, win_hbm, wsp_hbm, b_hbm, wout_hbm,
            fg_hbm, o_hbm,
            q_u, k_v, v_v, h_u, win_u, wsp_u, wout_u, fg_u,
            xn_u, z1_v, z2_u, p_v, hf_v, w_u, gg_u, xg_v, o_v, b32_v, b_v, sk_v, d_v,
            sem_q, sem_k, sem_v, sem_h, sem_w, sem_wsp, sem_o, sem_m):
    q_v = q_u.bitcast(BF)
    h_v = h_u.bitcast(BF)
    win_v = win_u.bitcast(BF)
    wsp_v = wsp_u.bitcast(BF)
    wout_v = wout_u.bitcast(BF)
    fg_v = fg_u.bitcast(BF)
    xn_v = xn_u.bitcast(BF)
    z2_v = z2_u.bitcast(BF)
    w_v = w_u.bitcast(BF)
    gg_v = gg_u.bitcast(BF)

    def ds(start, size):
        if isinstance(start, int):
            return pl.ds(start, size)
        return pl.ds(pl.multiple_of(start, size), size)

    def lanes(n):
        return slice(n * 128, (n + 1) * 128)

    def blocks(ch):
        return pl.ds(ch[0] * C, ch[1] * C)

    def brows(a):
        return ds(a * C, C)

    def cp_q(c):
        r = blocks(QCH[c])
        return pltpu.make_async_copy(q_hbm.at[r, :], q_v.at[r, :], sem_q.at[c])

    def cp_k(c):
        b0, n = KCH[c]
        return pltpu.make_async_copy(k_hbm.at[blocks(KCH[c]), :],
                                     k_v.at[pl.ds(b0 * C + HALO, n * C), :], sem_k.at[c])

    def cp_v(c):
        r = blocks(KCH[c])
        return pltpu.make_async_copy(v_hbm.at[r, :], v_v.at[r, :], sem_v.at[c])

    def cp_h(c):
        r = blocks(HCH[c])
        return pltpu.make_async_copy(h_hbm.at[:, r], h_v.at[:, r], sem_h.at[c])

    def cp_w(c):
        r = blocks(WCH[c])
        return pltpu.make_async_copy(win_hbm.at[:, r], win_v.at[:, r], sem_w.at[c])

    def cp_wsp(i):
        r = ds(i * TA, TA)
        return pltpu.make_async_copy(wsp_hbm.at[r, :], wsp_v.at[r, :], sem_wsp.at[i])

    def cp_o(a, cols=slice(None)):
        r = brows(a)
        return pltpu.make_async_copy(o_v.at[r, cols], o_hbm.at[r, cols], sem_o.at[0])

    cp_f = pltpu.make_async_copy(fg_hbm, fg_v, sem_m.at[0])
    cp_sk = pltpu.make_async_copy(sk_hbm, sk_v.at[:, 0:D], sem_m.at[1])
    cp_d = pltpu.make_async_copy(d_hbm, d_v, sem_m.at[2])
    cp_b = pltpu.make_async_copy(b_hbm, b_v, sem_m.at[3])
    cp_wout = pltpu.make_async_copy(wout_hbm, wout_v.at[0:FH, 0:D], sem_m.at[4])

    groups = [
        [cp_q(0)], [cp_w(0)], [cp_q(1), cp_w(1)], [cp_q(2), cp_w(2), cp_w(3)], [cp_q(3), cp_w(4)],
        [cp_f, cp_sk, cp_d, cp_b, cp_q(4), cp_h(0), cp_k(0), cp_v(0)],
        [cp_q(5), cp_h(1), cp_k(1), cp_v(1)],
    ]

    def wait(g):
        for cp in groups[g]:
            cp.wait()

    c0 = math.sqrt(2.0 / math.pi)
    c1 = c0 * 0.044715

    def gelu2(x):
        return x + x * jnp.tanh(x * (c0 + c1 * (x * x)))

    def fence(tok):
        t = tok[0:8, :]
        for g in range(1, tok.shape[0] // 8):
            t = t | tok[g * 8:(g + 1) * 8, :]
        return t & pltpu.bitcast(k_v[0:HALO, 0:128], U32)

    def z2_words(a):
        return pltpu.bitcast(z2_v[brows(a), 0:128], U32)

    def ln_q(a, gate=None, part=0, nparts=1):
        n = C // nparts
        r = pl.ds(a * C + part * n, n)
        x = q_v[r, :]
        if gate is not None:
            x = pltpu.bitcast(pltpu.bitcast(x, U32) | jnp.tile(gate, (n // 16, ND)), BF)
        x = x.astype(F32)
        mu = jnp.sum(x, axis=-1, keepdims=True) * (1.0 / D)
        ex2 = jnp.sum(x * x, axis=-1, keepdims=True) * (1.0 / D)
        var = jnp.maximum(ex2 - mu * mu, 0.0)
        mu = mu.astype(BF).astype(F32)
        xn_v[r, :] = ((x - mu) * jax.lax.rsqrt(var + EPS)).astype(BF)

    def h_dft(a, dt):
        res = jax.lax.dot_general(fg_v[0:2 * C, C:2 * C], h_v[lanes(dt), brows(a)],
                                  (((1,), (1,)), ((), ())), preferred_element_type=F32)
        spec = res.reshape(NB, 16, 128)
        if a == 0:
            dv = d_v[...].astype(F32)[dt:dt + 1, :]
            spec = jnp.concatenate([spec[:, 0:8, :] + dv[None], spec[:, 8:16, :]], axis=1)
        hf_v[:, a, :, lanes(dt)] = spec
        return res

    def u_dft(a, dt):
        cols = lanes(dt)
        kf = k_v[pl.ds(a * C + HALO - 8, C + 8), cols].astype(F32)
        sk = sk_v[:, cols].astype(F32)
        ks = kf[8:, :] * sk[0:1, :]
        for t in range(1, 4):
            ks = ks + pltpu.roll(kf, t, axis=0)[8:, :] * sk[t:t + 1, :]
        kv = (ks * v_v[brows(a), cols].astype(F32)).astype(BF)
        res = jnp.dot(fg_v[0:2 * C, 0:C], kv, preferred_element_type=F32)
        p_v[:, a, :, cols] = res.reshape(NB, 16, 128)

    def proj(a, n, gate=None):
        lhs = xn_v[brows(a), :]
        if gate is not None:
            top = pltpu.bitcast(pltpu.bitcast(lhs[0:16, :], U32) | jnp.tile(gate, (1, ND)), BF)
            lhs = jnp.concatenate([top, lhs[16:, :]], axis=0)
        return gelu2(jnp.dot(lhs, win_v[:, lanes(n)], preferred_element_type=F32))

    def w2_rows(a):
        return pl.ds(S + (a % 4) * C, C)

    def z2_tile(a, n, gate=None):
        z1_v[w2_rows(a), lanes(n)] = proj(a, NT + n, gate)

    def z1_tile(a, n, gate=None):
        t = proj(a, n, gate)
        z1_v[brows(a), lanes(n)] = t
        return t

    def ln_z2(a):
        w2 = z1_v[w2_rows(a), :]
        mu = jnp.sum(w2, axis=-1, keepdims=True) * (1.0 / FH)
        ex2 = jnp.sum(w2 * w2, axis=-1, keepdims=True) * (1.0 / FH)
        var = jnp.maximum(ex2 - mu * mu, 0.0)
        rs = 0.25 * jax.lax.rsqrt(var + 4.0 * EPS)
        z2_v[brows(a), :] = ((w2 - mu) * rs).astype(BF)

    def region(blks, hch=(0, 0), kch=(0, 0)):
        hs = [(a, dt) for a in range(hch[0], hch[0] + hch[1]) for dt in range(ND)]
        us = [(a, dt) for a in range(kch[0], kch[0] + kch[1]) for dt in range(ND)]

        def next_ln_q(a, n, t):
            tok = pltpu.bitcast(t, U32)
            if n == 0:
                tok = jnp.concatenate([tok, z2_words(a)], axis=0)
            ln_q(a + 1, fence(tok), n, NLQ)

        for bi, a in enumerate(blks):
            last = bi == len(blks) - 1
            nh = len(hs) // (len(blks) - bi)
            nu = len(us) // (len(blks) - bi)
            nh_mid = max(nh - 4, 0) if last else nh
            if a == NB - 1:
                slots, marks = U_SLOTS_FINAL, []
            elif nh_mid >= 6:
                slots, marks = U_SLOTS_EARLY, LNQ_MANY_H
            else:
                slots, marks = U_SLOTS, LNQ_SOME_H if nh_mid >= 4 else LNQ_NO_H
            slots = [x for x in slots if not (last and x == 2 * NT)]
            cnt = [0] * (2 * NT + 1)
            for j in range(nu):
                cnt[slots[j % len(slots)]] += 1
            for n in range(NT):
                z2_tile(a, n)
                for _ in range(cnt[n]):
                    u_dft(*us.pop(0))
            hres = [h_dft(*hs.pop(0)) for _ in range(nh_mid)]
            for _ in range(cnt[NT]):
                u_dft(*us.pop(0))
            ln_z2(a)
            for part, (kind, tile, row) in enumerate(marks):
                if kind == 'h':
                    next_ln_q(a, part, hres[tile][row:row + 8, :])
            for n in range(NT):
                t = z1_tile(a, n)
                for part, (kind, tile, row) in enumerate(marks):
                    if kind == 'z' and tile == n:
                        next_ln_q(a, part, t[row:row + 8, :])
                for _ in range(cnt[NT + 1 + n]):
                    u_dft(*us.pop(0))
            for _ in range(nh - nh_mid):
                h_dft(*hs.pop(0))
        assert not hs and not us

    def conv_pos(ft, ft2, par, dt, after):
        cols = lanes(dt)
        prev = None
        for a in range(NB):
            ar, ai = (None, None) if prev is None else (-prev[1], prev[0])
            for dl in range(a + 1):
                hr = hf_v[ft, dl, 0:8, cols]
                hi = hf_v[ft, dl, 8:16, cols]
                ur = p_v[ft, a - dl, 0:8, cols]
                ui = p_v[ft, a - dl, 8:16, cols]
                if ar is None:
                    ar, ai = ur * hr - ui * hi, ur * hi + ui * hr
                    if after is not None:
                        z = fence(pltpu.bitcast(after, U32))
                        ar = pltpu.bitcast(pltpu.bitcast(ar, U32) | z, F32)
                        ai = pltpu.bitcast(pltpu.bitcast(ai, U32) | z, F32)
                else:
                    ar = (ar + ur * hr) - ui * hi
                    ai = (ai + ur * hi) + ui * hr
            prev = (ar, ai) if prev is None else (ar + prev[1], ai - prev[0])
            w_v[a * 16 + ft2, par * 8:(par + 1) * 8, cols] = ar.astype(BF)
            w_v[a * 16 + 8 + ft2, par * 8:(par + 1) * 8, cols] = ai.astype(BF)
        return prev[0]

    gl_v = wout_v
    GL0 = FH

    def xn_gate(a, dt, g_ref, g_rows):
        rows = brows(a)
        hh = jnp.dot(g_ref[g_rows, :], wout_v[0:FH, lanes(dt)], preferred_element_type=F32)
        return xn_v[rows, lanes(dt)].astype(F32) * (hh + hh * jnp.tanh(hh))

    def phase2a(i, carry):
        cp_wsp(i).wait()
        eye = (jax.lax.broadcasted_iota(jnp.int32, (C, C), 0)
               == jax.lax.broadcasted_iota(jnp.int32, (C, C), 1))
        bcols = {}

        def g_tile(m, n):
            a = i * (TA // C) + m
            rows = brows(a)
            if m not in bcols:
                bcols[m] = jnp.sum(jnp.where(eye, b32_v[pl.ds(a, 1), :], 0.0), axis=-1, keepdims=True)
            g = jnp.dot(wsp_v[rows, :], z2_v[:, lanes(n)], preferred_element_type=F32) + bcols[m]
            g = (z1_v[rows, lanes(n)] * g).astype(BF)
            if m < NOP:
                gl_v[GL0 + m * C:GL0 + (m + 1) * C, lanes(n)] = g
            else:
                gg_v[ds(i * C, C), lanes(n)] = g

        tiles = [(m, n) for m in range(TA // C) for n in range(NT)]
        for m, n in tiles[:-1]:
            g_tile(m, n)
        for m in range(NOP):
            a = i * (TA // C) + m
            for dt in range(ND):
                xg_v[brows(a), lanes(dt)] = xn_gate(a, dt, gl_v, pl.ds(GL0 + m * C, C))
        g_tile(*tiles[-1])
        nft = NB * TA // S
        last = None
        for ft in range(nft):
            for dt in range(ND):
                last = conv_pos(i * nft + ft, i * (nft // 2) + ft // 2, ft % 2, dt, last)
        return carry

    step = pl.program_id(0)

    @pl.when(step == 0)
    def _():
        for grp in groups:
            for cp in grp:
                cp.start()
        cp_wout.start()
        for i in range(S // TA):
            cp_wsp(i).start()
        k_v[0:HALO, :] = jnp.zeros((HALO, D), BF)

    @pl.when(step == 1)
    def _():
        cp_wout.wait()
        jax.lax.fori_loop(0, S // TA, phase2a, 0)

        rev = 7 - jax.lax.broadcasted_iota(jnp.int32, (8, 128), 0)
        for a in range(NB):
            rows = brows(a)
            for dt in range(ND):
                cols = lanes(dt)
                ev = jnp.dot(fg_v[2 * C:2 * C + C // 2, 0:C],
                             w_v[ds(a * 16, 8), :, cols].reshape(C, 128), preferred_element_type=F32)
                od = jnp.dot(fg_v[2 * C:2 * C + C // 2, C:2 * C],
                             w_v[ds(a * 16 + 8, 8), :, cols].reshape(C, 128), preferred_element_type=F32)
                lo = ev - od
                ys = [jnp.take_along_axis(lo[g * 8:(g + 1) * 8, :], rev, axis=0)
                      for g in range(C // 16 - 1, -1, -1)]
                y = jnp.concatenate(ys + [ev + od], axis=0)
                xg = xg_v[rows, cols] if a % (TA // C) < NOP else xn_gate(a, dt, gg_v, brows(a // (TA // C)))
                o_v[rows, cols] = (q_v[rows, cols].astype(F32) + xg * y).astype(BF)
                if a == NB - 1:
                    cp_o(a, cols).start()
            if a < NB - 1:
                cp_o(a).start()
        pltpu.make_async_copy(o_v, o_hbm, sem_o.at[0]).wait()

    @pl.when(step == 0)
    def _():
        wait(0)
        ln_q(0)
        ln_q(1)
        wait(1)
        for n in (0, 1):
            z2_tile(0, n)
            z2_tile(1, n)
        wait(2)
        ln_q(2)
        for n in (2, 3):
            z2_tile(0, n)
            z2_tile(1, n)
        for n in range(4):
            z2_tile(2, n)
        wait(3)
        ln_q(3)
        seq = ([(z2_tile, a, n) for a in range(3) for n in (4, 5)] + [(z2_tile, 3, n) for n in range(NT)]
               + [(z1_tile, a, 0) for a in range(4)])
        for j, (tile, a, n) in enumerate(seq):
            if j == 3:
                gate = fence(pltpu.bitcast(xn_v[brows(3), 0:128], U32))
            else:
                gate = fence(z2_words((7, 10, 14).index(j))) if j in (7, 10, 14) else None
            tile(a, n, gate)
            if j in (1, 3, 5):
                ln_z2(a)
        wait(4)
        ln_z2(3)
        for j, (a, n) in enumerate((a, n) for n in range(1, NT) for a in range(4)):
            t = z1_tile(a, n, fence(z2_words(3)) if j == 3 else None)
            if j in (5, 8, 11, 14):
                ln_q(4, fence(pltpu.bitcast(t[0:8, :], U32)), (j - 5) // 3, NLQ)
        region([4])
        wait(5)
        b32_v[...] = b_v[...].astype(F32) * 0.25
        region(list(range(5, 11)), HCH[0], KCH[0])
        wait(6)
        region(list(range(11, NB)), HCH[1], KCH[1])


@jax.jit
def pallas_recurrent_scan__ssm_conv_h3__mixer_gmlp__prompt_kernel(
    A_q: jax.Array,
    A_k: jax.Array,
    A_v: jax.Array,
    A_shift_k: jax.Array,
    A_ssm_k: jax.Array,
    A_ssm_D: jax.Array,
    B_x: jax.Array,
    B_w_in: jax.Array,
    B_w_sp: jax.Array,
    B_b_sp: jax.Array,
    B_w_out: jax.Array,
):
    del B_x
    any_spec = pl.BlockSpec(memory_space=pl.ANY)
    vm = pltpu.VMEM
    dma = pltpu.SemaphoreType.DMA
    out = pl.pallas_call(
        _kernel,
        out_shape=jax.ShapeDtypeStruct((S, D), BF),
        grid=(2,),
        in_specs=[any_spec] * 11,
        out_specs=any_spec,
        scratch_shapes=[
            vm((S // 2, D), U32),
            vm((S + 64, D), BF),
            vm((S, D), BF),
            vm((D // 2, S), U32),
            vm((D // 2, 2 * FH), U32),
            vm((S // 2, S), U32),
            vm(((FH + 512) // 2, FH), U32),
            vm(((2 * C + C // 2) // 2, 2 * C), U32),
            vm((S // 2, D), U32),
            vm((S + 4 * C, FH), F32),
            vm((S // 2, FH), U32),
            vm((NB, NB, 16, D), F32),
            vm((NB, NB, 16, D), F32),
            vm((NB * 16, 8, 1024), U32),
            vm((S // TA * C // 2, FH), U32),
            vm((S, D), F32),
            vm((S, D), BF),
            vm((NB, 128), F32),
            vm((NB, 128), BF),
            vm((4, 18 * 128), BF),
            vm((ND, 128), BF),
            dma((len(QCH),)), dma((len(KCH),)), dma((len(KCH),)), dma((len(HCH),)),
            dma((len(WCH),)), dma((S // TA,)), dma((1,)), dma((5,)),
        ],
        compiler_params=pltpu.CompilerParams(
            dimension_semantics=("arbitrary",),
            vmem_limit_bytes=110 * 1024 * 1024,
            disable_bounds_checks=True,
            disable_semaphore_checks=True,
        ),
    )(
        A_q.reshape(S, D), A_k.reshape(S, D), A_v.reshape(S, D),
        A_shift_k.T, A_ssm_k, A_ssm_D.reshape(ND, 128),
        B_w_in, B_w_sp, B_b_sp.reshape(NB, 128), B_w_out,
        _dft_consts(),
    )
    return out.reshape(1, S, D)
```

```python
import math

import jax
import jax.numpy as jnp
import numpy as np
import jax.experimental.pallas as pl
import jax.experimental.pallas.tpu as pltpu

S = 2048
D = 640
FH = 768
C = 128
NB = S // C
ND = D // 128
NT = FH // 128
HALO = 16
EPS = 1e-5
TA = 512
NOP = 3
NLQ = 4

BF = jnp.bfloat16
F32 = jnp.float32
U32 = jnp.uint32

QCH = [(0, 2), (2, 1), (3, 1), (4, 2), (6, 6), (12, 4)]
HCH = [(0, 5), (5, 11)]
KCH = [(0, 3), (3, 13)]
WCH = [(6, 2), (8, 2), (10, 2), (0, 1), (1, 5)]
U_SLOTS = [1, 3, 0, 2, 4, 11, 12, 5, 6, 6, 10, 9]
U_SLOTS_EARLY = [1, 3, 7, 9, 0, 2, 11, 12, 4, 5, 8, 10, 6, 6]
U_SLOTS_FINAL = [1, 3, 8, 10, 0, 2, 9, 11, 4, 7, 5, 6, 6]
LNQ_MANY_H = [('h', 4, 128), ('h', 8, 128), ('z', 1, 0), ('z', 3, 0)]
LNQ_SOME_H = [('h', 3, 248), ('z', 0, 64), ('z', 1, 120), ('z', 3, 0)]
LNQ_NO_H = [('z', 0, 64), ('z', 1, 64), ('z', 2, 64), ('z', 3, 0)]


def _dft_consts():
    theta = np.pi * (4 * np.arange(C) + 1) / (2 * C)

    def fwd(t):
        ang = theta[:, None] * t[None, :]
        re = np.cos(ang).reshape(C // 8, 8, C)
        im = -np.sin(ang).reshape(C // 8, 8, C)
        return np.stack([re, im], axis=1).reshape(2 * C, C)

    fg = np.zeros((2 * C + C // 2, 2 * C), np.float64)
    fg[:2 * C, :C] = fwd(np.arange(C) - (C - 1) / 2)
    fg[:2 * C, C:] = fwd(np.arange(C))
    ang = (np.arange(C // 2) + 0.5)[:, None] * theta[None, :]
    fg[2 * C:, :C] = np.cos(ang) / C
    fg[2 * C:, C:] = -np.sin(ang) / C
    return fg.astype(np.float32).astype(BF)


def _kernel(q_hbm, k_hbm, v_hbm, sk_hbm, h_hbm, d_hbm, win_hbm, wsp_hbm, b_hbm, wout_hbm,
            fg_hbm, o_hbm,
            q_u, k_v, v_v, h_u, win_u, wsp_u, wout_u, fg_u,
            xn_u, z1_v, z2_u, p_v, hf_v, w_u, gg_u, xg_v, o_v, b32_v, b_v, sk_v, d_v,
            sem_q, sem_k, sem_v, sem_h, sem_w, sem_wsp, sem_o, sem_m):
    q_v = q_u.bitcast(BF)
    h_v = h_u.bitcast(BF)
    win_v = win_u.bitcast(BF)
    wsp_v = wsp_u.bitcast(BF)
    wout_v = wout_u.bitcast(BF)
    fg_v = fg_u.bitcast(BF)
    xn_v = xn_u.bitcast(BF)
    z2_v = z2_u.bitcast(BF)
    w_v = w_u.bitcast(BF)
    gg_v = gg_u.bitcast(BF)

    def ds(start, size):
        if isinstance(start, int):
            return pl.ds(start, size)
        return pl.ds(pl.multiple_of(start, size), size)

    def lanes(n):
        return slice(n * 128, (n + 1) * 128)

    def blocks(ch):
        return pl.ds(ch[0] * C, ch[1] * C)

    def brows(a):
        return ds(a * C, C)

    def cp_q(c):
        r = blocks(QCH[c])
        return pltpu.make_async_copy(q_hbm.at[r, :], q_v.at[r, :], sem_q.at[c])

    def cp_k(c):
        b0, n = KCH[c]
        return pltpu.make_async_copy(k_hbm.at[blocks(KCH[c]), :],
                                     k_v.at[pl.ds(b0 * C + HALO, n * C), :], sem_k.at[c])

    def cp_v(c):
        r = blocks(KCH[c])
        return pltpu.make_async_copy(v_hbm.at[r, :], v_v.at[r, :], sem_v.at[c])

    def cp_h(c):
        r = blocks(HCH[c])
        return pltpu.make_async_copy(h_hbm.at[:, r], h_v.at[:, r], sem_h.at[c])

    def cp_w(c):
        r = blocks(WCH[c])
        return pltpu.make_async_copy(win_hbm.at[:, r], win_v.at[:, r], sem_w.at[c])

    def cp_wsp(i):
        r = ds(i * TA, TA)
        return pltpu.make_async_copy(wsp_hbm.at[r, :], wsp_v.at[r, :], sem_wsp.at[i])

    def cp_o(a, cols=slice(None)):
        r = brows(a)
        return pltpu.make_async_copy(o_v.at[r, cols], o_hbm.at[r, cols], sem_o.at[0])

    cp_f = pltpu.make_async_copy(fg_hbm, fg_v, sem_m.at[0])
    cp_sk = pltpu.make_async_copy(sk_hbm, sk_v.at[:, 0:D], sem_m.at[1])
    cp_d = pltpu.make_async_copy(d_hbm, d_v, sem_m.at[2])
    cp_b = pltpu.make_async_copy(b_hbm, b_v, sem_m.at[3])
    cp_wout = pltpu.make_async_copy(wout_hbm, wout_v.at[0:FH, 0:D], sem_m.at[4])

    groups = [
        [cp_q(0)], [cp_w(0)], [cp_q(1), cp_w(1)], [cp_q(2), cp_w(2), cp_w(3)], [cp_q(3), cp_w(4)],
        [cp_f, cp_sk, cp_d, cp_b, cp_q(4), cp_h(0), cp_k(0), cp_v(0)],
        [cp_q(5), cp_h(1), cp_k(1), cp_v(1)],
    ]

    def wait(g):
        for cp in groups[g]:
            cp.wait()

    c0 = math.sqrt(2.0 / math.pi)
    c1 = c0 * 0.044715

    def gelu2(x):
        return x + x * jnp.tanh(x * (c0 + c1 * (x * x)))

    def fence(tok):
        t = tok[0:8, :]
        for g in range(1, tok.shape[0] // 8):
            t = t | tok[g * 8:(g + 1) * 8, :]
        return t & pltpu.bitcast(k_v[0:HALO, 0:128], U32)

    def z2_words(a, half=None):
        r = brows(a) if half is None else pl.ds(a * C + half * (C // 2), C // 2)
        return pltpu.bitcast(z2_v[r, 0:128], U32)

    def ln_q(a, gate=None, part=0, nparts=1):
        n = C // nparts
        r = pl.ds(a * C + part * n, n)
        x = q_v[r, :]
        if gate is not None:
            x = pltpu.bitcast(pltpu.bitcast(x, U32) | jnp.tile(gate, (n // 16, ND)), BF)
        x = x.astype(F32)
        mu = jnp.sum(x, axis=-1, keepdims=True) * (1.0 / D)
        ex2 = jnp.sum(x * x, axis=-1, keepdims=True) * (1.0 / D)
        var = jnp.maximum(ex2 - mu * mu, 0.0)
        mu = mu.astype(BF).astype(F32)
        xn_v[r, :] = ((x - mu) * jax.lax.rsqrt(var + EPS)).astype(BF)

    def h_dft(a, dt):
        res = jax.lax.dot_general(fg_v[0:2 * C, C:2 * C], h_v[lanes(dt), brows(a)],
                                  (((1,), (1,)), ((), ())), preferred_element_type=F32)
        spec = res.reshape(NB, 16, 128)
        if a == 0:
            dv = d_v[...].astype(F32)[dt:dt + 1, :]
            spec = jnp.concatenate([spec[:, 0:8, :] + dv[None], spec[:, 8:16, :]], axis=1)
        hf_v[:, a, :, lanes(dt)] = spec
        return res

    def u_dft(a, dt):
        cols = lanes(dt)
        kf = k_v[pl.ds(a * C + HALO - 8, C + 8), cols].astype(F32)
        sk = sk_v[:, cols].astype(F32)
        ks = kf[8:, :] * sk[0:1, :]
        for t in range(1, 4):
            ks = ks + pltpu.roll(kf, t, axis=0)[8:, :] * sk[t:t + 1, :]
        kv = (ks * v_v[brows(a), cols].astype(F32)).astype(BF)
        res = jnp.dot(fg_v[0:2 * C, 0:C], kv, preferred_element_type=F32)
        p_v[:, a, :, cols] = res.reshape(NB, 16, 128)

    def proj(a, n, gate=None):
        lhs = xn_v[brows(a), :]
        if gate is not None:
            top = pltpu.bitcast(pltpu.bitcast(lhs[0:16, :], U32) | jnp.tile(gate, (1, ND)), BF)
            lhs = jnp.concatenate([top, lhs[16:, :]], axis=0)
        return gelu2(jnp.dot(lhs, win_v[:, lanes(n)], preferred_element_type=F32))

    def w2_rows(a):
        return pl.ds(S + (a % 4) * C, C)

    def z2_tile(a, n, gate=None):
        z1_v[w2_rows(a), lanes(n)] = proj(a, NT + n, gate)

    def z1_tile(a, n, gate=None):
        t = proj(a, n, gate)
        z1_v[brows(a), lanes(n)] = t
        return t

    def ln_z2(a):
        w2 = z1_v[w2_rows(a), :]
        mu = jnp.sum(w2, axis=-1, keepdims=True) * (1.0 / FH)
        ex2 = jnp.sum(w2 * w2, axis=-1, keepdims=True) * (1.0 / FH)
        var = jnp.maximum(ex2 - mu * mu, 0.0)
        rs = 0.25 * jax.lax.rsqrt(var + 4.0 * EPS)
        z2_v[brows(a), :] = ((w2 - mu) * rs).astype(BF)

    def region(blks, hch=(0, 0), kch=(0, 0)):
        hs = [(a, dt) for a in range(hch[0], hch[0] + hch[1]) for dt in range(ND)]
        us = [(a, dt) for a in range(kch[0], kch[0] + kch[1]) for dt in range(ND)]

        def next_ln_q(a, n, t):
            tok = pltpu.bitcast(t, U32)
            if n == 0:
                tok = jnp.concatenate([tok, z2_words(a)], axis=0)
            ln_q(a + 1, fence(tok), n, NLQ)

        for bi, a in enumerate(blks):
            last = bi == len(blks) - 1
            nh = len(hs) // (len(blks) - bi)
            nu = len(us) // (len(blks) - bi)
            nh_mid = max(nh - 4, 0) if last else nh
            if a == NB - 1:
                slots, marks = U_SLOTS_FINAL, []
            elif nh_mid >= 6:
                slots, marks = U_SLOTS_EARLY, LNQ_MANY_H
            else:
                slots, marks = U_SLOTS, LNQ_SOME_H if nh_mid >= 4 else LNQ_NO_H
            slots = [x for x in slots if not (last and x == 2 * NT)]
            cnt = [0] * (2 * NT + 1)
            for j in range(nu):
                cnt[slots[j % len(slots)]] += 1
            for n in range(NT):
                z2_tile(a, n)
                for _ in range(cnt[n]):
                    u_dft(*us.pop(0))
            hres = [h_dft(*hs.pop(0)) for _ in range(nh_mid)]
            for _ in range(cnt[NT]):
                u_dft(*us.pop(0))
            ln_z2(a)
            for part, (kind, tile, row) in enumerate(marks):
                if kind == 'h':
                    next_ln_q(a, part, hres[tile][row:row + 8, :])
            for n in range(NT):
                t = z1_tile(a, n)
                for part, (kind, tile, row) in enumerate(marks):
                    if kind == 'z' and tile == n:
                        next_ln_q(a, part, t[row:row + 8, :])
                for _ in range(cnt[NT + 1 + n]):
                    u_dft(*us.pop(0))
            for _ in range(nh - nh_mid):
                h_dft(*hs.pop(0))
        assert not hs and not us

    def conv_pos(ft, ft2, par, dt, after):
        cols = lanes(dt)
        prev = None
        for a in range(NB):
            ar, ai = (None, None) if prev is None else (-prev[1], prev[0])
            for dl in range(a + 1):
                hr = hf_v[ft, dl, 0:8, cols]
                hi = hf_v[ft, dl, 8:16, cols]
                ur = p_v[ft, a - dl, 0:8, cols]
                ui = p_v[ft, a - dl, 8:16, cols]
                if ar is None:
                    ar, ai = ur * hr - ui * hi, ur * hi + ui * hr
                    if after is not None:
                        z = fence(pltpu.bitcast(after, U32))
                        ar = pltpu.bitcast(pltpu.bitcast(ar, U32) | z, F32)
                        ai = pltpu.bitcast(pltpu.bitcast(ai, U32) | z, F32)
                else:
                    ar = (ar + ur * hr) - ui * hi
                    ai = (ai + ur * hi) + ui * hr
            prev = (ar, ai) if prev is None else (ar + prev[1], ai - prev[0])
            w_v[a * 16 + ft2, par * 8:(par + 1) * 8, cols] = ar.astype(BF)
            w_v[a * 16 + 8 + ft2, par * 8:(par + 1) * 8, cols] = ai.astype(BF)
        return prev[0]

    gl_v = wout_v
    GL0 = FH

    def xn_gate(a, dt, g_ref, g_rows):
        rows = brows(a)
        hh = jnp.dot(g_ref[g_rows, :], wout_v[0:FH, lanes(dt)], preferred_element_type=F32)
        return xn_v[rows, lanes(dt)].astype(F32) * (hh + hh * jnp.tanh(hh))

    def phase2a(i, carry):
        cp_wsp(i).wait()
        eye = (jax.lax.broadcasted_iota(jnp.int32, (C, C), 0)
               == jax.lax.broadcasted_iota(jnp.int32, (C, C), 1))
        bcols = {}

        def g_tile(m, n):
            a = i * (TA // C) + m
            rows = brows(a)
            if m not in bcols:
                bcols[m] = jnp.sum(jnp.where(eye, b32_v[pl.ds(a, 1), :], 0.0), axis=-1, keepdims=True)
            g = jnp.dot(wsp_v[rows, :], z2_v[:, lanes(n)], preferred_element_type=F32) + bcols[m]
            g = (z1_v[rows, lanes(n)] * g).astype(BF)
            if m < NOP:
                gl_v[GL0 + m * C:GL0 + (m + 1) * C, lanes(n)] = g
            else:
                gg_v[ds(i * C, C), lanes(n)] = g

        tiles = [(m, n) for m in range(TA // C) for n in range(NT)]
        for m, n in tiles[:-1]:
            g_tile(m, n)
        for m in range(NOP):
            a = i * (TA // C) + m
            for dt in range(ND):
                xg_v[brows(a), lanes(dt)] = xn_gate(a, dt, gl_v, pl.ds(GL0 + m * C, C))
        g_tile(*tiles[-1])
        nft = NB * TA // S
        last = None
        for ft in range(nft):
            for dt in range(ND):
                last = conv_pos(i * nft + ft, i * (nft // 2) + ft // 2, ft % 2, dt, last)
        return carry

    step = pl.program_id(0)

    @pl.when(step == 0)
    def _():
        for grp in groups:
            for cp in grp:
                cp.start()
        cp_wout.start()
        for i in range(S // TA):
            cp_wsp(i).start()
        k_v[0:HALO, :] = jnp.zeros((HALO, D), BF)

    @pl.when(step == 1)
    def _():
        cp_wout.wait()
        jax.lax.fori_loop(0, S // TA, phase2a, 0)

        rev = 7 - jax.lax.broadcasted_iota(jnp.int32, (8, 128), 0)
        for a in range(NB):
            rows = brows(a)
            for dt in range(ND):
                cols = lanes(dt)
                ev = jnp.dot(fg_v[2 * C:2 * C + C // 2, 0:C],
                             w_v[ds(a * 16, 8), :, cols].reshape(C, 128), preferred_element_type=F32)
                od = jnp.dot(fg_v[2 * C:2 * C + C // 2, C:2 * C],
                             w_v[ds(a * 16 + 8, 8), :, cols].reshape(C, 128), preferred_element_type=F32)
                lo = ev - od
                ys = [jnp.take_along_axis(lo[g * 8:(g + 1) * 8, :], rev, axis=0)
                      for g in range(C // 16 - 1, -1, -1)]
                y = jnp.concatenate(ys + [ev + od], axis=0)
                xg = xg_v[rows, cols] if a % (TA // C) < NOP else xn_gate(a, dt, gg_v, brows(a // (TA // C)))
                o_v[rows, cols] = (q_v[rows, cols].astype(F32) + xg * y).astype(BF)
                if a == NB - 1:
                    cp_o(a, cols).start()
            if a < NB - 1:
                cp_o(a).start()
        pltpu.make_async_copy(o_v, o_hbm, sem_o.at[0]).wait()

    @pl.when(step == 0)
    def _():
        wait(0)
        ln_q(0)
        ln_q(1)
        wait(1)
        for n in (0, 1):
            z2_tile(0, n)
            z2_tile(1, n)
        wait(2)
        ln_q(2)
        for n in (2, 3):
            z2_tile(0, n)
            z2_tile(1, n)
        for n in range(4):
            z2_tile(2, n)
        wait(3)
        ln_q(3)
        seq = ([(z2_tile, a, n) for a in range(3) for n in (4, 5)] + [(z2_tile, 3, n) for n in range(NT)]
               + [(z1_tile, a, 0) for a in range(4)])
        for j, (tile, a, n) in enumerate(seq):
            if j == 3:
                gate = fence(pltpu.bitcast(xn_v[brows(3), 0:128], U32))
            else:
                gate = fence(z2_words(0, (7, 10).index(j))) if j in (7, 10) else None
            tile(a, n, gate)
            if j == 1:
                ln_z2(0)
        wait(4)
        for a in (1, 2, 3):
            ln_z2(a)
        for j, (a, n) in enumerate((a, n) for n in range(1, NT) for a in range(4)):
            gate = fence(z2_words(1 + (j - 2) // 4, (j // 2 - 1) % 2)) if j in (2, 4, 6, 8, 10, 12) else None
            t = z1_tile(a, n, gate)
            if j in (13, 14, 16, 17):
                ln_q(4, fence(pltpu.bitcast(t[0:8, :], U32)), (13, 14, 16, 17).index(j), NLQ)
        region([4])
        wait(5)
        b32_v[...] = b_v[...].astype(F32) * 0.25
        region(list(range(5, 11)), HCH[0], KCH[0])
        wait(6)
        region(list(range(11, NB)), HCH[1], KCH[1])


@jax.jit
def pallas_recurrent_scan__ssm_conv_h3__mixer_gmlp__prompt_kernel(
    A_q: jax.Array,
    A_k: jax.Array,
    A_v: jax.Array,
    A_shift_k: jax.Array,
    A_ssm_k: jax.Array,
    A_ssm_D: jax.Array,
    B_x: jax.Array,
    B_w_in: jax.Array,
    B_w_sp: jax.Array,
    B_b_sp: jax.Array,
    B_w_out: jax.Array,
):
    del B_x
    any_spec = pl.BlockSpec(memory_space=pl.ANY)
    vm = pltpu.VMEM
    dma = pltpu.SemaphoreType.DMA
    out = pl.pallas_call(
        _kernel,
        out_shape=jax.ShapeDtypeStruct((S, D), BF),
        grid=(2,),
        in_specs=[any_spec] * 11,
        out_specs=any_spec,
        scratch_shapes=[
            vm((S // 2, D), U32),
            vm((S + 64, D), BF),
            vm((S, D), BF),
            vm((D // 2, S), U32),
            vm((D // 2, 2 * FH), U32),
            vm((S // 2, S), U32),
            vm(((FH + 512) // 2, FH), U32),
            vm(((2 * C + C // 2) // 2, 2 * C), U32),
            vm((S // 2, D), U32),
            vm((S + 4 * C, FH), F32),
            vm((S // 2, FH), U32),
            vm((NB, NB, 16, D), F32),
            vm((NB, NB, 16, D), F32),
            vm((NB * 16, 8, 1024), U32),
            vm((S // TA * C // 2, FH), U32),
            vm((S, D), F32),
            vm((S, D), BF),
            vm((NB, 128), F32),
            vm((NB, 128), BF),
            vm((4, 18 * 128), BF),
            vm((ND, 128), BF),
            dma((len(QCH),)), dma((len(KCH),)), dma((len(KCH),)), dma((len(HCH),)),
            dma((len(WCH),)), dma((S // TA,)), dma((1,)), dma((5,)),
        ],
        compiler_params=pltpu.CompilerParams(
            dimension_semantics=("arbitrary",),
            vmem_limit_bytes=110 * 1024 * 1024,
            disable_bounds_checks=True,
            disable_semaphore_checks=True,
        ),
    )(
        A_q.reshape(S, D), A_k.reshape(S, D), A_v.reshape(S, D),
        A_shift_k.T, A_ssm_k, A_ssm_D.reshape(ND, 128),
        B_w_in, B_w_sp, B_b_sp.reshape(NB, 128), B_w_out,
        _dft_consts(),
    )
    return out.reshape(1, S, D)
```

```python
import math

import jax
import jax.numpy as jnp
import numpy as np
import jax.experimental.pallas as pl
import jax.experimental.pallas.tpu as pltpu

S = 2048
D = 640
FH = 768
C = 128
NB = S // C
ND = D // 128
NT = FH // 128
HALO = 16
EPS = 1e-5
HK = S // 2
HN = FH // 2
TA = 512
NOP = 3
NLQ = 4
H_LATE = 16
TREE = 12

BF = jnp.bfloat16
F32 = jnp.float32
U32 = jnp.uint32

QCH = [(0, 2), (2, 1), (3, 1), (4, 2), (6, 6), (12, 4)]
HCH = [(0, 5), (5, 11)]
KCH = [(0, 3), (3, 13)]
WCH = [(6, 2), (8, 2), (10, 2), (0, 1), (1, 5)]
DFT_PLAN = [[(4, 4), (4, 4), (4, 4), (4, 0), (4, 0), (5, 3)],
            [(7, 13), (7, 13), (7, 13), (7, 13), (11, 13)]]
U_SLOTS = [1, 3, 0, 2, 4, 11, 12, 5, 6, 6, 10, 9]
U_SLOTS_EARLY = [1, 3, 7, 9, 0, 2, 11, 12, 4, 5, 8, 10, 6, 6]
U_SLOTS_FINAL = [1, 3, 8, 10, 0, 2, 9, 11, 4, 7, 5, 6, 6]
LNQ_MANY_H = [('h', 4, 128), ('h', 6, 128), ('z', 1, 0), ('z', 3, 0)]
LNQ_SOME_H = [('h', 3, 248), ('z', 0, 64), ('z', 1, 120), ('z', 3, 0)]
LNQ_NO_H = [('z', 0, 64), ('z', 1, 64), ('z', 2, 64), ('z', 3, 0)]


def _dft_consts():
    theta = np.pi * (4 * np.arange(C) + 1) / (2 * C)

    def fwd(t):
        ang = theta[:, None] * t[None, :]
        re = np.cos(ang).reshape(C // 8, 8, C)
        im = -np.sin(ang).reshape(C // 8, 8, C)
        return np.stack([re, im], axis=1).reshape(2 * C, C)

    fg = np.zeros((2 * C + C // 2, 2 * C), np.float64)
    fg[:2 * C, :C] = fwd(np.arange(C) - (C - 1) / 2)
    fg[:2 * C, C:] = fwd(np.arange(C))
    ang = (np.arange(C // 2) + 0.5)[:, None] * theta[None, :]
    fg[2 * C:, :C] = np.cos(ang) / C
    fg[2 * C:, C:] = -np.sin(ang) / C
    return fg.astype(np.float32).astype(BF)


def _kernel(q_hbm, k_hbm, v_hbm, sk_hbm, h_hbm, d_hbm, win_hbm, wsp_hbm, b_hbm, wout_hbm,
            fg_hbm, o_hbm,
            q_u, k_v, v_v, h_u, win_u, wsp_u, wout_u, fg_u,
            xn_u, z1_v, z2_u, t_u, p_v, hf_v, w_u, gg_u, xg_v, o_v, b32_v, b_v, sk_v, d_v,
            sem_q, sem_k, sem_v, sem_h, sem_w, sem_wsp, sem_o, sem_m):
    q_v = q_u.bitcast(BF)
    h_v = h_u.bitcast(BF)
    win_v = win_u.bitcast(BF)
    wsp_v = wsp_u.bitcast(BF)
    wout_v = wout_u.bitcast(BF)
    fg_v = fg_u.bitcast(BF)
    xn_v = xn_u.bitcast(BF)
    z2_v = z2_u.bitcast(BF)
    t_v = t_u.bitcast(BF)
    w_v = w_u.bitcast(BF)
    gg_v = gg_u.bitcast(BF)

    def ds(start, size):
        if isinstance(start, int):
            return pl.ds(start, size)
        return pl.ds(pl.multiple_of(start, size), size)

    def lanes(n):
        return slice(n * 128, (n + 1) * 128)

    def blocks(ch):
        return pl.ds(ch[0] * C, ch[1] * C)

    def brows(a):
        return ds(a * C, C)

    def cp_q(c):
        r = blocks(QCH[c])
        return pltpu.make_async_copy(q_hbm.at[r, :], q_v.at[r, :], sem_q.at[c])

    def cp_k(c):
        b0, n = KCH[c]
        return pltpu.make_async_copy(k_hbm.at[blocks(KCH[c]), :],
                                     k_v.at[pl.ds(b0 * C + HALO, n * C), :], sem_k.at[c])

    def cp_v(c):
        r = blocks(KCH[c])
        return pltpu.make_async_copy(v_hbm.at[r, :], v_v.at[r, :], sem_v.at[c])

    def cp_h(c):
        r = blocks(HCH[c])
        return pltpu.make_async_copy(h_hbm.at[:, r], h_v.at[0:D, r], sem_h.at[c])

    def cp_w(c):
        r = blocks(WCH[c])
        return pltpu.make_async_copy(win_hbm.at[:, r], win_v.at[:, r], sem_w.at[c])

    def cp_wsp(i):
        r = ds(i * TA, TA)
        return pltpu.make_async_copy(wsp_hbm.at[r, :], wsp_v.at[r, :], sem_wsp.at[i])

    def cp_o(a, cols=slice(None)):
        r = brows(a)
        return pltpu.make_async_copy(o_v.at[r, cols], o_hbm.at[r, cols], sem_o.at[0])

    cp_f = pltpu.make_async_copy(fg_hbm, fg_v, sem_m.at[0])
    cp_sk = pltpu.make_async_copy(sk_hbm, sk_v.at[:, 0:D], sem_m.at[1])
    cp_d = pltpu.make_async_copy(d_hbm, d_v, sem_m.at[2])
    cp_b = pltpu.make_async_copy(b_hbm, b_v, sem_m.at[3])
    cp_wout = pltpu.make_async_copy(wout_hbm, wout_v.at[0:FH, 0:D], sem_m.at[4])

    groups = [
        [cp_q(0)], [cp_w(0)], [cp_q(1), cp_w(1)], [cp_q(2), cp_w(2), cp_w(3)], [cp_q(3), cp_w(4)],
        [cp_f, cp_sk, cp_d, cp_b, cp_q(4), cp_h(0), cp_k(0), cp_v(0)],
        [cp_q(5), cp_h(1), cp_k(1), cp_v(1)],
    ]

    def wait(g):
        for cp in groups[g]:
            cp.wait()

    c0 = math.sqrt(2.0 / math.pi)
    c1 = c0 * 0.044715

    def gelu2(x):
        return x + x * jnp.tanh(x * (c0 + c1 * (x * x)))

    def fence(tok):
        t = tok[0:8, :]
        for g in range(1, tok.shape[0] // 8):
            t = t | tok[g * 8:(g + 1) * 8, :]
        return t & pltpu.bitcast(k_v[0:HALO, 0:128], U32)

    def z2_words(a, half=None):
        r = brows(a) if half is None else pl.ds(a * C + half * (C // 2), C // 2)
        return pltpu.bitcast(z2_v[r, 0:128], U32)

    def ln_q(a, gate=None, part=0, nparts=1):
        n = C // nparts
        r = pl.ds(a * C + part * n, n)
        x = q_v[r, :]
        if gate is not None:
            x = pltpu.bitcast(pltpu.bitcast(x, U32) | jnp.tile(gate, (n // 16, ND)), BF)
        x = x.astype(F32)
        mu = jnp.sum(x, axis=-1, keepdims=True) * (1.0 / D)
        ex2 = jnp.sum(x * x, axis=-1, keepdims=True) * (1.0 / D)
        var = jnp.maximum(ex2 - mu * mu, 0.0)
        mu = mu.astype(BF).astype(F32)
        xn_v[r, :] = ((x - mu) * jax.lax.rsqrt(var + EPS)).astype(BF)

    def h_dft(a, dt):
        res = jax.lax.dot_general(fg_v[0:2 * C, C:2 * C], h_v[lanes(dt), brows(a)],
                                  (((1,), (1,)), ((), ())), preferred_element_type=F32)
        spec = res.reshape(NB, 16, 128)
        if a == 0:
            dv = d_v[...].astype(F32)[dt:dt + 1, :]
            spec = jnp.concatenate([spec[:, 0:8, :] + dv[None], spec[:, 8:16, :]], axis=1)
        hf_v[:, a, :, lanes(dt)] = spec
        return res

    def u_dft(a, dt):
        cols = lanes(dt)
        kf = k_v[pl.ds(a * C + HALO - 8, C + 8), cols].astype(F32)
        sk = sk_v[:, cols].astype(F32)
        ks = kf[8:, :] * sk[0:1, :]
        for t in range(1, 4):
            ks = ks + pltpu.roll(kf, t, axis=0)[8:, :] * sk[t:t + 1, :]
        kv = (ks * v_v[brows(a), cols].astype(F32)).astype(BF)
        res = jnp.dot(fg_v[0:2 * C, 0:C], kv, preferred_element_type=F32)
        p_v[:, a, :, cols] = res.reshape(NB, 16, 128)

    def proj(a, n, gate=None):
        lhs = xn_v[brows(a), :]
        if gate is not None:
            top = pltpu.bitcast(pltpu.bitcast(lhs[0:16, :], U32) | jnp.tile(gate, (1, ND)), BF)
            lhs = jnp.concatenate([top, lhs[16:, :]], axis=0)
        return gelu2(jnp.dot(lhs, win_v[:, lanes(n)], preferred_element_type=F32))

    def w2_rows(a):
        return pl.ds(S + (a % 4) * C, C)

    def z2_tile(a, n, gate=None):
        z1_v[w2_rows(a), lanes(n)] = proj(a, NT + n, gate)

    def z1_tile(a, n, gate=None):
        t = proj(a, n, gate)
        z1_v[brows(a), lanes(n)] = t
        return t

    def ln_z2(a):
        w2 = z1_v[w2_rows(a), :]
        mu = jnp.sum(w2, axis=-1, keepdims=True) * (1.0 / FH)
        ex2 = jnp.sum(w2 * w2, axis=-1, keepdims=True) * (1.0 / FH)
        var = jnp.maximum(ex2 - mu * mu, 0.0)
        rs = 0.25 * jax.lax.rsqrt(var + 4.0 * EPS)
        zn = (w2 - mu) * rs
        if a < NB // 2:
            z2_v[brows(a), 0:HN] = zn[:, :HN].astype(BF)
            t_v[brows(a), 0:HN] = (zn[:, HN:] - zn[:, :HN]).astype(BF)
        else:
            z2_v[brows(a), :] = zn.astype(BF)
            if a < NB - 1:
                t_rest(a - NB // 2, zn)

    def t_rest(r, bot):
        t2 = bot[:, HN:] - t_v[brows(r), 0:HN].astype(F32)
        t3 = t2 - z2_v[brows(r), 0:HN].astype(F32)
        t_v[brows(r), HN:4 * HN] = jnp.concatenate([t2, t3, bot[:, :HN] - t2], axis=1).astype(BF)

    def region(blks, hch=(0, 0), kch=(0, 0), plan=((0, 0),)):
        hs = [(a, dt) for a in range(hch[0], hch[0] + hch[1]) for dt in range(ND)]
        us = [(a, dt) for a in range(kch[0], kch[0] + kch[1]) for dt in range(ND)]

        def next_ln_q(a, n, t):
            tok = pltpu.bitcast(t, U32)
            if n == 0:
                tok = jnp.concatenate([tok, z2_words(a)], axis=0)
                if a >= NB // 2:
                    tw = pltpu.bitcast(t_v[brows(a - NB // 2), 4 * HN - 128:4 * HN], U32)
                    tok = jnp.concatenate([tok, tw], axis=0)
            ln_q(a + 1, fence(tok), n, NLQ)

        for bi, a in enumerate(blks):
            last = bi == len(blks) - 1
            nh, nu = plan[bi]
            nh_mid = max(nh - 4, 0) if last else nh
            if a == NB - 1:
                slots, marks = U_SLOTS_FINAL, []
            elif nh_mid >= 6:
                slots, marks = U_SLOTS_EARLY, LNQ_MANY_H
            else:
                slots, marks = U_SLOTS, LNQ_SOME_H if nh_mid >= 4 else LNQ_NO_H
            slots = [x for x in slots if not (last and x == 2 * NT)]
            cnt = [0] * (2 * NT + 1)
            for j in range(nu):
                cnt[slots[j % len(slots)]] += 1
            for n in range(NT):
                z2_tile(a, n)
                for _ in range(cnt[n]):
                    u_dft(*us.pop(0))
            hres = [h_dft(*hs.pop(0)) for _ in range(nh_mid)]
            for _ in range(cnt[NT]):
                u_dft(*us.pop(0))
            ln_z2(a)
            for part, (kind, tile, row) in enumerate(marks):
                if kind == 'h':
                    next_ln_q(a, part, hres[tile][row:row + 8, :])
            for n in range(NT):
                t = z1_tile(a, n)
                for part, (kind, tile, row) in enumerate(marks):
                    if kind == 'z' and tile == n:
                        next_ln_q(a, part, t[row:row + 8, :])
                for _ in range(cnt[NT + 1 + n]):
                    u_dft(*us.pop(0))
            for _ in range(nh - nh_mid):
                h_dft(*hs.pop(0))
        assert not us
        return hs

    def conv_pos(ft, ft2, par, dt, after):
        cols = lanes(dt)
        prev = None
        for a in range(NB):
            ar, ai = (None, None) if prev is None else (-prev[1], prev[0])
            for dl in range(a + 1):
                hr = hf_v[ft, dl, 0:8, cols]
                hi = hf_v[ft, dl, 8:16, cols]
                ur = p_v[ft, a - dl, 0:8, cols]
                ui = p_v[ft, a - dl, 8:16, cols]
                if ar is None:
                    ar, ai = ur * hr - ui * hi, ur * hi + ui * hr
                    if after is not None:
                        z = fence(after)
                        ar = pltpu.bitcast(pltpu.bitcast(ar, U32) | z, F32)
                        ai = pltpu.bitcast(pltpu.bitcast(ai, U32) | z, F32)
                elif (a * (a + 1) // 2 + dl) % TREE == 0:
                    ar = ar + (ur * hr - ui * hi)
                    ai = ai + (ur * hi + ui * hr)
                else:
                    ar = (ar + ur * hr) - ui * hi
                    ai = (ai + ur * hi) + ui * hr
            prev = (ar, ai) if prev is None else (ar + prev[1], ai - prev[0])
            w_v[a * 16 + ft2, par * 8:(par + 1) * 8, cols] = ar.astype(BF)
            w_v[a * 16 + 8 + ft2, par * 8:(par + 1) * 8, cols] = ai.astype(BF)
        return pltpu.bitcast(prev[0], U32)

    gl_v = wout_v
    GL0 = FH

    def xn_gate(a, dt, g_ref, g_rows):
        rows = brows(a)
        hh = jnp.dot(g_ref[g_rows, :], wout_v[0:FH, lanes(dt)], preferred_element_type=F32)
        return xn_v[rows, lanes(dt)].astype(F32) * (hh + hh * jnp.tanh(hh))

    def s_rows(slot, k):
        return D + (slot * 2 + k // 2) * C, (k % 2) * HK

    def s_val(slot, k):
        r0, c0_ = s_rows(slot, k)
        return h_v[r0:r0 + C, c0_:c0_ + HK]

    def s_sums(a0, nr, via_memory):
        last = None
        for slot in range(2):
            for c in range(HK // 128):
                for g in range(C // nr):
                    def ld(a, cols, gated):
                        x = wsp_v[ds(a * C + g * nr, nr), cols]
                        if gated and last is not None:
                            x = pltpu.bitcast(pltpu.bitcast(x, U32) | jnp.tile(fence(last), (nr // 16, 1)), BF)
                        return x.astype(F32)

                    a = a0 + 2 * slot
                    lo, hi = lanes(c), lanes(HK // 128 + c)
                    a11, a12 = ld(a, lo, not via_memory), ld(a, hi, not via_memory)
                    a21, a22 = ld(a + 1, lo, True), ld(a + 1, hi, not via_memory)
                    s1 = a21 + a22
                    s2 = s1 - a11
                    s4 = a12 - s2
                    words = []
                    for k, val in enumerate((s1, s2, a11 - a21, s4)):
                        r0, c0_ = s_rows(slot, k)
                        sl = (slice(r0 + g * nr, r0 + (g + 1) * nr), slice(c0_ + c * 128, c0_ + (c + 1) * 128))
                        h_v[sl] = val.astype(BF)
                        if via_memory:
                            words.append(pltpu.bitcast(h_v[sl], U32))
                    last = jnp.concatenate(words, axis=0) if via_memory else pltpu.bitcast(s4[nr - 8:nr, :], U32)

    def phase2a(i, carry):
        @pl.when(i + 1 < S // TA)
        def _():
            cp_wsp(i + 1).wait()

        eye = (jax.lax.broadcasted_iota(jnp.int32, (C, C), 0)
               == jax.lax.broadcasted_iota(jnp.int32, (C, C), 1))

        def bcol(a):
            return jnp.sum(jnp.where(eye, b32_v[pl.ds(a, 1), :], 0.0), axis=-1, keepdims=True)

        def mm(x, y):
            return jnp.dot(x, y, preferred_element_type=F32)

        def put(m, n, g):
            g = (z1_v[brows(i * (TA // C) + m), lanes(n)] * g).astype(BF)
            if m < NOP:
                gl_v[GL0 + m * C:GL0 + (m + 1) * C, lanes(n)] = g
            else:
                gg_v[ds(i * C, C), lanes(n)] = g

        for pp in range(2):
            m0 = 2 * pp
            a0 = i * (TA // C) + m0
            r0, r1 = brows(a0), brows(a0 + 1)
            b0 = bcol(a0)
            db = bcol(a0 + 1) - b0
            for j in range(NT // 2):
                jl, jr = lanes(j), lanes(NT // 2 + j)
                t1, t2, t3, t4 = (t_v[:, lanes(k * (NT // 2) + j)] for k in range(4))
                p1 = mm(wsp_v[r0, 0:HK], z2_v[0:HK, jl]) + b0
                put(m0, j, p1 + mm(wsp_v[r0, HK:S], z2_v[HK:S, jl]))
                u2 = p1 + mm(s_val(pp, 1), t2)
                u3 = (u2 + db) + mm(s_val(pp, 2), t3)
                put(m0 + 1, j, u3 + mm(wsp_v[r1, HK:S], t4))
                p5 = mm(s_val(pp, 0), t1)
                put(m0 + 1, NT // 2 + j, u3 + p5)
                put(m0, NT // 2 + j, (u2 + p5) + mm(s_val(pp, 3), z2_v[HK:S, jr]))
        for m in range(NOP):
            a = i * (TA // C) + m
            for dt in range(ND):
                xg_v[brows(a), lanes(dt)] = xn_gate(a, dt, gl_v, pl.ds(GL0 + m * C, C))
        s_sums(jnp.minimum(i + 1, S // TA - 1) * (TA // C), 16, True)
        nft = NB * TA // S
        last = None
        for ft in range(nft):
            for dt in range(ND):
                last = conv_pos(i * nft + ft, i * (nft // 2) + ft // 2, ft % 2, dt, last)
        return carry

    step = pl.program_id(0)

    @pl.when(step == 0)
    def _():
        for grp in groups:
            for cp in grp:
                cp.start()
        cp_wout.start()
        for i in range(S // TA):
            cp_wsp(i).start()
        k_v[0:HALO, :] = jnp.zeros((HALO, D), BF)

    @pl.when(step == 1)
    def _():
        cp_wsp(0).wait()
        cp_wout.wait()
        t_rest(NB // 2 - 1, z2_v[brows(NB - 1), :].astype(F32))
        for a, dt in [(a, dt) for a in range(NB) for dt in range(ND)][NB * ND - H_LATE:]:
            h_dft(a, dt)
        s_sums(0, 32, False)
        jax.lax.fori_loop(0, S // TA, phase2a, 0)

        rev = 7 - jax.lax.broadcasted_iota(jnp.int32, (8, 128), 0)
        for a in range(NB):
            rows = brows(a)
            for dt in range(ND):
                cols = lanes(dt)
                ev = jnp.dot(fg_v[2 * C:2 * C + C // 2, 0:C],
                             w_v[ds(a * 16, 8), :, cols].reshape(C, 128), preferred_element_type=F32)
                od = jnp.dot(fg_v[2 * C:2 * C + C // 2, C:2 * C],
                             w_v[ds(a * 16 + 8, 8), :, cols].reshape(C, 128), preferred_element_type=F32)
                lo = ev - od
                ys = [jnp.take_along_axis(lo[g * 8:(g + 1) * 8, :], rev, axis=0)
                      for g in range(C // 16 - 1, -1, -1)]
                y = jnp.concatenate(ys + [ev + od], axis=0)
                xg = xg_v[rows, cols] if a % (TA // C) < NOP else xn_gate(a, dt, gg_v, brows(a // (TA // C)))
                o_v[rows, cols] = (q_v[rows, cols].astype(F32) + xg * y).astype(BF)
                if a == NB - 1:
                    cp_o(a, cols).start()
            if a < NB - 1:
                cp_o(a).start()
        pltpu.make_async_copy(o_v, o_hbm, sem_o.at[0]).wait()

    @pl.when(step == 0)
    def _():
        wait(0)
        ln_q(0)
        ln_q(1)
        wait(1)
        for n in (0, 1):
            z2_tile(0, n)
            z2_tile(1, n)
        wait(2)
        ln_q(2)
        for n in (2, 3):
            z2_tile(0, n)
            z2_tile(1, n)
        for n in range(4):
            z2_tile(2, n)
        wait(3)
        ln_q(3)
        seq = ([(z2_tile, a, n) for a in range(3) for n in (4, 5)] + [(z2_tile, 3, n) for n in range(NT)]
               + [(z1_tile, a, 0) for a in range(4)])
        for j, (tile, a, n) in enumerate(seq):
            if j == 3:
                gate = fence(pltpu.bitcast(xn_v[brows(3), 0:128], U32))
            else:
                gate = fence(z2_words(0, (7, 10).index(j))) if j in (7, 10) else None
            tile(a, n, gate)
            if j == 1:
                ln_z2(0)
        wait(4)
        for a in (1, 2, 3):
            ln_z2(a)
        for j, (a, n) in enumerate((a, n) for n in range(1, NT) for a in range(4)):
            gate = fence(z2_words(1 + (j - 2) // 4, (j // 2 - 1) % 2)) if j in (2, 4, 6, 8, 10, 12) else None
            t = z1_tile(a, n, gate)
            if j in (13, 14, 16, 17):
                ln_q(4, fence(pltpu.bitcast(t[0:8, :], U32)), (13, 14, 16, 17).index(j), NLQ)
        region([4])
        wait(5)
        b32_v[...] = b_v[...].astype(F32) * 0.25
        assert not region(list(range(5, 11)), HCH[0], KCH[0], DFT_PLAN[0])
        wait(6)
        assert len(region(list(range(11, NB)), HCH[1], KCH[1], DFT_PLAN[1])) == H_LATE


@jax.jit
def pallas_recurrent_scan__ssm_conv_h3__mixer_gmlp__prompt_kernel(
    A_q: jax.Array,
    A_k: jax.Array,
    A_v: jax.Array,
    A_shift_k: jax.Array,
    A_ssm_k: jax.Array,
    A_ssm_D: jax.Array,
    B_x: jax.Array,
    B_w_in: jax.Array,
    B_w_sp: jax.Array,
    B_b_sp: jax.Array,
    B_w_out: jax.Array,
):
    del B_x
    any_spec = pl.BlockSpec(memory_space=pl.ANY)
    vm = pltpu.VMEM
    dma = pltpu.SemaphoreType.DMA
    out = pl.pallas_call(
        _kernel,
        out_shape=jax.ShapeDtypeStruct((S, D), BF),
        grid=(2,),
        in_specs=[any_spec] * 11,
        out_specs=any_spec,
        scratch_shapes=[
            vm((S // 2, D), U32),
            vm((S + 64, D), BF),
            vm((S, D), BF),
            vm(((D + 4 * C) // 2, S), U32),
            vm((D // 2, 2 * FH), U32),
            vm((S // 2, S), U32),
            vm(((FH + 512) // 2, FH), U32),
            vm(((2 * C + C // 2) // 2, 2 * C), U32),
            vm((S // 2, D), U32),
            vm((S + 4 * C, FH), F32),
            vm((S // 2, FH), U32),
            vm((S // 4, 2 * FH), U32),
            vm((NB, NB, 16, D), F32),
            vm((NB, NB, 16, D), F32),
            vm((NB * 16, 8, 1024), U32),
            vm((S // TA * C // 2, FH), U32),
            vm((S, D), F32),
            vm((S, D), BF),
            vm((NB, 128), F32),
            vm((NB, 128), BF),
            vm((4, 18 * 128), BF),
            vm((ND, 128), BF),
            dma((len(QCH),)), dma((len(KCH),)), dma((len(KCH),)), dma((len(HCH),)),
            dma((len(WCH),)), dma((S // TA,)), dma((1,)), dma((5,)),
        ],
        compiler_params=pltpu.CompilerParams(
            dimension_semantics=("arbitrary",),
            vmem_limit_bytes=110 * 1024 * 1024,
            disable_bounds_checks=True,
            disable_semaphore_checks=True,
        ),
    )(
        A_q.reshape(S, D), A_k.reshape(S, D), A_v.reshape(S, D),
        A_shift_k.T, A_ssm_k, A_ssm_D.reshape(ND, 128),
        B_w_in, B_w_sp, B_b_sp.reshape(NB, 128), B_w_out,
        _dft_consts(),
    )
    return out.reshape(1, S, D)
```

```python
import math

import jax
import jax.numpy as jnp
import numpy as np
import jax.experimental.pallas as pl
import jax.experimental.pallas.tpu as pltpu

S = 2048
D = 640
FH = 768
C = 128
NB = S // C
ND = D // 128
NT = FH // 128
EPS = 1e-5
HK = S // 2
HN = FH // 2
KS = 256
TA = 512
NOP = 3
NLQ = 4
H_LATE = 24
TREE = 11

BF = jnp.bfloat16
F32 = jnp.float32
U32 = jnp.uint32

QCH = [(0, 2), (2, 1), (3, 1), (4, 4), (8, 6), (14, 2)]
HCH = [(0, 5), (5, 11)]
KCH = [(0, 3), (3, 13)]
WCH = [(6, 2), (8, 2), (10, 2), (0, 1), (1, 5)]
DFT_PLAN = [[(8, 4), (8, 8), (9, 3)], [(16, 32), (15, 33)]]
U_SLOTS = [1, 5, 9, 3, 7, 14, 18, 22, 0, 4, 8, 16, 20, 2, 6, 10, 15, 19, 23, 11, 13, 17, 21, 12, 24]
LNQ_H = [('h', 4, 128)] + [('z', n, 120) for n in (0, 1, 3, 4, 5, 7, 8)]
LNQ_NO_H = [('z', n, 0) for n in (1, 2, 3, 4, 5, 6, 8, 9)]


def _dft_consts():
    theta = np.pi * (4 * np.arange(C) + 1) / (2 * C)

    def fwd(t):
        ang = theta[:, None] * t[None, :]
        re = np.cos(ang).reshape(C // 8, 8, C)
        im = -np.sin(ang).reshape(C // 8, 8, C)
        return np.stack([re, im], axis=1).reshape(2 * C, C)

    fg = np.zeros((2 * C + C // 2, 2 * C), np.float64)
    order = np.concatenate([np.arange(0, C, 2), np.arange(1, C, 2)])
    fg[:2 * C, :C] = fwd(order - (C - 1) / 2)
    fg[:2 * C, C:] = fwd(np.arange(C))
    ang = (np.arange(C // 2) + 0.5)[:, None] * theta[None, :]
    fg[2 * C:, :C] = np.cos(ang) / C
    fg[2 * C:, C:] = -np.sin(ang) / C
    return fg.astype(np.float32).astype(BF)


def _kernel(q_hbm, k_hbm, v_hbm, sk_hbm, h_hbm, d_hbm, win_hbm, wsp_hbm, b_hbm, wout_hbm,
            fg_hbm, o_hbm,
            q_u, k_u, v_u, h_u, win_u, wsp_u, wout_u, fg_u,
            xn_u, z1_v, z2_u, t_u, p_v, hf_v, w_u, gg_u, xg_v, o_v, b32_v, b_v, sk_v, d_v,
            sem_q, sem_k, sem_v, sem_h, sem_w, sem_wsp, sem_o, sem_m):
    q_v = q_u.bitcast(BF)
    v_v = v_u.bitcast(BF)
    k_w = k_hbm.bitcast(U32)
    h_v = h_u.bitcast(BF)
    win_v = win_u.bitcast(BF)
    wsp_v = wsp_u.bitcast(BF)
    wout_v = wout_u.bitcast(BF)
    fg_v = fg_u.bitcast(BF)
    xn_v = xn_u.bitcast(BF)
    z2_v = z2_u.bitcast(BF)
    t_v = t_u.bitcast(BF)
    w_v = w_u.bitcast(BF)
    gg_v = gg_u.bitcast(BF)

    def ds(start, size):
        if isinstance(start, int):
            return pl.ds(start, size)
        return pl.ds(pl.multiple_of(start, size), size)

    def lanes(n):
        return slice(n * 128, (n + 1) * 128)

    def blocks(ch):
        return pl.ds(ch[0] * C, ch[1] * C)

    def brows(a):
        return ds(a * C, C)

    def cp_q(c):
        r = blocks(QCH[c])
        return pltpu.make_async_copy(q_hbm.at[r, :], q_v.at[r, :], sem_q.at[c])

    def cp_k(c):
        b0, n = KCH[c]
        return [pltpu.make_async_copy(k_w.at[pl.ds(b0 * C // 2, n * C // 2), lanes(dt)],
                                      k_u.at[dt, pl.ds(b0 * C // 2 + 8, n * C // 2), :],
                                      sem_k.at[c * ND + dt])
                for dt in range(ND)]

    def cp_v(c):
        r = blocks(KCH[c])
        return pltpu.make_async_copy(v_hbm.at[r, :], v_v.at[r, :], sem_v.at[c])

    def cp_h(c):
        r = blocks(HCH[c])
        return pltpu.make_async_copy(h_hbm.at[:, r], h_v.at[0:D, r], sem_h.at[c])

    def cp_w(c):
        r = blocks(WCH[c])
        return pltpu.make_async_copy(win_hbm.at[:, r], win_v.at[0:D, r], sem_w.at[c])

    def cp_wsp(i):
        r = ds(i * TA, TA)
        return pltpu.make_async_copy(wsp_hbm.at[r, :], wsp_v.at[r, :], sem_wsp.at[i])

    def cp_o(a, cols=slice(None)):
        r = brows(a)
        return pltpu.make_async_copy(o_v.at[r, cols], o_hbm.at[r, cols], sem_o.at[0])

    cp_f = pltpu.make_async_copy(fg_hbm, fg_v, sem_m.at[0])
    cp_sk = pltpu.make_async_copy(sk_hbm, sk_v.at[:, 0:D], sem_m.at[1])
    cp_d = pltpu.make_async_copy(d_hbm, d_v, sem_m.at[2])
    cp_b = pltpu.make_async_copy(b_hbm, b_v, sem_m.at[3])
    cp_wout = pltpu.make_async_copy(wout_hbm, wout_v.at[0:FH, 0:D], sem_m.at[4])

    groups = [
        [cp_q(0)], [cp_w(0)], [cp_q(1), cp_w(1)], [cp_q(2), cp_w(2), cp_w(3)], [cp_q(3), cp_w(4)],
        [cp_f, cp_sk, cp_d, cp_b, cp_q(4), cp_h(0), *cp_k(0), cp_v(0)],
        [cp_q(5), cp_h(1), *cp_k(1), cp_v(1)],
    ]

    def wait(g):
        for cp in groups[g]:
            cp.wait()

    def mm(x, y):
        return jnp.dot(x, y, preferred_element_type=F32)

    def words(x):
        return pltpu.bitcast(x, U32)

    def fence(tok):
        t = tok[0:8, :]
        for g in range(1, tok.shape[0] // 8):
            t = t | tok[g * 8:(g + 1) * 8, :]
        return t & k_u[0, 0:8, :]

    def held(x, gate):
        if gate is None:
            return x
        w = words(x)
        return pltpu.bitcast(w | jnp.tile(gate, (w.shape[0] // 8, w.shape[1] // 128)), x.dtype)

    def a_sums(a11, a12, a21, a22):
        s1 = a21 + a22
        s2 = s1 - a11
        return s1, s2, a11 - a21, a12 - s2

    def b_sums(b11, b12, b21, b22):
        t1 = b12 - b11
        t2 = b22 - t1
        return t1, t2, t2 - b11, b21 - t2

    def chain_sums(units, quads, dest, combine, lead, via_memory):
        last = None
        for u in units:
            vals = []
            for n, (ref, idx) in enumerate(quads(u)):
                wait_here = last is not None and (n == lead or not via_memory)
                vals.append(held(ref[idx], fence(last) if wait_here else None).astype(F32))
            sums = combine(*vals)
            done = []
            for k, val in enumerate(sums):
                ref, idx = dest(u, k)
                ref[idx] = val.astype(BF)
                if via_memory:
                    done.append(words(ref[idx]))
            last = jnp.concatenate(done, axis=0) if via_memory else words(sums[-1][-8:, :])
        return last

    c0 = math.sqrt(2.0 / math.pi)
    c1 = c0 * 0.044715

    def gelu2(x):
        return x + x * jnp.tanh(x * (c0 + c1 * (x * x)))

    def z2_words(a, half=None):
        r = brows(a) if half is None else pl.ds(a * C + half * (C // 2), C // 2)
        return words(z2_v[r, 0:128])

    def xs_row(a0, k):
        return S + (a0 // 2 % 2) * 2 * C + k // 2 * C

    def ln_q(a, gate=None, part=0, nparts=1):
        n = C // nparts
        r = pl.ds(a * C + part * n, n)
        x = held(q_v[r, :], gate).astype(F32)
        mu = jnp.sum(x, axis=-1, keepdims=True) * (1.0 / D)
        ex2 = jnp.sum(x * x, axis=-1, keepdims=True) * (1.0 / D)
        var = jnp.maximum(ex2 - mu * mu, 0.0)
        mu = mu.astype(BF).astype(F32)
        xn = (x - mu) * jnp.exp(-0.5 * jnp.log(var + EPS))
        xn_v[r, :] = xn.astype(BF)
        if a >= 4 and a % 2 == 1:
            top = xn_v[pl.ds((a - 1) * C + part * n, n), 0:2 * KS].astype(F32)
            s1, s2, s3, s4 = a_sums(top[:, :KS], top[:, KS:], xn[:, :KS], xn[:, KS:2 * KS])
            xn_v[pl.ds(xs_row(a - 1, 0) + part * n, n), 0:2 * KS] = jnp.concatenate([s1, s2], axis=1).astype(BF)
            xn_v[pl.ds(xs_row(a - 1, 2) + part * n, n), 0:2 * KS] = jnp.concatenate([s3, s4], axis=1).astype(BF)

    def h_dft(a, dt):
        res = jax.lax.dot_general(fg_v[0:2 * C, C:2 * C], h_v[lanes(dt), brows(a)],
                                  (((1,), (1,)), ((), ())), preferred_element_type=F32)
        spec = res.reshape(NB, 16, 128)
        if a == 0:
            dv = d_v[...].astype(F32)[dt:dt + 1, :]
            spec = jnp.concatenate([spec[:, 0:8, :] + dv[None], spec[:, 8:16, :]], axis=1)
        hf_v[:, a, :, lanes(dt)] = spec
        return res

    def u_dft(a, dt):
        cols = lanes(dt)

        def even(w):
            return pltpu.bitcast(w << 16, F32)

        def odd(w):
            return pltpu.bitcast(w & jnp.uint32(0xFFFF0000), F32)

        w0, w1, w2 = (k_u[dt, pl.ds(8 + a * C // 2 - j, C // 2), :] for j in range(3))
        e0, o0, e1, o1 = even(w0), odd(w0), even(w1), odd(w1)
        sk = sk_v[:, cols].astype(F32)
        s0, s1, s2, s3 = (sk[j:j + 1, :] for j in range(4))
        vw = words(v_v[brows(a), cols])
        kve = (e0 * s0 + o1 * s1 + e1 * s2 + odd(w2) * s3) * even(vw)
        kvo = (o0 * s0 + e0 * s1 + o1 * s2 + e1 * s3) * odd(vw)
        kv = jnp.concatenate([kve, kvo], axis=0).astype(BF)
        p_v[:, a, :, cols] = mm(fg_v[0:2 * C, 0:C], kv).reshape(NB, 16, 128)

    def proj(a, n, gate=None):
        lhs = xn_v[brows(a), :]
        if gate is not None:
            lhs = jnp.concatenate([held(lhs[0:16, :], gate), lhs[16:, :]], axis=0)
        return gelu2(mm(lhs, win_v[0:D, lanes(n)]))

    def w2_rows(a):
        return pl.ds(S + (a % 4) * C, C)

    def z2_tile(a, n, gate=None):
        z1_v[w2_rows(a), lanes(n)] = proj(a, NT + n, gate)

    def z1_tile(a, n, gate=None):
        t = proj(a, n, gate)
        z1_v[brows(a), lanes(n)] = t
        return t

    def t_rest(r, bot, g=0, nr=C):
        rows = pl.ds(r * C + g * nr, nr)
        t2 = bot[:, HN:] - t_v[rows, 0:HN].astype(F32)
        t3 = t2 - z2_v[rows, 0:HN].astype(F32)
        t_v[rows, HN:4 * HN] = jnp.concatenate([t2, t3, bot[:, :HN] - t2], axis=1).astype(BF)

    def ln_z2(a, last=None):
        w2 = z1_v[w2_rows(a), :]
        mu = jnp.sum(w2, axis=-1, keepdims=True) * (1.0 / FH)
        ex2 = jnp.sum(w2 * w2, axis=-1, keepdims=True) * (1.0 / FH)
        var = jnp.maximum(ex2 - mu * mu, 0.0)
        rs = jnp.exp(-0.5 * jnp.log(16.0 * var + 64.0 * EPS))
        nr = 16 if 4 <= a < NB - 2 else C
        for g in range(C // nr):
            rr = slice(g * nr, (g + 1) * nr)
            m = held(jnp.broadcast_to(mu[rr], (nr, 128)), fence(last) if last is not None and nr < C else None)
            zn = (w2[rr] - jnp.tile(m, (1, NT))) * rs[rr]
            rows = pl.ds(a * C + g * nr, nr)
            if a < NB // 2:
                z2_v[rows, 0:HN] = zn[:, :HN].astype(BF)
                t_v[rows, 0:HN] = (zn[:, HN:] - zn[:, :HN]).astype(BF)
                done = [(z2_v, rows, k) for k in range(3)] + [(t_v, rows, k) for k in range(3)]
            else:
                z2_v[rows, :] = zn.astype(BF)
                done = [(z2_v, rows, k) for k in range(6)]
                if a < NB - 1:
                    t_rest(a - NB // 2, zn, g, nr)
                    done += [(t_v, pl.ds((a - NB // 2) * C + g * nr, nr), k) for k in range(3, 12)]
            if nr < C:
                last = jnp.concatenate([words(ref[r, lanes(k)]) for ref, r, k in done], axis=0)
        return last

    def tw_at(base, j, k):
        return D + (base // NT) * KS, lanes(j * 4 + k)

    def tw_sums(base):
        def quads(u):
            j, g = u
            return [(win_v, (slice(r0 + g * 16, r0 + (g + 1) * 16), lanes(n)))
                    for r0 in (0, KS) for n in (base + j, base + 3 + j)]

        def dest(u, k):
            j, g = u
            r0, cols = tw_at(base, j, k)
            return win_v, (slice(r0 + g * 16, r0 + (g + 1) * 16), cols)

        return chain_sums([(j, g) for j in range(3) for g in range(KS // 16)], quads, dest, b_sums, 0, True)

    def group(a0, base, j, hook, gate=None):
        r0, r1 = brows(a0), brows(a0 + 1)
        cl, cr = lanes(base + j), lanes(base + 3 + j)

        def out(a, n, val):
            t = gelu2(val)
            z1_v[w2_rows(a) if base else brows(a), lanes(n)] = t
            hook(t)

        def sx(k):
            return xn_v[xs_row(a0, k):xs_row(a0, k) + C, (k % 2) * KS:(k % 2 + 1) * KS]

        def tw(k):
            t0, cols = tw_at(base, j, k)
            return win_v[t0:t0 + KS, cols]

        def keep(slot, val):
            sl = (pl.ds(S + 4 * C + (j % 2) * C, C), lanes(slot))
            z1_v[sl] = val
            return lambda: z1_v[sl]

        a11 = xn_v[r0, 0:KS]
        if gate is not None:
            top = jnp.concatenate([held(a11[0:16, 0:128], gate), a11[0:16, 128:]], axis=1)
            a11 = jnp.concatenate([top, a11[16:, :]], axis=0)
        p1 = keep(0, mm(a11, win_v[0:KS, cl]))
        out(a0, j, p1() + mm(xn_v[r0, KS:D], win_v[KS:D, cl]))
        u2 = keep(1, p1() + mm(sx(1), tw(1)))
        u3 = keep(2, u2() + mm(sx(2), tw(2)))
        out(a0 + 1, j, u3() + mm(xn_v[r1, KS:D], jnp.concatenate([tw(3), win_v[2 * KS:D, cl]], axis=0)))
        p5 = mm(sx(0), tw(0))
        out(a0 + 1, 3 + j, (u3() + p5) + mm(xn_v[r1, 2 * KS:D], win_v[2 * KS:D, cr]))
        out(a0, 3 + j, (u2() + p5) + mm(jnp.concatenate([sx(3), xn_v[r0, 2 * KS:D]], axis=1), win_v[KS:D, cr]))

    def region(pairs, hch=(0, 0), kch=(0, 0), plan=((0, 0),)):
        hs = [(a, dt) for a in range(hch[0], hch[0] + hch[1]) for dt in range(ND)]
        us = [(a, dt) for a in range(kch[0], kch[0] + kch[1]) for dt in range(ND)]
        for bi, a0 in enumerate(pairs):
            nh, nu = plan[bi]
            nh_end = min(nh, 4) if bi == len(pairs) - 1 else 0
            nh_mid = min(8, nh - nh_end)
            nh_run = nh - nh_end - nh_mid
            nu_run = min(nu, 3 * nh_run)
            cnt = [0] * 25
            for j in range(nu - nu_run):
                cnt[U_SLOTS[j % len(U_SLOTS)]] += 1
            marks = [] if a0 + 2 >= NB else LNQ_H if nh_mid >= 5 else LNQ_NO_H
            seen = [0]

            def next_ln_q(part, t):
                tok = words(t)
                for a in (a0, a0 + 1):
                    if part == (0, 6)[a - a0]:
                        tok = jnp.concatenate([tok, z2_words(a)], axis=0)
                        if a >= NB // 2:
                            tw_ = words(t_v[brows(a - NB // 2), 4 * HN - 128:4 * HN])
                            tok = jnp.concatenate([tok, tw_], axis=0)
                ln_q(a0 + 2 + part // NLQ, fence(tok), part % NLQ, NLQ)

            def after_z2(t):
                for _ in range(cnt[seen[0]]):
                    u_dft(*us.pop(0))
                seen[0] += 1

            def after_z1(t):
                for part, (kind, idx, row) in enumerate(marks):
                    if kind == 'z' and idx == seen[0]:
                        next_ln_q(part, t[row:row + 8, :])
                for _ in range(cnt[13 + seen[0]]):
                    u_dft(*us.pop(0))
                seen[0] += 1

            for j in range(3):
                group(a0, NT, j, after_z2)
            hres = [h_dft(*hs.pop(0)) for _ in range(nh_mid)]
            for _ in range(cnt[12]):
                u_dft(*us.pop(0))
            ln_z2(a0 + 1, ln_z2(a0))
            for part, (kind, idx, row) in enumerate(marks):
                if kind == 'h':
                    next_ln_q(part, hres[idx][row:row + 8, :])
            seen[0] = 0
            for j in range(3):
                group(a0, 0, j, after_z1, fence(z2_words(a0 + j - 1)) if not marks and j >= 1 else None)
            ru, rh = nu_run, nh_run
            while ru or rh:
                if ru and ru * max(nh_run, 1) >= rh * max(nu_run, 1):
                    u_dft(*us.pop(0))
                    ru -= 1
                else:
                    h_dft(*hs.pop(0))
                    rh -= 1
            for _ in range(nh_end):
                h_dft(*hs.pop(0))
        assert not us
        return hs

    def conv_pos(ft, ft2, par, dt, after):
        cols = lanes(dt)
        prev = None
        for a in range(NB):
            ar, ai = (None, None) if prev is None else (-prev[1], prev[0])
            for dl in range(a + 1):
                hr = hf_v[ft, dl, 0:8, cols]
                hi = hf_v[ft, dl, 8:16, cols]
                ur = p_v[ft, a - dl, 0:8, cols]
                ui = p_v[ft, a - dl, 8:16, cols]
                if ar is None:
                    ar, ai = ur * hr - ui * hi, ur * hi + ui * hr
                    if after is not None:
                        z = fence(after)
                        ar, ai = held(ar, z), held(ai, z)
                elif (a * (a + 1) // 2 + dl) % TREE == 0:
                    ar = ar + (ur * hr - ui * hi)
                    ai = ai + (ur * hi + ui * hr)
                else:
                    ar = (ar + ur * hr) - ui * hi
                    ai = (ai + ur * hi) + ui * hr
            prev = (ar, ai) if prev is None else (ar + prev[1], ai - prev[0])
            w_v[a * 16 + ft2, par * 8:(par + 1) * 8, cols] = ar.astype(BF)
            w_v[a * 16 + 8 + ft2, par * 8:(par + 1) * 8, cols] = ai.astype(BF)
        return words(prev[0])

    gl_v = wout_v
    GL0 = FH
    GS0 = GL0 + NOP * C
    WS0 = GS0 + 2 * C

    def g_sums():
        def quads(u):
            c, g = u
            return [(gl_v, (pl.ds(GL0 + m * C + g * 16, 16), lanes(n))) for m in (0, 1) for n in (c, 3 + c)]

        def dest(u, k):
            c, g = u
            return gl_v, (pl.ds(GS0 + k // 2 * C + g * 16, 16), lanes(k % 2 * 3 + c))

        chain_sums([(c, g) for c in range(3) for g in range(C // 16)], quads, dest, a_sums, 2, True)

    def ws_at(jj, k):
        return WS0 + (jj * 4 + k) // 6 * HN, lanes((jj * 4 + k) % 6)

    def w_sums():
        def quads(u):
            jj, g = u
            return [(wout_v, (pl.ds(r0 + g * 16, 16), lanes(n))) for r0 in (0, HN) for n in (jj, 2 + jj)]

        def dest(u, k):
            jj, g = u
            r0, cols = ws_at(jj, k)
            return wout_v, (pl.ds(r0 + g * 16, 16), cols)

        chain_sums([(jj, g) for jj in range(2) for g in range(HN // 16)], quads, dest, b_sums, 0, False)

    def xn_gate(a, dt, hh):
        return xn_v[brows(a), lanes(dt)].astype(F32) * (hh + hh * jnp.tanh(hh))

    def o_pair(a0):
        r0, r1 = pl.ds(GL0, C), pl.ds(GL0 + C, C)

        def finish(a, dt, hh):
            xg_v[brows(a), lanes(dt)] = xn_gate(a, dt, hh)

        def gs(k):
            return gl_v[pl.ds(GS0 + k // 2 * C, C), (k % 2) * HN:(k % 2 + 1) * HN]

        def ws(jj, k):
            r, cols = ws_at(jj, k)
            return wout_v[r:r + HN, cols]

        finish(a0, 4, mm(gl_v[r0, :], wout_v[0:FH, lanes(4)]))
        finish(a0 + 1, 4, mm(gl_v[r1, :], wout_v[0:FH, lanes(4)]))
        for jj in range(2):
            p1 = mm(gl_v[r0, 0:HN], wout_v[0:HN, lanes(jj)])
            finish(a0, jj, p1 + mm(gl_v[r0, HN:FH], wout_v[HN:FH, lanes(jj)]))
            u2 = p1 + mm(gs(1), ws(jj, 1))
            u3 = u2 + mm(gs(2), ws(jj, 2))
            finish(a0 + 1, jj, u3 + mm(gl_v[r1, HN:FH], ws(jj, 3)))
            p5 = mm(gs(0), ws(jj, 0))
            finish(a0 + 1, 2 + jj, u3 + p5)
            finish(a0, 2 + jj, (u2 + p5) + mm(gs(3), wout_v[HN:FH, lanes(2 + jj)]))

    def s_at(slot, k):
        return D + (slot * 2 + k // 2) * C, (k % 2) * HK

    def s_val(slot, k):
        r0, col = s_at(slot, k)
        return h_v[r0:r0 + C, col:col + HK]

    def s_sums(a0, nr, via_memory):
        def quads(u):
            slot, c, g = u
            return [(wsp_v, (ds((a0 + 2 * slot + m) * C + g * nr, nr), lanes(n)))
                    for m in (0, 1) for n in (c, HK // 128 + c)]

        def dest(u, k):
            slot, c, g = u
            r0, col = s_at(slot, k)
            return h_v, (slice(r0 + g * nr, r0 + (g + 1) * nr), slice(col + c * 128, col + (c + 1) * 128))

        units = [(slot, c, g) for slot in range(2) for c in range(HK // 128) for g in range(C // nr)]
        chain_sums(units, quads, dest, a_sums, 2, via_memory)

    def phase2a(i, carry):
        @pl.when(i + 1 < S // TA)
        def _():
            cp_wsp(i + 1).wait()

        eye = (jax.lax.broadcasted_iota(jnp.int32, (C, C), 0)
               == jax.lax.broadcasted_iota(jnp.int32, (C, C), 1))

        def bcol(a):
            return jnp.sum(jnp.where(eye, b32_v[pl.ds(a, 1), :], 0.0), axis=-1, keepdims=True)

        def put(m, n, g):
            g = (z1_v[brows(i * (TA // C) + m), lanes(n)] * g).astype(BF)
            if m < NOP:
                gl_v[GL0 + m * C:GL0 + (m + 1) * C, lanes(n)] = g
            else:
                gg_v[ds(i * C, C), lanes(n)] = g

        for pp in range(2):
            if pp == 1:
                g_sums()
            m0 = 2 * pp
            a0 = i * (TA // C) + m0
            r0, r1 = brows(a0), brows(a0 + 1)
            b0 = bcol(a0)
            db = bcol(a0 + 1) - b0
            for j in range(NT // 2):
                jl, jr = lanes(j), lanes(NT // 2 + j)
                t1, t2, t3, t4 = (t_v[:, lanes(k * (NT // 2) + j)] for k in range(4))
                p1 = mm(wsp_v[r0, 0:HK], z2_v[0:HK, jl]) + b0
                put(m0, j, p1 + mm(wsp_v[r0, HK:S], z2_v[HK:S, jl]))
                u2 = p1 + mm(s_val(pp, 1), t2)
                u3 = (u2 + db) + mm(s_val(pp, 2), t3)
                put(m0 + 1, j, u3 + mm(wsp_v[r1, HK:S], t4))
                p5 = mm(s_val(pp, 0), t1)
                put(m0 + 1, NT // 2 + j, u3 + p5)
                put(m0, NT // 2 + j, (u2 + p5) + mm(s_val(pp, 3), z2_v[HK:S, jr]))
        o_pair(i * (TA // C))
        for m in range(2, NOP):
            a = i * (TA // C) + m
            for dt in range(ND):
                hh = mm(gl_v[pl.ds(GL0 + m * C, C), :], wout_v[0:FH, lanes(dt)])
                xg_v[brows(a), lanes(dt)] = xn_gate(a, dt, hh)
        s_sums(jnp.minimum(i + 1, S // TA - 1) * (TA // C), 16, True)
        nft = NB * TA // S
        last = None
        for ft in range(nft):
            for dt in range(ND):
                last = conv_pos(i * nft + ft, i * (nft // 2) + ft // 2, ft % 2, dt, last)
        return carry

    step = pl.program_id(0)

    @pl.when(step == 0)
    def _():
        for grp in groups:
            for cp in grp:
                cp.start()
        cp_wout.start()
        for i in range(S // TA):
            cp_wsp(i).start()
        k_u[:, 0:8, :] = jnp.zeros((ND, 8, 128), U32)

    @pl.when(step == 1)
    def _():
        cp_wsp(0).wait()
        cp_wout.wait()
        t_rest(NB // 2 - 1, z2_v[brows(NB - 1), :].astype(F32))
        for a, dt in [(a, dt) for a in range(NB) for dt in range(ND)][NB * ND - H_LATE:]:
            h_dft(a, dt)
        w_sums()
        s_sums(0, 32, False)
        jax.lax.fori_loop(0, S // TA, phase2a, 0)

        rev = 7 - jax.lax.broadcasted_iota(jnp.int32, (8, 128), 0)
        for a in range(NB):
            rows = brows(a)
            for dt in range(ND):
                cols = lanes(dt)
                ev = mm(fg_v[2 * C:2 * C + C // 2, 0:C], w_v[ds(a * 16, 8), :, cols].reshape(C, 128))
                od = mm(fg_v[2 * C:2 * C + C // 2, C:2 * C], w_v[ds(a * 16 + 8, 8), :, cols].reshape(C, 128))
                lo = ev - od
                ys = [jnp.take_along_axis(lo[g * 8:(g + 1) * 8, :], rev, axis=0)
                      for g in range(C // 16 - 1, -1, -1)]
                y = jnp.concatenate(ys + [ev + od], axis=0)
                if a % (TA // C) < NOP:
                    xg = xg_v[rows, cols]
                else:
                    xg = xn_gate(a, dt, mm(gg_v[brows(a // (TA // C)), :], wout_v[0:FH, cols]))
                o_v[rows, cols] = (q_v[rows, cols].astype(F32) + xg * y).astype(BF)
                if a == NB - 1:
                    cp_o(a, cols).start()
            if a < NB - 1:
                cp_o(a).start()
        pltpu.make_async_copy(o_v, o_hbm, sem_o.at[0]).wait()

    @pl.when(step == 0)
    def _():
        wait(0)
        ln_q(0)
        ln_q(1)
        wait(1)
        for n in (0, 1):
            z2_tile(0, n)
            z2_tile(1, n)
        wait(2)
        ln_q(2)
        for n in (2, 3):
            z2_tile(0, n)
            z2_tile(1, n)
        for n in range(4):
            z2_tile(2, n)
        wait(3)
        ln_q(3)
        seq = ([(z2_tile, a, n) for a in range(3) for n in (4, 5)] + [(z2_tile, 3, n) for n in range(NT)]
               + [(z1_tile, a, 0) for a in range(4)])
        tw_done = tw_sums(NT)
        for j, (tile, a, n) in enumerate(seq):
            if j == 15:
                gate = fence(tw_done)
            elif j == 3:
                gate = fence(words(xn_v[brows(3), 0:128]))
            else:
                gate = fence(z2_words(0, (7, 10).index(j))) if j in (7, 10) else None
            tile(a, n, gate)
            if j == 1:
                ln_z2(0)
        wait(4)
        for a in (1, 2, 3):
            ln_z2(a)
        tw_sums(0)
        release = (9, 10, 11, 12, 14, 15, 16, 17)
        for j, (a, n) in enumerate((a, n) for n in range(1, NT) for a in range(4)):
            gate = fence(z2_words(1 + (j - 2) // 4, (j // 2 - 1) % 2)) if j in (2, 4, 6, 8, 10, 12) else None
            t = z1_tile(a, n, gate)
            if j in release:
                part = release.index(j)
                ln_q(4 + part // NLQ, fence(words(t[0:8, :])), part % NLQ, NLQ)
        region([4])
        wait(5)
        b32_v[...] = b_v[...].astype(F32) * 0.25
        assert not region([6, 8, 10], HCH[0], KCH[0], DFT_PLAN[0])
        wait(6)
        assert len(region([12, 14], HCH[1], KCH[1], DFT_PLAN[1])) == H_LATE


@jax.jit
def pallas_recurrent_scan__ssm_conv_h3__mixer_gmlp__prompt_kernel(
    A_q: jax.Array,
    A_k: jax.Array,
    A_v: jax.Array,
    A_shift_k: jax.Array,
    A_ssm_k: jax.Array,
    A_ssm_D: jax.Array,
    B_x: jax.Array,
    B_w_in: jax.Array,
    B_w_sp: jax.Array,
    B_b_sp: jax.Array,
    B_w_out: jax.Array,
):
    del B_x
    any_spec = pl.BlockSpec(memory_space=pl.ANY)
    vm = pltpu.VMEM
    dma = pltpu.SemaphoreType.DMA
    out = pl.pallas_call(
        _kernel,
        out_shape=jax.ShapeDtypeStruct((S, D), BF),
        grid=(2,),
        in_specs=[any_spec] * 11,
        out_specs=any_spec,
        scratch_shapes=[
            vm((S // 2, D), U32),
            vm((ND, S // 2 + 32, 128), U32),
            vm((S // 2, D), U32),
            vm(((D + 4 * C) // 2, S), U32),
            vm(((D + 2 * KS) // 2, 2 * FH), U32),
            vm((S // 2, S), U32),
            vm(((FH + 6 * C + 2 * HN) // 2, FH), U32),
            vm(((2 * C + C // 2) // 2, 2 * C), U32),
            vm(((S + 4 * C) // 2, D), U32),
            vm((S + 6 * C, FH), F32),
            vm((S // 2, FH), U32),
            vm((S // 4, 2 * FH), U32),
            vm((NB, NB, 16, D), F32),
            vm((NB, NB, 16, D), F32),
            vm((NB * 16, 8, 1024), U32),
            vm((S // TA * C // 2, FH), U32),
            vm((S, D), F32),
            vm((S, D), BF),
            vm((NB, 128), F32),
            vm((NB, 128), BF),
            vm((4, 18 * 128), BF),
            vm((ND, 128), BF),
            dma((len(QCH),)), dma((len(KCH) * ND,)), dma((len(KCH),)), dma((len(HCH),)),
            dma((len(WCH),)), dma((S // TA,)), dma((1,)), dma((5,)),
        ],
        compiler_params=pltpu.CompilerParams(
            dimension_semantics=("arbitrary",),
            vmem_limit_bytes=110 * 1024 * 1024,
            disable_bounds_checks=True,
            disable_semaphore_checks=True,
        ),
    )(
        A_q.reshape(S, D), A_k.reshape(S, D), A_v.reshape(S, D),
        A_shift_k.T, A_ssm_k, A_ssm_D.reshape(ND, 128),
        B_w_in, B_w_sp, B_b_sp.reshape(NB, 128), B_w_out,
        _dft_consts(),
    )
    return out.reshape(1, S, D)
```

```python
import math

import jax
import jax.numpy as jnp
import numpy as np
import jax.experimental.pallas as pl
import jax.experimental.pallas.tpu as pltpu

S = 2048
D = 640
FH = 768
C = 128
NB = S // C
ND = D // 128
NT = FH // 128
EPS = 1e-5
HK = S // 2
HN = FH // 2
KS = 256
TA = 512
NOP = 2
NLQ = 4
H_LATE = 24
TREE = 10

BF = jnp.bfloat16
F32 = jnp.float32
U32 = jnp.uint32

QCH = [(0, 2), (2, 1), (3, 1), (4, 4), (8, 6), (14, 2)]
HCH = [(0, 5), (5, 11)]
KCH = [(0, 3), (3, 13)]
WCH = [(6, 2), (8, 2), (10, 2), (0, 1), (1, 5)]
DFT_PLAN = [[(8, 4), (8, 8), (9, 3)], [(16, 32), (15, 33)]]
U_SLOTS = [1, 5, 9, 3, 7, 14, 18, 22, 0, 4, 8, 16, 20, 2, 6, 10, 15, 19, 23, 11, 13, 17, 21, 12, 24]
LNQ_H = [('h', 4, 128)] + [('z', n, 120) for n in (0, 1, 3, 4, 5, 7, 8)]
LNQ_NO_H = [('z', n, 0) for n in (1, 2, 3, 4, 5, 6, 8, 9)]


def _dft_consts():
    theta = np.pi * (4 * np.arange(C) + 1) / (2 * C)

    def fwd(t):
        ang = theta[:, None] * t[None, :]
        re = np.cos(ang).reshape(C // 8, 8, C)
        im = -np.sin(ang).reshape(C // 8, 8, C)
        return np.stack([re, im], axis=1).reshape(2 * C, C)

    fg = np.zeros((2 * C + C // 2, 2 * C), np.float64)
    order = np.concatenate([np.arange(0, C, 2), np.arange(1, C, 2)])
    fg[:2 * C, :C] = fwd(order - (C - 1) / 2)
    fg[:2 * C, C:] = fwd(np.arange(C))
    ang = (np.arange(C // 2) + 0.5)[:, None] * theta[None, :]
    fg[2 * C:, :C] = np.cos(ang) / C
    fg[2 * C:, C:] = -np.sin(ang) / C
    return fg.astype(np.float32).astype(BF)


def _kernel(q_hbm, k_hbm, v_hbm, sk_hbm, h_hbm, d_hbm, win_hbm, wsp_hbm, b_hbm, wout_hbm,
            fg_hbm, o_hbm,
            q_u, k_u, v_u, h_u, win_u, wsp_u, wout_u, fg_u,
            xn_u, z1_v, z2_u, t_u, p_v, hf_v, w_u, gg_u, xg_v, o_v, b32_v, b_v, sk_v, d_v,
            sem_q, sem_k, sem_v, sem_h, sem_w, sem_wsp, sem_o, sem_m):
    q_v = q_u.bitcast(BF)
    v_v = v_u.bitcast(BF)
    k_w = k_hbm.bitcast(U32)
    h_v = h_u.bitcast(BF)
    win_v = win_u.bitcast(BF)
    wsp_v = wsp_u.bitcast(BF)
    wout_v = wout_u.bitcast(BF)
    fg_v = fg_u.bitcast(BF)
    xn_v = xn_u.bitcast(BF)
    z2_v = z2_u.bitcast(BF)
    t_v = t_u.bitcast(BF)
    w_v = w_u.bitcast(BF)
    gg_v = gg_u.bitcast(BF)

    def ds(start, size):
        if isinstance(start, int):
            return pl.ds(start, size)
        return pl.ds(pl.multiple_of(start, size), size)

    def lanes(n):
        return slice(n * 128, (n + 1) * 128)

    def blocks(ch):
        return pl.ds(ch[0] * C, ch[1] * C)

    def brows(a):
        return ds(a * C, C)

    def cp_q(c):
        r = blocks(QCH[c])
        return pltpu.make_async_copy(q_hbm.at[r, :], q_v.at[r, :], sem_q.at[c])

    def cp_k(c):
        b0, n = KCH[c]
        return [pltpu.make_async_copy(k_w.at[pl.ds(b0 * C // 2, n * C // 2), lanes(dt)],
                                      k_u.at[dt, pl.ds(b0 * C // 2 + 8, n * C // 2), :],
                                      sem_k.at[c * ND + dt])
                for dt in range(ND)]

    def cp_v(c):
        r = blocks(KCH[c])
        return pltpu.make_async_copy(v_hbm.at[r, :], v_v.at[r, :], sem_v.at[c])

    def cp_h(c):
        r = blocks(HCH[c])
        return pltpu.make_async_copy(h_hbm.at[:, r], h_v.at[0:D, r], sem_h.at[c])

    def cp_w(c):
        r = blocks(WCH[c])
        return pltpu.make_async_copy(win_hbm.at[:, r], win_v.at[0:D, r], sem_w.at[c])

    def cp_wsp(i):
        r = ds(i * TA, TA)
        return pltpu.make_async_copy(wsp_hbm.at[r, :], wsp_v.at[r, :], sem_wsp.at[i])

    def cp_o(a, cols=slice(None)):
        r = brows(a)
        return pltpu.make_async_copy(o_v.at[r, cols], o_hbm.at[r, cols], sem_o.at[0])

    cp_f = pltpu.make_async_copy(fg_hbm, fg_v, sem_m.at[0])
    cp_sk = pltpu.make_async_copy(sk_hbm, sk_v.at[:, 0:D], sem_m.at[1])
    cp_d = pltpu.make_async_copy(d_hbm, d_v, sem_m.at[2])
    cp_b = pltpu.make_async_copy(b_hbm, b_v, sem_m.at[3])
    cp_wout = pltpu.make_async_copy(wout_hbm, wout_v.at[0:FH, 0:D], sem_m.at[4])

    groups = [
        [cp_q(0)], [cp_w(0)], [cp_q(1), cp_w(1)], [cp_q(2), cp_w(2), cp_w(3)], [cp_q(3), cp_w(4)],
        [cp_f, cp_sk, cp_d, cp_b, cp_q(4), cp_h(0), *cp_k(0), cp_v(0)],
        [cp_q(5), cp_h(1), *cp_k(1), cp_v(1)],
    ]

    def wait(g):
        for cp in groups[g]:
            cp.wait()

    def mm(x, y):
        return jnp.dot(x, y, preferred_element_type=F32)

    def words(x):
        return pltpu.bitcast(x, U32)

    def fence(tok):
        t = tok[0:8, :]
        for g in range(1, tok.shape[0] // 8):
            t = t | tok[g * 8:(g + 1) * 8, :]
        return t & k_u[0, 0:8, :]

    def held(x, gate):
        if gate is None:
            return x
        w = words(x)
        return pltpu.bitcast(w | jnp.tile(gate, (w.shape[0] // 8, w.shape[1] // 128)), x.dtype)

    def a_sums(a11, a12, a21, a22):
        s1 = a21 + a22
        s2 = s1 - a11
        return s1, s2, a11 - a21, a12 - s2

    def b_sums(b11, b12, b21, b22):
        t1 = b12 - b11
        t2 = b22 - t1
        return t1, t2, t2 - b11, b21 - t2

    def chain_sums(units, quads, dest, combine, lead, via_memory):
        last = None
        for u in units:
            vals = []
            for n, (ref, idx) in enumerate(quads(u)):
                wait_here = last is not None and (n == lead or not via_memory)
                vals.append(held(ref[idx], fence(last) if wait_here else None).astype(F32))
            sums = combine(*vals)
            done = []
            for k, val in enumerate(sums):
                ref, idx = dest(u, k)
                ref[idx] = val.astype(BF)
                if via_memory:
                    done.append(words(ref[idx]))
            last = jnp.concatenate(done, axis=0) if via_memory else words(sums[-1][-8:, :])
        return last

    c0 = math.sqrt(2.0 / math.pi)
    c1 = c0 * 0.044715

    def gelu2(x):
        return x + x * jnp.tanh(x * (c0 + c1 * (x * x)))

    def z2_words(a, half=None):
        r = brows(a) if half is None else pl.ds(a * C + half * (C // 2), C // 2)
        return words(z2_v[r, 0:128])

    def xs_row(a0, k):
        return S + (a0 // 2 % 2) * 2 * C + k // 2 * C

    def ln_q(a, gate=None, part=0, nparts=1):
        n = C // nparts
        r = pl.ds(a * C + part * n, n)
        x = held(q_v[r, :], gate).astype(F32)
        mu = jnp.sum(x, axis=-1, keepdims=True) * (1.0 / D)
        ex2 = jnp.sum(x * x, axis=-1, keepdims=True) * (1.0 / D)
        var = jnp.maximum(ex2 - mu * mu, 0.0)
        mu = mu.astype(BF).astype(F32)
        xn = (x - mu) * jnp.exp(-0.5 * jnp.log(var + EPS))
        xn_v[r, :] = xn.astype(BF)
        if a >= 4 and a % 2 == 1:
            top = xn_v[pl.ds((a - 1) * C + part * n, n), 0:2 * KS].astype(F32)
            s1, s2, s3, s4 = a_sums(top[:, :KS], top[:, KS:], xn[:, :KS], xn[:, KS:2 * KS])
            xn_v[pl.ds(xs_row(a - 1, 0) + part * n, n), 0:2 * KS] = jnp.concatenate([s1, s2], axis=1).astype(BF)
            xn_v[pl.ds(xs_row(a - 1, 2) + part * n, n), 0:2 * KS] = jnp.concatenate([s3, s4], axis=1).astype(BF)

    def h_dft(a, dt):
        res = jax.lax.dot_general(fg_v[0:2 * C, C:2 * C], h_v[lanes(dt), brows(a)],
                                  (((1,), (1,)), ((), ())), preferred_element_type=F32)
        spec = res.reshape(NB, 16, 128)
        if a == 0:
            dv = d_v[...].astype(F32)[dt:dt + 1, :]
            spec = jnp.concatenate([spec[:, 0:8, :] + dv[None], spec[:, 8:16, :]], axis=1)
        hf_v[:, a, :, lanes(dt)] = spec
        return res

    def u_dft(a, dt):
        cols = lanes(dt)

        def even(w):
            return pltpu.bitcast(w << 16, F32)

        def odd(w):
            return pltpu.bitcast(w & jnp.uint32(0xFFFF0000), F32)

        w0, w1, w2 = (k_u[dt, pl.ds(8 + a * C // 2 - j, C // 2), :] for j in range(3))
        e0, o0, e1, o1 = even(w0), odd(w0), even(w1), odd(w1)
        sk = sk_v[:, cols].astype(F32)
        s0, s1, s2, s3 = (sk[j:j + 1, :] for j in range(4))
        vw = words(v_v[brows(a), cols])
        kve = (e0 * s0 + o1 * s1 + e1 * s2 + odd(w2) * s3) * even(vw)
        kvo = (o0 * s0 + e0 * s1 + o1 * s2 + e1 * s3) * odd(vw)
        kv = jnp.concatenate([kve, kvo], axis=0).astype(BF)
        p_v[:, a, :, cols] = mm(fg_v[0:2 * C, 0:C], kv).reshape(NB, 16, 128)

    def proj(a, n, gate=None):
        lhs = xn_v[brows(a), :]
        if gate is not None:
            lhs = jnp.concatenate([held(lhs[0:16, :], gate), lhs[16:, :]], axis=0)
        return gelu2(mm(lhs, win_v[0:D, lanes(n)]))

    def w2_rows(a):
        return pl.ds(S + (a % 4) * C, C)

    def z2_tile(a, n, gate=None):
        z1_v[w2_rows(a), lanes(n)] = proj(a, NT + n, gate)

    def z1_tile(a, n, gate=None):
        t = proj(a, n, gate)
        z1_v[brows(a), lanes(n)] = t
        return t

    def t_rest(r, bot, g=0, nr=C):
        rows = pl.ds(r * C + g * nr, nr)
        t2 = bot[:, HN:] - t_v[rows, 0:HN].astype(F32)
        t3 = t2 - z2_v[rows, 0:HN].astype(F32)
        t_v[rows, HN:4 * HN] = jnp.concatenate([t2, t3, bot[:, :HN] - t2], axis=1).astype(BF)

    def ln_z2(a, last=None):
        w2 = z1_v[w2_rows(a), :]
        mu = jnp.sum(w2, axis=-1, keepdims=True) * (1.0 / FH)
        ex2 = jnp.sum(w2 * w2, axis=-1, keepdims=True) * (1.0 / FH)
        var = jnp.maximum(ex2 - mu * mu, 0.0)
        rs = jnp.exp(-0.5 * jnp.log(16.0 * var + 64.0 * EPS))
        nr = 16 if 4 <= a < NB - 2 else C
        for g in range(C // nr):
            rr = slice(g * nr, (g + 1) * nr)
            m = held(jnp.broadcast_to(mu[rr], (nr, 128)), fence(last) if last is not None and nr < C else None)
            zn = (w2[rr] - jnp.tile(m, (1, NT))) * rs[rr]
            rows = pl.ds(a * C + g * nr, nr)
            if a < NB // 2:
                z2_v[rows, 0:HN] = zn[:, :HN].astype(BF)
                t_v[rows, 0:HN] = (zn[:, HN:] - zn[:, :HN]).astype(BF)
                done = [(z2_v, rows, k) for k in range(3)] + [(t_v, rows, k) for k in range(3)]
            else:
                z2_v[rows, :] = zn.astype(BF)
                done = [(z2_v, rows, k) for k in range(6)]
                if a < NB - 1:
                    t_rest(a - NB // 2, zn, g, nr)
                    done += [(t_v, pl.ds((a - NB // 2) * C + g * nr, nr), k) for k in range(3, 12)]
            if nr < C:
                last = jnp.concatenate([words(ref[r, lanes(k)]) for ref, r, k in done], axis=0)
        return last

    def tw_at(base, j, k):
        return D + (base // NT) * KS, lanes(j * 4 + k)

    def tw_sums(base):
        def quads(u):
            j, g = u
            return [(win_v, (slice(r0 + g * 16, r0 + (g + 1) * 16), lanes(n)))
                    for r0 in (0, KS) for n in (base + j, base + 3 + j)]

        def dest(u, k):
            j, g = u
            r0, cols = tw_at(base, j, k)
            return win_v, (slice(r0 + g * 16, r0 + (g + 1) * 16), cols)

        return chain_sums([(j, g) for j in range(3) for g in range(KS // 16)], quads, dest, b_sums, 0, True)

    def group(a0, base, j, hook, gate=None):
        r0, r1 = brows(a0), brows(a0 + 1)
        cl, cr = lanes(base + j), lanes(base + 3 + j)

        def out(a, n, val):
            t = gelu2(val)
            z1_v[w2_rows(a) if base else brows(a), lanes(n)] = t
            hook(t)

        def sx(k):
            return xn_v[xs_row(a0, k):xs_row(a0, k) + C, (k % 2) * KS:(k % 2 + 1) * KS]

        def tw(k):
            t0, cols = tw_at(base, j, k)
            return win_v[t0:t0 + KS, cols]

        def keep(slot, val):
            sl = (pl.ds(S + 4 * C + (j % 2) * C, C), lanes(slot))
            z1_v[sl] = val
            return lambda: z1_v[sl]

        a11 = xn_v[r0, 0:KS]
        if gate is not None:
            top = jnp.concatenate([held(a11[0:16, 0:128], gate), a11[0:16, 128:]], axis=1)
            a11 = jnp.concatenate([top, a11[16:, :]], axis=0)
        p1 = keep(0, mm(a11, win_v[0:KS, cl]))
        out(a0, j, p1() + mm(xn_v[r0, KS:D], win_v[KS:D, cl]))
        u2 = keep(1, p1() + mm(sx(1), tw(1)))
        u3 = keep(2, u2() + mm(sx(2), tw(2)))
        out(a0 + 1, j, u3() + mm(xn_v[r1, KS:D], jnp.concatenate([tw(3), win_v[2 * KS:D, cl]], axis=0)))
        p5 = mm(sx(0), tw(0))
        out(a0 + 1, 3 + j, (u3() + p5) + mm(xn_v[r1, 2 * KS:D], win_v[2 * KS:D, cr]))
        out(a0, 3 + j, (u2() + p5) + mm(jnp.concatenate([sx(3), xn_v[r0, 2 * KS:D]], axis=1), win_v[KS:D, cr]))

    def region(pairs, hch=(0, 0), kch=(0, 0), plan=((0, 0),)):
        hs = [(a, dt) for a in range(hch[0], hch[0] + hch[1]) for dt in range(ND)]
        us = [(a, dt) for a in range(kch[0], kch[0] + kch[1]) for dt in range(ND)]
        for bi, a0 in enumerate(pairs):
            nh, nu = plan[bi]
            nh_end = min(nh, 4) if bi == len(pairs) - 1 else 0
            nh_mid = min(8, nh - nh_end)
            nh_run = nh - nh_end - nh_mid
            nu_run = min(nu, 3 * nh_run)
            cnt = [0] * 25
            for j in range(nu - nu_run):
                cnt[U_SLOTS[j % len(U_SLOTS)]] += 1
            marks = [] if a0 + 2 >= NB else LNQ_H if nh_mid >= 5 else LNQ_NO_H
            seen = [0]

            def next_ln_q(part, t):
                tok = words(t)
                for a in (a0, a0 + 1):
                    if part == (0, 6)[a - a0]:
                        tok = jnp.concatenate([tok, z2_words(a)], axis=0)
                        if a >= NB // 2:
                            tw_ = words(t_v[brows(a - NB // 2), 4 * HN - 128:4 * HN])
                            tok = jnp.concatenate([tok, tw_], axis=0)
                ln_q(a0 + 2 + part // NLQ, fence(tok), part % NLQ, NLQ)

            def after_z2(t):
                for _ in range(cnt[seen[0]]):
                    u_dft(*us.pop(0))
                seen[0] += 1

            def after_z1(t):
                for part, (kind, idx, row) in enumerate(marks):
                    if kind == 'z' and idx == seen[0]:
                        next_ln_q(part, t[row:row + 8, :])
                for _ in range(cnt[13 + seen[0]]):
                    u_dft(*us.pop(0))
                seen[0] += 1

            for j in range(3):
                group(a0, NT, j, after_z2)
            hres = [h_dft(*hs.pop(0)) for _ in range(nh_mid)]
            for _ in range(cnt[12]):
                u_dft(*us.pop(0))
            ln_z2(a0 + 1, ln_z2(a0))
            for part, (kind, idx, row) in enumerate(marks):
                if kind == 'h':
                    next_ln_q(part, hres[idx][row:row + 8, :])
            seen[0] = 0
            for j in range(3):
                group(a0, 0, j, after_z1, fence(z2_words(a0 + j - 1)) if not marks and j >= 1 else None)
            ru, rh = nu_run, nh_run
            while ru or rh:
                if ru and ru * max(nh_run, 1) >= rh * max(nu_run, 1):
                    u_dft(*us.pop(0))
                    ru -= 1
                else:
                    h_dft(*hs.pop(0))
                    rh -= 1
            for _ in range(nh_end):
                h_dft(*hs.pop(0))
        assert not us
        return hs

    def conv_pos(ft, ft2, par, dt, after):
        cols = lanes(dt)
        prev = None
        for a in range(NB):
            ar, ai = (None, None) if prev is None else (-prev[1], prev[0])
            for dl in range(a + 1):
                hr = hf_v[ft, dl, 0:8, cols]
                hi = hf_v[ft, dl, 8:16, cols]
                ur = p_v[ft, a - dl, 0:8, cols]
                ui = p_v[ft, a - dl, 8:16, cols]
                if ar is None:
                    ar, ai = ur * hr - ui * hi, ur * hi + ui * hr
                    if after is not None:
                        z = fence(after)
                        ar, ai = held(ar, z), held(ai, z)
                elif (a * (a + 1) // 2 + dl) % TREE == 0:
                    ar = ar + (ur * hr - ui * hi)
                    ai = ai + (ur * hi + ui * hr)
                else:
                    ar = (ar + ur * hr) - ui * hi
                    ai = (ai + ur * hi) + ui * hr
            prev = (ar, ai) if prev is None else (ar + prev[1], ai - prev[0])
            w_v[a * 16 + ft2, par * 8:(par + 1) * 8, cols] = ar.astype(BF)
            w_v[a * 16 + 8 + ft2, par * 8:(par + 1) * 8, cols] = ai.astype(BF)
        return words(prev[0])

    gl_v = wout_v
    GL0 = FH
    GS0 = GL0 + NOP * C
    WS0 = GS0 + 4 * C
    GX0 = WS0 + 2 * HN

    def g_sums(ref, g0, s0):
        def quads(u):
            c, g = u
            return [(ref, (pl.ds(g0 + m * C + g * 16, 16), lanes(n))) for m in (0, 1) for n in (c, 3 + c)]

        def dest(u, k):
            c, g = u
            return gl_v, (pl.ds(s0 + k // 2 * C + g * 16, 16), lanes(k % 2 * 3 + c))

        chain_sums([(c, g) for c in range(3) for g in range(C // 16)], quads, dest, a_sums, 2, True)

    def ws_at(jj, k):
        return WS0 + (jj * 4 + k) // 6 * HN, lanes((jj * 4 + k) % 6)

    def w_sums():
        def quads(u):
            jj, g = u
            return [(wout_v, (pl.ds(r0 + g * 16, 16), lanes(n))) for r0 in (0, HN) for n in (jj, 2 + jj)]

        def dest(u, k):
            jj, g = u
            r0, cols = ws_at(jj, k)
            return wout_v, (pl.ds(r0 + g * 16, 16), cols)

        chain_sums([(jj, g) for jj in range(2) for g in range(HN // 16)], quads, dest, b_sums, 0, False)

    def xn_gate(a, dt, hh):
        return xn_v[brows(a), lanes(dt)].astype(F32) * (hh + hh * jnp.tanh(hh))

    def o_pair(a0, ref, g0, s0, finish, skip=False):
        r0, r1 = pl.ds(g0, C), pl.ds(g0 + C, C)

        def gs(k):
            return gl_v[pl.ds(s0 + k // 2 * C, C), (k % 2) * HN:(k % 2 + 1) * HN]

        def ws(jj, k):
            r, cols = ws_at(jj, k)
            return wout_v[r:r + HN, cols]

        finish(a0, 4, None if skip else mm(ref[r0, :], wout_v[0:FH, lanes(4)]))
        finish(a0 + 1, 4, mm(ref[r1, :], wout_v[0:FH, lanes(4)]))
        for jj in range(2):
            p1 = mm(ref[r0, 0:HN], wout_v[0:HN, lanes(jj)])
            finish(a0, jj, p1 + mm(ref[r0, HN:FH], wout_v[HN:FH, lanes(jj)]))
            u2 = p1 + mm(gs(1), ws(jj, 1))
            u3 = u2 + mm(gs(2), ws(jj, 2))
            finish(a0 + 1, jj, u3 + mm(ref[r1, HN:FH], ws(jj, 3)))
            p5 = mm(gs(0), ws(jj, 0))
            finish(a0 + 1, 2 + jj, u3 + p5)
            finish(a0, 2 + jj, (u2 + p5) + mm(gs(3), wout_v[HN:FH, lanes(2 + jj)]))

    def s_at(slot, k):
        return D + (slot * 2 + k // 2) * C, (k % 2) * HK

    def s_val(slot, k):
        r0, col = s_at(slot, k)
        return h_v[r0:r0 + C, col:col + HK]

    def s_sums(a0, nr, via_memory):
        def quads(u):
            slot, c, g = u
            return [(wsp_v, (ds((a0 + 2 * slot + m) * C + g * nr, nr), lanes(n)))
                    for m in (0, 1) for n in (c, HK // 128 + c)]

        def dest(u, k):
            slot, c, g = u
            r0, col = s_at(slot, k)
            return h_v, (slice(r0 + g * nr, r0 + (g + 1) * nr), slice(col + c * 128, col + (c + 1) * 128))

        units = [(slot, c, g) for slot in range(2) for c in range(HK // 128) for g in range(C // nr)]
        for part in (units[:len(units) // 2], units[len(units) // 2:]) if via_memory else (units,):
            chain_sums(part, quads, dest, a_sums, 2, via_memory)

    def phase2a(i, carry):
        @pl.when(i + 1 < S // TA)
        def _():
            cp_wsp(i + 1).wait()

        eye = (jax.lax.broadcasted_iota(jnp.int32, (C, C), 0)
               == jax.lax.broadcasted_iota(jnp.int32, (C, C), 1))

        def bcol(a):
            return jnp.sum(jnp.where(eye, b32_v[pl.ds(a, 1), :], 0.0), axis=-1, keepdims=True)

        def put(m, n, g):
            g = (z1_v[brows(i * (TA // C) + m), lanes(n)] * g).astype(BF)
            if m < NOP:
                gl_v[GL0 + m * C:GL0 + (m + 1) * C, lanes(n)] = g
            else:
                gg_v[ds((2 * i + m - NOP) * C, C), lanes(n)] = g
                if m == NOP:
                    gl_v[GX0:GX0 + C, lanes(n)] = g

        for pp in range(2):
            if pp == 1:
                g_sums(gl_v, GL0, GS0)
            m0 = 2 * pp
            a0 = i * (TA // C) + m0
            r0, r1 = brows(a0), brows(a0 + 1)
            b0 = bcol(a0)
            db = bcol(a0 + 1) - b0
            for j in range(NT // 2):
                jl, jr = lanes(j), lanes(NT // 2 + j)
                t1, t2, t3, t4 = (t_v[:, lanes(k * (NT // 2) + j)] for k in range(4))
                p1 = mm(wsp_v[r0, 0:HK], z2_v[0:HK, jl]) + b0
                put(m0, j, p1 + mm(wsp_v[r0, HK:S], z2_v[HK:S, jl]))
                u2 = p1 + mm(s_val(pp, 1), t2)
                u3 = (u2 + db) + mm(s_val(pp, 2), t3)
                put(m0 + 1, j, u3 + mm(wsp_v[r1, HK:S], t4))
                p5 = mm(s_val(pp, 0), t1)
                put(m0 + 1, NT // 2 + j, u3 + p5)
                put(m0, NT // 2 + j, (u2 + p5) + mm(s_val(pp, 3), z2_v[HK:S, jr]))
        def finish(a, dt, hh):
            xg_v[brows(a), lanes(dt)] = xn_gate(a, dt, hh)

        o_pair(i * (TA // C), gl_v, GL0, GS0, finish)
        finish(i * (TA // C) + 2, 4, mm(gl_v[GX0:GX0 + C, :], wout_v[0:FH, lanes(4)]))
        s_sums(jnp.minimum(i + 1, S // TA - 1) * (TA // C), 16, True)
        nft = NB * TA // S
        last = None
        for ft in range(nft):
            for dt in range(ND):
                last = conv_pos(i * nft + ft, i * (nft // 2) + ft // 2, ft % 2, dt, last)
        return carry

    step = pl.program_id(0)

    @pl.when(step == 0)
    def _():
        for grp in groups:
            for cp in grp:
                cp.start()
        cp_wout.start()
        for i in range(S // TA):
            cp_wsp(i).start()
        k_u[:, 0:8, :] = jnp.zeros((ND, 8, 128), U32)

    @pl.when(step == 1)
    def _():
        cp_wsp(0).wait()
        cp_wout.wait()
        t_rest(NB // 2 - 1, z2_v[brows(NB - 1), :].astype(F32))
        for a, dt in [(a, dt) for a in range(NB) for dt in range(ND)][NB * ND - H_LATE:]:
            h_dft(a, dt)
        w_sums()
        s_sums(0, 32, False)
        jax.lax.fori_loop(0, S // TA, phase2a, 0)

        rev = 7 - jax.lax.broadcasted_iota(jnp.int32, (8, 128), 0)
        done = {}

        def emit(a, dt, hh):
            rows, cols = brows(a), lanes(dt)
            ev = mm(fg_v[2 * C:2 * C + C // 2, 0:C], w_v[ds(a * 16, 8), :, cols].reshape(C, 128))
            od = mm(fg_v[2 * C:2 * C + C // 2, C:2 * C], w_v[ds(a * 16 + 8, 8), :, cols].reshape(C, 128))
            lo = ev - od
            ys = [jnp.take_along_axis(lo[g * 8:(g + 1) * 8, :], rev, axis=0)
                  for g in range(C // 16 - 1, -1, -1)]
            y = jnp.concatenate(ys + [ev + od], axis=0)
            xg = xg_v[rows, cols] if hh is None else xn_gate(a, dt, hh)
            o_v[rows, cols] = (q_v[rows, cols].astype(F32) + xg * y).astype(BF)
            done[a] = done.get(a, 0) + 1
            if a >= NB - 2:
                cp_o(a, cols).start()
            elif done[a] == ND:
                cp_o(a).start()

        g_sums(gg_v, 0, GS0)
        for k in range(S // TA):
            if k + 1 < S // TA:
                g_sums(gg_v, (k + 1) * 2 * C, GS0 + ((k + 1) % 2) * 2 * C)
            for a in (4 * k, 4 * k + 1):
                for dt in range(ND):
                    emit(a, dt, None)
            o_pair(4 * k + 2, gg_v, k * 2 * C, GS0 + (k % 2) * 2 * C, emit, skip=True)
        pltpu.make_async_copy(o_v, o_hbm, sem_o.at[0]).wait()

    @pl.when(step == 0)
    def _():
        wait(0)
        ln_q(0)
        ln_q(1)
        wait(1)
        for n in (0, 1):
            z2_tile(0, n)
            z2_tile(1, n)
        wait(2)
        ln_q(2)
        for n in (2, 3):
            z2_tile(0, n)
            z2_tile(1, n)
        for n in range(4):
            z2_tile(2, n)
        wait(3)
        ln_q(3)
        seq = ([(z2_tile, a, n) for a in range(3) for n in (4, 5)] + [(z2_tile, 3, n) for n in range(NT)]
               + [(z1_tile, a, 0) for a in range(4)])
        tw_done = tw_sums(NT)
        for j, (tile, a, n) in enumerate(seq):
            if j == 15:
                gate = fence(tw_done)
            elif j == 3:
                gate = fence(words(xn_v[brows(3), 0:128]))
            else:
                gate = fence(z2_words(0, (7, 10).index(j))) if j in (7, 10) else None
            tile(a, n, gate)
            if j == 1:
                ln_z2(0)
        wait(4)
        for a in (1, 2, 3):
            ln_z2(a)
        tw_sums(0)
        release = (9, 10, 11, 12, 14, 15, 16, 17)
        for j, (a, n) in enumerate((a, n) for n in range(1, NT) for a in range(4)):
            gate = fence(z2_words(1 + (j - 2) // 4, (j // 2 - 1) % 2)) if j in (2, 4, 6, 8, 10, 12) else None
            t = z1_tile(a, n, gate)
            if j in release:
                part = release.index(j)
                ln_q(4 + part // NLQ, fence(words(t[0:8, :])), part % NLQ, NLQ)
        region([4])
        wait(5)
        b32_v[...] = b_v[...].astype(F32) * 0.25
        assert not region([6, 8, 10], HCH[0], KCH[0], DFT_PLAN[0])
        wait(6)
        assert len(region([12, 14], HCH[1], KCH[1], DFT_PLAN[1])) == H_LATE


@jax.jit
def pallas_recurrent_scan__ssm_conv_h3__mixer_gmlp__prompt_kernel(
    A_q: jax.Array,
    A_k: jax.Array,
    A_v: jax.Array,
    A_shift_k: jax.Array,
    A_ssm_k: jax.Array,
    A_ssm_D: jax.Array,
    B_x: jax.Array,
    B_w_in: jax.Array,
    B_w_sp: jax.Array,
    B_b_sp: jax.Array,
    B_w_out: jax.Array,
):
    del B_x
    any_spec = pl.BlockSpec(memory_space=pl.ANY)
    vm = pltpu.VMEM
    dma = pltpu.SemaphoreType.DMA
    out = pl.pallas_call(
        _kernel,
        out_shape=jax.ShapeDtypeStruct((S, D), BF),
        grid=(2,),
        in_specs=[any_spec] * 11,
        out_specs=any_spec,
        scratch_shapes=[
            vm((S // 2, D), U32),
            vm((ND, S // 2 + 32, 128), U32),
            vm((S // 2, D), U32),
            vm(((D + 4 * C) // 2, S), U32),
            vm(((D + 2 * KS) // 2, 2 * FH), U32),
            vm((S // 2, S), U32),
            vm(((FH + 8 * C + 2 * HN) // 2, FH), U32),
            vm(((2 * C + C // 2) // 2, 2 * C), U32),
            vm(((S + 4 * C) // 2, D), U32),
            vm((S + 6 * C, FH), F32),
            vm((S // 2, FH), U32),
            vm((S // 4, 2 * FH), U32),
            vm((NB, NB, 16, D), F32),
            vm((NB, NB, 16, D), F32),
            vm((NB * 16, 8, 1024), U32),
            vm((S // 4, FH), U32),
            vm((S, D), F32),
            vm((S, D), BF),
            vm((NB, 128), F32),
            vm((NB, 128), BF),
            vm((4, 18 * 128), BF),
            vm((ND, 128), BF),
            dma((len(QCH),)), dma((len(KCH) * ND,)), dma((len(KCH),)), dma((len(HCH),)),
            dma((len(WCH),)), dma((S // TA,)), dma((1,)), dma((5,)),
        ],
        compiler_params=pltpu.CompilerParams(
            dimension_semantics=("arbitrary",),
            vmem_limit_bytes=110 * 1024 * 1024,
            disable_bounds_checks=True,
            disable_semaphore_checks=True,
        ),
    )(
        A_q.reshape(S, D), A_k.reshape(S, D), A_v.reshape(S, D),
        A_shift_k.T, A_ssm_k, A_ssm_D.reshape(ND, 128),
        B_w_in, B_w_sp, B_b_sp.reshape(NB, 128), B_w_out,
        _dft_consts(),
    )
    return out.reshape(1, S, D)
```

```python
import math

import jax
import jax.numpy as jnp
import numpy as np
import jax.experimental.pallas as pl
import jax.experimental.pallas.tpu as pltpu

S = 2048
D = 640
FH = 768
C = 128
NB = S // C
ND = D // 128
NT = FH // 128
EPS = 1e-5
HK = S // 2
HN = FH // 2
KS = 256
TA = 512
NOP = 2
NLQ = 4
H_LATE = 24
TREE = 10

BF = jnp.bfloat16
F32 = jnp.float32
U32 = jnp.uint32

QCH = [(0, 2), (2, 1), (3, 1), (4, 4), (8, 6), (14, 2)]
HCH = [(0, 5), (5, 11)]
KCH = [(0, 3), (3, 13)]
WCH = [(6, 2), (8, 2), (10, 2), (0, 1), (1, 5)]
DFT_PLAN = [[(8, 4), (8, 8), (9, 3)], [(16, 32), (15, 33)]]
U_SLOTS = [1, 5, 9, 3, 7, 14, 18, 22, 0, 4, 8, 16, 20, 2, 6, 10, 15, 19, 23, 11, 13, 17, 21, 12, 24]
LNQ_H = [('h', 4, 128)] + [('z', n, 120) for n in (0, 1, 3, 4, 5, 7, 8)]
LNQ_NO_H = [('z', n, 0) for n in (1, 2, 3, 4, 5, 6, 8, 9)]


def _dft_consts():
    theta = np.pi * (4 * np.arange(C) + 1) / (2 * C)

    def fwd(t):
        ang = theta[:, None] * t[None, :]
        re = np.cos(ang).reshape(C // 8, 8, C)
        im = -np.sin(ang).reshape(C // 8, 8, C)
        return np.stack([re, im], axis=1).reshape(2 * C, C)

    fg = np.zeros((2 * C + C // 2, 2 * C), np.float64)
    order = np.concatenate([np.arange(0, C, 2), np.arange(1, C, 2)])
    fg[:2 * C, :C] = fwd(order - (C - 1) / 2)
    fg[:2 * C, C:] = fwd(np.arange(C))
    ang = (np.arange(C // 2) + 0.5)[:, None] * theta[None, :]
    fg[2 * C:, :C] = np.cos(ang) / C
    fg[2 * C:, C:] = -np.sin(ang) / C
    return fg.astype(np.float32).astype(BF)


def _kernel(q_hbm, k_hbm, v_hbm, sk_hbm, h_hbm, d_hbm, win_hbm, wsp_hbm, b_hbm, wout_hbm,
            fg_hbm, o_hbm,
            q_u, k_u, v_u, h_u, win_u, wsp_u, wout_u, fg_u,
            xn_u, z1_v, z2_u, t_u, p_v, hf_v, w_u, gg_u, xg_v, o_v, b32_v, b_v, sk_v, d_v,
            sem_q, sem_k, sem_v, sem_h, sem_w, sem_wsp, sem_o, sem_m):
    q_v = q_u.bitcast(BF)
    v_v = v_u.bitcast(BF)
    k_w = k_hbm.bitcast(U32)
    h_v = h_u.bitcast(BF)
    win_v = win_u.bitcast(BF)
    wsp_v = wsp_u.bitcast(BF)
    wout_v = wout_u.bitcast(BF)
    fg_v = fg_u.bitcast(BF)
    xn_v = xn_u.bitcast(BF)
    z2_v = z2_u.bitcast(BF)
    t_v = t_u.bitcast(BF)
    w_v = w_u.bitcast(BF)
    gg_v = gg_u.bitcast(BF)

    def ds(start, size):
        if isinstance(start, int):
            return pl.ds(start, size)
        return pl.ds(pl.multiple_of(start, size), size)

    def lanes(n):
        return slice(n * 128, (n + 1) * 128)

    def blocks(ch):
        return pl.ds(ch[0] * C, ch[1] * C)

    def brows(a):
        return ds(a * C, C)

    def cp_q(c):
        r = blocks(QCH[c])
        return pltpu.make_async_copy(q_hbm.at[r, :], q_v.at[r, :], sem_q.at[c])

    def cp_k(c):
        b0, n = KCH[c]
        return [pltpu.make_async_copy(k_w.at[pl.ds(b0 * C // 2, n * C // 2), lanes(dt)],
                                      k_u.at[dt, pl.ds(b0 * C // 2 + 8, n * C // 2), :],
                                      sem_k.at[c * ND + dt])
                for dt in range(ND)]

    def cp_v(c):
        r = blocks(KCH[c])
        return pltpu.make_async_copy(v_hbm.at[r, :], v_v.at[r, :], sem_v.at[c])

    def cp_h(c):
        r = blocks(HCH[c])
        return pltpu.make_async_copy(h_hbm.at[:, r], h_v.at[0:D, r], sem_h.at[c])

    def cp_w(c):
        r = blocks(WCH[c])
        return pltpu.make_async_copy(win_hbm.at[:, r], win_v.at[0:D, r], sem_w.at[c])

    def cp_wsp(i):
        r = ds(i * TA, TA)
        return pltpu.make_async_copy(wsp_hbm.at[r, :], wsp_v.at[r, :], sem_wsp.at[i])

    def cp_o(a, cols=slice(None)):
        r = brows(a)
        return pltpu.make_async_copy(o_v.at[r, cols], o_hbm.at[r, cols], sem_o.at[0])

    cp_f = pltpu.make_async_copy(fg_hbm, fg_v, sem_m.at[0])
    cp_sk = pltpu.make_async_copy(sk_hbm, sk_v.at[:, 0:D], sem_m.at[1])
    cp_d = pltpu.make_async_copy(d_hbm, d_v, sem_m.at[2])
    cp_b = pltpu.make_async_copy(b_hbm, b_v, sem_m.at[3])
    cp_wout = pltpu.make_async_copy(wout_hbm, wout_v.at[0:FH, 0:D], sem_m.at[4])

    groups = [
        [cp_q(0)], [cp_w(0)], [cp_q(1), cp_w(1)], [cp_q(2), cp_w(2), cp_w(3)], [cp_q(3), cp_w(4)],
        [cp_f, cp_sk, cp_d, cp_b, cp_q(4), cp_h(0), *cp_k(0), cp_v(0)],
        [cp_q(5), cp_h(1), *cp_k(1), cp_v(1)],
    ]

    def wait(g):
        for cp in groups[g]:
            cp.wait()

    def mm(x, y):
        return jnp.dot(x, y, preferred_element_type=F32)

    def words(x):
        return pltpu.bitcast(x, U32)

    def fence(tok):
        t = tok[0:8, :]
        for g in range(1, tok.shape[0] // 8):
            t = t | tok[g * 8:(g + 1) * 8, :]
        return t & k_u[0, 0:8, :]

    def held(x, gate):
        if gate is None:
            return x
        w = words(x)
        return pltpu.bitcast(w | jnp.tile(gate, (w.shape[0] // 8, w.shape[1] // 128)), x.dtype)

    def a_sums(a11, a12, a21, a22):
        s1 = a21 + a22
        s2 = s1 - a11
        return s1, s2, a11 - a21, a12 - s2

    def b_sums(b11, b12, b21, b22):
        t1 = b12 - b11
        t2 = b22 - t1
        return t1, t2, t2 - b11, b21 - t2

    def chain_sums(units, quads, dest, combine, lead, via_memory):
        last = None
        for u in units:
            vals = []
            for n, (ref, idx) in enumerate(quads(u)):
                wait_here = last is not None and (n == lead or not via_memory)
                vals.append(held(ref[idx], fence(last) if wait_here else None).astype(F32))
            sums = combine(*vals)
            done = []
            for k, val in enumerate(sums):
                ref, idx = dest(u, k)
                ref[idx] = val.astype(BF)
                if via_memory:
                    done.append(words(ref[idx]))
            last = jnp.concatenate(done, axis=0) if via_memory else words(sums[-1][-8:, :])
        return last

    c0 = math.sqrt(2.0 / math.pi)
    c1 = c0 * 0.044715

    def gelu2(x):
        return x + x * jnp.tanh(x * (c0 + c1 * (x * x)))

    def z2_words(a, half=None):
        r = brows(a) if half is None else pl.ds(a * C + half * (C // 2), C // 2)
        return words(z2_v[r, 0:128])

    def xs_row(a0, k):
        return S + (a0 // 2 % 2) * 2 * C + k // 2 * C

    def ln_q(a, gate=None, part=0, nparts=1):
        n = C // nparts
        r = pl.ds(a * C + part * n, n)
        x = held(q_v[r, :], gate).astype(F32)
        mu = jnp.sum(x, axis=-1, keepdims=True) * (1.0 / D)
        ex2 = jnp.sum(x * x, axis=-1, keepdims=True) * (1.0 / D)
        var = jnp.maximum(ex2 - mu * mu, 0.0)
        mu = mu.astype(BF).astype(F32)
        xn = (x - mu) * jnp.exp(-0.5 * jnp.log(var + EPS))
        xn_v[r, :] = xn.astype(BF)
        if a >= 4 and a % 2 == 1:
            top = xn_v[pl.ds((a - 1) * C + part * n, n), 0:2 * KS].astype(F32)
            s1, s2, s3, s4 = a_sums(top[:, :KS], top[:, KS:], xn[:, :KS], xn[:, KS:2 * KS])
            xn_v[pl.ds(xs_row(a - 1, 0) + part * n, n), 0:2 * KS] = jnp.concatenate([s1, s2], axis=1).astype(BF)
            xn_v[pl.ds(xs_row(a - 1, 2) + part * n, n), 0:2 * KS] = jnp.concatenate([s3, s4], axis=1).astype(BF)

    def h_dft(a, dt):
        res = jax.lax.dot_general(fg_v[0:2 * C, C:2 * C], h_v[lanes(dt), brows(a)],
                                  (((1,), (1,)), ((), ())), preferred_element_type=F32)
        spec = res.reshape(NB, 16, 128)
        if a == 0:
            dv = d_v[...].astype(F32)[dt:dt + 1, :]
            spec = jnp.concatenate([spec[:, 0:8, :] + dv[None], spec[:, 8:16, :]], axis=1)
        hf_v[:, a, :, lanes(dt)] = spec
        return res

    def u_dft(a, dt):
        cols = lanes(dt)

        def even(w):
            return pltpu.bitcast(w << 16, F32)

        def odd(w):
            return pltpu.bitcast(w & jnp.uint32(0xFFFF0000), F32)

        w0, w1, w2 = (k_u[dt, pl.ds(8 + a * C // 2 - j, C // 2), :] for j in range(3))
        e0, o0, e1, o1 = even(w0), odd(w0), even(w1), odd(w1)
        sk = sk_v[:, cols].astype(F32)
        s0, s1, s2, s3 = (sk[j:j + 1, :] for j in range(4))
        vw = words(v_v[brows(a), cols])
        kve = (e0 * s0 + o1 * s1 + e1 * s2 + odd(w2) * s3) * even(vw)
        kvo = (o0 * s0 + e0 * s1 + o1 * s2 + e1 * s3) * odd(vw)
        kv = jnp.concatenate([kve, kvo], axis=0).astype(BF)
        p_v[:, a, :, cols] = mm(fg_v[0:2 * C, 0:C], kv).reshape(NB, 16, 128)

    def proj(a, n, gate=None):
        lhs = xn_v[brows(a), :]
        if gate is not None:
            lhs = jnp.concatenate([held(lhs[0:16, :], gate), lhs[16:, :]], axis=0)
        return gelu2(mm(lhs, win_v[0:D, lanes(n)]))

    def w2_rows(a):
        return pl.ds(S + (a % 4) * C, C)

    def z2_tile(a, n, gate=None):
        z1_v[w2_rows(a), lanes(n)] = proj(a, NT + n, gate)

    def z1_tile(a, n, gate=None):
        t = proj(a, n, gate)
        z1_v[brows(a), lanes(n)] = t
        return t

    def t_rest(r, bot, g=0, nr=C):
        rows = pl.ds(r * C + g * nr, nr)
        t2 = bot[:, HN:] - t_v[rows, 0:HN].astype(F32)
        t3 = t2 - z2_v[rows, 0:HN].astype(F32)
        t_v[rows, HN:4 * HN] = jnp.concatenate([t2, t3, bot[:, :HN] - t2], axis=1).astype(BF)

    def ln_z2(a, last=None):
        w2 = z1_v[w2_rows(a), :]
        mu = jnp.sum(w2, axis=-1, keepdims=True) * (1.0 / FH)
        ex2 = jnp.sum(w2 * w2, axis=-1, keepdims=True) * (1.0 / FH)
        var = jnp.maximum(ex2 - mu * mu, 0.0)
        rs = jnp.exp(-0.5 * jnp.log(16.0 * var + 64.0 * EPS))
        nr = 16 if 4 <= a < NB - 2 else C
        for g in range(C // nr):
            rr = slice(g * nr, (g + 1) * nr)
            m = held(jnp.broadcast_to(mu[rr], (nr, 128)), fence(last) if last is not None and nr < C else None)
            zn = (w2[rr] - jnp.tile(m, (1, NT))) * rs[rr]
            rows = pl.ds(a * C + g * nr, nr)
            if a < NB // 2:
                z2_v[rows, 0:HN] = zn[:, :HN].astype(BF)
                t_v[rows, 0:HN] = (zn[:, HN:] - zn[:, :HN]).astype(BF)
                done = [(z2_v, rows, k) for k in range(3)] + [(t_v, rows, k) for k in range(3)]
            else:
                z2_v[rows, :] = zn.astype(BF)
                done = [(z2_v, rows, k) for k in range(6)]
                if a < NB - 1:
                    t_rest(a - NB // 2, zn, g, nr)
                    done += [(t_v, pl.ds((a - NB // 2) * C + g * nr, nr), k) for k in range(3, 12)]
            if nr < C:
                last = jnp.concatenate([words(ref[r, lanes(k)]) for ref, r, k in done], axis=0)
        return last

    def tw_at(base, j, k):
        return D + (base // NT) * KS, lanes(j * 4 + k)

    def tw_sums(base):
        def quads(u):
            j, g = u
            return [(win_v, (slice(r0 + g * 16, r0 + (g + 1) * 16), lanes(n)))
                    for r0 in (0, KS) for n in (base + j, base + 3 + j)]

        def dest(u, k):
            j, g = u
            r0, cols = tw_at(base, j, k)
            return win_v, (slice(r0 + g * 16, r0 + (g + 1) * 16), cols)

        return chain_sums([(j, g) for j in range(3) for g in range(KS // 16)], quads, dest, b_sums, 0, True)

    def group(a0, base, j, hook, gate=None):
        r0, r1 = brows(a0), brows(a0 + 1)
        cl, cr = lanes(base + j), lanes(base + 3 + j)

        def out(a, n, val):
            t = gelu2(val)
            z1_v[w2_rows(a) if base else brows(a), lanes(n)] = t
            hook(t)

        def sx(k):
            return xn_v[xs_row(a0, k):xs_row(a0, k) + C, (k % 2) * KS:(k % 2 + 1) * KS]

        def tw(k):
            t0, cols = tw_at(base, j, k)
            return win_v[t0:t0 + KS, cols]

        def keep(slot, val):
            sl = (pl.ds(S + 4 * C + (j % 2) * C, C), lanes(slot))
            z1_v[sl] = val
            return lambda: z1_v[sl]

        a11 = xn_v[r0, 0:KS]
        if gate is not None:
            top = jnp.concatenate([held(a11[0:16, 0:128], gate), a11[0:16, 128:]], axis=1)
            a11 = jnp.concatenate([top, a11[16:, :]], axis=0)
        p1 = keep(0, mm(a11, win_v[0:KS, cl]))
        out(a0, j, p1() + mm(xn_v[r0, KS:D], win_v[KS:D, cl]))
        u2 = keep(1, p1() + mm(sx(1), tw(1)))
        u3 = keep(2, u2() + mm(sx(2), tw(2)))
        out(a0 + 1, j, u3() + mm(xn_v[r1, KS:D], jnp.concatenate([tw(3), win_v[2 * KS:D, cl]], axis=0)))
        p5 = mm(sx(0), tw(0))
        out(a0 + 1, 3 + j, (u3() + p5) + mm(xn_v[r1, 2 * KS:D], win_v[2 * KS:D, cr]))
        out(a0, 3 + j, (u2() + p5) + mm(jnp.concatenate([sx(3), xn_v[r0, 2 * KS:D]], axis=1), win_v[KS:D, cr]))

    def region(pairs, hch=(0, 0), kch=(0, 0), plan=((0, 0),)):
        hs = [(a, dt) for a in range(hch[0], hch[0] + hch[1]) for dt in range(ND)]
        us = [(a, dt) for a in range(kch[0], kch[0] + kch[1]) for dt in range(ND)]
        for bi, a0 in enumerate(pairs):
            nh, nu = plan[bi]
            nh_end = min(nh, 4) if bi == len(pairs) - 1 else 0
            nh_mid = min(8, nh - nh_end)
            nh_run = nh - nh_end - nh_mid
            nu_run = min(nu, 3 * nh_run)
            cnt = [0] * 25
            for j in range(nu - nu_run):
                cnt[U_SLOTS[j % len(U_SLOTS)]] += 1
            marks = [] if a0 + 2 >= NB else LNQ_H if nh_mid >= 5 else LNQ_NO_H
            seen = [0]

            def next_ln_q(part, t):
                tok = words(t)
                for a in (a0, a0 + 1):
                    if part == (0, 6)[a - a0]:
                        tok = jnp.concatenate([tok, z2_words(a)], axis=0)
                        if a >= NB // 2:
                            tw_ = words(t_v[brows(a - NB // 2), 4 * HN - 128:4 * HN])
                            tok = jnp.concatenate([tok, tw_], axis=0)
                ln_q(a0 + 2 + part // NLQ, fence(tok), part % NLQ, NLQ)

            def after_z2(t):
                for _ in range(cnt[seen[0]]):
                    u_dft(*us.pop(0))
                seen[0] += 1

            def after_z1(t):
                for part, (kind, idx, row) in enumerate(marks):
                    if kind == 'z' and idx == seen[0]:
                        next_ln_q(part, t[row:row + 8, :])
                for _ in range(cnt[13 + seen[0]]):
                    u_dft(*us.pop(0))
                seen[0] += 1

            for j in range(3):
                group(a0, NT, j, after_z2)
            hres = [h_dft(*hs.pop(0)) for _ in range(nh_mid)]
            for _ in range(cnt[12]):
                u_dft(*us.pop(0))
            ln_z2(a0 + 1, ln_z2(a0))
            for part, (kind, idx, row) in enumerate(marks):
                if kind == 'h':
                    next_ln_q(part, hres[idx][row:row + 8, :])
            seen[0] = 0
            for j in range(3):
                group(a0, 0, j, after_z1, fence(z2_words(a0 + j - 1)) if not marks and j >= 1 else None)
            ru, rh = nu_run, nh_run
            while ru or rh:
                if ru and ru * max(nh_run, 1) >= rh * max(nu_run, 1):
                    u_dft(*us.pop(0))
                    ru -= 1
                else:
                    h_dft(*hs.pop(0))
                    rh -= 1
            for _ in range(nh_end):
                h_dft(*hs.pop(0))
        assert not us
        return hs

    def conv_pos(ft, ft2, par, dt, after):
        cols = lanes(dt)
        prev = None
        for a in range(NB):
            ar, ai = (None, None) if prev is None else (-prev[1], prev[0])
            for dl in range(a + 1):
                hr = hf_v[ft, dl, 0:8, cols]
                hi = hf_v[ft, dl, 8:16, cols]
                ur = p_v[ft, a - dl, 0:8, cols]
                ui = p_v[ft, a - dl, 8:16, cols]
                if ar is None:
                    ar, ai = ur * hr - ui * hi, ur * hi + ui * hr
                    if after is not None:
                        z = fence(after)
                        ar, ai = held(ar, z), held(ai, z)
                elif (a * (a + 1) // 2 + dl) % TREE == 0:
                    ar = ar + (ur * hr - ui * hi)
                    ai = ai + (ur * hi + ui * hr)
                else:
                    ar = (ar + ur * hr) - ui * hi
                    ai = (ai + ur * hi) + ui * hr
            prev = (ar, ai) if prev is None else (ar + prev[1], ai - prev[0])
            w_v[a * 16 + ft2, par * 8:(par + 1) * 8, cols] = ar.astype(BF)
            w_v[a * 16 + 8 + ft2, par * 8:(par + 1) * 8, cols] = ai.astype(BF)
        return words(prev[0])

    gl_v = wout_v
    GL0 = FH
    GS0 = GL0 + NOP * C
    WS0 = GS0 + 4 * C
    GX0 = WS0 + 2 * HN

    def g_sums(ref, g0, s0):
        def quads(u):
            c, g = u
            return [(ref, (pl.ds(g0 + m * C + g * 16, 16), lanes(n))) for m in (0, 1) for n in (c, 3 + c)]

        def dest(u, k):
            c, g = u
            return gl_v, (pl.ds(s0 + k // 2 * C + g * 16, 16), lanes(k % 2 * 3 + c))

        chain_sums([(c, g) for c in range(3) for g in range(C // 16)], quads, dest, a_sums, 2, True)

    def ws_at(jj, k):
        return WS0 + (jj * 4 + k) // 6 * HN, lanes((jj * 4 + k) % 6)

    def w_sums():
        def quads(u):
            jj, g = u
            return [(wout_v, (pl.ds(r0 + g * 16, 16), lanes(n))) for r0 in (0, HN) for n in (jj, 2 + jj)]

        def dest(u, k):
            jj, g = u
            r0, cols = ws_at(jj, k)
            return wout_v, (pl.ds(r0 + g * 16, 16), cols)

        chain_sums([(jj, g) for jj in range(2) for g in range(HN // 16)], quads, dest, b_sums, 0, False)

    def xn_gate(a, dt, hh):
        return xn_v[brows(a), lanes(dt)].astype(F32) * (hh + hh * jnp.tanh(hh))

    def o_pair(a0, ref, g0, s0, finish, skip=False):
        r0, r1 = pl.ds(g0, C), pl.ds(g0 + C, C)

        def gs(k):
            return gl_v[pl.ds(s0 + k // 2 * C, C), (k % 2) * HN:(k % 2 + 1) * HN]

        def ws(jj, k):
            r, cols = ws_at(jj, k)
            return wout_v[r:r + HN, cols]

        for jj in range(2):
            if jj == (0 if skip else 1):
                finish(a0, 4, None if skip else mm(ref[r0, :], wout_v[0:FH, lanes(4)]))
                finish(a0 + 1, 4, mm(ref[r1, :], wout_v[0:FH, lanes(4)]))
            p1 = mm(ref[r0, 0:HN], wout_v[0:HN, lanes(jj)])
            finish(a0, jj, p1 + mm(ref[r0, HN:FH], wout_v[HN:FH, lanes(jj)]))
            u2 = p1 + mm(gs(1), ws(jj, 1))
            u3 = u2 + mm(gs(2), ws(jj, 2))
            finish(a0 + 1, jj, u3 + mm(ref[r1, HN:FH], ws(jj, 3)))
            p5 = mm(gs(0), ws(jj, 0))
            finish(a0 + 1, 2 + jj, u3 + p5)
            finish(a0, 2 + jj, (u2 + p5) + mm(gs(3), wout_v[HN:FH, lanes(2 + jj)]))

    def s_at(slot, k):
        return D + (slot * 2 + k // 2) * C, (k % 2) * HK

    def s_val(slot, k):
        r0, col = s_at(slot, k)
        return h_v[r0:r0 + C, col:col + HK]

    def s_sums(a0, nr, via_memory):
        def quads(u):
            slot, c, g = u
            return [(wsp_v, (ds((a0 + 2 * slot + m) * C + g * nr, nr), lanes(n)))
                    for m in (0, 1) for n in (c, HK // 128 + c)]

        def dest(u, k):
            slot, c, g = u
            r0, col = s_at(slot, k)
            return h_v, (slice(r0 + g * nr, r0 + (g + 1) * nr), slice(col + c * 128, col + (c + 1) * 128))

        units = [(slot, c, g) for slot in range(2) for c in range(HK // 128) for g in range(C // nr)]
        for part in (units[:48], units[48:]) if via_memory else (units,):
            chain_sums(part, quads, dest, a_sums, 2, via_memory)

    def phase2a(i, carry):
        @pl.when(i + 1 < S // TA)
        def _():
            cp_wsp(i + 1).wait()

        eye = (jax.lax.broadcasted_iota(jnp.int32, (C, C), 0)
               == jax.lax.broadcasted_iota(jnp.int32, (C, C), 1))

        def bcol(a):
            return jnp.sum(jnp.where(eye, b32_v[pl.ds(a, 1), :], 0.0), axis=-1, keepdims=True)

        def put(m, n, g):
            g = (z1_v[brows(i * (TA // C) + m), lanes(n)] * g).astype(BF)
            if m < NOP:
                gl_v[GL0 + m * C:GL0 + (m + 1) * C, lanes(n)] = g
            else:
                gg_v[ds((2 * i + m - NOP) * C, C), lanes(n)] = g
                if m == NOP:
                    gl_v[GX0:GX0 + C, lanes(n)] = g

        for pp in range(2):
            if pp == 1:
                g_sums(gl_v, GL0, GS0)
            m0 = 2 * pp
            a0 = i * (TA // C) + m0
            r0, r1 = brows(a0), brows(a0 + 1)
            b0 = bcol(a0)
            db = bcol(a0 + 1) - b0
            for j in range(NT // 2):
                jl, jr = lanes(j), lanes(NT // 2 + j)
                t1, t2, t3, t4 = (t_v[:, lanes(k * (NT // 2) + j)] for k in range(4))
                p1 = mm(wsp_v[r0, 0:HK], z2_v[0:HK, jl]) + b0
                put(m0, j, p1 + mm(wsp_v[r0, HK:S], z2_v[HK:S, jl]))
                u2 = p1 + mm(s_val(pp, 1), t2)
                u3 = (u2 + db) + mm(s_val(pp, 2), t3)
                put(m0 + 1, j, u3 + mm(wsp_v[r1, HK:S], t4))
                p5 = mm(s_val(pp, 0), t1)
                put(m0 + 1, NT // 2 + j, u3 + p5)
                put(m0, NT // 2 + j, (u2 + p5) + mm(s_val(pp, 3), z2_v[HK:S, jr]))
        def finish(a, dt, hh):
            xg_v[brows(a), lanes(dt)] = xn_gate(a, dt, hh)

        o_pair(i * (TA // C), gl_v, GL0, GS0, finish)
        finish(i * (TA // C) + 2, 4, mm(gl_v[GX0:GX0 + C, :], wout_v[0:FH, lanes(4)]))
        s_sums(jnp.minimum(i + 1, S // TA - 1) * (TA // C), 16, True)
        nft = NB * TA // S
        last = None
        for ft in range(nft):
            for dt in range(ND):
                last = conv_pos(i * nft + ft, i * (nft // 2) + ft // 2, ft % 2, dt, last)
        return carry

    step = pl.program_id(0)

    @pl.when(step == 0)
    def _():
        for grp in groups:
            for cp in grp:
                cp.start()
        cp_wout.start()
        for i in range(S // TA):
            cp_wsp(i).start()
        k_u[:, 0:8, :] = jnp.zeros((ND, 8, 128), U32)

    @pl.when(step == 1)
    def _():
        cp_wsp(0).wait()
        cp_wout.wait()
        t_rest(NB // 2 - 1, z2_v[brows(NB - 1), :].astype(F32))
        for a, dt in [(a, dt) for a in range(NB) for dt in range(ND)][NB * ND - H_LATE:]:
            h_dft(a, dt)
        w_sums()
        s_sums(0, 32, False)
        jax.lax.fori_loop(0, S // TA, phase2a, 0)

        rev = 7 - jax.lax.broadcasted_iota(jnp.int32, (8, 128), 0)
        done = {}

        def emit(a, dt, hh):
            rows, cols = brows(a), lanes(dt)
            ev = mm(fg_v[2 * C:2 * C + C // 2, 0:C], w_v[ds(a * 16, 8), :, cols].reshape(C, 128))
            od = mm(fg_v[2 * C:2 * C + C // 2, C:2 * C], w_v[ds(a * 16 + 8, 8), :, cols].reshape(C, 128))
            lo = ev - od
            ys = [jnp.take_along_axis(lo[g * 8:(g + 1) * 8, :], rev, axis=0)
                  for g in range(C // 16 - 1, -1, -1)]
            y = jnp.concatenate(ys + [ev + od], axis=0)
            xg = xg_v[rows, cols] if hh is None else xn_gate(a, dt, hh)
            o_v[rows, cols] = (q_v[rows, cols].astype(F32) + xg * y).astype(BF)
            done[a] = done.get(a, 0) + 1
            if a >= NB - 2:
                cp_o(a, cols).start()
            elif done[a] == ND:
                cp_o(a).start()

        g_sums(gg_v, 0, GS0)
        for k in range(S // TA):
            if k + 1 < S // TA:
                g_sums(gg_v, (k + 1) * 2 * C, GS0 + ((k + 1) % 2) * 2 * C)
            for a in (4 * k, 4 * k + 1):
                for dt in range(ND):
                    emit(a, dt, None)
            o_pair(4 * k + 2, gg_v, k * 2 * C, GS0 + (k % 2) * 2 * C, emit, skip=True)
        pltpu.make_async_copy(o_v, o_hbm, sem_o.at[0]).wait()

    @pl.when(step == 0)
    def _():
        wait(0)
        ln_q(0)
        ln_q(1)
        wait(1)
        for n in (0, 1):
            z2_tile(0, n)
            z2_tile(1, n)
        wait(2)
        ln_q(2)
        for n in (2, 3):
            z2_tile(0, n)
            z2_tile(1, n)
        for n in range(4):
            z2_tile(2, n)
        wait(3)
        ln_q(3)
        seq = ([(z2_tile, a, n) for a in range(3) for n in (4, 5)] + [(z2_tile, 3, n) for n in range(NT)]
               + [(z1_tile, a, 0) for a in range(4)])
        tw_done = tw_sums(NT)
        for j, (tile, a, n) in enumerate(seq):
            if j == 15:
                gate = fence(tw_done)
            elif j == 3:
                gate = fence(words(xn_v[brows(3), 0:128]))
            else:
                gate = fence(z2_words(0, (7, 10).index(j))) if j in (7, 10) else None
            tile(a, n, gate)
            if j == 1:
                ln_z2(0)
        wait(4)
        for a in (1, 2, 3):
            ln_z2(a)
        tw_sums(0)
        release = (9, 10, 11, 12, 14, 15, 16, 17)
        for j, (a, n) in enumerate((a, n) for n in range(1, NT) for a in range(4)):
            gate = fence(z2_words(1 + (j - 2) // 4, (j // 2 - 1) % 2)) if j in (2, 4, 6, 8, 10, 12) else None
            t = z1_tile(a, n, gate)
            if j in release:
                part = release.index(j)
                ln_q(4 + part // NLQ, fence(words(t[0:8, :])), part % NLQ, NLQ)
        region([4])
        wait(5)
        b32_v[...] = b_v[...].astype(F32) * 0.25
        assert not region([6, 8, 10], HCH[0], KCH[0], DFT_PLAN[0])
        wait(6)
        assert len(region([12, 14], HCH[1], KCH[1], DFT_PLAN[1])) == H_LATE


@jax.jit
def pallas_recurrent_scan__ssm_conv_h3__mixer_gmlp__prompt_kernel(
    A_q: jax.Array,
    A_k: jax.Array,
    A_v: jax.Array,
    A_shift_k: jax.Array,
    A_ssm_k: jax.Array,
    A_ssm_D: jax.Array,
    B_x: jax.Array,
    B_w_in: jax.Array,
    B_w_sp: jax.Array,
    B_b_sp: jax.Array,
    B_w_out: jax.Array,
):
    del B_x
    any_spec = pl.BlockSpec(memory_space=pl.ANY)
    vm = pltpu.VMEM
    dma = pltpu.SemaphoreType.DMA
    out = pl.pallas_call(
        _kernel,
        out_shape=jax.ShapeDtypeStruct((S, D), BF),
        grid=(2,),
        in_specs=[any_spec] * 11,
        out_specs=any_spec,
        scratch_shapes=[
            vm((S // 2, D), U32),
            vm((ND, S // 2 + 32, 128), U32),
            vm((S // 2, D), U32),
            vm(((D + 4 * C) // 2, S), U32),
            vm(((D + 2 * KS) // 2, 2 * FH), U32),
            vm((S // 2, S), U32),
            vm(((FH + 8 * C + 2 * HN) // 2, FH), U32),
            vm(((2 * C + C // 2) // 2, 2 * C), U32),
            vm(((S + 4 * C) // 2, D), U32),
            vm((S + 6 * C, FH), F32),
            vm((S // 2, FH), U32),
            vm((S // 4, 2 * FH), U32),
            vm((NB, NB, 16, D), F32),
            vm((NB, NB, 16, D), F32),
            vm((NB * 16, 8, 1024), U32),
            vm((S // 4, FH), U32),
            vm((S, D), F32),
            vm((S, D), BF),
            vm((NB, 128), F32),
            vm((NB, 128), BF),
            vm((4, 18 * 128), BF),
            vm((ND, 128), BF),
            dma((len(QCH),)), dma((len(KCH) * ND,)), dma((len(KCH),)), dma((len(HCH),)),
            dma((len(WCH),)), dma((S // TA,)), dma((1,)), dma((5,)),
        ],
        compiler_params=pltpu.CompilerParams(
            dimension_semantics=("arbitrary",),
            vmem_limit_bytes=110 * 1024 * 1024,
            disable_bounds_checks=True,
            disable_semaphore_checks=True,
        ),
    )(
        A_q.reshape(S, D), A_k.reshape(S, D), A_v.reshape(S, D),
        A_shift_k.T, A_ssm_k, A_ssm_D.reshape(ND, 128),
        B_w_in, B_w_sp, B_b_sp.reshape(NB, 128), B_w_out,
        _dft_consts(),
    )
    return out.reshape(1, S, D)
```

```python
import math

import jax
import jax.numpy as jnp
import numpy as np
import jax.experimental.pallas as pl
import jax.experimental.pallas.tpu as pltpu

S = 2048
D = 640
FH = 768
C = 128
NB = S // C
ND = D // 128
NT = FH // 128
EPS = 1e-5
HK = S // 2
HN = FH // 2
KS = 256
TA = 512
NOP = 2
NLQ = 4
H_LATE = 24
TREE = 10

BF = jnp.bfloat16
F32 = jnp.float32
U32 = jnp.uint32

QCH = [(0, 2), (2, 1), (3, 1), (4, 4), (8, 6), (14, 2)]
HCH = [(0, 5), (5, 11)]
KCH = [(0, 3), (3, 13)]
WCH = [(6, 2), (8, 2), (10, 2), (0, 1), (1, 5)]
DFT_PLAN = [[(8, 4), (8, 8), (9, 3)], [(16, 32), (15, 33)]]
HINTS = {
    4: dict(slots=[], after=(0, 6), stash=7,
             marks=[('z', 2, 0), ('z', 2, 0), ('z', 2, 0), ('z', 4, 0), ('z', 5, 0), ('z', 6, 0), ('z', 8, 0), ('z', 9, 0)]),
    6: dict(slots=[1, 5, 7, 3], after=(0, 6), stash=2,
             marks=[('h', 4, 128), ('z', 0, 120), ('z', 1, 120), ('z', 3, 64), ('z', 4, 120), ('z', 5, 120), ('z', 7, 120), ('z', 9, 120)]),
    8: dict(slots=[1, 5, 9, 3, 7, 14, 18, 22], after=(2, 6), stash=3,
             marks=[('h', 4, 128), ('z', 0, 120), ('z', 1, 120), ('z', 3, 120), ('z', 4, 48), ('z', 5, 120), ('z', 7, 120), ('z', 8, 120)]),
    10: dict(slots=[1, 5, 9], after=(1, 6), stash=7,
             marks=[('z', 0, 56), ('z', 0, 120), ('z', 1, 120), ('z', 3, 120), ('z', 4, 120), ('z', 5, 64), ('z', 7, 120), ('z', 9, 56)]),
    12: dict(slots=[1, 5, 9, 3, 7, 14, 18, 22], after=(1, 6), stash=3,
             marks=[('h', 4, 128), ('z', 0, 120), ('z', 2, 56), ('z', 3, 120), ('z', 4, 120), ('z', 5, 48), ('z', 7, 120), ('z', 8, 120)]),
    14: dict(slots=[0, 5, 9, 3, 7, 10, 18, 22, 4, 1, 8, 16, 20, 2, 6, 14, 15, 19, 23, 11, 13, 17, 21, 12], after=(0, 6), stash=1,
             marks=[]),
}


def _dft_consts():
    theta = np.pi * (4 * np.arange(C) + 1) / (2 * C)

    def fwd(t):
        ang = theta[:, None] * t[None, :]
        re = np.cos(ang).reshape(C // 8, 8, C)
        im = -np.sin(ang).reshape(C // 8, 8, C)
        return np.stack([re, im], axis=1).reshape(2 * C, C)

    fg = np.zeros((2 * C + C // 2, 2 * C), np.float64)
    order = np.concatenate([np.arange(0, C, 2), np.arange(1, C, 2)])
    fg[:2 * C, :C] = fwd(order - (C - 1) / 2)
    fg[:2 * C, C:] = fwd(np.arange(C))
    ang = (np.arange(C // 2) + 0.5)[:, None] * theta[None, :]
    fg[2 * C:, :C] = np.cos(ang) / C
    fg[2 * C:, C:] = -np.sin(ang) / C
    return fg.astype(np.float32).astype(BF)


def _kernel(q_hbm, k_hbm, v_hbm, sk_hbm, h_hbm, d_hbm, win_hbm, wsp_hbm, b_hbm, wout_hbm,
            fg_hbm, o_hbm,
            q_u, k_u, v_u, h_u, win_u, wsp_u, wout_u, fg_u,
            xn_u, z1_v, z2_u, t_u, p_v, hf_v, w_u, gg_u, xg_v, o_v, b32_v, b_v, sk_v, d_v,
            sem_q, sem_k, sem_v, sem_h, sem_w, sem_wsp, sem_o, sem_m):
    q_v = q_u.bitcast(BF)
    v_v = v_u.bitcast(BF)
    k_w = k_hbm.bitcast(U32)
    h_v = h_u.bitcast(BF)
    win_v = win_u.bitcast(BF)
    wsp_v = wsp_u.bitcast(BF)
    wout_v = wout_u.bitcast(BF)
    fg_v = fg_u.bitcast(BF)
    xn_v = xn_u.bitcast(BF)
    z2_v = z2_u.bitcast(BF)
    t_v = t_u.bitcast(BF)
    w_v = w_u.bitcast(BF)
    gg_v = gg_u.bitcast(BF)

    def ds(start, size):
        if isinstance(start, int):
            return pl.ds(start, size)
        return pl.ds(pl.multiple_of(start, size), size)

    def lanes(n):
        return slice(n * 128, (n + 1) * 128)

    def blocks(ch):
        return pl.ds(ch[0] * C, ch[1] * C)

    def brows(a):
        return ds(a * C, C)

    def cp_q(c):
        r = blocks(QCH[c])
        return pltpu.make_async_copy(q_hbm.at[r, :], q_v.at[r, :], sem_q.at[c])

    def cp_k(c):
        b0, n = KCH[c]
        return [pltpu.make_async_copy(k_w.at[pl.ds(b0 * C // 2, n * C // 2), lanes(dt)],
                                      k_u.at[dt, pl.ds(b0 * C // 2 + 8, n * C // 2), :],
                                      sem_k.at[c * ND + dt])
                for dt in range(ND)]

    def cp_v(c):
        r = blocks(KCH[c])
        return pltpu.make_async_copy(v_hbm.at[r, :], v_v.at[r, :], sem_v.at[c])

    def cp_h(c):
        r = blocks(HCH[c])
        return pltpu.make_async_copy(h_hbm.at[:, r], h_v.at[0:D, r], sem_h.at[c])

    def cp_w(c):
        r = blocks(WCH[c])
        return pltpu.make_async_copy(win_hbm.at[:, r], win_v.at[0:D, r], sem_w.at[c])

    def cp_wsp(i):
        r = ds(i * TA, TA)
        return pltpu.make_async_copy(wsp_hbm.at[r, :], wsp_v.at[r, :], sem_wsp.at[i])

    def cp_o(a, cols=slice(None)):
        r = brows(a)
        return pltpu.make_async_copy(o_v.at[r, cols], o_hbm.at[r, cols], sem_o.at[0])

    cp_f = pltpu.make_async_copy(fg_hbm, fg_v, sem_m.at[0])
    cp_sk = pltpu.make_async_copy(sk_hbm, sk_v.at[:, 0:D], sem_m.at[1])
    cp_d = pltpu.make_async_copy(d_hbm, d_v, sem_m.at[2])
    cp_b = pltpu.make_async_copy(b_hbm, b_v, sem_m.at[3])
    cp_wout = pltpu.make_async_copy(wout_hbm, wout_v.at[0:FH, 0:D], sem_m.at[4])

    groups = [
        [cp_q(0)], [cp_w(0)], [cp_q(1), cp_w(1)], [cp_q(2), cp_w(2), cp_w(3)], [cp_q(3), cp_w(4)],
        [cp_f, cp_sk, cp_d, cp_b, cp_q(4), cp_h(0), *cp_k(0), cp_v(0)],
        [cp_q(5), cp_h(1), *cp_k(1), cp_v(1)],
    ]

    def wait(g):
        for cp in groups[g]:
            cp.wait()

    def mm(x, y):
        return jnp.dot(x, y, preferred_element_type=F32)

    def words(x):
        return pltpu.bitcast(x, U32)

    def fence(tok):
        t = tok[0:8, :]
        for g in range(1, tok.shape[0] // 8):
            t = t | tok[g * 8:(g + 1) * 8, :]
        return t & k_u[0, 0:8, :]

    def held(x, gate):
        if gate is None:
            return x
        w = words(x)
        return pltpu.bitcast(w | jnp.tile(gate, (w.shape[0] // 8, w.shape[1] // 128)), x.dtype)

    def a_sums(a11, a12, a21, a22):
        s1 = a21 + a22
        s2 = s1 - a11
        return s1, s2, a11 - a21, a12 - s2

    def b_sums(b11, b12, b21, b22):
        t1 = b12 - b11
        t2 = b22 - t1
        return t1, t2, t2 - b11, b21 - t2

    def chain_sums(units, quads, dest, combine, lead, via_memory):
        last = None
        for u in units:
            vals = []
            for n, (ref, idx) in enumerate(quads(u)):
                wait_here = last is not None and (n == lead or not via_memory)
                vals.append(held(ref[idx], fence(last) if wait_here else None).astype(F32))
            sums = combine(*vals)
            done = []
            for k, val in enumerate(sums):
                ref, idx = dest(u, k)
                ref[idx] = val.astype(BF)
                if via_memory:
                    done.append(words(ref[idx]))
            last = jnp.concatenate(done, axis=0) if via_memory else words(sums[-1][-8:, :])
        return last

    c0 = math.sqrt(2.0 / math.pi)
    c1 = c0 * 0.044715

    def gelu2(x):
        return x + x * jnp.tanh(x * (c0 + c1 * (x * x)))

    def z2_words(a, half=None):
        r = brows(a) if half is None else pl.ds(a * C + half * (C // 2), C // 2)
        return words(z2_v[r, 0:128])

    def xs_row(a0, k):
        return S + (a0 // 2 % 2) * 2 * C + k // 2 * C

    def ln_q(a, gate=None, part=0, nparts=1):
        n = C // nparts
        r = pl.ds(a * C + part * n, n)
        x = held(q_v[r, :], gate).astype(F32)
        mu = jnp.sum(x, axis=-1, keepdims=True) * (1.0 / D)
        ex2 = jnp.sum(x * x, axis=-1, keepdims=True) * (1.0 / D)
        var = jnp.maximum(ex2 - mu * mu, 0.0)
        mu = mu.astype(BF).astype(F32)
        xn = (x - mu) * jnp.exp(-0.5 * jnp.log(var + EPS))
        xn_v[r, :] = xn.astype(BF)
        if a >= 4 and a % 2 == 1:
            top = xn_v[pl.ds((a - 1) * C + part * n, n), 0:2 * KS].astype(F32)
            s1, s2, s3, s4 = a_sums(top[:, :KS], top[:, KS:], xn[:, :KS], xn[:, KS:2 * KS])
            xn_v[pl.ds(xs_row(a - 1, 0) + part * n, n), 0:2 * KS] = jnp.concatenate([s1, s2], axis=1).astype(BF)
            xn_v[pl.ds(xs_row(a - 1, 2) + part * n, n), 0:2 * KS] = jnp.concatenate([s3, s4], axis=1).astype(BF)

    def h_dft(a, dt):
        res = jax.lax.dot_general(fg_v[0:2 * C, C:2 * C], h_v[lanes(dt), brows(a)],
                                  (((1,), (1,)), ((), ())), preferred_element_type=F32)
        spec = res.reshape(NB, 16, 128)
        if a == 0:
            dv = d_v[...].astype(F32)[dt:dt + 1, :]
            spec = jnp.concatenate([spec[:, 0:8, :] + dv[None], spec[:, 8:16, :]], axis=1)
        hf_v[:, a, :, lanes(dt)] = spec
        return res

    def u_dft(a, dt):
        cols = lanes(dt)

        def even(w):
            return pltpu.bitcast(w << 16, F32)

        def odd(w):
            return pltpu.bitcast(w & jnp.uint32(0xFFFF0000), F32)

        w0, w1, w2 = (k_u[dt, pl.ds(8 + a * C // 2 - j, C // 2), :] for j in range(3))
        e0, o0, e1, o1 = even(w0), odd(w0), even(w1), odd(w1)
        sk = sk_v[:, cols].astype(F32)
        s0, s1, s2, s3 = (sk[j:j + 1, :] for j in range(4))
        vw = words(v_v[brows(a), cols])
        kve = (e0 * s0 + o1 * s1 + e1 * s2 + odd(w2) * s3) * even(vw)
        kvo = (o0 * s0 + e0 * s1 + o1 * s2 + e1 * s3) * odd(vw)
        kv = jnp.concatenate([kve, kvo], axis=0).astype(BF)
        p_v[:, a, :, cols] = mm(fg_v[0:2 * C, 0:C], kv).reshape(NB, 16, 128)

    def proj(a, n, gate=None):
        lhs = xn_v[brows(a), :]
        if gate is not None:
            lhs = jnp.concatenate([held(lhs[0:16, :], gate), lhs[16:, :]], axis=0)
        return gelu2(mm(lhs, win_v[0:D, lanes(n)]))

    def w2_rows(a):
        return pl.ds(S + (a % 4) * C, C)

    def z2_tile(a, n, gate=None):
        z1_v[w2_rows(a), lanes(n)] = proj(a, NT + n, gate)

    def z1_tile(a, n, gate=None):
        t = proj(a, n, gate)
        z1_v[brows(a), lanes(n)] = t
        return t

    def t_rest(r, bot, g=0, nr=C):
        rows = pl.ds(r * C + g * nr, nr)
        t2 = bot[:, HN:] - t_v[rows, 0:HN].astype(F32)
        t3 = t2 - z2_v[rows, 0:HN].astype(F32)
        t_v[rows, HN:4 * HN] = jnp.concatenate([t2, t3, bot[:, :HN] - t2], axis=1).astype(BF)

    def ln_z2(a, last=None):
        w2 = z1_v[w2_rows(a), :]
        mu = jnp.sum(w2, axis=-1, keepdims=True) * (1.0 / FH)
        ex2 = jnp.sum(w2 * w2, axis=-1, keepdims=True) * (1.0 / FH)
        var = jnp.maximum(ex2 - mu * mu, 0.0)
        rs = jnp.exp(-0.5 * jnp.log(16.0 * var + 64.0 * EPS))
        nr = 16 if 4 <= a < NB - 2 else C
        for g in range(C // nr):
            rr = slice(g * nr, (g + 1) * nr)
            m = held(jnp.broadcast_to(mu[rr], (nr, 128)), fence(last) if last is not None and nr < C else None)
            zn = (w2[rr] - jnp.tile(m, (1, NT))) * rs[rr]
            rows = pl.ds(a * C + g * nr, nr)
            if a < NB // 2:
                z2_v[rows, 0:HN] = zn[:, :HN].astype(BF)
                t_v[rows, 0:HN] = (zn[:, HN:] - zn[:, :HN]).astype(BF)
                done = [(z2_v, rows, k) for k in range(3)] + [(t_v, rows, k) for k in range(3)]
            else:
                z2_v[rows, :] = zn.astype(BF)
                done = [(z2_v, rows, k) for k in range(6)]
                if a < NB - 1:
                    t_rest(a - NB // 2, zn, g, nr)
                    done += [(t_v, pl.ds((a - NB // 2) * C + g * nr, nr), k) for k in range(3, 12)]
            if nr < C:
                last = jnp.concatenate([words(ref[r, lanes(k)]) for ref, r, k in done], axis=0)
        return last

    def tw_at(base, j, k):
        return D + (base // NT) * KS, lanes(j * 4 + k)

    def tw_sums(base):
        def quads(u):
            j, g = u
            return [(win_v, (slice(r0 + g * 16, r0 + (g + 1) * 16), lanes(n)))
                    for r0 in (0, KS) for n in (base + j, base + 3 + j)]

        def dest(u, k):
            j, g = u
            r0, cols = tw_at(base, j, k)
            return win_v, (slice(r0 + g * 16, r0 + (g + 1) * 16), cols)

        return chain_sums([(j, g) for j in range(3) for g in range(KS // 16)], quads, dest, b_sums, 0, True)

    def group(a0, base, j, hook, gate=None):
        r0, r1 = brows(a0), brows(a0 + 1)
        cl, cr = lanes(base + j), lanes(base + 3 + j)

        def out(a, n, val):
            t = gelu2(val)
            z1_v[w2_rows(a) if base else brows(a), lanes(n)] = t
            hook(t)

        def sx(k):
            return xn_v[xs_row(a0, k):xs_row(a0, k) + C, (k % 2) * KS:(k % 2 + 1) * KS]

        def tw(k):
            t0, cols = tw_at(base, j, k)
            return win_v[t0:t0 + KS, cols]

        def keep(slot, val):
            if not (HINTS[a0]['stash'] >> slot) & 1:
                return lambda: val
            sl = (pl.ds(S + 4 * C + (j % 2) * C, C), lanes(slot))
            z1_v[sl] = val
            return lambda: z1_v[sl]

        a11 = xn_v[r0, 0:KS]
        if gate is not None:
            top = jnp.concatenate([held(a11[0:16, 0:128], gate), a11[0:16, 128:]], axis=1)
            a11 = jnp.concatenate([top, a11[16:, :]], axis=0)
        p1 = keep(0, mm(a11, win_v[0:KS, cl]))
        out(a0, j, p1() + mm(xn_v[r0, KS:D], win_v[KS:D, cl]))
        u2 = keep(1, p1() + mm(sx(1), tw(1)))
        u3 = keep(2, u2() + mm(sx(2), tw(2)))
        out(a0 + 1, j, u3() + mm(xn_v[r1, KS:D], jnp.concatenate([tw(3), win_v[2 * KS:D, cl]], axis=0)))
        p5 = mm(sx(0), tw(0))
        out(a0 + 1, 3 + j, (u3() + p5) + mm(xn_v[r1, 2 * KS:D], win_v[2 * KS:D, cr]))
        out(a0, 3 + j, (u2() + p5) + mm(jnp.concatenate([sx(3), xn_v[r0, 2 * KS:D]], axis=1), win_v[KS:D, cr]))

    def region(pairs, hch=(0, 0), kch=(0, 0), plan=((0, 0),)):
        hs = [(a, dt) for a in range(hch[0], hch[0] + hch[1]) for dt in range(ND)]
        us = [(a, dt) for a in range(kch[0], kch[0] + kch[1]) for dt in range(ND)]
        for bi, a0 in enumerate(pairs):
            nh, nu = plan[bi]
            nh_end = min(nh, 4) if bi == len(pairs) - 1 else 0
            nh_mid = min(8, nh - nh_end)
            nh_run = nh - nh_end - nh_mid
            nu_run = min(nu, 3 * nh_run)
            cnt = [0] * 25
            for j in range(nu - nu_run):
                cnt[HINTS[a0]['slots'][j]] += 1
            marks = HINTS[a0]['marks']
            seen = [0]

            def next_ln_q(part, t):
                tok = words(t)
                for a in (a0, a0 + 1):
                    if part == HINTS[a0]['after'][a - a0]:
                        tok = jnp.concatenate([tok, z2_words(a)], axis=0)
                        if a >= NB // 2:
                            tw_ = words(t_v[brows(a - NB // 2), 4 * HN - 128:4 * HN])
                            tok = jnp.concatenate([tok, tw_], axis=0)
                ln_q(a0 + 2 + part // NLQ, fence(tok), part % NLQ, NLQ)

            def after_z2(t):
                for _ in range(cnt[seen[0]]):
                    u_dft(*us.pop(0))
                seen[0] += 1

            def after_z1(t):
                for part, (kind, idx, row) in enumerate(marks):
                    if kind == 'z' and idx == seen[0]:
                        next_ln_q(part, t[row:row + 8, :])
                for _ in range(cnt[13 + seen[0]]):
                    u_dft(*us.pop(0))
                seen[0] += 1

            for j in range(3):
                group(a0, NT, j, after_z2)
            hres = [h_dft(*hs.pop(0)) for _ in range(nh_mid)]
            for _ in range(cnt[12]):
                u_dft(*us.pop(0))
            ln_z2(a0 + 1, ln_z2(a0))
            for part, (kind, idx, row) in enumerate(marks):
                if kind == 'h':
                    next_ln_q(part, hres[idx][row:row + 8, :])
            seen[0] = 0
            for j in range(3):
                group(a0, 0, j, after_z1, fence(z2_words(a0 + j - 1)) if not marks and j >= 1 else None)
            ru, rh = nu_run, nh_run
            while ru or rh:
                if ru and ru * max(nh_run, 1) >= rh * max(nu_run, 1):
                    u_dft(*us.pop(0))
                    ru -= 1
                else:
                    h_dft(*hs.pop(0))
                    rh -= 1
            for _ in range(nh_end):
                h_dft(*hs.pop(0))
        assert not us
        return hs

    def conv_pos(ft, ft2, par, dt, after):
        cols = lanes(dt)
        prev = None
        for a in range(NB):
            ar, ai = (None, None) if prev is None else (-prev[1], prev[0])
            for dl in range(a + 1):
                hr = hf_v[ft, dl, 0:8, cols]
                hi = hf_v[ft, dl, 8:16, cols]
                ur = p_v[ft, a - dl, 0:8, cols]
                ui = p_v[ft, a - dl, 8:16, cols]
                if ar is None:
                    ar, ai = ur * hr - ui * hi, ur * hi + ui * hr
                    if after is not None:
                        z = fence(after)
                        ar, ai = held(ar, z), held(ai, z)
                elif (a * (a + 1) // 2 + dl) % TREE == 0:
                    ar = ar + (ur * hr - ui * hi)
                    ai = ai + (ur * hi + ui * hr)
                else:
                    ar = (ar + ur * hr) - ui * hi
                    ai = (ai + ur * hi) + ui * hr
            prev = (ar, ai) if prev is None else (ar + prev[1], ai - prev[0])
            w_v[a * 16 + ft2, par * 8:(par + 1) * 8, cols] = ar.astype(BF)
            w_v[a * 16 + 8 + ft2, par * 8:(par + 1) * 8, cols] = ai.astype(BF)
        return words(prev[0])

    gl_v = wout_v
    GL0 = FH
    GS0 = GL0 + NOP * C
    WS0 = GS0 + 4 * C
    GX0 = WS0 + 2 * HN

    def g_sums(ref, g0, s0):
        def quads(u):
            c, g = u
            return [(ref, (pl.ds(g0 + m * C + g * 16, 16), lanes(n))) for m in (0, 1) for n in (c, 3 + c)]

        def dest(u, k):
            c, g = u
            return gl_v, (pl.ds(s0 + k // 2 * C + g * 16, 16), lanes(k % 2 * 3 + c))

        chain_sums([(c, g) for c in range(3) for g in range(C // 16)], quads, dest, a_sums, 2, True)

    def ws_at(jj, k):
        return WS0 + (jj * 4 + k) // 6 * HN, lanes((jj * 4 + k) % 6)

    def w_sums():
        def quads(u):
            jj, g = u
            return [(wout_v, (pl.ds(r0 + g * 16, 16), lanes(n))) for r0 in (0, HN) for n in (jj, 2 + jj)]

        def dest(u, k):
            jj, g = u
            r0, cols = ws_at(jj, k)
            return wout_v, (pl.ds(r0 + g * 16, 16), cols)

        chain_sums([(jj, g) for jj in range(2) for g in range(HN // 16)], quads, dest, b_sums, 0, False)

    def xn_gate(a, dt, hh):
        return xn_v[brows(a), lanes(dt)].astype(F32) * (hh + hh * jnp.tanh(hh))

    def o_pair(a0, ref, g0, s0, finish, skip=False):
        r0, r1 = pl.ds(g0, C), pl.ds(g0 + C, C)

        def gs(k):
            return gl_v[pl.ds(s0 + k // 2 * C, C), (k % 2) * HN:(k % 2 + 1) * HN]

        def ws(jj, k):
            r, cols = ws_at(jj, k)
            return wout_v[r:r + HN, cols]

        for jj in range(2):
            if jj == (0 if skip else 1):
                finish(a0, 4, None if skip else mm(ref[r0, :], wout_v[0:FH, lanes(4)]))
                finish(a0 + 1, 4, mm(ref[r1, :], wout_v[0:FH, lanes(4)]))
            p1 = mm(ref[r0, 0:HN], wout_v[0:HN, lanes(jj)])
            finish(a0, jj, p1 + mm(ref[r0, HN:FH], wout_v[HN:FH, lanes(jj)]))
            u2 = p1 + mm(gs(1), ws(jj, 1))
            u3 = u2 + mm(gs(2), ws(jj, 2))
            finish(a0 + 1, jj, u3 + mm(ref[r1, HN:FH], ws(jj, 3)))
            p5 = mm(gs(0), ws(jj, 0))
            finish(a0 + 1, 2 + jj, u3 + p5)
            finish(a0, 2 + jj, (u2 + p5) + mm(gs(3), wout_v[HN:FH, lanes(2 + jj)]))

    def s_at(slot, k):
        return D + (slot * 2 + k // 2) * C, (k % 2) * HK

    def s_val(slot, k):
        r0, col = s_at(slot, k)
        return h_v[r0:r0 + C, col:col + HK]

    def s_sums(a0, nr, via_memory):
        def quads(u):
            slot, c, g = u
            return [(wsp_v, (ds((a0 + 2 * slot + m) * C + g * nr, nr), lanes(n)))
                    for m in (0, 1) for n in (c, HK // 128 + c)]

        def dest(u, k):
            slot, c, g = u
            r0, col = s_at(slot, k)
            return h_v, (slice(r0 + g * nr, r0 + (g + 1) * nr), slice(col + c * 128, col + (c + 1) * 128))

        units = [(slot, c, g) for slot in range(2) for c in range(HK // 128) for g in range(C // nr)]
        for part in (units[:48], units[48:]) if via_memory else (units,):
            chain_sums(part, quads, dest, a_sums, 2, via_memory)

    def phase2a(i, carry):
        @pl.when(i + 1 < S // TA)
        def _():
            cp_wsp(i + 1).wait()

        eye = (jax.lax.broadcasted_iota(jnp.int32, (C, C), 0)
               == jax.lax.broadcasted_iota(jnp.int32, (C, C), 1))

        def bcol(a):
            return jnp.sum(jnp.where(eye, b32_v[pl.ds(a, 1), :], 0.0), axis=-1, keepdims=True)

        def put(m, n, g):
            g = (z1_v[brows(i * (TA // C) + m), lanes(n)] * g).astype(BF)
            if m < NOP:
                gl_v[GL0 + m * C:GL0 + (m + 1) * C, lanes(n)] = g
            else:
                gg_v[ds((2 * i + m - NOP) * C, C), lanes(n)] = g
                if m == NOP:
                    gl_v[GX0:GX0 + C, lanes(n)] = g

        for pp in range(2):
            if pp == 1:
                g_sums(gl_v, GL0, GS0)
            m0 = 2 * pp
            a0 = i * (TA // C) + m0
            r0, r1 = brows(a0), brows(a0 + 1)
            b0 = bcol(a0)
            db = bcol(a0 + 1) - b0
            for j in range(NT // 2):
                jl, jr = lanes(j), lanes(NT // 2 + j)
                t1, t2, t3, t4 = (t_v[:, lanes(k * (NT // 2) + j)] for k in range(4))
                p1 = mm(wsp_v[r0, 0:HK], z2_v[0:HK, jl]) + b0
                put(m0, j, p1 + mm(wsp_v[r0, HK:S], z2_v[HK:S, jl]))
                u2 = p1 + mm(s_val(pp, 1), t2)
                u3 = (u2 + db) + mm(s_val(pp, 2), t3)
                put(m0 + 1, j, u3 + mm(wsp_v[r1, HK:S], t4))
                p5 = mm(s_val(pp, 0), t1)
                put(m0 + 1, NT // 2 + j, u3 + p5)
                put(m0, NT // 2 + j, (u2 + p5) + mm(s_val(pp, 3), z2_v[HK:S, jr]))
        def finish(a, dt, hh):
            xg_v[brows(a), lanes(dt)] = xn_gate(a, dt, hh)

        o_pair(i * (TA // C), gl_v, GL0, GS0, finish)
        finish(i * (TA // C) + 2, 4, mm(gl_v[GX0:GX0 + C, :], wout_v[0:FH, lanes(4)]))
        s_sums(jnp.minimum(i + 1, S // TA - 1) * (TA // C), 16, True)
        nft = NB * TA // S
        last = None
        for ft in range(nft):
            for dt in range(ND):
                last = conv_pos(i * nft + ft, i * (nft // 2) + ft // 2, ft % 2, dt, last)
        return carry

    step = pl.program_id(0)

    @pl.when(step == 0)
    def _():
        for grp in groups:
            for cp in grp:
                cp.start()
        cp_wout.start()
        for i in range(S // TA):
            cp_wsp(i).start()
        k_u[:, 0:8, :] = jnp.zeros((ND, 8, 128), U32)

    @pl.when(step == 1)
    def _():
        cp_wsp(0).wait()
        cp_wout.wait()
        t_rest(NB // 2 - 1, z2_v[brows(NB - 1), :].astype(F32))
        for a, dt in [(a, dt) for a in range(NB) for dt in range(ND)][NB * ND - H_LATE:]:
            h_dft(a, dt)
        w_sums()
        s_sums(0, 32, False)
        jax.lax.fori_loop(0, S // TA, phase2a, 0)

        rev = 7 - jax.lax.broadcasted_iota(jnp.int32, (8, 128), 0)
        done = {}

        def emit(a, dt, hh):
            rows, cols = brows(a), lanes(dt)
            ev = mm(fg_v[2 * C:2 * C + C // 2, 0:C], w_v[ds(a * 16, 8), :, cols].reshape(C, 128))
            od = mm(fg_v[2 * C:2 * C + C // 2, C:2 * C], w_v[ds(a * 16 + 8, 8), :, cols].reshape(C, 128))
            lo = ev - od
            ys = [jnp.take_along_axis(lo[g * 8:(g + 1) * 8, :], rev, axis=0)
                  for g in range(C // 16 - 1, -1, -1)]
            y = jnp.concatenate(ys + [ev + od], axis=0)
            xg = xg_v[rows, cols] if hh is None else xn_gate(a, dt, hh)
            o_v[rows, cols] = (q_v[rows, cols].astype(F32) + xg * y).astype(BF)
            done[a] = done.get(a, 0) + 1
            if a >= NB - 2:
                cp_o(a, cols).start()
            elif done[a] == ND:
                cp_o(a).start()

        g_sums(gg_v, 0, GS0)
        for k in range(S // TA):
            if k + 1 < S // TA:
                g_sums(gg_v, (k + 1) * 2 * C, GS0 + ((k + 1) % 2) * 2 * C)
            for a in (4 * k, 4 * k + 1):
                for dt in range(ND):
                    emit(a, dt, None)
            o_pair(4 * k + 2, gg_v, k * 2 * C, GS0 + (k % 2) * 2 * C, emit, skip=True)
        pltpu.make_async_copy(o_v, o_hbm, sem_o.at[0]).wait()

    @pl.when(step == 0)
    def _():
        wait(0)
        ln_q(0)
        ln_q(1)
        wait(1)
        for n in (0, 1):
            z2_tile(0, n)
            z2_tile(1, n)
        wait(2)
        ln_q(2)
        for n in (2, 3):
            z2_tile(0, n)
            z2_tile(1, n)
        for n in range(4):
            z2_tile(2, n)
        wait(3)
        ln_q(3)
        seq = ([(z2_tile, a, n) for a in range(3) for n in (4, 5)] + [(z2_tile, 3, n) for n in range(NT)]
               + [(z1_tile, a, 0) for a in range(4)])
        tw_done = tw_sums(NT)
        for j, (tile, a, n) in enumerate(seq):
            if j == 15:
                gate = fence(tw_done)
            elif j == 3:
                gate = fence(words(xn_v[brows(3), 0:128]))
            else:
                gate = fence(z2_words(0, (7, 10).index(j))) if j in (7, 10) else None
            tile(a, n, gate)
            if j == 1:
                ln_z2(0)
        wait(4)
        for a in (1, 2, 3):
            ln_z2(a)
        tw_sums(0)
        release = (9, 10, 11, 12, 13, 15, 16, 17)
        waits = (3, 4, 6, 8, 10, 11)
        for j, (a, n) in enumerate((a, n) for n in range(1, NT) for a in range(4)):
            gate = fence(z2_words(1 + waits.index(j) // 2, waits.index(j) % 2)) if j in waits else None
            t = z1_tile(a, n, gate)
            if j in release:
                part = release.index(j)
                ln_q(4 + part // NLQ, fence(words(t[0:8, :])), part % NLQ, NLQ)
        region([4])
        wait(5)
        b32_v[...] = b_v[...].astype(F32) * 0.25
        assert not region([6, 8, 10], HCH[0], KCH[0], DFT_PLAN[0])
        wait(6)
        assert len(region([12, 14], HCH[1], KCH[1], DFT_PLAN[1])) == H_LATE


@jax.jit
def pallas_recurrent_scan__ssm_conv_h3__mixer_gmlp__prompt_kernel(
    A_q: jax.Array,
    A_k: jax.Array,
    A_v: jax.Array,
    A_shift_k: jax.Array,
    A_ssm_k: jax.Array,
    A_ssm_D: jax.Array,
    B_x: jax.Array,
    B_w_in: jax.Array,
    B_w_sp: jax.Array,
    B_b_sp: jax.Array,
    B_w_out: jax.Array,
):
    del B_x
    any_spec = pl.BlockSpec(memory_space=pl.ANY)
    vm = pltpu.VMEM
    dma = pltpu.SemaphoreType.DMA
    out = pl.pallas_call(
        _kernel,
        out_shape=jax.ShapeDtypeStruct((S, D), BF),
        grid=(2,),
        in_specs=[any_spec] * 11,
        out_specs=any_spec,
        scratch_shapes=[
            vm((S // 2, D), U32),
            vm((ND, S // 2 + 32, 128), U32),
            vm((S // 2, D), U32),
            vm(((D + 4 * C) // 2, S), U32),
            vm(((D + 2 * KS) // 2, 2 * FH), U32),
            vm((S // 2, S), U32),
            vm(((FH + 8 * C + 2 * HN) // 2, FH), U32),
            vm(((2 * C + C // 2) // 2, 2 * C), U32),
            vm(((S + 4 * C) // 2, D), U32),
            vm((S + 6 * C, FH), F32),
            vm((S // 2, FH), U32),
            vm((S // 4, 2 * FH), U32),
            vm((NB, NB, 16, D), F32),
            vm((NB, NB, 16, D), F32),
            vm((NB * 16, 8, 1024), U32),
            vm((S // 4, FH), U32),
            vm((S, D), F32),
            vm((S, D), BF),
            vm((NB, 128), F32),
            vm((NB, 128), BF),
            vm((4, 18 * 128), BF),
            vm((ND, 128), BF),
            dma((len(QCH),)), dma((len(KCH) * ND,)), dma((len(KCH),)), dma((len(HCH),)),
            dma((len(WCH),)), dma((S // TA,)), dma((1,)), dma((5,)),
        ],
        compiler_params=pltpu.CompilerParams(
            dimension_semantics=("arbitrary",),
            vmem_limit_bytes=110 * 1024 * 1024,
            disable_bounds_checks=True,
            disable_semaphore_checks=True,
        ),
    )(
        A_q.reshape(S, D), A_k.reshape(S, D), A_v.reshape(S, D),
        A_shift_k.T, A_ssm_k, A_ssm_D.reshape(ND, 128),
        B_w_in, B_w_sp, B_b_sp.reshape(NB, 128), B_w_out,
        _dft_consts(),
    )
    return out.reshape(1, S, D)
```

```python
import math

import jax
import jax.numpy as jnp
import numpy as np
import jax.experimental.pallas as pl
import jax.experimental.pallas.tpu as pltpu

S = 2048
D = 640
FH = 768
C = 128
NB = S // C
ND = D // 128
NT = FH // 128
EPS = 1e-5
HK = S // 2
HN = FH // 2
KS = 256
TA = 512
NOP = 2
NLQ = 4
H_LATE = 24
TREE = 10

BF = jnp.bfloat16
F32 = jnp.float32
U32 = jnp.uint32

QCH = [(0, 2), (2, 1), (3, 1), (4, 4), (8, 6), (14, 2)]
HCH = [(0, 5), (5, 11)]
KCH = [(0, 3), (3, 13)]
WCH = [(6, 2), (8, 2), (10, 2), (0, 1), (1, 5)]
DFT_PLAN = [[(8, 4), (8, 8), (9, 3)], [(16, 32), (15, 33)]]
HINTS = {
    4: dict(slots=[], after=(0, 6), stash=7,
             marks=[('z', 2, 0), ('z', 2, 0), ('z', 2, 0), ('z', 4, 0), ('z', 5, 0), ('z', 6, 0), ('z', 8, 0), ('z', 9, 0)]),
    6: dict(slots=[1, 5, 7, 3], after=(0, 6), stash=2,
             marks=[('h', 4, 128), ('z', 0, 120), ('z', 1, 120), ('z', 3, 64), ('z', 4, 120), ('z', 5, 120), ('z', 7, 120), ('z', 9, 120)]),
    8: dict(slots=[1, 5, 9, 3, 7, 14, 18, 22], after=(2, 6), stash=3,
             marks=[('h', 4, 128), ('z', 0, 120), ('z', 1, 120), ('z', 3, 120), ('z', 4, 48), ('z', 5, 120), ('z', 7, 120), ('z', 8, 120)]),
    10: dict(slots=[1, 5, 9], after=(1, 6), stash=7,
             marks=[('z', 0, 56), ('z', 0, 120), ('z', 1, 120), ('z', 3, 120), ('z', 4, 120), ('z', 5, 64), ('z', 7, 120), ('z', 9, 56)]),
    12: dict(slots=[1, 5, 9, 3, 7, 14, 18, 22], after=(1, 6), stash=3,
             marks=[('h', 4, 128), ('z', 0, 120), ('z', 2, 56), ('z', 3, 120), ('z', 4, 120), ('z', 5, 48), ('z', 7, 120), ('z', 8, 120)]),
    14: dict(slots=[0, 5, 9, 3, 7, 10, 18, 22, 4, 1, 8, 16, 20, 2, 6, 14, 15, 19, 23, 11, 13, 17, 21, 12], after=(0, 6), stash=1,
             marks=[]),
}


def _dft_consts():
    theta = np.pi * (4 * np.arange(C) + 1) / (2 * C)

    def fwd(t):
        ang = theta[:, None] * t[None, :]
        re = np.cos(ang).reshape(C // 8, 8, C)
        im = -np.sin(ang).reshape(C // 8, 8, C)
        return np.stack([re, im], axis=1).reshape(2 * C, C)

    fg = np.zeros((2 * C + C // 2, 2 * C), np.float64)
    order = np.concatenate([np.arange(0, C, 2), np.arange(1, C, 2)])
    fg[:2 * C, :C] = fwd(order - (C - 1) / 2)
    fg[:2 * C, C:] = fwd(np.arange(C))
    ang = (np.arange(C // 2) + 0.5)[:, None] * theta[None, :]
    fg[2 * C:, :C] = np.cos(ang) / C
    fg[2 * C:, C:] = -np.sin(ang) / C
    return fg.astype(np.float32).astype(BF)


def _kernel(q_hbm, k_hbm, v_hbm, sk_hbm, h_hbm, d_hbm, win_hbm, wsp_hbm, b_hbm, wout_hbm,
            fg_hbm, o_hbm,
            q_u, k_u, v_u, h_u, win_u, wsp_u, wout_u, fg_u,
            xn_u, z1_v, z2_u, t_u, p_v, hf_v, w_u, gg_u, xg_v, o_v, b32_v, b_v, sk_v, d_v,
            sem_q, sem_k, sem_v, sem_h, sem_w, sem_wsp, sem_o, sem_m):
    q_v = q_u.bitcast(BF)
    v_v = v_u.bitcast(BF)
    k_w = k_hbm.bitcast(U32)
    h_v = h_u.bitcast(BF)
    win_v = win_u.bitcast(BF)
    wsp_v = wsp_u.bitcast(BF)
    wout_v = wout_u.bitcast(BF)
    fg_v = fg_u.bitcast(BF)
    xn_v = xn_u.bitcast(BF)
    z2_v = z2_u.bitcast(BF)
    t_v = t_u.bitcast(BF)
    w_v = w_u.bitcast(BF)
    gg_v = gg_u.bitcast(BF)

    def ds(start, size):
        if isinstance(start, int):
            return pl.ds(start, size)
        return pl.ds(pl.multiple_of(start, size), size)

    def lanes(n):
        return slice(n * 128, (n + 1) * 128)

    def blocks(ch):
        return pl.ds(ch[0] * C, ch[1] * C)

    def brows(a):
        return ds(a * C, C)

    def cp_q(c):
        r = blocks(QCH[c])
        return pltpu.make_async_copy(q_hbm.at[r, :], q_v.at[r, :], sem_q.at[c])

    def cp_k(c):
        b0, n = KCH[c]
        return [pltpu.make_async_copy(k_w.at[pl.ds(b0 * C // 2, n * C // 2), lanes(dt)],
                                      k_u.at[dt, pl.ds(b0 * C // 2 + 8, n * C // 2), :],
                                      sem_k.at[c * ND + dt])
                for dt in range(ND)]

    def cp_v(c):
        r = blocks(KCH[c])
        return pltpu.make_async_copy(v_hbm.at[r, :], v_v.at[r, :], sem_v.at[c])

    def cp_h(c):
        r = blocks(HCH[c])
        return pltpu.make_async_copy(h_hbm.at[:, r], h_v.at[0:D, r], sem_h.at[c])

    def cp_w(c):
        r = blocks(WCH[c])
        return pltpu.make_async_copy(win_hbm.at[:, r], win_v.at[0:D, r], sem_w.at[c])

    def cp_wsp(i):
        r = ds(i * TA, TA)
        return pltpu.make_async_copy(wsp_hbm.at[r, :], wsp_v.at[r, :], sem_wsp.at[i])

    def cp_o(a, cols=slice(None)):
        r = brows(a)
        return pltpu.make_async_copy(o_v.at[r, cols], o_hbm.at[r, cols], sem_o.at[0])

    cp_f = pltpu.make_async_copy(fg_hbm, fg_v, sem_m.at[0])
    cp_sk = pltpu.make_async_copy(sk_hbm, sk_v.at[:, 0:D], sem_m.at[1])
    cp_d = pltpu.make_async_copy(d_hbm, d_v, sem_m.at[2])
    cp_b = pltpu.make_async_copy(b_hbm, b_v, sem_m.at[3])
    cp_wout = pltpu.make_async_copy(wout_hbm, wout_v.at[0:FH, 0:D], sem_m.at[4])

    groups = [
        [cp_q(0)], [cp_w(0)], [cp_q(1), cp_w(1)], [cp_q(2), cp_w(2), cp_w(3)], [cp_q(3), cp_w(4)],
        [cp_f, cp_sk, cp_d, cp_b, cp_q(4), cp_h(0), *cp_k(0), cp_v(0)],
        [cp_q(5), cp_h(1), *cp_k(1), cp_v(1)],
    ]

    def wait(g):
        for cp in groups[g]:
            cp.wait()

    def mm(x, y):
        return jnp.dot(x, y, preferred_element_type=F32)

    def words(x):
        return pltpu.bitcast(x, U32)

    def fence(tok):
        t = tok[0:8, :]
        for g in range(1, tok.shape[0] // 8):
            t = t | tok[g * 8:(g + 1) * 8, :]
        return t & k_u[0, 0:8, :]

    def held(x, gate):
        if gate is None:
            return x
        w = words(x)
        return pltpu.bitcast(w | jnp.tile(gate, (w.shape[0] // 8, w.shape[1] // 128)), x.dtype)

    def a_sums(a11, a12, a21, a22):
        s1 = a21 + a22
        s2 = s1 - a11
        return s1, s2, a11 - a21, a12 - s2

    def b_sums(b11, b12, b21, b22):
        t1 = b12 - b11
        t2 = b22 - t1
        return t1, t2, t2 - b11, b21 - t2

    def chain_sums(units, quads, dest, combine, lead, via_memory, last=None):
        for u in units:
            vals = []
            for n, (ref, idx) in enumerate(quads(u)):
                wait_here = last is not None and (n == lead or not via_memory)
                vals.append(held(ref[idx], fence(last) if wait_here else None).astype(F32))
            sums = combine(*vals)
            done = []
            for k, val in enumerate(sums):
                ref, idx = dest(u, k)
                ref[idx] = val.astype(BF)
                if via_memory:
                    done.append(words(ref[idx]))
            last = jnp.concatenate(done, axis=0) if via_memory else words(sums[-1][-8:, :])
        return last

    c0 = math.sqrt(2.0 / math.pi)
    c1 = c0 * 0.044715

    def gelu2(x):
        return x + x * jnp.tanh(x * (c0 + c1 * (x * x)))

    def z2_words(a, half=None):
        r = brows(a) if half is None else pl.ds(a * C + half * (C // 2), C // 2)
        return words(z2_v[r, 0:128])

    def xs_row(a0, k):
        return S + (a0 // 2 % 2) * 2 * C + k // 2 * C

    def ln_q(a, gate=None, part=0, nparts=1):
        n = C // nparts
        r = pl.ds(a * C + part * n, n)
        x = held(q_v[r, :], gate).astype(F32)
        mu = jnp.sum(x, axis=-1, keepdims=True) * (1.0 / D)
        ex2 = jnp.sum(x * x, axis=-1, keepdims=True) * (1.0 / D)
        var = jnp.maximum(ex2 - mu * mu, 0.0)
        mu = mu.astype(BF).astype(F32)
        xn = (x - mu) * jnp.exp(-0.5 * jnp.log(var + EPS))
        xn_v[r, :] = xn.astype(BF)
        if a >= 4 and a % 2 == 1:
            top = xn_v[pl.ds((a - 1) * C + part * n, n), 0:2 * KS].astype(F32)
            s1, s2, s3, s4 = a_sums(top[:, :KS], top[:, KS:], xn[:, :KS], xn[:, KS:2 * KS])
            xn_v[pl.ds(xs_row(a - 1, 0) + part * n, n), 0:2 * KS] = jnp.concatenate([s1, s2], axis=1).astype(BF)
            xn_v[pl.ds(xs_row(a - 1, 2) + part * n, n), 0:2 * KS] = jnp.concatenate([s3, s4], axis=1).astype(BF)

    def h_dft(a, dt):
        res = jax.lax.dot_general(fg_v[0:2 * C, C:2 * C], h_v[lanes(dt), brows(a)],
                                  (((1,), (1,)), ((), ())), preferred_element_type=F32)
        spec = res.reshape(NB, 16, 128)
        if a == 0:
            dv = d_v[...].astype(F32)[dt:dt + 1, :]
            spec = jnp.concatenate([spec[:, 0:8, :] + dv[None], spec[:, 8:16, :]], axis=1)
        hf_v[:, a, :, lanes(dt)] = spec
        return res

    def u_dft(a, dt):
        cols = lanes(dt)

        def even(w):
            return pltpu.bitcast(w << 16, F32)

        def odd(w):
            return pltpu.bitcast(w & jnp.uint32(0xFFFF0000), F32)

        w0, w1, w2 = (k_u[dt, pl.ds(8 + a * C // 2 - j, C // 2), :] for j in range(3))
        e0, o0, e1, o1 = even(w0), odd(w0), even(w1), odd(w1)
        sk = sk_v[:, cols].astype(F32)
        s0, s1, s2, s3 = (sk[j:j + 1, :] for j in range(4))
        vw = words(v_v[brows(a), cols])
        kve = (e0 * s0 + o1 * s1 + e1 * s2 + odd(w2) * s3) * even(vw)
        kvo = (o0 * s0 + e0 * s1 + o1 * s2 + e1 * s3) * odd(vw)
        kv = jnp.concatenate([kve, kvo], axis=0).astype(BF)
        p_v[:, a, :, cols] = mm(fg_v[0:2 * C, 0:C], kv).reshape(NB, 16, 128)

    def proj(a, n, gate=None):
        lhs = xn_v[brows(a), :]
        if gate is not None:
            lhs = jnp.concatenate([held(lhs[0:16, :], gate), lhs[16:, :]], axis=0)
        return gelu2(mm(lhs, win_v[0:D, lanes(n)]))

    def w2_rows(a):
        return pl.ds(S + (a % 4) * C, C)

    def z2_tile(a, n, gate=None):
        z1_v[w2_rows(a), lanes(n)] = proj(a, NT + n, gate)

    def z1_tile(a, n, gate=None):
        t = proj(a, n, gate)
        z1_v[brows(a), lanes(n)] = t
        return t

    def t_rest(r, bot, g=0, nr=C):
        rows = pl.ds(r * C + g * nr, nr)
        t2 = bot[:, HN:] - t_v[rows, 0:HN].astype(F32)
        t3 = t2 - z2_v[rows, 0:HN].astype(F32)
        t_v[rows, HN:4 * HN] = jnp.concatenate([t2, t3, bot[:, :HN] - t2], axis=1).astype(BF)

    def ln_z2(a, last=None):
        w2 = z1_v[w2_rows(a), :]
        mu = jnp.sum(w2, axis=-1, keepdims=True) * (1.0 / FH)
        ex2 = jnp.sum(w2 * w2, axis=-1, keepdims=True) * (1.0 / FH)
        var = jnp.maximum(ex2 - mu * mu, 0.0)
        rs = jnp.exp(-0.5 * jnp.log(16.0 * var + 64.0 * EPS))
        nr = 16 if 4 <= a < NB - 2 else C
        for g in range(C // nr):
            rr = slice(g * nr, (g + 1) * nr)
            m = held(jnp.broadcast_to(mu[rr], (nr, 128)), fence(last) if last is not None and nr < C else None)
            zn = (w2[rr] - jnp.tile(m, (1, NT))) * rs[rr]
            rows = pl.ds(a * C + g * nr, nr)
            if a < NB // 2:
                z2_v[rows, 0:HN] = zn[:, :HN].astype(BF)
                t_v[rows, 0:HN] = (zn[:, HN:] - zn[:, :HN]).astype(BF)
                done = [(z2_v, rows, k) for k in range(3)] + [(t_v, rows, k) for k in range(3)]
            else:
                z2_v[rows, :] = zn.astype(BF)
                done = [(z2_v, rows, k) for k in range(6)]
                if a < NB - 1:
                    t_rest(a - NB // 2, zn, g, nr)
                    done += [(t_v, pl.ds((a - NB // 2) * C + g * nr, nr), k) for k in range(3, 12)]
            if nr < C:
                last = jnp.concatenate([words(ref[r, lanes(k)]) for ref, r, k in done], axis=0)
        return last

    def tw_at(base, j, k):
        return D + (base // NT) * KS, lanes(j * 4 + k)

    def tw_sums(base):
        def quads(u):
            j, g = u
            return [(win_v, (slice(r0 + g * 16, r0 + (g + 1) * 16), lanes(n)))
                    for r0 in (0, KS) for n in (base + j, base + 3 + j)]

        def dest(u, k):
            j, g = u
            r0, cols = tw_at(base, j, k)
            return win_v, (slice(r0 + g * 16, r0 + (g + 1) * 16), cols)

        return chain_sums([(j, g) for j in range(3) for g in range(KS // 16)], quads, dest, b_sums, 0, True)

    def group(a0, base, j, hook, gate=None):
        r0, r1 = brows(a0), brows(a0 + 1)
        cl, cr = lanes(base + j), lanes(base + 3 + j)

        def out(a, n, val):
            t = gelu2(val)
            z1_v[w2_rows(a) if base else brows(a), lanes(n)] = t
            hook(t)

        def sx(k):
            return xn_v[xs_row(a0, k):xs_row(a0, k) + C, (k % 2) * KS:(k % 2 + 1) * KS]

        def tw(k):
            t0, cols = tw_at(base, j, k)
            return win_v[t0:t0 + KS, cols]

        def keep(slot, val):
            if not (HINTS[a0]['stash'] >> slot) & 1:
                return lambda: val
            sl = (pl.ds(S + 4 * C + (j % 2) * C, C), lanes(slot))
            z1_v[sl] = val
            return lambda: z1_v[sl]

        a11 = xn_v[r0, 0:KS]
        if gate is not None:
            top = jnp.concatenate([held(a11[0:16, 0:128], gate), a11[0:16, 128:]], axis=1)
            a11 = jnp.concatenate([top, a11[16:, :]], axis=0)
        p1 = keep(0, mm(a11, win_v[0:KS, cl]))
        out(a0, j, p1() + mm(xn_v[r0, KS:D], win_v[KS:D, cl]))
        u2 = keep(1, p1() + mm(sx(1), tw(1)))
        u3 = keep(2, u2() + mm(sx(2), tw(2)))
        out(a0 + 1, j, u3() + mm(xn_v[r1, KS:D], jnp.concatenate([tw(3), win_v[2 * KS:D, cl]], axis=0)))
        p5 = mm(sx(0), tw(0))
        out(a0 + 1, 3 + j, (u3() + p5) + mm(xn_v[r1, 2 * KS:D], win_v[2 * KS:D, cr]))
        out(a0, 3 + j, (u2() + p5) + mm(jnp.concatenate([sx(3), xn_v[r0, 2 * KS:D]], axis=1), win_v[KS:D, cr]))

    def region(pairs, hch=(0, 0), kch=(0, 0), plan=((0, 0),)):
        hs = [(a, dt) for a in range(hch[0], hch[0] + hch[1]) for dt in range(ND)]
        us = [(a, dt) for a in range(kch[0], kch[0] + kch[1]) for dt in range(ND)]
        for bi, a0 in enumerate(pairs):
            nh, nu = plan[bi]
            nh_end = min(nh, 4) if bi == len(pairs) - 1 else 0
            nh_mid = min(8, nh - nh_end)
            nh_run = nh - nh_end - nh_mid
            nu_run = min(nu, 3 * nh_run)
            cnt = [0] * 25
            for j in range(nu - nu_run):
                cnt[HINTS[a0]['slots'][j]] += 1
            marks = HINTS[a0]['marks']
            seen = [0]

            def next_ln_q(part, t):
                tok = words(t)
                for a in (a0, a0 + 1):
                    if part == HINTS[a0]['after'][a - a0]:
                        tok = jnp.concatenate([tok, z2_words(a)], axis=0)
                        if a >= NB // 2:
                            tw_ = words(t_v[brows(a - NB // 2), 4 * HN - 128:4 * HN])
                            tok = jnp.concatenate([tok, tw_], axis=0)
                ln_q(a0 + 2 + part // NLQ, fence(tok), part % NLQ, NLQ)

            def after_z2(t):
                for _ in range(cnt[seen[0]]):
                    u_dft(*us.pop(0))
                seen[0] += 1

            def after_z1(t):
                for part, (kind, idx, row) in enumerate(marks):
                    if kind == 'z' and idx == seen[0]:
                        next_ln_q(part, t[row:row + 8, :])
                for _ in range(cnt[13 + seen[0]]):
                    u_dft(*us.pop(0))
                seen[0] += 1

            for j in range(3):
                group(a0, NT, j, after_z2)
            hres = [h_dft(*hs.pop(0)) for _ in range(nh_mid)]
            for _ in range(cnt[12]):
                u_dft(*us.pop(0))
            ln_z2(a0 + 1, ln_z2(a0))
            for part, (kind, idx, row) in enumerate(marks):
                if kind == 'h':
                    next_ln_q(part, hres[idx][row:row + 8, :])
            seen[0] = 0
            for j in range(3):
                group(a0, 0, j, after_z1, fence(z2_words(a0 + j - 1)) if not marks and j >= 1 else None)
            ru, rh = nu_run, nh_run
            while ru or rh:
                if ru and ru * max(nh_run, 1) >= rh * max(nu_run, 1):
                    u_dft(*us.pop(0))
                    ru -= 1
                else:
                    h_dft(*hs.pop(0))
                    rh -= 1
            for _ in range(nh_end):
                h_dft(*hs.pop(0))
        assert not us
        return hs

    def conv_pos(ft, ft2, par, dt, after):
        cols = lanes(dt)
        prev = None
        for a in range(NB):
            ar, ai = (None, None) if prev is None else (-prev[1], prev[0])
            for dl in range(a + 1):
                hr = hf_v[ft, dl, 0:8, cols]
                hi = hf_v[ft, dl, 8:16, cols]
                ur = p_v[ft, a - dl, 0:8, cols]
                ui = p_v[ft, a - dl, 8:16, cols]
                if ar is None:
                    ar, ai = ur * hr - ui * hi, ur * hi + ui * hr
                    if after is not None:
                        z = fence(after)
                        ar, ai = held(ar, z), held(ai, z)
                elif (a * (a + 1) // 2 + dl) % TREE == 0:
                    ar = ar + (ur * hr - ui * hi)
                    ai = ai + (ur * hi + ui * hr)
                else:
                    ar = (ar + ur * hr) - ui * hi
                    ai = (ai + ur * hi) + ui * hr
            prev = (ar, ai) if prev is None else (ar + prev[1], ai - prev[0])
            w_v[a * 16 + ft2, par * 8:(par + 1) * 8, cols] = ar.astype(BF)
            w_v[a * 16 + 8 + ft2, par * 8:(par + 1) * 8, cols] = ai.astype(BF)
        return words(prev[0])

    gl_v = wout_v
    GL0 = FH
    GS0 = GL0 + NOP * C
    WS0 = GS0 + 4 * C
    GX0 = WS0 + 2 * HN

    def g_sums(ref, g0, s0):
        def quads(u):
            c, g = u
            return [(ref, (pl.ds(g0 + m * C + g * 16, 16), lanes(n))) for m in (0, 1) for n in (c, 3 + c)]

        def dest(u, k):
            c, g = u
            return gl_v, (pl.ds(s0 + k // 2 * C + g * 16, 16), lanes(k % 2 * 3 + c))

        chain_sums([(c, g) for c in range(3) for g in range(C // 16)], quads, dest, a_sums, 2, True)

    def ws_at(jj, k):
        return WS0 + (jj * 4 + k) // 6 * HN, lanes((jj * 4 + k) % 6)

    def w_sums(after):
        def quads(u):
            jj, g = u
            return [(wout_v, (pl.ds(r0 + g * 16, 16), lanes(n))) for r0 in (0, HN) for n in (jj, 2 + jj)]

        def dest(u, k):
            jj, g = u
            r0, cols = ws_at(jj, k)
            return wout_v, (pl.ds(r0 + g * 16, 16), cols)

        chain_sums([(jj, g) for jj in range(2) for g in range(HN // 16)], quads, dest, b_sums, 0, False, after)

    def xn_gate(a, dt, hh):
        return xn_v[brows(a), lanes(dt)].astype(F32) * (hh + hh * jnp.tanh(hh))

    def o_pair(a0, ref, g0, s0, finish, skip=False):
        r0, r1 = pl.ds(g0, C), pl.ds(g0 + C, C)

        def gs(k):
            return gl_v[pl.ds(s0 + k // 2 * C, C), (k % 2) * HN:(k % 2 + 1) * HN]

        def ws(jj, k):
            r, cols = ws_at(jj, k)
            return wout_v[r:r + HN, cols]

        for jj in range(2):
            if jj == (0 if skip else 1):
                finish(a0, 4, None if skip else mm(ref[r0, :], wout_v[0:FH, lanes(4)]))
                finish(a0 + 1, 4, mm(ref[r1, :], wout_v[0:FH, lanes(4)]))
            p1 = mm(ref[r0, 0:HN], wout_v[0:HN, lanes(jj)])
            finish(a0, jj, p1 + mm(ref[r0, HN:FH], wout_v[HN:FH, lanes(jj)]))
            u2 = p1 + mm(gs(1), ws(jj, 1))
            u3 = u2 + mm(gs(2), ws(jj, 2))
            finish(a0 + 1, jj, u3 + mm(ref[r1, HN:FH], ws(jj, 3)))
            p5 = mm(gs(0), ws(jj, 0))
            finish(a0 + 1, 2 + jj, u3 + p5)
            finish(a0, 2 + jj, (u2 + p5) + mm(gs(3), wout_v[HN:FH, lanes(2 + jj)]))

    def s_at(slot, k):
        return D + (slot * 2 + k // 2) * C, (k % 2) * HK

    def s_val(slot, k):
        r0, col = s_at(slot, k)
        return h_v[r0:r0 + C, col:col + HK]

    def s_sums(a0, nr, via_memory):
        def quads(u):
            slot, c, g = u
            return [(wsp_v, (ds((a0 + 2 * slot + m) * C + g * nr, nr), lanes(n)))
                    for m in (0, 1) for n in (c, HK // 128 + c)]

        def dest(u, k):
            slot, c, g = u
            r0, col = s_at(slot, k)
            return h_v, (slice(r0 + g * nr, r0 + (g + 1) * nr), slice(col + c * 128, col + (c + 1) * 128))

        units = [(slot, c, g) for slot in range(2) for c in range(HK // 128) for g in range(C // nr)]
        for part in (units[:48], units[48:]) if via_memory else (units,):
            chain_sums(part, quads, dest, a_sums, 2, via_memory)

    def phase2a(i, carry):
        @pl.when(i + 1 < S // TA)
        def _():
            cp_wsp(i + 1).wait()

        eye = (jax.lax.broadcasted_iota(jnp.int32, (C, C), 0)
               == jax.lax.broadcasted_iota(jnp.int32, (C, C), 1))

        def bcol(a):
            return jnp.sum(jnp.where(eye, b32_v[pl.ds(a, 1), :], 0.0), axis=-1, keepdims=True)

        def put(m, n, g):
            g = (z1_v[brows(i * (TA // C) + m), lanes(n)] * g).astype(BF)
            if m < NOP:
                gl_v[GL0 + m * C:GL0 + (m + 1) * C, lanes(n)] = g
            else:
                gg_v[ds((2 * i + m - NOP) * C, C), lanes(n)] = g
                if m == NOP:
                    gl_v[GX0:GX0 + C, lanes(n)] = g

        for pp in range(2):
            if pp == 1:
                g_sums(gl_v, GL0, GS0)
            m0 = 2 * pp
            a0 = i * (TA // C) + m0
            r0, r1 = brows(a0), brows(a0 + 1)
            b0 = bcol(a0)
            db = bcol(a0 + 1) - b0
            for j in range(NT // 2):
                jl, jr = lanes(j), lanes(NT // 2 + j)
                t1, t2, t3, t4 = (t_v[:, lanes(k * (NT // 2) + j)] for k in range(4))
                p1 = mm(wsp_v[r0, 0:HK], z2_v[0:HK, jl]) + b0
                put(m0, j, p1 + mm(wsp_v[r0, HK:S], z2_v[HK:S, jl]))
                u2 = p1 + mm(s_val(pp, 1), t2)
                u3 = (u2 + db) + mm(s_val(pp, 2), t3)
                put(m0 + 1, j, u3 + mm(wsp_v[r1, HK:S], t4))
                p5 = mm(s_val(pp, 0), t1)
                put(m0 + 1, NT // 2 + j, u3 + p5)
                put(m0, NT // 2 + j, (u2 + p5) + mm(s_val(pp, 3), z2_v[HK:S, jr]))
        def finish(a, dt, hh):
            xg_v[brows(a), lanes(dt)] = xn_gate(a, dt, hh)

        o_pair(i * (TA // C), gl_v, GL0, GS0, finish)
        finish(i * (TA // C) + 2, 4, mm(gl_v[GX0:GX0 + C, :], wout_v[0:FH, lanes(4)]))
        s_sums(jnp.minimum(i + 1, S // TA - 1) * (TA // C), 16, True)
        nft = NB * TA // S
        last = None
        for ft in range(nft):
            for dt in range(ND):
                last = conv_pos(i * nft + ft, i * (nft // 2) + ft // 2, ft % 2, dt, last)
        return carry

    step = pl.program_id(0)

    @pl.when(step == 0)
    def _():
        for grp in groups:
            for cp in grp:
                cp.start()
        cp_wout.start()
        for i in range(S // TA):
            cp_wsp(i).start()
        k_u[:, 0:8, :] = jnp.zeros((ND, 8, 128), U32)

    @pl.when(step == 1)
    def _():
        cp_wsp(0).wait()
        cp_wout.wait()
        for a, dt in [(a, dt) for a in range(NB) for dt in range(ND)][NB * ND - H_LATE:]:
            h_dft(a, dt)
        last = None
        for g in range(C // 16):
            bot = held(z2_v[pl.ds((NB - 1) * C + g * 16, 16), :], None if last is None else fence(last))
            t_rest(NB // 2 - 1, bot.astype(F32), g, 16)
            rows = pl.ds((NB // 2 - 1) * C + g * 16, 16)
            last = jnp.concatenate([words(t_v[rows, lanes(k)]) for k in range(3, 12)], axis=0)
        w_sums(last)
        s_sums(0, 32, False)
        jax.lax.fori_loop(0, S // TA, phase2a, 0)

        rev = 7 - jax.lax.broadcasted_iota(jnp.int32, (8, 128), 0)
        done = {}

        def emit(a, dt, hh):
            rows, cols = brows(a), lanes(dt)
            ev = mm(fg_v[2 * C:2 * C + C // 2, 0:C], w_v[ds(a * 16, 8), :, cols].reshape(C, 128))
            od = mm(fg_v[2 * C:2 * C + C // 2, C:2 * C], w_v[ds(a * 16 + 8, 8), :, cols].reshape(C, 128))
            lo = ev - od
            ys = [jnp.take_along_axis(lo[g * 8:(g + 1) * 8, :], rev, axis=0)
                  for g in range(C // 16 - 1, -1, -1)]
            y = jnp.concatenate(ys + [ev + od], axis=0)
            xg = xg_v[rows, cols] if hh is None else xn_gate(a, dt, hh)
            o_v[rows, cols] = (q_v[rows, cols].astype(F32) + xg * y).astype(BF)
            done[a] = done.get(a, 0) + 1
            if a >= NB - 2:
                cp_o(a, cols).start()
            elif done[a] == ND:
                cp_o(a).start()

        g_sums(gg_v, 0, GS0)
        for k in range(S // TA):
            if k + 1 < S // TA:
                g_sums(gg_v, (k + 1) * 2 * C, GS0 + ((k + 1) % 2) * 2 * C)
            for a in (4 * k, 4 * k + 1):
                for dt in range(ND):
                    emit(a, dt, None)
            o_pair(4 * k + 2, gg_v, k * 2 * C, GS0 + (k % 2) * 2 * C, emit, skip=True)
        pltpu.make_async_copy(o_v, o_hbm, sem_o.at[0]).wait()

    @pl.when(step == 0)
    def _():
        wait(0)
        ln_q(0)
        ln_q(1)
        wait(1)
        for n in (0, 1):
            z2_tile(0, n)
            z2_tile(1, n)
        wait(2)
        ln_q(2)
        for n in (2, 3):
            z2_tile(0, n)
            z2_tile(1, n)
        for n in range(4):
            z2_tile(2, n)
        wait(3)
        ln_q(3)
        seq = ([(z2_tile, a, n) for a in range(3) for n in (4, 5)] + [(z2_tile, 3, n) for n in range(NT)]
               + [(z1_tile, a, 0) for a in range(4)])
        tw_done = tw_sums(NT)
        for j, (tile, a, n) in enumerate(seq):
            if j == 15:
                gate = fence(tw_done)
            elif j == 3:
                gate = fence(words(xn_v[brows(3), 0:128]))
            else:
                gate = fence(z2_words(0, (7, 10).index(j))) if j in (7, 10) else None
            tile(a, n, gate)
            if j == 1:
                ln_z2(0)
        wait(4)
        for a in (1, 2, 3):
            ln_z2(a)
        tw_sums(0)
        release = (9, 10, 11, 12, 13, 15, 16, 17)
        waits = (3, 4, 6, 8, 10, 11)
        for j, (a, n) in enumerate((a, n) for n in range(1, NT) for a in range(4)):
            gate = fence(z2_words(1 + waits.index(j) // 2, waits.index(j) % 2)) if j in waits else None
            t = z1_tile(a, n, gate)
            if j in release:
                part = release.index(j)
                ln_q(4 + part // NLQ, fence(words(t[0:8, :])), part % NLQ, NLQ)
        region([4])
        wait(5)
        b32_v[...] = b_v[...].astype(F32) * 0.25
        assert not region([6, 8, 10], HCH[0], KCH[0], DFT_PLAN[0])
        wait(6)
        assert len(region([12, 14], HCH[1], KCH[1], DFT_PLAN[1])) == H_LATE


@jax.jit
def pallas_recurrent_scan__ssm_conv_h3__mixer_gmlp__prompt_kernel(
    A_q: jax.Array,
    A_k: jax.Array,
    A_v: jax.Array,
    A_shift_k: jax.Array,
    A_ssm_k: jax.Array,
    A_ssm_D: jax.Array,
    B_x: jax.Array,
    B_w_in: jax.Array,
    B_w_sp: jax.Array,
    B_b_sp: jax.Array,
    B_w_out: jax.Array,
):
    del B_x
    any_spec = pl.BlockSpec(memory_space=pl.ANY)
    vm = pltpu.VMEM
    dma = pltpu.SemaphoreType.DMA
    out = pl.pallas_call(
        _kernel,
        out_shape=jax.ShapeDtypeStruct((S, D), BF),
        grid=(2,),
        in_specs=[any_spec] * 11,
        out_specs=any_spec,
        scratch_shapes=[
            vm((S // 2, D), U32),
            vm((ND, S // 2 + 32, 128), U32),
            vm((S // 2, D), U32),
            vm(((D + 4 * C) // 2, S), U32),
            vm(((D + 2 * KS) // 2, 2 * FH), U32),
            vm((S // 2, S), U32),
            vm(((FH + 8 * C + 2 * HN) // 2, FH), U32),
            vm(((2 * C + C // 2) // 2, 2 * C), U32),
            vm(((S + 4 * C) // 2, D), U32),
            vm((S + 6 * C, FH), F32),
            vm((S // 2, FH), U32),
            vm((S // 4, 2 * FH), U32),
            vm((NB, NB, 16, D), F32),
            vm((NB, NB, 16, D), F32),
            vm((NB * 16, 8, 1024), U32),
            vm((S // 4, FH), U32),
            vm((S, D), F32),
            vm((S, D), BF),
            vm((NB, 128), F32),
            vm((NB, 128), BF),
            vm((4, 18 * 128), BF),
            vm((ND, 128), BF),
            dma((len(QCH),)), dma((len(KCH) * ND,)), dma((len(KCH),)), dma((len(HCH),)),
            dma((len(WCH),)), dma((S // TA,)), dma((1,)), dma((5,)),
        ],
        compiler_params=pltpu.CompilerParams(
            dimension_semantics=("arbitrary",),
            vmem_limit_bytes=110 * 1024 * 1024,
            disable_bounds_checks=True,
            disable_semaphore_checks=True,
        ),
    )(
        A_q.reshape(S, D), A_k.reshape(S, D), A_v.reshape(S, D),
        A_shift_k.T, A_ssm_k, A_ssm_D.reshape(ND, 128),
        B_w_in, B_w_sp, B_b_sp.reshape(NB, 128), B_w_out,
        _dft_consts(),
    )
    return out.reshape(1, S, D)
```

```python
import math

import jax
import jax.numpy as jnp
import numpy as np
import jax.experimental.pallas as pl
import jax.experimental.pallas.tpu as pltpu

S = 2048
D = 640
FH = 768
C = 128
NB = S // C
ND = D // 128
NT = FH // 128
EPS = 1e-5
HK = S // 2
HN = FH // 2
KS = 256
TA = 512
NOP = 2
NLQ = 4
H_LATE = 24
TREE = 10

BF = jnp.bfloat16
F32 = jnp.float32
U32 = jnp.uint32

QCH = [(0, 2), (2, 1), (3, 1), (4, 4), (8, 6), (14, 2)]
HCH = [(0, 5), (5, 11)]
KCH = [(0, 3), (3, 13)]
WCH = [(6, 2), (8, 2), (10, 2), (0, 1), (1, 5)]
HINTS = {
    4: dict(h=(0, 0, 0), u_run=0, after=(0, 6), stash=7,
             slots=[],
             marks=[('z', 2, 0), ('z', 2, 0), ('z', 2, 0), ('z', 4, 0),
                    ('z', 4, 64), ('z', 6, 0), ('z', 8, 0), ('z', 9, 0)]),
    6: dict(h=(5, 0, 0), u_run=0, after=(0, 6), stash=6,
             slots=[1, 5, 7, 10, 4, 14, 18],
             marks=[('h', 4, 128), ('z', 0, 120), ('z', 1, 120), ('z', 3, 64),
                    ('z', 4, 120), ('z', 5, 120), ('z', 7, 120), ('z', 9, 56)]),
    8: dict(h=(8, 0, 0), u_run=0, after=(2, 6), stash=7,
             slots=[1, 5, 9, 3],
             marks=[('z', 0, 0), ('z', 0, 120), ('z', 1, 56), ('z', 3, 120),
                    ('z', 4, 48), ('z', 5, 120), ('z', 7, 120), ('z', 8, 120)]),
    10: dict(h=(8, 0, 4), u_run=0, after=(1, 6), stash=7,
             slots=[1, 5, 9, 18],
             marks=[('z', 0, 56), ('z', 0, 120), ('z', 1, 120), ('z', 3, 120),
                    ('z', 4, 120), ('z', 6, 64), ('z', 7, 120), ('z', 9, 56)]),
    12: dict(h=(8, 4, 0), u_run=23, after=(1, 6), stash=3,
             slots=[1, 5, 9, 3, 7, 14, 18, 22, 0],
             marks=[('h', 4, 128), ('z', 0, 120), ('z', 2, 56), ('z', 3, 120),
                    ('z', 4, 120), ('z', 5, 48), ('z', 7, 120), ('z', 8, 64)]),
    14: dict(h=(10, 5, 4), u_run=11, after=(0, 6), stash=7,
             slots=[0, 5, 9, 3, 7, 10, 20, 22, 4, 1, 8, 16, 18, 2, 6, 14, 15, 19, 23, 11, 13, 17],
             marks=[]),
}
LNZ_ROWS = [128, 16, 32, 16, 16, 16, 16, 16, 16, 16, 16, 16, 16, 16, 128, 128]


def _dft_consts():
    theta = np.pi * (4 * np.arange(C) + 1) / (2 * C)

    def fwd(t):
        ang = theta[:, None] * t[None, :]
        re = np.cos(ang).reshape(C // 8, 8, C)
        im = -np.sin(ang).reshape(C // 8, 8, C)
        return np.stack([re, im], axis=1).reshape(2 * C, C)

    fg = np.zeros((2 * C + C // 2, 2 * C), np.float64)
    order = np.concatenate([np.arange(0, C, 2), np.arange(1, C, 2)])
    fg[:2 * C, :C] = fwd(order - (C - 1) / 2)
    fg[:2 * C, C:] = fwd(np.arange(C))
    ang = (np.arange(C // 2) + 0.5)[:, None] * theta[None, :]
    fg[2 * C:, :C] = np.cos(ang) / C
    fg[2 * C:, C:] = -np.sin(ang) / C
    return fg.astype(np.float32).astype(BF)


def _kernel(q_hbm, k_hbm, v_hbm, sk_hbm, h_hbm, d_hbm, win_hbm, wsp_hbm, b_hbm, wout_hbm,
            fg_hbm, o_hbm,
            q_u, k_u, v_u, h_u, win_u, wsp_u, wout_u, fg_u,
            xn_u, z1_v, z2_u, t_u, p_v, hf_v, w_u, gg_u, xg_v, o_v, b32_v, b_v, sk_v, d_v,
            sem_q, sem_k, sem_v, sem_h, sem_w, sem_wsp, sem_o, sem_m):
    q_v = q_u.bitcast(BF)
    v_v = v_u.bitcast(BF)
    k_w = k_hbm.bitcast(U32)
    h_v = h_u.bitcast(BF)
    win_v = win_u.bitcast(BF)
    wsp_v = wsp_u.bitcast(BF)
    wout_v = wout_u.bitcast(BF)
    fg_v = fg_u.bitcast(BF)
    xn_v = xn_u.bitcast(BF)
    z2_v = z2_u.bitcast(BF)
    t_v = t_u.bitcast(BF)
    w_v = w_u.bitcast(BF)
    gg_v = gg_u.bitcast(BF)

    def ds(start, size):
        if isinstance(start, int):
            return pl.ds(start, size)
        return pl.ds(pl.multiple_of(start, size), size)

    def lanes(n):
        return slice(n * 128, (n + 1) * 128)

    def blocks(ch):
        return pl.ds(ch[0] * C, ch[1] * C)

    def brows(a):
        return ds(a * C, C)

    def cp_q(c):
        r = blocks(QCH[c])
        return pltpu.make_async_copy(q_hbm.at[r, :], q_v.at[r, :], sem_q.at[c])

    def cp_k(c):
        b0, n = KCH[c]
        return [pltpu.make_async_copy(k_w.at[pl.ds(b0 * C // 2, n * C // 2), lanes(dt)],
                                      k_u.at[dt, pl.ds(b0 * C // 2 + 8, n * C // 2), :],
                                      sem_k.at[c * ND + dt])
                for dt in range(ND)]

    def cp_v(c):
        r = blocks(KCH[c])
        return pltpu.make_async_copy(v_hbm.at[r, :], v_v.at[r, :], sem_v.at[c])

    def cp_h(c):
        r = blocks(HCH[c])
        return pltpu.make_async_copy(h_hbm.at[:, r], h_v.at[0:D, r], sem_h.at[c])

    def cp_w(c):
        r = blocks(WCH[c])
        return pltpu.make_async_copy(win_hbm.at[:, r], win_v.at[0:D, r], sem_w.at[c])

    def cp_wsp(i):
        r = ds(i * TA, TA)
        return pltpu.make_async_copy(wsp_hbm.at[r, :], wsp_v.at[r, :], sem_wsp.at[i])

    def cp_o(a, cols=slice(None)):
        r = brows(a)
        return pltpu.make_async_copy(o_v.at[r, cols], o_hbm.at[r, cols], sem_o.at[0])

    cp_f = pltpu.make_async_copy(fg_hbm, fg_v, sem_m.at[0])
    cp_sk = pltpu.make_async_copy(sk_hbm, sk_v.at[:, 0:D], sem_m.at[1])
    cp_d = pltpu.make_async_copy(d_hbm, d_v, sem_m.at[2])
    cp_b = pltpu.make_async_copy(b_hbm, b_v, sem_m.at[3])
    cp_wout = pltpu.make_async_copy(wout_hbm, wout_v.at[0:FH, 0:D], sem_m.at[4])

    groups = [
        [cp_q(0)], [cp_w(0)], [cp_q(1), cp_w(1)], [cp_q(2), cp_w(2), cp_w(3)], [cp_q(3), cp_w(4)],
        [cp_f, cp_sk, cp_d, cp_b, cp_q(4), cp_h(0), *cp_k(0), cp_v(0)],
        [cp_q(5), cp_h(1), *cp_k(1), cp_v(1)],
    ]

    def wait(g):
        for cp in groups[g]:
            cp.wait()

    def mm(x, y):
        return jnp.dot(x, y, preferred_element_type=F32)

    def words(x):
        return pltpu.bitcast(x, U32)

    def fence(tok):
        t = tok[0:8, :]
        for g in range(1, tok.shape[0] // 8):
            t = t | tok[g * 8:(g + 1) * 8, :]
        return t & k_u[0, 0:8, :]

    def held(x, gate):
        if gate is None:
            return x
        w = words(x)
        return pltpu.bitcast(w | jnp.tile(gate, (w.shape[0] // 8, w.shape[1] // 128)), x.dtype)

    def a_sums(a11, a12, a21, a22):
        s1 = a21 + a22
        s2 = s1 - a11
        return s1, s2, a11 - a21, a12 - s2

    def b_sums(b11, b12, b21, b22):
        t1 = b12 - b11
        t2 = b22 - t1
        return t1, t2, t2 - b11, b21 - t2

    def chain_sums(units, quads, dest, combine, lead, via_memory, last=None):
        for u in units:
            vals = []
            for n, (ref, idx) in enumerate(quads(u)):
                wait_here = last is not None and (n == lead or not via_memory)
                vals.append(held(ref[idx], fence(last) if wait_here else None).astype(F32))
            sums = combine(*vals)
            done = []
            for k, val in enumerate(sums):
                ref, idx = dest(u, k)
                ref[idx] = val.astype(BF)
                if via_memory:
                    done.append(words(ref[idx]))
            last = jnp.concatenate(done, axis=0) if via_memory else words(sums[-1][-8:, :])
        return last

    c0 = math.sqrt(2.0 / math.pi)
    c1 = c0 * 0.044715

    def gelu2(x):
        return x + x * jnp.tanh(x * (c0 + c1 * (x * x)))

    def z2_words(a, half=None):
        r = brows(a) if half is None else pl.ds(a * C + half * (C // 2), C // 2)
        return words(z2_v[r, 0:128])

    def xs_row(a0, k):
        return S + (a0 // 2 % 2) * 2 * C + k // 2 * C

    def ln_q(a, gate=None, part=0, nparts=1):
        n = C // nparts
        r = pl.ds(a * C + part * n, n)
        x = held(q_v[r, :], gate).astype(F32)
        mu = jnp.sum(x, axis=-1, keepdims=True) * (1.0 / D)
        ex2 = jnp.sum(x * x, axis=-1, keepdims=True) * (1.0 / D)
        var = jnp.maximum(ex2 - mu * mu, 0.0)
        mu = mu.astype(BF).astype(F32)
        xn = (x - mu) * jnp.exp(-0.5 * jnp.log(var + EPS))
        xn_v[r, :] = xn.astype(BF)
        if a >= 4 and a % 2 == 1:
            top = xn_v[pl.ds((a - 1) * C + part * n, n), 0:2 * KS].astype(F32)
            s1, s2, s3, s4 = a_sums(top[:, :KS], top[:, KS:], xn[:, :KS], xn[:, KS:2 * KS])
            xn_v[pl.ds(xs_row(a - 1, 0) + part * n, n), 0:2 * KS] = jnp.concatenate([s1, s2], axis=1).astype(BF)
            xn_v[pl.ds(xs_row(a - 1, 2) + part * n, n), 0:2 * KS] = jnp.concatenate([s3, s4], axis=1).astype(BF)

    def h_dft(a, dt):
        res = jax.lax.dot_general(fg_v[0:2 * C, C:2 * C], h_v[lanes(dt), brows(a)],
                                  (((1,), (1,)), ((), ())), preferred_element_type=F32)
        spec = res.reshape(NB, 16, 128)
        if a == 0:
            dv = d_v[...].astype(F32)[dt:dt + 1, :]
            spec = jnp.concatenate([spec[:, 0:8, :] + dv[None], spec[:, 8:16, :]], axis=1)
        hf_v[:, a, :, lanes(dt)] = spec
        return res

    def u_dft(a, dt):
        cols = lanes(dt)

        def even(w):
            return pltpu.bitcast(w << 16, F32)

        def odd(w):
            return pltpu.bitcast(w & jnp.uint32(0xFFFF0000), F32)

        w0, w1, w2 = (k_u[dt, pl.ds(8 + a * C // 2 - j, C // 2), :] for j in range(3))
        e0, o0, e1, o1 = even(w0), odd(w0), even(w1), odd(w1)
        sk = sk_v[:, cols].astype(F32)
        s0, s1, s2, s3 = (sk[j:j + 1, :] for j in range(4))
        vw = words(v_v[brows(a), cols])
        kve = (e0 * s0 + o1 * s1 + e1 * s2 + odd(w2) * s3) * even(vw)
        kvo = (o0 * s0 + e0 * s1 + o1 * s2 + e1 * s3) * odd(vw)
        kv = jnp.concatenate([kve, kvo], axis=0).astype(BF)
        p_v[:, a, :, cols] = mm(fg_v[0:2 * C, 0:C], kv).reshape(NB, 16, 128)

    def proj(a, n, gate=None):
        lhs = xn_v[brows(a), :]
        if gate is not None:
            lhs = jnp.concatenate([held(lhs[0:16, :], gate), lhs[16:, :]], axis=0)
        return gelu2(mm(lhs, win_v[0:D, lanes(n)]))

    def w2_rows(a):
        return pl.ds(S + (a % 4) * C, C)

    def z2_tile(a, n, gate=None):
        z1_v[w2_rows(a), lanes(n)] = proj(a, NT + n, gate)

    def z1_tile(a, n, gate=None):
        t = proj(a, n, gate)
        z1_v[brows(a), lanes(n)] = t
        return t

    def t_rest(r, bot, g=0, nr=C):
        rows = pl.ds(r * C + g * nr, nr)
        t2 = bot[:, HN:] - t_v[rows, 0:HN].astype(F32)
        t3 = t2 - z2_v[rows, 0:HN].astype(F32)
        t_v[rows, HN:4 * HN] = jnp.concatenate([t2, t3, bot[:, :HN] - t2], axis=1).astype(BF)

    def ln_z2(a, last=None):
        w2 = z1_v[w2_rows(a), :]
        mu = jnp.sum(w2, axis=-1, keepdims=True) * (1.0 / FH)
        ex2 = jnp.sum(w2 * w2, axis=-1, keepdims=True) * (1.0 / FH)
        var = jnp.maximum(ex2 - mu * mu, 0.0)
        rs = jnp.exp(-0.5 * jnp.log(16.0 * var + 64.0 * EPS))
        nr = LNZ_ROWS[a]
        for g in range(C // nr):
            rr = slice(g * nr, (g + 1) * nr)
            m = held(jnp.broadcast_to(mu[rr], (nr, 128)), fence(last) if last is not None and nr < C else None)
            zn = (w2[rr] - jnp.tile(m, (1, NT))) * rs[rr]
            rows = pl.ds(a * C + g * nr, nr)
            if a < NB // 2:
                z2_v[rows, 0:HN] = zn[:, :HN].astype(BF)
                t_v[rows, 0:HN] = (zn[:, HN:] - zn[:, :HN]).astype(BF)
                done = [(z2_v, rows, k) for k in range(3)] + [(t_v, rows, k) for k in range(3)]
            else:
                z2_v[rows, :] = zn.astype(BF)
                done = [(z2_v, rows, k) for k in range(6)]
                if a < NB - 1:
                    t_rest(a - NB // 2, zn, g, nr)
                    done += [(t_v, pl.ds((a - NB // 2) * C + g * nr, nr), k) for k in range(3, 12)]
            if nr < C:
                last = jnp.concatenate([words(ref[r, lanes(k)]) for ref, r, k in done], axis=0)
        return last

    def tw_at(base, j, k):
        return D + (base // NT) * KS, lanes(j * 4 + k)

    def tw_sums(base):
        def quads(u):
            j, g = u
            return [(win_v, (slice(r0 + g * 16, r0 + (g + 1) * 16), lanes(n)))
                    for r0 in (0, KS) for n in (base + j, base + 3 + j)]

        def dest(u, k):
            j, g = u
            r0, cols = tw_at(base, j, k)
            return win_v, (slice(r0 + g * 16, r0 + (g + 1) * 16), cols)

        return chain_sums([(j, g) for j in range(3) for g in range(KS // 16)], quads, dest, b_sums, 0, True)

    def group(a0, base, j, hook, gate=None):
        r0, r1 = brows(a0), brows(a0 + 1)
        cl, cr = lanes(base + j), lanes(base + 3 + j)

        def out(a, n, val):
            t = gelu2(val)
            z1_v[w2_rows(a) if base else brows(a), lanes(n)] = t
            hook(t)

        def sx(k):
            return xn_v[xs_row(a0, k):xs_row(a0, k) + C, (k % 2) * KS:(k % 2 + 1) * KS]

        def tw(k):
            t0, cols = tw_at(base, j, k)
            return win_v[t0:t0 + KS, cols]

        def keep(slot, val):
            if not (HINTS[a0]['stash'] >> slot) & 1:
                return lambda: val
            sl = (pl.ds(S + 4 * C + (j % 2) * C, C), lanes(slot))
            z1_v[sl] = val
            return lambda: z1_v[sl]

        a11 = xn_v[r0, 0:KS]
        if gate is not None:
            top = jnp.concatenate([held(a11[0:16, 0:128], gate), a11[0:16, 128:]], axis=1)
            a11 = jnp.concatenate([top, a11[16:, :]], axis=0)
        p1 = keep(0, mm(a11, win_v[0:KS, cl]))
        out(a0, j, p1() + mm(xn_v[r0, KS:D], win_v[KS:D, cl]))
        u2 = keep(1, p1() + mm(sx(1), tw(1)))
        u3 = keep(2, u2() + mm(sx(2), tw(2)))
        out(a0 + 1, j, u3() + mm(xn_v[r1, KS:D], jnp.concatenate([tw(3), win_v[2 * KS:D, cl]], axis=0)))
        p5 = mm(sx(0), tw(0))
        out(a0 + 1, 3 + j, (u3() + p5) + mm(xn_v[r1, 2 * KS:D], win_v[2 * KS:D, cr]))
        out(a0, 3 + j, (u2() + p5) + mm(jnp.concatenate([sx(3), xn_v[r0, 2 * KS:D]], axis=1), win_v[KS:D, cr]))

    def region(pairs, hch=(0, 0), kch=(0, 0)):
        hs = [(a, dt) for a in range(hch[0], hch[0] + hch[1]) for dt in range(ND)]
        us = [(a, dt) for a in range(kch[0], kch[0] + kch[1]) for dt in range(ND)]
        for a0 in pairs:
            nh_mid, nh_run, nh_end = HINTS[a0]['h']
            nu_run = HINTS[a0]['u_run']
            cnt = [HINTS[a0]['slots'].count(j) for j in range(25)]
            marks = HINTS[a0]['marks']
            seen = [0]

            def next_ln_q(part, t):
                tok = words(t)
                for a in (a0, a0 + 1):
                    if part == HINTS[a0]['after'][a - a0]:
                        tok = jnp.concatenate([tok, z2_words(a)], axis=0)
                        if a >= NB // 2:
                            tw_ = words(t_v[brows(a - NB // 2), 4 * HN - 128:4 * HN])
                            tok = jnp.concatenate([tok, tw_], axis=0)
                ln_q(a0 + 2 + part // NLQ, fence(tok), part % NLQ, NLQ)

            def after_z2(t):
                for _ in range(cnt[seen[0]]):
                    u_dft(*us.pop(0))
                seen[0] += 1

            def after_z1(t):
                for part, (kind, idx, row) in enumerate(marks):
                    if kind == 'z' and idx == seen[0]:
                        next_ln_q(part, t[row:row + 8, :])
                for _ in range(cnt[13 + seen[0]]):
                    u_dft(*us.pop(0))
                seen[0] += 1

            for j in range(3):
                group(a0, NT, j, after_z2)
            hres = [h_dft(*hs.pop(0)) for _ in range(nh_mid)]
            for _ in range(cnt[12]):
                u_dft(*us.pop(0))
            ln_z2(a0 + 1, ln_z2(a0))
            for part, (kind, idx, row) in enumerate(marks):
                if kind == 'h':
                    next_ln_q(part, hres[idx][row:row + 8, :])
            seen[0] = 0
            for j in range(3):
                group(a0, 0, j, after_z1, fence(z2_words(a0 + j - 1)) if not marks and j >= 1 else None)
            ru, rh = nu_run, nh_run
            while ru or rh:
                if ru and ru * max(nh_run, 1) >= rh * max(nu_run, 1):
                    u_dft(*us.pop(0))
                    ru -= 1
                else:
                    h_dft(*hs.pop(0))
                    rh -= 1
            for _ in range(nh_end):
                h_dft(*hs.pop(0))
        assert not us
        return hs

    def conv_pos(ft, ft2, par, dt, after):
        cols = lanes(dt)
        prev = None
        for a in range(NB):
            ar, ai = (None, None) if prev is None else (-prev[1], prev[0])
            for dl in range(a + 1):
                hr = hf_v[ft, dl, 0:8, cols]
                hi = hf_v[ft, dl, 8:16, cols]
                ur = p_v[ft, a - dl, 0:8, cols]
                ui = p_v[ft, a - dl, 8:16, cols]
                if ar is None:
                    ar, ai = ur * hr - ui * hi, ur * hi + ui * hr
                    if after is not None:
                        z = fence(after)
                        ar, ai = held(ar, z), held(ai, z)
                elif (a * (a + 1) // 2 + dl) % TREE == 0:
                    ar = ar + (ur * hr - ui * hi)
                    ai = ai + (ur * hi + ui * hr)
                else:
                    ar = (ar + ur * hr) - ui * hi
                    ai = (ai + ur * hi) + ui * hr
            prev = (ar, ai) if prev is None else (ar + prev[1], ai - prev[0])
            w_v[a * 16 + ft2, par * 8:(par + 1) * 8, cols] = ar.astype(BF)
            w_v[a * 16 + 8 + ft2, par * 8:(par + 1) * 8, cols] = ai.astype(BF)
        return words(prev[0])

    gl_v = wout_v
    GL0 = FH
    GS0 = GL0 + NOP * C
    WS0 = GS0 + 4 * C
    GX0 = WS0 + 2 * HN

    def g_sums(ref, g0, s0):
        def quads(u):
            c, g = u
            return [(ref, (pl.ds(g0 + m * C + g * 16, 16), lanes(n))) for m in (0, 1) for n in (c, 3 + c)]

        def dest(u, k):
            c, g = u
            return gl_v, (pl.ds(s0 + k // 2 * C + g * 16, 16), lanes(k % 2 * 3 + c))

        chain_sums([(c, g) for c in range(3) for g in range(C // 16)], quads, dest, a_sums, 2, True)

    def ws_at(jj, k):
        return WS0 + (jj * 4 + k) // 6 * HN, lanes((jj * 4 + k) % 6)

    def w_sums(after):
        def quads(u):
            jj, g = u
            return [(wout_v, (pl.ds(r0 + g * 16, 16), lanes(n))) for r0 in (0, HN) for n in (jj, 2 + jj)]

        def dest(u, k):
            jj, g = u
            r0, cols = ws_at(jj, k)
            return wout_v, (pl.ds(r0 + g * 16, 16), cols)

        chain_sums([(jj, g) for jj in range(2) for g in range(HN // 16)], quads, dest, b_sums, 0, False, after)

    def xn_gate(a, dt, hh):
        return xn_v[brows(a), lanes(dt)].astype(F32) * (hh + hh * jnp.tanh(hh))

    def o_pair(a0, ref, g0, s0, finish, skip=False):
        r0, r1 = pl.ds(g0, C), pl.ds(g0 + C, C)

        def gs(k):
            return gl_v[pl.ds(s0 + k // 2 * C, C), (k % 2) * HN:(k % 2 + 1) * HN]

        def ws(jj, k):
            r, cols = ws_at(jj, k)
            return wout_v[r:r + HN, cols]

        for jj in range(2):
            if jj == (0 if skip else 1):
                finish(a0, 4, None if skip else mm(ref[r0, :], wout_v[0:FH, lanes(4)]))
                finish(a0 + 1, 4, mm(ref[r1, :], wout_v[0:FH, lanes(4)]))
            p1 = mm(ref[r0, 0:HN], wout_v[0:HN, lanes(jj)])
            finish(a0, jj, p1 + mm(ref[r0, HN:FH], wout_v[HN:FH, lanes(jj)]))
            u2 = p1 + mm(gs(1), ws(jj, 1))
            u3 = u2 + mm(gs(2), ws(jj, 2))
            finish(a0 + 1, jj, u3 + mm(ref[r1, HN:FH], ws(jj, 3)))
            p5 = mm(gs(0), ws(jj, 0))
            finish(a0 + 1, 2 + jj, u3 + p5)
            finish(a0, 2 + jj, (u2 + p5) + mm(gs(3), wout_v[HN:FH, lanes(2 + jj)]))

    def s_at(slot, k):
        return D + (slot * 2 + k // 2) * C, (k % 2) * HK

    def s_val(slot, k):
        r0, col = s_at(slot, k)
        return h_v[r0:r0 + C, col:col + HK]

    def s_sums(a0, nr, via_memory):
        def quads(u):
            slot, c, g = u
            return [(wsp_v, (ds((a0 + 2 * slot + m) * C + g * nr, nr), lanes(n)))
                    for m in (0, 1) for n in (c, HK // 128 + c)]

        def dest(u, k):
            slot, c, g = u
            r0, col = s_at(slot, k)
            return h_v, (slice(r0 + g * nr, r0 + (g + 1) * nr), slice(col + c * 128, col + (c + 1) * 128))

        units = [(slot, c, g) for slot in range(2) for c in range(HK // 128) for g in range(C // nr)]
        for part in (units[:48], units[48:]) if via_memory else (units,):
            chain_sums(part, quads, dest, a_sums, 2, via_memory)

    def phase2a(i, carry):
        @pl.when(i + 1 < S // TA)
        def _():
            cp_wsp(i + 1).wait()

        eye = (jax.lax.broadcasted_iota(jnp.int32, (C, C), 0)
               == jax.lax.broadcasted_iota(jnp.int32, (C, C), 1))

        def bcol(a):
            return jnp.sum(jnp.where(eye, b32_v[pl.ds(a, 1), :], 0.0), axis=-1, keepdims=True)

        def put(m, n, g):
            g = (z1_v[brows(i * (TA // C) + m), lanes(n)] * g).astype(BF)
            if m < NOP:
                gl_v[GL0 + m * C:GL0 + (m + 1) * C, lanes(n)] = g
            else:
                gg_v[ds((2 * i + m - NOP) * C, C), lanes(n)] = g
                if m == NOP:
                    gl_v[GX0:GX0 + C, lanes(n)] = g

        for pp in range(2):
            if pp == 1:
                g_sums(gl_v, GL0, GS0)
            m0 = 2 * pp
            a0 = i * (TA // C) + m0
            r0, r1 = brows(a0), brows(a0 + 1)
            b0 = bcol(a0)
            db = bcol(a0 + 1) - b0
            for j in range(NT // 2):
                jl, jr = lanes(j), lanes(NT // 2 + j)
                t1, t2, t3, t4 = (t_v[:, lanes(k * (NT // 2) + j)] for k in range(4))
                p1 = mm(wsp_v[r0, 0:HK], z2_v[0:HK, jl]) + b0
                put(m0, j, p1 + mm(wsp_v[r0, HK:S], z2_v[HK:S, jl]))
                u2 = p1 + mm(s_val(pp, 1), t2)
                u3 = (u2 + db) + mm(s_val(pp, 2), t3)
                put(m0 + 1, j, u3 + mm(wsp_v[r1, HK:S], t4))
                p5 = mm(s_val(pp, 0), t1)
                put(m0 + 1, NT // 2 + j, u3 + p5)
                put(m0, NT // 2 + j, (u2 + p5) + mm(s_val(pp, 3), z2_v[HK:S, jr]))
        def finish(a, dt, hh):
            xg_v[brows(a), lanes(dt)] = xn_gate(a, dt, hh)

        o_pair(i * (TA // C), gl_v, GL0, GS0, finish)
        finish(i * (TA // C) + 2, 4, mm(gl_v[GX0:GX0 + C, :], wout_v[0:FH, lanes(4)]))
        s_sums(jnp.minimum(i + 1, S // TA - 1) * (TA // C), 16, True)
        nft = NB * TA // S
        last = None
        for ft in range(nft):
            for dt in range(ND):
                last = conv_pos(i * nft + ft, i * (nft // 2) + ft // 2, ft % 2, dt, last)
        return carry

    step = pl.program_id(0)

    @pl.when(step == 0)
    def _():
        for grp in groups:
            for cp in grp:
                cp.start()
        cp_wout.start()
        for i in range(S // TA):
            cp_wsp(i).start()
        k_u[:, 0:8, :] = jnp.zeros((ND, 8, 128), U32)

    @pl.when(step == 1)
    def _():
        cp_wsp(0).wait()
        cp_wout.wait()
        for a, dt in [(a, dt) for a in range(NB) for dt in range(ND)][NB * ND - H_LATE:]:
            h_dft(a, dt)
        last = None
        for g in range(C // 16):
            bot = held(z2_v[pl.ds((NB - 1) * C + g * 16, 16), :], None if last is None else fence(last))
            t_rest(NB // 2 - 1, bot.astype(F32), g, 16)
            rows = pl.ds((NB // 2 - 1) * C + g * 16, 16)
            last = jnp.concatenate([words(t_v[rows, lanes(k)]) for k in range(3, 12)], axis=0)
        w_sums(last)
        s_sums(0, 32, False)
        jax.lax.fori_loop(0, S // TA, phase2a, 0)

        rev = 7 - jax.lax.broadcasted_iota(jnp.int32, (8, 128), 0)
        done = {}

        def emit(a, dt, hh):
            rows, cols = brows(a), lanes(dt)
            ev = mm(fg_v[2 * C:2 * C + C // 2, 0:C], w_v[ds(a * 16, 8), :, cols].reshape(C, 128))
            od = mm(fg_v[2 * C:2 * C + C // 2, C:2 * C], w_v[ds(a * 16 + 8, 8), :, cols].reshape(C, 128))
            lo = ev - od
            ys = [jnp.take_along_axis(lo[g * 8:(g + 1) * 8, :], rev, axis=0)
                  for g in range(C // 16 - 1, -1, -1)]
            y = jnp.concatenate(ys + [ev + od], axis=0)
            xg = xg_v[rows, cols] if hh is None else xn_gate(a, dt, hh)
            o_v[rows, cols] = (q_v[rows, cols].astype(F32) + xg * y).astype(BF)
            done[a] = done.get(a, 0) + 1
            if a >= NB - 2:
                cp_o(a, cols).start()
            elif done[a] == ND:
                cp_o(a).start()

        g_sums(gg_v, 0, GS0)
        for k in range(S // TA):
            if k + 1 < S // TA:
                g_sums(gg_v, (k + 1) * 2 * C, GS0 + ((k + 1) % 2) * 2 * C)
            for a in (4 * k, 4 * k + 1):
                for dt in range(ND):
                    emit(a, dt, None)
            o_pair(4 * k + 2, gg_v, k * 2 * C, GS0 + (k % 2) * 2 * C, emit, skip=True)
        pltpu.make_async_copy(o_v, o_hbm, sem_o.at[0]).wait()

    @pl.when(step == 0)
    def _():
        wait(0)
        ln_q(0)
        ln_q(1)
        wait(1)
        for n in (0, 1):
            z2_tile(0, n)
            z2_tile(1, n)
        wait(2)
        ln_q(2)
        for n in (2, 3):
            z2_tile(0, n)
            z2_tile(1, n)
        for n in range(4):
            z2_tile(2, n)
        wait(3)
        ln_q(3)
        seq = ([(z2_tile, a, n) for a in range(3) for n in (4, 5)] + [(z2_tile, 3, n) for n in range(NT)]
               + [(z1_tile, a, 0) for a in range(4)])
        tw_done = tw_sums(NT)
        for j, (tile, a, n) in enumerate(seq):
            if j == 15:
                gate = fence(tw_done)
            elif j == 3:
                gate = fence(words(xn_v[brows(3), 0:128]))
            else:
                gate = fence(z2_words(0, (7, 10).index(j))) if j in (7, 10) else None
            tile(a, n, gate)
            if j == 1:
                ln_z2(0)
        wait(4)
        for a in (1, 2, 3):
            ln_z2(a)
        tw_sums(0)
        release = (8, 10, 11, 12, 13, 15, 16, 17)
        waits = (3, 4, 6, 8, 10, 11)
        for j, (a, n) in enumerate((a, n) for n in range(1, NT) for a in range(4)):
            gate = fence(z2_words(1 + waits.index(j) // 2, waits.index(j) % 2)) if j in waits else None
            t = z1_tile(a, n, gate)
            if j in release:
                part = release.index(j)
                ln_q(4 + part // NLQ, fence(words(t[0:8, :])), part % NLQ, NLQ)
        region([4])
        wait(5)
        b32_v[...] = b_v[...].astype(F32) * 0.25
        assert not region([6, 8, 10], HCH[0], KCH[0])
        wait(6)
        assert len(region([12, 14], HCH[1], KCH[1])) == H_LATE


@jax.jit
def pallas_recurrent_scan__ssm_conv_h3__mixer_gmlp__prompt_kernel(
    A_q: jax.Array,
    A_k: jax.Array,
    A_v: jax.Array,
    A_shift_k: jax.Array,
    A_ssm_k: jax.Array,
    A_ssm_D: jax.Array,
    B_x: jax.Array,
    B_w_in: jax.Array,
    B_w_sp: jax.Array,
    B_b_sp: jax.Array,
    B_w_out: jax.Array,
):
    del B_x
    any_spec = pl.BlockSpec(memory_space=pl.ANY)
    vm = pltpu.VMEM
    dma = pltpu.SemaphoreType.DMA
    out = pl.pallas_call(
        _kernel,
        out_shape=jax.ShapeDtypeStruct((S, D), BF),
        grid=(2,),
        in_specs=[any_spec] * 11,
        out_specs=any_spec,
        scratch_shapes=[
            vm((S // 2, D), U32),
            vm((ND, S // 2 + 32, 128), U32),
            vm((S // 2, D), U32),
            vm(((D + 4 * C) // 2, S), U32),
            vm(((D + 2 * KS) // 2, 2 * FH), U32),
            vm((S // 2, S), U32),
            vm(((FH + 8 * C + 2 * HN) // 2, FH), U32),
            vm(((2 * C + C // 2) // 2, 2 * C), U32),
            vm(((S + 4 * C) // 2, D), U32),
            vm((S + 6 * C, FH), F32),
            vm((S // 2, FH), U32),
            vm((S // 4, 2 * FH), U32),
            vm((NB, NB, 16, D), F32),
            vm((NB, NB, 16, D), F32),
            vm((NB * 16, 8, 1024), U32),
            vm((S // 4, FH), U32),
            vm((S, D), F32),
            vm((S, D), BF),
            vm((NB, 128), F32),
            vm((NB, 128), BF),
            vm((4, 18 * 128), BF),
            vm((ND, 128), BF),
            dma((len(QCH),)), dma((len(KCH) * ND,)), dma((len(KCH),)), dma((len(HCH),)),
            dma((len(WCH),)), dma((S // TA,)), dma((1,)), dma((5,)),
        ],
        compiler_params=pltpu.CompilerParams(
            dimension_semantics=("arbitrary",),
            vmem_limit_bytes=110 * 1024 * 1024,
            disable_bounds_checks=True,
            disable_semaphore_checks=True,
        ),
    )(
        A_q.reshape(S, D), A_k.reshape(S, D), A_v.reshape(S, D),
        A_shift_k.T, A_ssm_k, A_ssm_D.reshape(ND, 128),
        B_w_in, B_w_sp, B_b_sp.reshape(NB, 128), B_w_out,
        _dft_consts(),
    )
    return out.reshape(1, S, D)
```

```python
import math

import jax
import jax.numpy as jnp
import numpy as np
import jax.experimental.pallas as pl
import jax.experimental.pallas.tpu as pltpu

S = 2048
D = 640
FH = 768
C = 128
NB = S // C
ND = D // 128
NT = FH // 128
EPS = 1e-5
HK = S // 2
HN = FH // 2
KS = 256
TA = 512
NOP = 2
NLQ = 4
H_LATE = 24
TREE = 10

BF = jnp.bfloat16
F32 = jnp.float32
U32 = jnp.uint32

QCH = [(0, 2), (2, 1), (3, 1), (4, 4), (8, 6), (14, 2)]
HCH = [(0, 5), (5, 11)]
KCH = [(0, 3), (3, 13)]
WCH = [(6, 2), (8, 2), (10, 2), (0, 1), (1, 5)]
HINTS = {
    4: dict(h=(0, 0, 0), u_run=0, after=(0, 6), stash=7,
             slots=[],
             marks=[('z', 2, 0), ('z', 2, 0), ('z', 2, 0), ('z', 4, 0),
                    ('z', 4, 64), ('z', 6, 0), ('z', 8, 0), ('z', 9, 0)]),
    6: dict(h=(5, 0, 0), u_run=0, after=(0, 6), stash=6,
             slots=[1, 5, 7, 10, 4, 14, 18],
             marks=[('h', 4, 128), ('z', 0, 120), ('z', 1, 120), ('z', 3, 64),
                    ('z', 4, 120), ('z', 5, 120), ('z', 7, 120), ('z', 9, 56)]),
    8: dict(h=(8, 0, 0), u_run=0, after=(2, 6), stash=7,
             slots=[1, 5, 9, 3],
             marks=[('z', 0, 0), ('z', 0, 120), ('z', 1, 56), ('z', 3, 120),
                    ('z', 4, 48), ('z', 5, 120), ('z', 7, 120), ('z', 8, 120)]),
    10: dict(h=(8, 0, 4), u_run=0, after=(1, 6), stash=7,
             slots=[1, 5, 9, 18],
             marks=[('z', 0, 56), ('z', 0, 120), ('z', 1, 120), ('z', 3, 120),
                    ('z', 4, 120), ('z', 6, 64), ('z', 7, 120), ('z', 9, 56)]),
    12: dict(h=(8, 4, 0), u_run=23, after=(1, 6), stash=3,
             slots=[1, 5, 9, 3, 7, 14, 18, 22, 0],
             marks=[('h', 4, 128), ('z', 0, 120), ('z', 2, 56), ('z', 3, 120),
                    ('z', 4, 120), ('z', 5, 48), ('z', 7, 120), ('z', 8, 64)]),
    14: dict(h=(10, 5, 4), u_run=11, after=(0, 6), stash=7,
             slots=[0, 5, 9, 3, 7, 10, 20, 22, 4, 1, 8, 16, 18, 2, 6, 14, 15, 19, 23, 11, 13, 17],
             marks=[]),
}
LNZ_ROWS = [128, 16, 32, 16, 16, 16, 16, 16, 16, 16, 16, 16, 16, 16, 128, 128]


def _dft_consts():
    theta = np.pi * (4 * np.arange(C) + 1) / (2 * C)

    def fwd(t):
        ang = theta[:, None] * t[None, :]
        re = np.cos(ang).reshape(C // 8, 8, C)
        im = -np.sin(ang).reshape(C // 8, 8, C)
        return np.stack([re, im], axis=1).reshape(2 * C, C)

    fg = np.zeros((2 * C + C // 2, 2 * C), np.float64)
    order = np.concatenate([np.arange(0, C, 2), np.arange(1, C, 2)])
    fg[:2 * C, :C] = fwd(order - (C - 1) / 2)
    fg[:2 * C, C:] = fwd(np.arange(C))
    ang = (np.arange(C // 2) + 0.5)[:, None] * theta[None, :]
    fg[2 * C:, :C] = np.cos(ang) / C
    fg[2 * C:, C:] = -np.sin(ang) / C
    return fg.astype(np.float32).astype(BF)


def _kernel(q_hbm, k_hbm, v_hbm, sk_hbm, h_hbm, d_hbm, win_hbm, wsp_hbm, b_hbm, wout_hbm,
            fg_hbm, o_hbm,
            q_u, k_u, v_u, h_u, win_u, wsp_u, wout_u, fg_u,
            xn_u, z1_v, z2_u, t_u, p_v, hf_v, w_u, gg_u, xg_v, o_v, b32_v, b_v, sk_v, d_v,
            sem_q, sem_k, sem_v, sem_h, sem_w, sem_wsp, sem_o, sem_m):
    q_v = q_u.bitcast(BF)
    v_v = v_u.bitcast(BF)
    k_w = k_hbm.bitcast(U32)
    h_v = h_u.bitcast(BF)
    win_v = win_u.bitcast(BF)
    wsp_v = wsp_u.bitcast(BF)
    wout_v = wout_u.bitcast(BF)
    fg_v = fg_u.bitcast(BF)
    xn_v = xn_u.bitcast(BF)
    z2_v = z2_u.bitcast(BF)
    t_v = t_u.bitcast(BF)
    w_v = w_u.bitcast(BF)
    gg_v = gg_u.bitcast(BF)

    def ds(start, size):
        if isinstance(start, int):
            return pl.ds(start, size)
        return pl.ds(pl.multiple_of(start, size), size)

    def lanes(n):
        return slice(n * 128, (n + 1) * 128)

    def blocks(ch):
        return pl.ds(ch[0] * C, ch[1] * C)

    def brows(a):
        return ds(a * C, C)

    def cp_q(c):
        r = blocks(QCH[c])
        return pltpu.make_async_copy(q_hbm.at[r, :], q_v.at[r, :], sem_q.at[c])

    def cp_k(c):
        b0, n = KCH[c]
        return [pltpu.make_async_copy(k_w.at[pl.ds(b0 * C // 2, n * C // 2), lanes(dt)],
                                      k_u.at[dt, pl.ds(b0 * C // 2 + 8, n * C // 2), :],
                                      sem_k.at[c * ND + dt])
                for dt in range(ND)]

    def cp_v(c):
        r = blocks(KCH[c])
        return pltpu.make_async_copy(v_hbm.at[r, :], v_v.at[r, :], sem_v.at[c])

    def cp_h(c):
        r = blocks(HCH[c])
        return pltpu.make_async_copy(h_hbm.at[:, r], h_v.at[0:D, r], sem_h.at[c])

    def cp_w(c):
        r = blocks(WCH[c])
        return pltpu.make_async_copy(win_hbm.at[:, r], win_v.at[0:D, r], sem_w.at[c])

    def cp_wsp(i):
        r = ds(i * TA, TA)
        return pltpu.make_async_copy(wsp_hbm.at[r, :], wsp_v.at[r, :], sem_wsp.at[i])

    def cp_o(a, cols=slice(None)):
        r = brows(a)
        return pltpu.make_async_copy(o_v.at[r, cols], o_hbm.at[r, cols], sem_o.at[0])

    cp_f = pltpu.make_async_copy(fg_hbm, fg_v, sem_m.at[0])
    cp_sk = pltpu.make_async_copy(sk_hbm, sk_v.at[:, 0:D], sem_m.at[1])
    cp_d = pltpu.make_async_copy(d_hbm, d_v, sem_m.at[2])
    cp_b = pltpu.make_async_copy(b_hbm, b_v, sem_m.at[3])
    cp_wout = pltpu.make_async_copy(wout_hbm, wout_v.at[0:FH, 0:D], sem_m.at[4])

    groups = [
        [cp_q(0)], [cp_w(0)], [cp_q(1), cp_w(1)], [cp_q(2), cp_w(2), cp_w(3)], [cp_q(3), cp_w(4)],
        [cp_f, cp_sk, cp_d, cp_b, cp_q(4), cp_h(0), *cp_k(0), cp_v(0)],
        [cp_q(5), cp_h(1), *cp_k(1), cp_v(1)],
    ]

    def wait(g):
        for cp in groups[g]:
            cp.wait()

    def mm(x, y):
        return jnp.dot(x, y, preferred_element_type=F32)

    def words(x):
        return pltpu.bitcast(x, U32)

    def fence(tok):
        t = tok[0:8, :]
        for g in range(1, tok.shape[0] // 8):
            t = t | tok[g * 8:(g + 1) * 8, :]
        return t & k_u[0, 0:8, :]

    def held(x, gate):
        if gate is None:
            return x
        w = words(x)
        return pltpu.bitcast(w | jnp.tile(gate, (w.shape[0] // 8, w.shape[1] // 128)), x.dtype)

    def a_sums(a11, a12, a21, a22):
        s1 = a21 + a22
        s2 = s1 - a11
        return s1, s2, a11 - a21, a12 - s2

    def b_sums(b11, b12, b21, b22):
        t1 = b12 - b11
        t2 = b22 - t1
        return t1, t2, t2 - b11, b21 - t2

    def chain_sums(units, quads, dest, combine, lead, via_memory, last=None, first=0):
        for u in units:
            vals = []
            for n, (ref, idx) in enumerate(quads(u)):
                wait_here = last is not None and (n == lead or not via_memory)
                vals.append(held(ref[idx], fence(last) if wait_here else None).astype(F32))
            sums = combine(*vals)
            done = []
            for k, val in enumerate(sums):
                ref, idx = dest(u, k)
                ref[idx] = val.astype(BF)
                if via_memory and k >= first:
                    done.append(words(ref[idx]))
            last = jnp.concatenate(done, axis=0) if via_memory else words(sums[-1][-8:, :])
        return last

    c0 = math.sqrt(2.0 / math.pi)
    c1 = c0 * 0.044715

    def gelu2(x):
        return x + x * jnp.tanh(x * (c0 + c1 * (x * x)))

    def z2_words(a, half=None):
        r = brows(a) if half is None else pl.ds(a * C + half * (C // 2), C // 2)
        return words(z2_v[r, 0:128])

    def xs_row(a0, k):
        return S + (a0 // 2 % 2) * 2 * C + k // 2 * C

    def ln_q(a, gate=None, part=0, nparts=1):
        n = C // nparts
        r = pl.ds(a * C + part * n, n)
        x = held(q_v[r, :], gate).astype(F32)
        mu = jnp.sum(x, axis=-1, keepdims=True) * (1.0 / D)
        ex2 = jnp.sum(x * x, axis=-1, keepdims=True) * (1.0 / D)
        var = jnp.maximum(ex2 - mu * mu, 0.0)
        mu = mu.astype(BF).astype(F32)
        xn = (x - mu) * jnp.exp(-0.5 * jnp.log(var + EPS))
        xn_v[r, :] = xn.astype(BF)
        if a >= 4 and a % 2 == 1:
            top = xn_v[pl.ds((a - 1) * C + part * n, n), 0:2 * KS].astype(F32)
            s1, s2, s3, s4 = a_sums(top[:, :KS], top[:, KS:], xn[:, :KS], xn[:, KS:2 * KS])
            xn_v[pl.ds(xs_row(a - 1, 0) + part * n, n), 0:2 * KS] = jnp.concatenate([s1, s2], axis=1).astype(BF)
            xn_v[pl.ds(xs_row(a - 1, 2) + part * n, n), 0:2 * KS] = jnp.concatenate([s3, s4], axis=1).astype(BF)

    def h_dft(a, dt):
        res = jax.lax.dot_general(fg_v[0:2 * C, C:2 * C], h_v[lanes(dt), brows(a)],
                                  (((1,), (1,)), ((), ())), preferred_element_type=F32)
        spec = res.reshape(NB, 16, 128)
        if a == 0:
            dv = d_v[...].astype(F32)[dt:dt + 1, :]
            spec = jnp.concatenate([spec[:, 0:8, :] + dv[None], spec[:, 8:16, :]], axis=1)
        hf_v[:, a, :, lanes(dt)] = spec
        return res

    def u_dft(a, dt):
        cols = lanes(dt)

        def even(w):
            return pltpu.bitcast(w << 16, F32)

        def odd(w):
            return pltpu.bitcast(w & jnp.uint32(0xFFFF0000), F32)

        w0, w1, w2 = (k_u[dt, pl.ds(8 + a * C // 2 - j, C // 2), :] for j in range(3))
        e0, o0, e1, o1 = even(w0), odd(w0), even(w1), odd(w1)
        sk = sk_v[:, cols].astype(F32)
        s0, s1, s2, s3 = (sk[j:j + 1, :] for j in range(4))
        vw = words(v_v[brows(a), cols])
        kve = (e0 * s0 + o1 * s1 + e1 * s2 + odd(w2) * s3) * even(vw)
        kvo = (o0 * s0 + e0 * s1 + o1 * s2 + e1 * s3) * odd(vw)
        kv = jnp.concatenate([kve, kvo], axis=0).astype(BF)
        p_v[:, a, :, cols] = mm(fg_v[0:2 * C, 0:C], kv).reshape(NB, 16, 128)

    def proj(a, n, gate=None):
        lhs = xn_v[brows(a), :]
        if gate is not None:
            lhs = jnp.concatenate([held(lhs[0:16, :], gate), lhs[16:, :]], axis=0)
        return gelu2(mm(lhs, win_v[0:D, lanes(n)]))

    def w2_rows(a):
        return pl.ds(S + (a % 4) * C, C)

    def z2_tile(a, n, gate=None):
        z1_v[w2_rows(a), lanes(n)] = proj(a, NT + n, gate)

    def z1_tile(a, n, gate=None):
        t = proj(a, n, gate)
        z1_v[brows(a), lanes(n)] = t
        return t

    def t_rest(r, bot, g=0, nr=C):
        rows = pl.ds(r * C + g * nr, nr)
        t2 = bot[:, HN:] - t_v[rows, 0:HN].astype(F32)
        t3 = t2 - z2_v[rows, 0:HN].astype(F32)
        t_v[rows, HN:4 * HN] = jnp.concatenate([t2, t3, bot[:, :HN] - t2], axis=1).astype(BF)

    def ln_z2(a, last=None):
        w2 = z1_v[w2_rows(a), :]
        mu = jnp.sum(w2, axis=-1, keepdims=True) * (1.0 / FH)
        ex2 = jnp.sum(w2 * w2, axis=-1, keepdims=True) * (1.0 / FH)
        var = jnp.maximum(ex2 - mu * mu, 0.0)
        rs = jnp.exp(-0.5 * jnp.log(16.0 * var + 64.0 * EPS))
        nr = LNZ_ROWS[a]
        for g in range(C // nr):
            rr = slice(g * nr, (g + 1) * nr)
            m = held(jnp.broadcast_to(mu[rr], (nr, 128)), fence(last) if last is not None and nr < C else None)
            zn = (w2[rr] - jnp.tile(m, (1, NT))) * rs[rr]
            rows = pl.ds(a * C + g * nr, nr)
            if a < NB // 2:
                z2_v[rows, 0:HN] = zn[:, :HN].astype(BF)
                t_v[rows, 0:HN] = (zn[:, HN:] - zn[:, :HN]).astype(BF)
                done = [(z2_v, rows, k) for k in range(3)] + [(t_v, rows, k) for k in range(3)]
            else:
                z2_v[rows, :] = zn.astype(BF)
                done = [(z2_v, rows, k) for k in range(6)]
                if a < NB - 1:
                    t_rest(a - NB // 2, zn, g, nr)
                    done += [(t_v, pl.ds((a - NB // 2) * C + g * nr, nr), k) for k in range(3, 12)]
            if nr < C:
                last = jnp.concatenate([words(ref[r, lanes(k)]) for ref, r, k in done], axis=0)
        return last

    def tw_at(base, j, k):
        return D + (base // NT) * KS, lanes(j * 4 + k)

    def tw_sums(base):
        def quads(u):
            j, g = u
            return [(win_v, (slice(r0 + g * 16, r0 + (g + 1) * 16), lanes(n)))
                    for r0 in (0, KS) for n in (base + j, base + 3 + j)]

        def dest(u, k):
            j, g = u
            r0, cols = tw_at(base, j, k)
            return win_v, (slice(r0 + g * 16, r0 + (g + 1) * 16), cols)

        return chain_sums([(j, g) for j in range(3) for g in range(KS // 16)], quads, dest, b_sums, 0, True)

    def group(a0, base, j, hook, gate=None):
        r0, r1 = brows(a0), brows(a0 + 1)
        cl, cr = lanes(base + j), lanes(base + 3 + j)

        def out(a, n, val):
            t = gelu2(val)
            z1_v[w2_rows(a) if base else brows(a), lanes(n)] = t
            hook(t)

        def sx(k):
            return xn_v[xs_row(a0, k):xs_row(a0, k) + C, (k % 2) * KS:(k % 2 + 1) * KS]

        def tw(k):
            t0, cols = tw_at(base, j, k)
            return win_v[t0:t0 + KS, cols]

        def keep(slot, val):
            if not (HINTS[a0]['stash'] >> slot) & 1:
                return lambda: val
            sl = (pl.ds(S + 4 * C + (j % 2) * C, C), lanes(slot))
            z1_v[sl] = val
            return lambda: z1_v[sl]

        a11 = xn_v[r0, 0:KS]
        if gate is not None:
            top = jnp.concatenate([held(a11[0:16, 0:128], gate), a11[0:16, 128:]], axis=1)
            a11 = jnp.concatenate([top, a11[16:, :]], axis=0)
        p1 = keep(0, mm(a11, win_v[0:KS, cl]))
        out(a0, j, p1() + mm(xn_v[r0, KS:D], win_v[KS:D, cl]))
        u2 = keep(1, p1() + mm(sx(1), tw(1)))
        u3 = keep(2, u2() + mm(sx(2), tw(2)))
        out(a0 + 1, j, u3() + mm(xn_v[r1, KS:D], jnp.concatenate([tw(3), win_v[2 * KS:D, cl]], axis=0)))
        p5 = mm(sx(0), tw(0))
        out(a0 + 1, 3 + j, (u3() + p5) + mm(xn_v[r1, 2 * KS:D], win_v[2 * KS:D, cr]))
        out(a0, 3 + j, (u2() + p5) + mm(jnp.concatenate([sx(3), xn_v[r0, 2 * KS:D]], axis=1), win_v[KS:D, cr]))

    def region(pairs, hch=(0, 0), kch=(0, 0)):
        hs = [(a, dt) for a in range(hch[0], hch[0] + hch[1]) for dt in range(ND)]
        us = [(a, dt) for a in range(kch[0], kch[0] + kch[1]) for dt in range(ND)]
        for a0 in pairs:
            nh_mid, nh_run, nh_end = HINTS[a0]['h']
            nu_run = HINTS[a0]['u_run']
            cnt = [HINTS[a0]['slots'].count(j) for j in range(25)]
            marks = HINTS[a0]['marks']
            seen = [0]

            def next_ln_q(part, t):
                tok = words(t)
                for a in (a0, a0 + 1):
                    if part == HINTS[a0]['after'][a - a0]:
                        tok = jnp.concatenate([tok, z2_words(a)], axis=0)
                        if a >= NB // 2:
                            tw_ = words(t_v[brows(a - NB // 2), 4 * HN - 128:4 * HN])
                            tok = jnp.concatenate([tok, tw_], axis=0)
                ln_q(a0 + 2 + part // NLQ, fence(tok), part % NLQ, NLQ)

            def after_z2(t):
                for _ in range(cnt[seen[0]]):
                    u_dft(*us.pop(0))
                seen[0] += 1

            def after_z1(t):
                for part, (kind, idx, row) in enumerate(marks):
                    if kind == 'z' and idx == seen[0]:
                        next_ln_q(part, t[row:row + 8, :])
                for _ in range(cnt[13 + seen[0]]):
                    u_dft(*us.pop(0))
                seen[0] += 1

            for j in range(3):
                group(a0, NT, j, after_z2)
            hres = [h_dft(*hs.pop(0)) for _ in range(nh_mid)]
            for _ in range(cnt[12]):
                u_dft(*us.pop(0))
            ln_z2(a0 + 1, ln_z2(a0))
            for part, (kind, idx, row) in enumerate(marks):
                if kind == 'h':
                    next_ln_q(part, hres[idx][row:row + 8, :])
            seen[0] = 0
            for j in range(3):
                group(a0, 0, j, after_z1, fence(z2_words(a0 + j - 1)) if not marks and j >= 1 else None)
            ru, rh = nu_run, nh_run
            while ru or rh:
                if ru and ru * max(nh_run, 1) >= rh * max(nu_run, 1):
                    u_dft(*us.pop(0))
                    ru -= 1
                else:
                    h_dft(*hs.pop(0))
                    rh -= 1
            for _ in range(nh_end):
                h_dft(*hs.pop(0))
        assert not us
        return hs

    def conv_pos(ft, ft2, par, dt, after):
        cols = lanes(dt)
        prev = None
        for a in range(NB):
            ar, ai = (None, None) if prev is None else (-prev[1], prev[0])
            for dl in range(a + 1):
                hr = hf_v[ft, dl, 0:8, cols]
                hi = hf_v[ft, dl, 8:16, cols]
                ur = p_v[ft, a - dl, 0:8, cols]
                ui = p_v[ft, a - dl, 8:16, cols]
                if ar is None:
                    ar, ai = ur * hr - ui * hi, ur * hi + ui * hr
                    if after is not None:
                        z = fence(after)
                        ar, ai = held(ar, z), held(ai, z)
                elif (a * (a + 1) // 2 + dl) % TREE == 0:
                    ar = ar + (ur * hr - ui * hi)
                    ai = ai + (ur * hi + ui * hr)
                else:
                    ar = (ar + ur * hr) - ui * hi
                    ai = (ai + ur * hi) + ui * hr
            prev = (ar, ai) if prev is None else (ar + prev[1], ai - prev[0])
            w_v[a * 16 + ft2, par * 8:(par + 1) * 8, cols] = ar.astype(BF)
            w_v[a * 16 + 8 + ft2, par * 8:(par + 1) * 8, cols] = ai.astype(BF)
        return words(prev[0])

    gl_v = wout_v
    GL0 = FH
    GS0 = GL0 + NOP * C
    WS0 = GS0 + 4 * C
    GX0 = WS0 + 2 * HN

    def g_sums(ref, g0, s0):
        def quads(u):
            c, g = u
            return [(ref, (pl.ds(g0 + m * C + g * 16, 16), lanes(n))) for m in (0, 1) for n in (c, 3 + c)]

        def dest(u, k):
            c, g = u
            return gl_v, (pl.ds(s0 + k // 2 * C + g * 16, 16), lanes(k % 2 * 3 + c))

        units = [(c, g) for c in range(3) for g in range(C // 16)]
        chain_sums(units, quads, dest, a_sums, 2, True, first=2 if ref is gl_v else 0)

    def ws_at(jj, k):
        return WS0 + (jj * 4 + k) // 6 * HN, lanes((jj * 4 + k) % 6)

    def w_sums(after):
        def quads(u):
            jj, g = u
            return [(wout_v, (pl.ds(r0 + g * 16, 16), lanes(n))) for r0 in (0, HN) for n in (jj, 2 + jj)]

        def dest(u, k):
            jj, g = u
            r0, cols = ws_at(jj, k)
            return wout_v, (pl.ds(r0 + g * 16, 16), cols)

        chain_sums([(jj, g) for jj in range(2) for g in range(HN // 16)], quads, dest, b_sums, 0, False, after)

    def xn_gate(a, dt, hh):
        return xn_v[brows(a), lanes(dt)].astype(F32) * (hh + hh * jnp.tanh(hh))

    def o_pair(a0, ref, g0, s0, finish, skip=False):
        r0, r1 = pl.ds(g0, C), pl.ds(g0 + C, C)

        def gs(k):
            return gl_v[pl.ds(s0 + k // 2 * C, C), (k % 2) * HN:(k % 2 + 1) * HN]

        def ws(jj, k):
            r, cols = ws_at(jj, k)
            return wout_v[r:r + HN, cols]

        for jj in range(2):
            if jj == (0 if skip else 1):
                finish(a0, 4, None if skip else mm(ref[r0, :], wout_v[0:FH, lanes(4)]))
                finish(a0 + 1, 4, mm(ref[r1, :], wout_v[0:FH, lanes(4)]))
            p1 = mm(ref[r0, 0:HN], wout_v[0:HN, lanes(jj)])
            finish(a0, jj, p1 + mm(ref[r0, HN:FH], wout_v[HN:FH, lanes(jj)]))
            u2 = p1 + mm(gs(1), ws(jj, 1))
            u3 = u2 + mm(gs(2), ws(jj, 2))
            finish(a0 + 1, jj, u3 + mm(ref[r1, HN:FH], ws(jj, 3)))
            p5 = mm(gs(0), ws(jj, 0))
            finish(a0 + 1, 2 + jj, u3 + p5)
            finish(a0, 2 + jj, (u2 + p5) + mm(gs(3), wout_v[HN:FH, lanes(2 + jj)]))

    def s_at(slot, k):
        return D + (slot * 2 + k // 2) * C, (k % 2) * HK

    def s_val(slot, k):
        r0, col = s_at(slot, k)
        return h_v[r0:r0 + C, col:col + HK]

    def s_sums(a0, nr, via_memory):
        def quads(u):
            slot, c, g = u
            return [(wsp_v, (ds((a0 + 2 * slot + m) * C + g * nr, nr), lanes(n)))
                    for m in (0, 1) for n in (c, HK // 128 + c)]

        def dest(u, k):
            slot, c, g = u
            r0, col = s_at(slot, k)
            return h_v, (slice(r0 + g * nr, r0 + (g + 1) * nr), slice(col + c * 128, col + (c + 1) * 128))

        units = [(slot, c, g) for slot in range(2) for c in range(HK // 128) for g in range(C // nr)]
        for part in (units[:56], units[56:]) if via_memory else (units,):
            chain_sums(part, quads, dest, a_sums, 2, via_memory, first=2)

    def phase2a(i, carry):
        @pl.when(i + 1 < S // TA)
        def _():
            cp_wsp(i + 1).wait()

        eye = (jax.lax.broadcasted_iota(jnp.int32, (C, C), 0)
               == jax.lax.broadcasted_iota(jnp.int32, (C, C), 1))

        def bcol(a):
            return jnp.sum(jnp.where(eye, b32_v[pl.ds(a, 1), :], 0.0), axis=-1, keepdims=True)

        def put(m, n, g):
            g = (z1_v[brows(i * (TA // C) + m), lanes(n)] * g).astype(BF)
            if m < NOP:
                gl_v[GL0 + m * C:GL0 + (m + 1) * C, lanes(n)] = g
            else:
                gg_v[ds((2 * i + m - NOP) * C, C), lanes(n)] = g
                if m == NOP:
                    gl_v[GX0:GX0 + C, lanes(n)] = g

        for pp in range(2):
            if pp == 1:
                g_sums(gl_v, GL0, GS0)
            m0 = 2 * pp
            a0 = i * (TA // C) + m0
            r0, r1 = brows(a0), brows(a0 + 1)
            b0 = bcol(a0)
            db = bcol(a0 + 1) - b0
            for j in range(NT // 2):
                jl, jr = lanes(j), lanes(NT // 2 + j)
                t1, t2, t3, t4 = (t_v[:, lanes(k * (NT // 2) + j)] for k in range(4))
                p1 = mm(wsp_v[r0, 0:HK], z2_v[0:HK, jl]) + b0
                put(m0, j, p1 + mm(wsp_v[r0, HK:S], z2_v[HK:S, jl]))
                u2 = p1 + mm(s_val(pp, 1), t2)
                u3 = (u2 + db) + mm(s_val(pp, 2), t3)
                put(m0 + 1, j, u3 + mm(wsp_v[r1, HK:S], t4))
                p5 = mm(s_val(pp, 0), t1)
                put(m0 + 1, NT // 2 + j, u3 + p5)
                put(m0, NT // 2 + j, (u2 + p5) + mm(s_val(pp, 3), z2_v[HK:S, jr]))
        def finish(a, dt, hh):
            xg_v[brows(a), lanes(dt)] = xn_gate(a, dt, hh)

        o_pair(i * (TA // C), gl_v, GL0, GS0, finish)
        finish(i * (TA // C) + 2, 4, mm(gl_v[GX0:GX0 + C, :], wout_v[0:FH, lanes(4)]))
        s_sums(jnp.minimum(i + 1, S // TA - 1) * (TA // C), 16, True)
        nft = NB * TA // S
        last = None
        for ft in range(nft):
            for dt in range(ND):
                last = conv_pos(i * nft + ft, i * (nft // 2) + ft // 2, ft % 2, dt, last)
        return carry

    step = pl.program_id(0)

    @pl.when(step == 0)
    def _():
        for grp in groups:
            for cp in grp:
                cp.start()
        cp_wout.start()
        for i in range(S // TA):
            cp_wsp(i).start()
        k_u[:, 0:8, :] = jnp.zeros((ND, 8, 128), U32)

    @pl.when(step == 1)
    def _():
        cp_wsp(0).wait()
        cp_wout.wait()
        for a, dt in [(a, dt) for a in range(NB) for dt in range(ND)][NB * ND - H_LATE:]:
            h_dft(a, dt)
        last = None
        for g in range(C // 16):
            bot = held(z2_v[pl.ds((NB - 1) * C + g * 16, 16), :], None if last is None else fence(last))
            t_rest(NB // 2 - 1, bot.astype(F32), g, 16)
            rows = pl.ds((NB // 2 - 1) * C + g * 16, 16)
            last = jnp.concatenate([words(t_v[rows, lanes(k)]) for k in range(3, 12)], axis=0)
        w_sums(last)
        s_sums(0, 32, False)
        jax.lax.fori_loop(0, S // TA, phase2a, 0)

        rev = 7 - jax.lax.broadcasted_iota(jnp.int32, (8, 128), 0)
        done = {}

        def emit(a, dt, hh):
            rows, cols = brows(a), lanes(dt)
            ev = mm(fg_v[2 * C:2 * C + C // 2, 0:C], w_v[ds(a * 16, 8), :, cols].reshape(C, 128))
            od = mm(fg_v[2 * C:2 * C + C // 2, C:2 * C], w_v[ds(a * 16 + 8, 8), :, cols].reshape(C, 128))
            lo = ev - od
            ys = [jnp.take_along_axis(lo[g * 8:(g + 1) * 8, :], rev, axis=0)
                  for g in range(C // 16 - 1, -1, -1)]
            y = jnp.concatenate(ys + [ev + od], axis=0)
            xg = xg_v[rows, cols] if hh is None else xn_gate(a, dt, hh)
            o_v[rows, cols] = (q_v[rows, cols].astype(F32) + xg * y).astype(BF)
            done[a] = done.get(a, 0) + 1
            if a >= NB - 2:
                cp_o(a, cols).start()
            elif done[a] == ND:
                cp_o(a).start()

        g_sums(gg_v, 0, GS0)
        for k in range(S // TA):
            if k + 1 < S // TA:
                g_sums(gg_v, (k + 1) * 2 * C, GS0 + ((k + 1) % 2) * 2 * C)
            for a in (4 * k, 4 * k + 1):
                for dt in range(ND):
                    emit(a, dt, None)
            o_pair(4 * k + 2, gg_v, k * 2 * C, GS0 + (k % 2) * 2 * C, emit, skip=True)
        pltpu.make_async_copy(o_v, o_hbm, sem_o.at[0]).wait()

    @pl.when(step == 0)
    def _():
        wait(0)
        ln_q(0)
        ln_q(1)
        wait(1)
        for n in (0, 1):
            z2_tile(0, n)
            z2_tile(1, n)
        wait(2)
        ln_q(2)
        for n in (2, 3):
            z2_tile(0, n)
            z2_tile(1, n)
        for n in range(4):
            z2_tile(2, n)
        wait(3)
        ln_q(3)
        seq = ([(z2_tile, a, n) for a in range(3) for n in (4, 5)] + [(z2_tile, 3, n) for n in range(NT)]
               + [(z1_tile, a, 0) for a in range(4)])
        tw_done = tw_sums(NT)
        for j, (tile, a, n) in enumerate(seq):
            if j == 15:
                gate = fence(tw_done)
            elif j == 3:
                gate = fence(words(xn_v[brows(3), 0:128]))
            else:
                gate = fence(z2_words(0, (7, 10).index(j))) if j in (7, 10) else None
            tile(a, n, gate)
            if j == 1:
                ln_z2(0)
        wait(4)
        for a in (1, 2, 3):
            ln_z2(a)
        tw_sums(0)
        release = (8, 10, 11, 12, 13, 15, 16, 17)
        waits = (3, 4, 6, 8, 10, 11)
        for j, (a, n) in enumerate((a, n) for n in range(1, NT) for a in range(4)):
            gate = fence(z2_words(1 + waits.index(j) // 2, waits.index(j) % 2)) if j in waits else None
            t = z1_tile(a, n, gate)
            if j in release:
                part = release.index(j)
                ln_q(4 + part // NLQ, fence(words(t[0:8, :])), part % NLQ, NLQ)
        region([4])
        wait(5)
        b32_v[...] = b_v[...].astype(F32) * 0.25
        assert not region([6, 8, 10], HCH[0], KCH[0])
        wait(6)
        assert len(region([12, 14], HCH[1], KCH[1])) == H_LATE


@jax.jit
def pallas_recurrent_scan__ssm_conv_h3__mixer_gmlp__prompt_kernel(
    A_q: jax.Array,
    A_k: jax.Array,
    A_v: jax.Array,
    A_shift_k: jax.Array,
    A_ssm_k: jax.Array,
    A_ssm_D: jax.Array,
    B_x: jax.Array,
    B_w_in: jax.Array,
    B_w_sp: jax.Array,
    B_b_sp: jax.Array,
    B_w_out: jax.Array,
):
    del B_x
    any_spec = pl.BlockSpec(memory_space=pl.ANY)
    vm = pltpu.VMEM
    dma = pltpu.SemaphoreType.DMA
    out = pl.pallas_call(
        _kernel,
        out_shape=jax.ShapeDtypeStruct((S, D), BF),
        grid=(2,),
        in_specs=[any_spec] * 11,
        out_specs=any_spec,
        scratch_shapes=[
            vm((S // 2, D), U32),
            vm((ND, S // 2 + 32, 128), U32),
            vm((S // 2, D), U32),
            vm(((D + 4 * C) // 2, S), U32),
            vm(((D + 2 * KS) // 2, 2 * FH), U32),
            vm((S // 2, S), U32),
            vm(((FH + 8 * C + 2 * HN) // 2, FH), U32),
            vm(((2 * C + C // 2) // 2, 2 * C), U32),
            vm(((S + 4 * C) // 2, D), U32),
            vm((S + 6 * C, FH), F32),
            vm((S // 2, FH), U32),
            vm((S // 4, 2 * FH), U32),
            vm((NB, NB, 16, D), F32),
            vm((NB, NB, 16, D), F32),
            vm((NB * 16, 8, 1024), U32),
            vm((S // 4, FH), U32),
            vm((S, D), F32),
            vm((S, D), BF),
            vm((NB, 128), F32),
            vm((NB, 128), BF),
            vm((4, 18 * 128), BF),
            vm((ND, 128), BF),
            dma((len(QCH),)), dma((len(KCH) * ND,)), dma((len(KCH),)), dma((len(HCH),)),
            dma((len(WCH),)), dma((S // TA,)), dma((1,)), dma((5,)),
        ],
        compiler_params=pltpu.CompilerParams(
            dimension_semantics=("arbitrary",),
            vmem_limit_bytes=110 * 1024 * 1024,
            disable_bounds_checks=True,
            disable_semaphore_checks=True,
        ),
    )(
        A_q.reshape(S, D), A_k.reshape(S, D), A_v.reshape(S, D),
        A_shift_k.T, A_ssm_k, A_ssm_D.reshape(ND, 128),
        B_w_in, B_w_sp, B_b_sp.reshape(NB, 128), B_w_out,
        _dft_consts(),
    )
    return out.reshape(1, S, D)
```

```python
import math

import jax
import jax.numpy as jnp
import numpy as np
import jax.experimental.pallas as pl
import jax.experimental.pallas.tpu as pltpu

S = 2048
D = 640
FH = 768
C = 128
NB = S // C
ND = D // 128
NT = FH // 128
EPS = 1e-5
HK = S // 2
HN = FH // 2
KS = 256
TA = 512
NOP = 2
NLQ = 4
H_LATE = 24
TREE = 10

BF = jnp.bfloat16
F32 = jnp.float32
U32 = jnp.uint32

QCH = [(0, 2), (2, 1), (3, 1), (4, 4), (8, 6), (14, 2)]
HCH = [(0, 5), (5, 11)]
KCH = [(0, 3), (3, 13)]
WCH = [(6, 2), (8, 2), (10, 2), (0, 1), (1, 5)]
HINTS = {
    4: dict(h=(0, 0, 0), u_run=0, after=(0, 6), stash=7,
             slots=[],
             marks=[('z', 2, 0), ('z', 2, 0), ('z', 2, 0), ('z', 4, 0),
                    ('z', 4, 64), ('z', 6, 64), ('z', 8, 0), ('z', 9, 0)]),
    6: dict(h=(5, 0, 0), u_run=0, after=(0, 6), stash=6,
             slots=[1, 5, 7, 10, 4, 14, 18],
             marks=[('h', 4, 128), ('z', 0, 120), ('z', 1, 120), ('z', 3, 64),
                    ('z', 4, 120), ('z', 5, 120), ('z', 7, 120), ('z', 9, 56)]),
    8: dict(h=(8, 0, 0), u_run=0, after=(2, 6), stash=7,
             slots=[1, 5, 9, 3],
             marks=[('z', 0, 0), ('z', 0, 120), ('z', 1, 56), ('z', 3, 120),
                    ('z', 4, 48), ('z', 5, 120), ('z', 7, 120), ('z', 8, 120)]),
    10: dict(h=(8, 0, 4), u_run=0, after=(1, 6), stash=2,
             slots=[11, 5, 9, 18],
             marks=[('z', 0, 56), ('z', 0, 120), ('z', 1, 120), ('z', 3, 120),
                    ('z', 4, 120), ('z', 6, 64), ('z', 7, 120), ('z', 9, 56)]),
    12: dict(h=(8, 4, 0), u_run=23, after=(1, 6), stash=3,
             slots=[1, 5, 9, 3, 7, 14, 18, 22, 0],
             marks=[('h', 4, 128), ('z', 0, 120), ('z', 2, 56), ('z', 3, 120),
                    ('z', 4, 120), ('z', 5, 48), ('z', 7, 120), ('z', 8, 64)]),
    14: dict(h=(10, 5, 4), u_run=11, after=(0, 6), stash=7,
             slots=[0, 5, 9, 3, 7, 10, 20, 22, 4, 1, 8, 16, 18, 2, 6, 14, 15, 19, 23, 11, 13, 17],
             marks=[]),
}
LNZ_ROWS = [128, 16, 32, 16, 16, 16, 16, 16, 16, 16, 16, 16, 16, 16, 16, 16]


def _dft_consts():
    theta = np.pi * (4 * np.arange(C) + 1) / (2 * C)

    def fwd(t):
        ang = theta[:, None] * t[None, :]
        re = np.cos(ang).reshape(C // 8, 8, C)
        im = -np.sin(ang).reshape(C // 8, 8, C)
        return np.stack([re, im], axis=1).reshape(2 * C, C)

    fg = np.zeros((2 * C + C // 2, 2 * C), np.float64)
    order = np.concatenate([np.arange(0, C, 2), np.arange(1, C, 2)])
    fg[:2 * C, :C] = fwd(order - (C - 1) / 2)
    fg[:2 * C, C:] = fwd(np.arange(C))
    ang = (np.arange(C // 2) + 0.5)[:, None] * theta[None, :]
    fg[2 * C:, :C] = np.cos(ang) / C
    fg[2 * C:, C:] = -np.sin(ang) / C
    return fg.astype(np.float32).astype(BF)


def _kernel(q_hbm, k_hbm, v_hbm, sk_hbm, h_hbm, d_hbm, win_hbm, wsp_hbm, b_hbm, wout_hbm,
            fg_hbm, o_hbm,
            q_u, k_u, v_u, h_u, win_u, wsp_u, wout_u, fg_u,
            xn_u, z1_v, z2_u, t_u, p_v, hf_v, w_u, gg_u, xg_v, o_v, b32_v, b_v, sk_v, d_v,
            sem_q, sem_k, sem_v, sem_h, sem_w, sem_wsp, sem_o, sem_m):
    q_v = q_u.bitcast(BF)
    v_v = v_u.bitcast(BF)
    k_w = k_hbm.bitcast(U32)
    h_v = h_u.bitcast(BF)
    win_v = win_u.bitcast(BF)
    wsp_v = wsp_u.bitcast(BF)
    wout_v = wout_u.bitcast(BF)
    fg_v = fg_u.bitcast(BF)
    xn_v = xn_u.bitcast(BF)
    z2_v = z2_u.bitcast(BF)
    t_v = t_u.bitcast(BF)
    w_v = w_u.bitcast(BF)
    gg_v = gg_u.bitcast(BF)

    def ds(start, size):
        if isinstance(start, int):
            return pl.ds(start, size)
        return pl.ds(pl.multiple_of(start, size), size)

    def lanes(n):
        return slice(n * 128, (n + 1) * 128)

    def blocks(ch):
        return pl.ds(ch[0] * C, ch[1] * C)

    def brows(a):
        return ds(a * C, C)

    def cp_q(c):
        r = blocks(QCH[c])
        return pltpu.make_async_copy(q_hbm.at[r, :], q_v.at[r, :], sem_q.at[c])

    def cp_k(c):
        b0, n = KCH[c]
        return [pltpu.make_async_copy(k_w.at[pl.ds(b0 * C // 2, n * C // 2), lanes(dt)],
                                      k_u.at[dt, pl.ds(b0 * C // 2 + 8, n * C // 2), :],
                                      sem_k.at[c * ND + dt])
                for dt in range(ND)]

    def cp_v(c):
        r = blocks(KCH[c])
        return pltpu.make_async_copy(v_hbm.at[r, :], v_v.at[r, :], sem_v.at[c])

    def cp_h(c):
        r = blocks(HCH[c])
        return pltpu.make_async_copy(h_hbm.at[:, r], h_v.at[0:D, r], sem_h.at[c])

    def cp_w(c):
        r = blocks(WCH[c])
        return pltpu.make_async_copy(win_hbm.at[:, r], win_v.at[0:D, r], sem_w.at[c])

    def cp_wsp(i):
        r = ds(i * TA, TA)
        return pltpu.make_async_copy(wsp_hbm.at[r, :], wsp_v.at[r, :], sem_wsp.at[i])

    def cp_o(a, cols=slice(None)):
        r = brows(a)
        return pltpu.make_async_copy(o_v.at[r, cols], o_hbm.at[r, cols], sem_o.at[0])

    cp_f = pltpu.make_async_copy(fg_hbm, fg_v, sem_m.at[0])
    cp_sk = pltpu.make_async_copy(sk_hbm, sk_v.at[:, 0:D], sem_m.at[1])
    cp_d = pltpu.make_async_copy(d_hbm, d_v, sem_m.at[2])
    cp_b = pltpu.make_async_copy(b_hbm, b_v, sem_m.at[3])
    cp_wout = pltpu.make_async_copy(wout_hbm, wout_v.at[0:FH, 0:D], sem_m.at[4])

    groups = [
        [cp_q(0)], [cp_w(0)], [cp_q(1), cp_w(1)], [cp_q(2), cp_w(2), cp_w(3)], [cp_q(3), cp_w(4)],
        [cp_f, cp_sk, cp_d, cp_b, cp_q(4), cp_h(0), *cp_k(0), cp_v(0)],
        [cp_q(5), cp_h(1), *cp_k(1), cp_v(1)],
    ]

    def wait(g):
        for cp in groups[g]:
            cp.wait()

    def mm(x, y):
        return jnp.dot(x, y, preferred_element_type=F32)

    def words(x):
        return pltpu.bitcast(x, U32)

    def fence(tok):
        t = tok[0:8, :]
        for g in range(1, tok.shape[0] // 8):
            t = t | tok[g * 8:(g + 1) * 8, :]
        return t & k_u[0, 0:8, :]

    def held(x, gate):
        if gate is None:
            return x
        w = words(x)
        return pltpu.bitcast(w | jnp.tile(gate, (w.shape[0] // 8, w.shape[1] // 128)), x.dtype)

    def a_sums(a11, a12, a21, a22):
        s1 = a21 + a22
        s2 = s1 - a11
        return s1, s2, a11 - a21, a12 - s2

    def b_sums(b11, b12, b21, b22):
        t1 = b12 - b11
        t2 = b22 - t1
        return t1, t2, t2 - b11, b21 - t2

    def chain_sums(units, quads, dest, combine, lead, via_memory, last=None, first=0):
        for u in units:
            vals = []
            for n, (ref, idx) in enumerate(quads(u)):
                wait_here = last is not None and (n == lead or not via_memory)
                vals.append(held(ref[idx], fence(last) if wait_here else None).astype(F32))
            sums = combine(*vals)
            done = []
            for k, val in enumerate(sums):
                ref, idx = dest(u, k)
                ref[idx] = val.astype(BF)
                if via_memory and k >= first:
                    done.append(words(ref[idx]))
            last = jnp.concatenate(done, axis=0) if via_memory else words(sums[-1][-8:, :])
        return last

    c0 = math.sqrt(2.0 / math.pi)
    c1 = c0 * 0.044715

    def gelu2(x):
        return x + x * jnp.tanh(x * (c0 + c1 * (x * x)))

    def z2_words(a, half=None):
        r = brows(a) if half is None else pl.ds(a * C + half * (C // 2), C // 2)
        return words(z2_v[r, 0:128])

    def xs_row(a0, k):
        return S + (a0 // 2 % 2) * 2 * C + k // 2 * C

    def ln_q(a, gate=None, part=0, nparts=1):
        n = C // nparts
        r = pl.ds(a * C + part * n, n)
        x = held(q_v[r, :], gate).astype(F32)
        mu = jnp.sum(x, axis=-1, keepdims=True) * (1.0 / D)
        ex2 = jnp.sum(x * x, axis=-1, keepdims=True) * (1.0 / D)
        var = jnp.maximum(ex2 - mu * mu, 0.0)
        mu = mu.astype(BF).astype(F32)
        xn = (x - mu) * jnp.exp(-0.5 * jnp.log(var + EPS))
        xn_v[r, :] = xn.astype(BF)
        if a >= 4 and a % 2 == 1:
            top = xn_v[pl.ds((a - 1) * C + part * n, n), 0:2 * KS].astype(F32)
            s1, s2, s3, s4 = a_sums(top[:, :KS], top[:, KS:], xn[:, :KS], xn[:, KS:2 * KS])
            xn_v[pl.ds(xs_row(a - 1, 0) + part * n, n), 0:2 * KS] = jnp.concatenate([s1, s2], axis=1).astype(BF)
            xn_v[pl.ds(xs_row(a - 1, 2) + part * n, n), 0:2 * KS] = jnp.concatenate([s3, s4], axis=1).astype(BF)

    def h_dft(a, dt):
        res = jax.lax.dot_general(fg_v[0:2 * C, C:2 * C], h_v[lanes(dt), brows(a)],
                                  (((1,), (1,)), ((), ())), preferred_element_type=F32)
        spec = res.reshape(NB, 16, 128)
        if a == 0:
            dv = d_v[...].astype(F32)[dt:dt + 1, :]
            spec = jnp.concatenate([spec[:, 0:8, :] + dv[None], spec[:, 8:16, :]], axis=1)
        hf_v[:, a, :, lanes(dt)] = spec
        return res

    def u_dft(a, dt):
        cols = lanes(dt)

        def even(w):
            return pltpu.bitcast(w << 16, F32)

        def odd(w):
            return pltpu.bitcast(w & jnp.uint32(0xFFFF0000), F32)

        w0, w1, w2 = (k_u[dt, pl.ds(8 + a * C // 2 - j, C // 2), :] for j in range(3))
        e0, o0, e1, o1 = even(w0), odd(w0), even(w1), odd(w1)
        sk = sk_v[:, cols].astype(F32)
        s0, s1, s2, s3 = (sk[j:j + 1, :] for j in range(4))
        vw = words(v_v[brows(a), cols])
        kve = (e0 * s0 + o1 * s1 + e1 * s2 + odd(w2) * s3) * even(vw)
        kvo = (o0 * s0 + e0 * s1 + o1 * s2 + e1 * s3) * odd(vw)
        kv = jnp.concatenate([kve, kvo], axis=0).astype(BF)
        p_v[:, a, :, cols] = mm(fg_v[0:2 * C, 0:C], kv).reshape(NB, 16, 128)

    def proj(a, n, gate=None):
        lhs = xn_v[brows(a), :]
        if gate is not None:
            lhs = jnp.concatenate([held(lhs[0:16, :], gate), lhs[16:, :]], axis=0)
        return gelu2(mm(lhs, win_v[0:D, lanes(n)]))

    def w2_rows(a):
        return pl.ds(S + (a % 4) * C, C)

    def z2_tile(a, n, gate=None):
        z1_v[w2_rows(a), lanes(n)] = proj(a, NT + n, gate)

    def z1_tile(a, n, gate=None):
        t = proj(a, n, gate)
        z1_v[brows(a), lanes(n)] = t
        return t

    def t_rest(r, bot, g=0, nr=C):
        rows = pl.ds(r * C + g * nr, nr)
        t2 = bot[:, HN:] - t_v[rows, 0:HN].astype(F32)
        t3 = t2 - z2_v[rows, 0:HN].astype(F32)
        t_v[rows, HN:4 * HN] = jnp.concatenate([t2, t3, bot[:, :HN] - t2], axis=1).astype(BF)

    def ln_z2(a, last=None):
        w2 = z1_v[w2_rows(a), :]
        mu = jnp.sum(w2, axis=-1, keepdims=True) * (1.0 / FH)
        ex2 = jnp.sum(w2 * w2, axis=-1, keepdims=True) * (1.0 / FH)
        var = jnp.maximum(ex2 - mu * mu, 0.0)
        rs = jnp.exp(-0.5 * jnp.log(16.0 * var + 64.0 * EPS))
        nr = LNZ_ROWS[a]
        for g in range(C // nr):
            rr = slice(g * nr, (g + 1) * nr)
            m = held(jnp.broadcast_to(mu[rr], (nr, 128)), fence(last) if last is not None and nr < C else None)
            zn = (w2[rr] - jnp.tile(m, (1, NT))) * rs[rr]
            rows = pl.ds(a * C + g * nr, nr)
            if a < NB // 2:
                z2_v[rows, 0:HN] = zn[:, :HN].astype(BF)
                t_v[rows, 0:HN] = (zn[:, HN:] - zn[:, :HN]).astype(BF)
                done = [(z2_v, rows, k) for k in range(3)] + [(t_v, rows, k) for k in range(3)]
            else:
                z2_v[rows, :] = zn.astype(BF)
                done = [(z2_v, rows, k) for k in range(6)]
                if a < NB - 1:
                    t_rest(a - NB // 2, zn, g, nr)
                    done += [(t_v, pl.ds((a - NB // 2) * C + g * nr, nr), k) for k in range(3, 12)]
            if nr < C:
                last = jnp.concatenate([words(ref[r, lanes(k)]) for ref, r, k in done], axis=0)
        return last

    def tw_at(base, j, k):
        return D + (base // NT) * KS, lanes(j * 4 + k)

    def tw_sums(base):
        def quads(u):
            j, g = u
            return [(win_v, (slice(r0 + g * 16, r0 + (g + 1) * 16), lanes(n)))
                    for r0 in (0, KS) for n in (base + j, base + 3 + j)]

        def dest(u, k):
            j, g = u
            r0, cols = tw_at(base, j, k)
            return win_v, (slice(r0 + g * 16, r0 + (g + 1) * 16), cols)

        return chain_sums([(j, g) for j in range(3) for g in range(KS // 16)], quads, dest, b_sums, 0, True)

    def group(a0, base, j, hook, gate=None):
        r0, r1 = brows(a0), brows(a0 + 1)
        cl, cr = lanes(base + j), lanes(base + 3 + j)

        def out(a, n, val):
            t = gelu2(val)
            z1_v[w2_rows(a) if base else brows(a), lanes(n)] = t
            hook(t)

        def sx(k):
            return xn_v[xs_row(a0, k):xs_row(a0, k) + C, (k % 2) * KS:(k % 2 + 1) * KS]

        def tw(k):
            t0, cols = tw_at(base, j, k)
            return win_v[t0:t0 + KS, cols]

        def keep(slot, val):
            if not (HINTS[a0]['stash'] >> slot) & 1:
                return lambda: val
            sl = (pl.ds(S + 4 * C + (j % 2) * C, C), lanes(slot))
            z1_v[sl] = val
            return lambda: z1_v[sl]

        a11 = xn_v[r0, 0:KS]
        if gate is not None:
            top = jnp.concatenate([held(a11[0:16, 0:128], gate), a11[0:16, 128:]], axis=1)
            a11 = jnp.concatenate([top, a11[16:, :]], axis=0)
        p1 = keep(0, mm(a11, win_v[0:KS, cl]))
        out(a0, j, p1() + mm(xn_v[r0, KS:D], win_v[KS:D, cl]))
        u2 = keep(1, p1() + mm(sx(1), tw(1)))
        u3 = keep(2, u2() + mm(sx(2), tw(2)))
        out(a0 + 1, j, u3() + mm(xn_v[r1, KS:D], jnp.concatenate([tw(3), win_v[2 * KS:D, cl]], axis=0)))
        p5 = mm(sx(0), tw(0))
        out(a0 + 1, 3 + j, (u3() + p5) + mm(xn_v[r1, 2 * KS:D], win_v[2 * KS:D, cr]))
        out(a0, 3 + j, (u2() + p5) + mm(jnp.concatenate([sx(3), xn_v[r0, 2 * KS:D]], axis=1), win_v[KS:D, cr]))

    def region(pairs, hch=(0, 0), kch=(0, 0)):
        hs = [(a, dt) for a in range(hch[0], hch[0] + hch[1]) for dt in range(ND)]
        us = [(a, dt) for a in range(kch[0], kch[0] + kch[1]) for dt in range(ND)]
        for a0 in pairs:
            nh_mid, nh_run, nh_end = HINTS[a0]['h']
            nu_run = HINTS[a0]['u_run']
            cnt = [HINTS[a0]['slots'].count(j) for j in range(25)]
            marks = HINTS[a0]['marks']
            seen = [0]

            def next_ln_q(part, t):
                tok = words(t)
                for a in (a0, a0 + 1):
                    if part == HINTS[a0]['after'][a - a0]:
                        tok = jnp.concatenate([tok, z2_words(a)], axis=0)
                        if a >= NB // 2:
                            tw_ = words(t_v[brows(a - NB // 2), 4 * HN - 128:4 * HN])
                            tok = jnp.concatenate([tok, tw_], axis=0)
                ln_q(a0 + 2 + part // NLQ, fence(tok), part % NLQ, NLQ)

            def after_z2(t):
                for _ in range(cnt[seen[0]]):
                    u_dft(*us.pop(0))
                seen[0] += 1

            def after_z1(t):
                for part, (kind, idx, row) in enumerate(marks):
                    if kind == 'z' and idx == seen[0]:
                        next_ln_q(part, t[row:row + 8, :])
                for _ in range(cnt[13 + seen[0]]):
                    u_dft(*us.pop(0))
                seen[0] += 1

            for j in range(3):
                group(a0, NT, j, after_z2)
            hres = [h_dft(*hs.pop(0)) for _ in range(nh_mid)]
            for _ in range(cnt[12]):
                u_dft(*us.pop(0))
            ln_z2(a0 + 1, ln_z2(a0))
            for part, (kind, idx, row) in enumerate(marks):
                if kind == 'h':
                    next_ln_q(part, hres[idx][row:row + 8, :])
            seen[0] = 0

            def dft_run():
                ru, rh = nu_run, nh_run
                while ru or rh:
                    if ru and ru * max(nh_run, 1) >= rh * max(nu_run, 1):
                        u_dft(*us.pop(0))
                        ru -= 1
                    else:
                        h_dft(*hs.pop(0))
                        rh -= 1

            if not marks:
                dft_run()
            for j in range(3):
                group(a0, 0, j, after_z1, fence(z2_words(a0 + 1)) if not marks and j == 1 else None)
            if marks:
                dft_run()
            for _ in range(nh_end):
                h_dft(*hs.pop(0))
        assert not us
        return hs

    def conv_pos(ft, ft2, par, dt, after):
        cols = lanes(dt)
        prev = None
        for a in range(NB):
            ar, ai = (None, None) if prev is None else (-prev[1], prev[0])
            for dl in range(a + 1):
                hr = hf_v[ft, dl, 0:8, cols]
                hi = hf_v[ft, dl, 8:16, cols]
                ur = p_v[ft, a - dl, 0:8, cols]
                ui = p_v[ft, a - dl, 8:16, cols]
                if ar is None:
                    ar, ai = ur * hr - ui * hi, ur * hi + ui * hr
                    if after is not None:
                        z = fence(after)
                        ar, ai = held(ar, z), held(ai, z)
                elif (a * (a + 1) // 2 + dl) % TREE == 0:
                    ar = ar + (ur * hr - ui * hi)
                    ai = ai + (ur * hi + ui * hr)
                else:
                    ar = (ar + ur * hr) - ui * hi
                    ai = (ai + ur * hi) + ui * hr
            prev = (ar, ai) if prev is None else (ar + prev[1], ai - prev[0])
            w_v[a * 16 + ft2, par * 8:(par + 1) * 8, cols] = ar.astype(BF)
            w_v[a * 16 + 8 + ft2, par * 8:(par + 1) * 8, cols] = ai.astype(BF)
        return words(prev[0])

    gl_v = wout_v
    GL0 = FH
    GS0 = GL0 + NOP * C
    WS0 = GS0 + 4 * C
    GX0 = WS0 + 2 * HN

    def g_sums(ref, g0, s0):
        def quads(u):
            c, g = u
            return [(ref, (pl.ds(g0 + m * C + g * 16, 16), lanes(n))) for m in (0, 1) for n in (c, 3 + c)]

        def dest(u, k):
            c, g = u
            return gl_v, (pl.ds(s0 + k // 2 * C + g * 16, 16), lanes(k % 2 * 3 + c))

        units = [(c, g) for c in range(3) for g in range(C // 16)]
        chain_sums(units, quads, dest, a_sums, 2, True, first=2 if ref is gl_v else 0)

    def ws_at(jj, k):
        return WS0 + (jj * 4 + k) // 6 * HN, lanes((jj * 4 + k) % 6)

    def w_sums(after):
        def quads(u):
            jj, g = u
            return [(wout_v, (pl.ds(r0 + g * 16, 16), lanes(n))) for r0 in (0, HN) for n in (jj, 2 + jj)]

        def dest(u, k):
            jj, g = u
            r0, cols = ws_at(jj, k)
            return wout_v, (pl.ds(r0 + g * 16, 16), cols)

        chain_sums([(jj, g) for jj in range(2) for g in range(HN // 16)], quads, dest, b_sums, 0, False, after)

    def xn_gate(a, dt, hh):
        return xn_v[brows(a), lanes(dt)].astype(F32) * (hh + hh * jnp.tanh(hh))

    def o_pair(a0, ref, g0, s0, finish, skip=False):
        r0, r1 = pl.ds(g0, C), pl.ds(g0 + C, C)

        def gs(k):
            return gl_v[pl.ds(s0 + k // 2 * C, C), (k % 2) * HN:(k % 2 + 1) * HN]

        def ws(jj, k):
            r, cols = ws_at(jj, k)
            return wout_v[r:r + HN, cols]

        for jj in range(2):
            if jj == (0 if skip else 1):
                finish(a0, 4, None if skip else mm(ref[r0, :], wout_v[0:FH, lanes(4)]))
                finish(a0 + 1, 4, mm(ref[r1, :], wout_v[0:FH, lanes(4)]))
            p1 = mm(ref[r0, 0:HN], wout_v[0:HN, lanes(jj)])
            finish(a0, jj, p1 + mm(ref[r0, HN:FH], wout_v[HN:FH, lanes(jj)]))
            u2 = p1 + mm(gs(1), ws(jj, 1))
            u3 = u2 + mm(gs(2), ws(jj, 2))
            finish(a0 + 1, jj, u3 + mm(ref[r1, HN:FH], ws(jj, 3)))
            p5 = mm(gs(0), ws(jj, 0))
            finish(a0 + 1, 2 + jj, u3 + p5)
            finish(a0, 2 + jj, (u2 + p5) + mm(gs(3), wout_v[HN:FH, lanes(2 + jj)]))

    def s_at(slot, k):
        return D + (slot * 2 + k // 2) * C, (k % 2) * HK

    def s_val(slot, k):
        r0, col = s_at(slot, k)
        return h_v[r0:r0 + C, col:col + HK]

    def s_sums(a0, nr, via_memory):
        def quads(u):
            slot, c, g = u
            return [(wsp_v, (ds((a0 + 2 * slot + m) * C + g * nr, nr), lanes(n)))
                    for m in (0, 1) for n in (c, HK // 128 + c)]

        def dest(u, k):
            slot, c, g = u
            r0, col = s_at(slot, k)
            return h_v, (slice(r0 + g * nr, r0 + (g + 1) * nr), slice(col + c * 128, col + (c + 1) * 128))

        units = [(slot, c, g) for slot in range(2) for c in range(HK // 128) for g in range(C // nr)]
        for part in (units[:56], units[56:]) if via_memory else (units,):
            chain_sums(part, quads, dest, a_sums, 2, via_memory, first=2)

    def phase2a(i, carry):
        @pl.when(i + 1 < S // TA)
        def _():
            cp_wsp(i + 1).wait()

        eye = (jax.lax.broadcasted_iota(jnp.int32, (C, C), 0)
               == jax.lax.broadcasted_iota(jnp.int32, (C, C), 1))

        def bcol(a):
            return jnp.sum(jnp.where(eye, b32_v[pl.ds(a, 1), :], 0.0), axis=-1, keepdims=True)

        def put(m, n, g):
            g = (z1_v[brows(i * (TA // C) + m), lanes(n)] * g).astype(BF)
            if m < NOP:
                gl_v[GL0 + m * C:GL0 + (m + 1) * C, lanes(n)] = g
            else:
                gg_v[ds((2 * i + m - NOP) * C, C), lanes(n)] = g
                if m == NOP:
                    gl_v[GX0:GX0 + C, lanes(n)] = g

        for pp in range(2):
            if pp == 1:
                g_sums(gl_v, GL0, GS0)
            m0 = 2 * pp
            a0 = i * (TA // C) + m0
            r0, r1 = brows(a0), brows(a0 + 1)
            b0 = bcol(a0)
            db = bcol(a0 + 1) - b0
            for j in range(NT // 2):
                jl, jr = lanes(j), lanes(NT // 2 + j)
                t1, t2, t3, t4 = (t_v[:, lanes(k * (NT // 2) + j)] for k in range(4))
                p1 = mm(wsp_v[r0, 0:HK], z2_v[0:HK, jl]) + b0
                put(m0, j, p1 + mm(wsp_v[r0, HK:S], z2_v[HK:S, jl]))
                u2 = p1 + mm(s_val(pp, 1), t2)
                u3 = (u2 + db) + mm(s_val(pp, 2), t3)
                put(m0 + 1, j, u3 + mm(wsp_v[r1, HK:S], t4))
                p5 = mm(s_val(pp, 0), t1)
                put(m0 + 1, NT // 2 + j, u3 + p5)
                put(m0, NT // 2 + j, (u2 + p5) + mm(s_val(pp, 3), z2_v[HK:S, jr]))
        def finish(a, dt, hh):
            xg_v[brows(a), lanes(dt)] = xn_gate(a, dt, hh)

        o_pair(i * (TA // C), gl_v, GL0, GS0, finish)
        finish(i * (TA // C) + 2, 4, mm(gl_v[GX0:GX0 + C, :], wout_v[0:FH, lanes(4)]))
        s_sums(jnp.minimum(i + 1, S // TA - 1) * (TA // C), 16, True)
        nft = NB * TA // S
        last = None
        for ft in range(nft):
            for dt in range(ND):
                last = conv_pos(i * nft + ft, i * (nft // 2) + ft // 2, ft % 2, dt, last)
        return carry

    step = pl.program_id(0)

    @pl.when(step == 0)
    def _():
        for grp in groups:
            for cp in grp:
                cp.start()
        cp_wout.start()
        for i in range(S // TA):
            cp_wsp(i).start()
        k_u[:, 0:8, :] = jnp.zeros((ND, 8, 128), U32)

    @pl.when(step == 1)
    def _():
        cp_wsp(0).wait()
        cp_wout.wait()
        for a, dt in [(a, dt) for a in range(NB) for dt in range(ND)][NB * ND - H_LATE:]:
            h_dft(a, dt)
        last = None
        for g in range(C // 16):
            bot = held(z2_v[pl.ds((NB - 1) * C + g * 16, 16), :], None if last is None else fence(last))
            t_rest(NB // 2 - 1, bot.astype(F32), g, 16)
            rows = pl.ds((NB // 2 - 1) * C + g * 16, 16)
            last = jnp.concatenate([words(t_v[rows, lanes(k)]) for k in range(3, 12)], axis=0)
        w_sums(last)
        s_sums(0, 32, False)
        jax.lax.fori_loop(0, S // TA, phase2a, 0)

        rev = 7 - jax.lax.broadcasted_iota(jnp.int32, (8, 128), 0)
        done = {}

        def emit(a, dt, hh):
            rows, cols = brows(a), lanes(dt)
            ev = mm(fg_v[2 * C:2 * C + C // 2, 0:C], w_v[ds(a * 16, 8), :, cols].reshape(C, 128))
            od = mm(fg_v[2 * C:2 * C + C // 2, C:2 * C], w_v[ds(a * 16 + 8, 8), :, cols].reshape(C, 128))
            lo = ev - od
            ys = [jnp.take_along_axis(lo[g * 8:(g + 1) * 8, :], rev, axis=0)
                  for g in range(C // 16 - 1, -1, -1)]
            y = jnp.concatenate(ys + [ev + od], axis=0)
            xg = xg_v[rows, cols] if hh is None else xn_gate(a, dt, hh)
            o_v[rows, cols] = (q_v[rows, cols].astype(F32) + xg * y).astype(BF)
            done[a] = done.get(a, 0) + 1
            if a >= NB - 2:
                cp_o(a, cols).start()
            elif done[a] == ND:
                cp_o(a).start()

        g_sums(gg_v, 0, GS0)
        for k in range(S // TA):
            if k + 1 < S // TA:
                g_sums(gg_v, (k + 1) * 2 * C, GS0 + ((k + 1) % 2) * 2 * C)
            for a in (4 * k, 4 * k + 1):
                for dt in range(ND):
                    emit(a, dt, None)
            o_pair(4 * k + 2, gg_v, k * 2 * C, GS0 + (k % 2) * 2 * C, emit, skip=True)
        pltpu.make_async_copy(o_v, o_hbm, sem_o.at[0]).wait()

    @pl.when(step == 0)
    def _():
        wait(0)
        ln_q(0)
        ln_q(1)
        wait(1)
        for n in (0, 1):
            z2_tile(0, n)
            z2_tile(1, n)
        wait(2)
        ln_q(2)
        for n in (2, 3):
            z2_tile(0, n)
            z2_tile(1, n)
        for n in range(4):
            z2_tile(2, n)
        wait(3)
        ln_q(3)
        seq = ([(z2_tile, a, n) for a in range(3) for n in (4, 5)] + [(z2_tile, 3, n) for n in range(NT)]
               + [(z1_tile, a, 0) for a in range(4)])
        tw_done = tw_sums(NT)
        for j, (tile, a, n) in enumerate(seq):
            if j == 15:
                gate = fence(tw_done)
            elif j == 3:
                gate = fence(words(xn_v[brows(3), 0:128]))
            else:
                gate = fence(z2_words(0, (7, 10).index(j))) if j in (7, 10) else None
            tile(a, n, gate)
            if j == 1:
                ln_z2(0)
        wait(4)
        for a in (1, 2, 3):
            ln_z2(a)
        tw_sums(0)
        release = (8, 10, 11, 12, 13, 15, 16, 17)
        waits = (3, 4, 6, 8, 10, 11)
        for j, (a, n) in enumerate((a, n) for n in range(1, NT) for a in range(4)):
            gate = fence(z2_words(1 + waits.index(j) // 2, waits.index(j) % 2)) if j in waits else None
            t = z1_tile(a, n, gate)
            if j in release:
                part = release.index(j)
                ln_q(4 + part // NLQ, fence(words(t[0:8, :])), part % NLQ, NLQ)
        region([4])
        wait(5)
        b32_v[...] = b_v[...].astype(F32) * 0.25
        assert not region([6, 8, 10], HCH[0], KCH[0])
        wait(6)
        assert len(region([12, 14], HCH[1], KCH[1])) == H_LATE


@jax.jit
def pallas_recurrent_scan__ssm_conv_h3__mixer_gmlp__prompt_kernel(
    A_q: jax.Array,
    A_k: jax.Array,
    A_v: jax.Array,
    A_shift_k: jax.Array,
    A_ssm_k: jax.Array,
    A_ssm_D: jax.Array,
    B_x: jax.Array,
    B_w_in: jax.Array,
    B_w_sp: jax.Array,
    B_b_sp: jax.Array,
    B_w_out: jax.Array,
):
    del B_x
    any_spec = pl.BlockSpec(memory_space=pl.ANY)
    vm = pltpu.VMEM
    dma = pltpu.SemaphoreType.DMA
    out = pl.pallas_call(
        _kernel,
        out_shape=jax.ShapeDtypeStruct((S, D), BF),
        grid=(2,),
        in_specs=[any_spec] * 11,
        out_specs=any_spec,
        scratch_shapes=[
            vm((S // 2, D), U32),
            vm((ND, S // 2 + 32, 128), U32),
            vm((S // 2, D), U32),
            vm(((D + 4 * C) // 2, S), U32),
            vm(((D + 2 * KS) // 2, 2 * FH), U32),
            vm((S // 2, S), U32),
            vm(((FH + 8 * C + 2 * HN) // 2, FH), U32),
            vm(((2 * C + C // 2) // 2, 2 * C), U32),
            vm(((S + 4 * C) // 2, D), U32),
            vm((S + 6 * C, FH), F32),
            vm((S // 2, FH), U32),
            vm((S // 4, 2 * FH), U32),
            vm((NB, NB, 16, D), F32),
            vm((NB, NB, 16, D), F32),
            vm((NB * 16, 8, 1024), U32),
            vm((S // 4, FH), U32),
            vm((S, D), F32),
            vm((S, D), BF),
            vm((NB, 128), F32),
            vm((NB, 128), BF),
            vm((4, 18 * 128), BF),
            vm((ND, 128), BF),
            dma((len(QCH),)), dma((len(KCH) * ND,)), dma((len(KCH),)), dma((len(HCH),)),
            dma((len(WCH),)), dma((S // TA,)), dma((1,)), dma((5,)),
        ],
        compiler_params=pltpu.CompilerParams(
            dimension_semantics=("arbitrary",),
            vmem_limit_bytes=110 * 1024 * 1024,
            disable_bounds_checks=True,
            disable_semaphore_checks=True,
        ),
    )(
        A_q.reshape(S, D), A_k.reshape(S, D), A_v.reshape(S, D),
        A_shift_k.T, A_ssm_k, A_ssm_D.reshape(ND, 128),
        B_w_in, B_w_sp, B_b_sp.reshape(NB, 128), B_w_out,
        _dft_consts(),
    )
    return out.reshape(1, S, D)
```
